```python
import jax
import jax.numpy as jnp

def _softmax(x, axis=-1):
    return jax.nn.softmax(x, axis=axis)

def _gelu(x):
    return jax.nn.gelu(x, approximate=True)

def _silu(x):
    return jax.nn.silu(x)

def _sigmoid(x):
    return jax.nn.sigmoid(x)

def _layernorm(x, axis=-1, eps=1e-05):
    m = jnp.mean(x, axis=axis, keepdims=True)
    v = jnp.var(x, axis=axis, keepdims=True)
    return (x - m) / jnp.sqrt(v + eps)

def _scatter_add(tgt, idx, src, axis=0):
    return tgt.at[idx].add(src)

def _segment_sum(src, seg, n):
    return jax.ops.segment_sum(src, seg, n)

class _Rng:

    def __init__(self, key):
        self._k = key

    def _next(self):
        self._k, sub = jax.random.split(self._k)
        return sub

    def normal(self, shape):
        return jax.random.normal(self._next(), shape, dtype=jnp.bfloat16)

    def randint(self, lo, hi, shape):
        return jax.random.randint(self._next(), shape, lo, hi, dtype=jnp.int32)

    def uniform(self, shape, lo=0.0, hi=1.0):
        return jax.random.uniform(self._next(), shape, jnp.bfloat16, lo, hi)

    def permutation(self, n):
        return jax.random.permutation(self._next(), n)
kernel_name = 'concat_heads__ssm_conv_h3__memory_aug_recurrent_mem_tr__prompt'

def setup_inputs():
    _rng = _Rng(jax.random.key(int.from_bytes(__import__("os").urandom(4), "little")))
    _w = lambda a: (lambda t: t.astype(jnp.bfloat16) if jnp.issubdtype(t.dtype, jnp.floating) else t)(jnp.asarray(a))

    def _A_setup():
        B, S, D = (1, 2048, 1024)
        ks = 4
        return {'q': _w((lambda *s: _rng.normal(s) * 0.05)(B, S, D)), 'k': _w((lambda *s: _rng.normal(s) * 0.05)(B, S, D)), 'v': _w((lambda *s: _rng.normal(s) * 0.05)(B, S, D)), 'shift_k': _w((lambda *s: _rng.normal(s) * 0.05)(D, ks) * 0.5), 'ssm_k': _w((lambda *s: _rng.normal(s) * 0.05)(D, S) * (1.0 / S ** 0.5)), 'ssm_D': _w((lambda *s: _rng.normal(s) * 0.05)(D))}
    _A_in = _A_setup()

    def _B_setup():
        B, S, Dm = (1, 2048, 1024)
        H, Dh = (32, 128)
        M, seg = (8, 32)
        seg = min(seg, S)
        S = S // seg * seg
        return {'x': _w((lambda *s: _rng.normal(s) * 0.05)(B, S, Dm)), 'mem0': _w((lambda *s: _rng.normal(s) * 0.05)(B, M, Dm)), 'Wq': _w((lambda *s: _rng.normal(s) * 0.05)(Dm, H, Dh) * Dm ** (-0.5)), 'Wk': _w((lambda *s: _rng.normal(s) * 0.05)(Dm, H, Dh) * Dm ** (-0.5)), 'Wv': _w((lambda *s: _rng.normal(s) * 0.05)(Dm, H, Dh) * Dm ** (-0.5)), 'Wo': _w((lambda *s: _rng.normal(s) * 0.05)(H, Dh, Dm) * (H * Dh) ** (-0.5)), 'seg_len': seg}
    _B_in = _B_setup()
    return {'A_q': _A_in['q'], 'A_k': _A_in['k'], 'A_v': _A_in['v'], 'A_shift_k': _A_in['shift_k'], 'A_ssm_k': _A_in['ssm_k'], 'A_ssm_D': _A_in['ssm_D'], 'B_x': _B_in['x'], 'B_mem0': _B_in['mem0'], 'B_Wq': _B_in['Wq'], 'B_Wk': _B_in['Wk'], 'B_Wv': _B_in['Wv'], 'B_Wo': _B_in['Wo'], 'B_seg_len': _B_in['seg_len']}

def reference(A_q, A_k, A_v, A_shift_k, A_ssm_k, A_ssm_D, B_x, B_mem0, B_Wq, B_Wk, B_Wv, B_Wo, B_seg_len):

    def _A_ref(q, k, v, shift_k, ssm_k, ssm_D):
        B, S, D = q.shape
        ks = shift_k.shape[-1]
        k_pad = jnp.pad(k, ((0, 0), (ks - 1, 0), (0, 0)))
        k_shift = jnp.zeros_like(k)
        for t in range(ks):
            k_shift = k_shift + k_pad[:, t:t + S, :] * shift_k[:, ks - 1 - t][None, None, :]
        kv = k_shift * v
        L = 2 * S
        kv_pad = jnp.pad(kv, ((0, 0), (0, S), (0, 0)))
        kf_pad = jnp.pad(ssm_k, ((0, 0), (0, S)))
        kv_f = (lambda x, axes=(-2, -1): jnp.fft.rfft2(x.astype(jnp.float32), axes=axes))(kv_pad[:, None, :, :], axes=(1, 2))
        kf_f = (lambda x, axes=(-2, -1): jnp.fft.rfft2(x.astype(jnp.float32), axes=axes))(kf_pad[:, None, :], axes=(1, 2))
        kf_f = (lambda x, *d: x.transpose(*d))(kf_f, 1, 2, 0)
        y_f = kv_f * kf_f[None, :, :, :]
        y = (lambda x, s, axes=(-2, -1): jnp.fft.irfft2(x, s=s, axes=axes).astype(jnp.bfloat16))(y_f, (1, L), axes=(1, 2))[:, 0, :S, :]
        y = y + kv * ssm_D[None, None, :]
        return q * y

    def _B_ref(x, mem0, Wq, Wk, Wv, Wo, seg_len):
        B, S, Dm = x.shape
        H, Dh = (Wq.shape[1], Wq.shape[2])
        M = mem0.shape[1]
        scale = Dh ** (-0.5)
        n_seg = S // seg_len
        L = M + seg_len
        idx = jnp.arange(L)
        mask = (idx[:, None] < M) | (idx[:, None] >= idx[None, :])
        mem = mem0
        outs = []
        for s in range(n_seg):
            xs = x[:, s * seg_len:(s + 1) * seg_len, :].copy()
            h = jnp.concatenate([mem, xs], axis=1)
            q = jnp.einsum('btd,dhe->bhte', h, Wq)
            k = jnp.einsum('btd,dhe->bhte', h, Wk)
            v = jnp.einsum('btd,dhe->bhte', h, Wv)
            scores = jnp.einsum('bhqe,bhke->bhqk', q, k) * scale
            scores = jnp.where(mask[None, None], scores, -1000000000.0)
            p = _softmax(scores, axis=-1)
            o = jnp.einsum('bhqk,bhke->bhqe', p, v)
            o = jnp.einsum('bhte,hed->btd', o, Wo)
            mem = o[:, :M, :].copy()
            outs.append(o[:, M:, :])
        return jnp.concatenate(outs, axis=1)
    a = _A_ref(A_q, A_k, A_v, A_shift_k, A_ssm_k, A_ssm_D)
    b = _B_ref(B_x, B_mem0, B_Wq, B_Wk, B_Wv, B_Wo, B_seg_len)
    return jnp.concatenate([a, b], axis=-1)
```

```python
import functools

import numpy as np
import jax
import jax.numpy as jnp
from jax import lax
import jax.experimental.pallas as pl
import jax.experimental.pallas.tpu as pltpu

F32 = jnp.float32
BF16 = jnp.bfloat16
U32 = jnp.uint32

LANES = 128
BLK = 128
NFFT = 2 * BLK
WPITCH = 520
TOL = 2.0 ** -10


def _dft_mats():
    order = np.concatenate([np.arange(0, BLK, 2), np.arange(1, BLK, 2)])
    theta = 2.0 * np.pi * (order + 0.5) / NFFT
    n = np.arange(BLK)
    c = np.cos(theta[:, None] * n[None, :])
    s = np.sin(theta[:, None] * n[None, :])
    fwd = np.zeros((NFFT, BLK))
    inv = np.zeros((BLK, NFFT))
    for m in range(BLK // 8):
        fwd[16 * m:16 * m + 8] = c[8 * m:8 * m + 8]
        fwd[16 * m + 8:16 * m + 16] = -s[8 * m:8 * m + 8]
        inv[:, 16 * m:16 * m + 8] = c[8 * m:8 * m + 8].T * (2.0 / NFFT)
        inv[:, 16 * m + 8:16 * m + 16] = -s[8 * m:8 * m + 8].T * (2.0 / NFFT)
    return fwd.astype(np.float32), inv.astype(np.float32)


def _kernel(q_hbm, k_hbm, v_hbm, shift_ref, h_hbm, d_ref, x_hbm, mem0_ref,
            wq_hbm, wk_hbm, wv_hbm, wo_hbm, fwd_ref, inv_ref,
            out_hbm,
            hbuf, vbuf, wq32, wk32, wv32, wo, stage, acc, obuf, mhat, mnew, tsum,
            aq, ak, av, ah, kf, kvb, xf, hf, wf, aout,
            sem_x, sem_wo, sem_stage, sem_a, sem_aout, sem_o,
            *, S, D, DM, H, M, SEG):
    E = LANES
    NSEG = S // SEG
    NP = NSEG // 2
    MR = 2 * M
    XR = 2 * SEG
    PR = MR + XR
    L = M + SEG
    NB = S // BLK
    NT = D // LANES
    PPB = 8
    NRB = NP // PPB
    G = 4
    scale = float(E) ** -0.5

    def slot_head(sl):
        return 16 * (sl // 16) + 2 * (sl % 8) + (sl % 16) // 8

    def x_copy():
        return pltpu.make_async_copy(x_hbm, hbuf.at[:, MR:PR, :], sem_x)

    def wo_copy(sl):
        return pltpu.make_async_copy(
            wo_hbm.at[pl.ds(slot_head(sl) * E, E), :],
            wo.at[pl.ds(sl * E, E), :], sem_wo)

    w_srcs = [wv_hbm, wq_hbm, wk_hbm]
    w_dsts = [wv32, wq32, wk32]

    def stage_copy(i):
        return pltpu.make_async_copy(
            w_srcs[i // 2].at[:, pl.ds(16 * (i % 2), 16), :],
            stage.at[i % 2], sem_stage.at[i % 2])

    def a_copies(t, sl):
        c = pl.ds(pl.multiple_of(t * LANES, LANES), LANES)
        return [
            pltpu.make_async_copy(k_hbm.at[:, c], ak.at[sl], sem_a.at[sl, 0]),
            pltpu.make_async_copy(v_hbm.at[:, c], av.at[sl], sem_a.at[sl, 1]),
            pltpu.make_async_copy(h_hbm.at[c, :], ah.at[sl], sem_a.at[sl, 2]),
            pltpu.make_async_copy(q_hbm.at[:, c], aq.at[sl], sem_a.at[sl, 3]),
        ]

    def aout_copy(t, sl):
        c = pl.ds(pl.multiple_of(t * LANES, LANES), LANES)
        return pltpu.make_async_copy(aout.at[sl], out_hbm.at[:, c], sem_aout.at[sl])

    def o_copy(rb, sl):
        r = pl.ds(pl.multiple_of(rb * (PPB * XR), PPB * XR), PPB * XR)
        return pltpu.make_async_copy(obuf.at[sl], out_hbm.at[r, pl.ds(D, DM)], sem_o.at[sl])

    for cp in a_copies(0, 0):
        cp.start()
    stage_copy(0).start()
    stage_copy(1).start()
    x_copy().start()
    for sl in range(H):
        wo_copy(sl).start()

    kf[0:8, :] = jnp.zeros((8, LANES), F32)

    def a_tile(t, carry):
        sl = t % 2

        @pl.when(t + 1 < NT)
        def _():
            for cp in a_copies(t + 1, 1 - sl):
                cp.start()

        for cp in a_copies(t, sl):
            cp.wait()

        c = pl.ds(pl.multiple_of(t * LANES, LANES), LANES)
        taps = shift_ref[:, c].astype(F32)
        dcol = d_ref[...].astype(F32)
        rows = lax.broadcasted_iota(jnp.int32, dcol.shape, 0)
        dvec = jnp.sum(jnp.where(rows == t, dcol, 0.0), axis=0, keepdims=True)

        kf[8:8 + S, :] = ak[sl].astype(F32)
        for b in range(NB):
            r0 = b * BLK
            ks = kf[8 + r0:8 + r0 + BLK, :] * taps[0:1, :]
            for j in range(1, 4):
                ks = ks + kf[8 + r0 - j:8 + r0 - j + BLK, :] * taps[j:j + 1, :]
            kvb[r0:r0 + BLK, :] = (ks * av[sl, r0:r0 + BLK, :].astype(F32)).astype(BF16)

        fwd = fwd_ref[...]
        rhs = jnp.concatenate([kvb[b * BLK:(b + 1) * BLK, :] for b in range(NB)], axis=1)
        xf[...] = jnp.dot(fwd, rhs, preferred_element_type=F32)
        hst = jnp.concatenate([ah[sl, :, b * BLK:(b + 1) * BLK] for b in range(NB)], axis=0)
        hf[...] = lax.dot_general(fwd, hst, (((1,), (1,)), ((), ())), preferred_element_type=F32)

        def freq_chunk(m, sign):
            r_re = pl.ds(pl.multiple_of(16 * m, 16), 8)
            r_im = pl.ds(pl.multiple_of(16 * m + 8, 8), 8)
            hr = [hf[r_re, b * BLK:(b + 1) * BLK] for b in range(NB)]
            hi = [hf[r_im, b * BLK:(b + 1) * BLK] for b in range(NB)]
            gr = [hr[0]]
            gi = [hi[0]]
            for b in range(1, NB):
                if sign > 0:
                    gr.append(hr[b] - hi[b - 1])
                    gi.append(hi[b] + hr[b - 1])
                else:
                    gr.append(hr[b] + hi[b - 1])
                    gi.append(hi[b] - hr[b - 1])
            for a in range(NB):
                wr = wi = None
                for cc in range(a + 1):
                    xr = xf[r_re, cc * BLK:(cc + 1) * BLK]
                    xi = xf[r_im, cc * BLK:(cc + 1) * BLK]
                    pr = xr * gr[a - cc] - xi * gi[a - cc]
                    pi = xr * gi[a - cc] + xi * gr[a - cc]
                    wr = pr if wr is None else wr + pr
                    wi = pi if wi is None else wi + pi
                wf[pl.ds(pl.multiple_of(16 * m, 16), 16), a * BLK:(a + 1) * BLK] = (
                    jnp.concatenate([wr, wi], axis=0).astype(BF16))

        def even_body(m, cy):
            freq_chunk(m, 1)
            return cy

        def odd_body(m, cy):
            freq_chunk(m, -1)
            return cy

        lax.fori_loop(0, BLK // 16, even_body, 0)
        lax.fori_loop(BLK // 16, BLK // 8, odd_body, 0)

        @pl.when(t >= 2)
        def _():
            aout_copy(t - 2, sl).wait()

        y = jnp.dot(inv_ref[...], wf[...], preferred_element_type=F32)
        for b in range(NB):
            r0 = b * BLK
            yb = y[:, r0:r0 + BLK] + kvb[r0:r0 + BLK, :].astype(F32) * dvec
            aout[sl, r0:r0 + BLK, :] = (aq[sl, r0:r0 + BLK, :].astype(F32) * yb).astype(BF16)
        aout_copy(t, sl).start()
        return carry

    lax.fori_loop(0, NT, a_tile, 0)
    aout_copy(NT - 2, 0).wait()
    aout_copy(NT - 1, 1).wait()

    CH = 16

    def relayout(i):
        dst = w_dsts[i // 2]
        g = i % 2

        def body(tt, cy):
            i0 = pl.multiple_of(tt * CH, CH)
            win = dst.at[pl.ds(16 * g * WPITCH + i0, 15 * WPITCH + CH), :]
            for ii in range(CH):
                a = pltpu.bitcast(stage[g, 2 * i0 + 2 * ii], U32)
                b = pltpu.bitcast(stage[g, 2 * i0 + 2 * ii + 1], U32)
                lo = (a & jnp.uint32(0xFFFF)) | (b << 16)
                hi = (a >> 16) | (b & jnp.uint32(0xFFFF0000))
                win[pl.ds(ii, 8, stride=WPITCH), :] = lo
                win[pl.ds(8 * WPITCH + ii, 8, stride=WPITCH), :] = hi
            return cy

        lax.fori_loop(0, DM // 2 // CH, body, 0)

    for i in range(6):
        stage_copy(i).wait()
        relayout(i)
        if i + 2 < 6:
            stage_copy(i + 2).start()

    def wmat(w32, sl0, n):
        parts = []
        for j in range(n):
            r0 = pl.multiple_of((sl0 + j) * WPITCH, 8)
            parts.append(pltpu.bitcast(w32[pl.ds(r0, DM // 2), :], BF16))
        return parts[0] if n == 1 else jnp.concatenate(parts, axis=1)

    x_copy().wait()
    for sl in range(H):
        wo_copy(sl).wait()

    mem0 = mem0_ref[...].astype(F32)
    hbuf[0, 0:MR, :] = jnp.concatenate([mem0, jnp.zeros_like(mem0)], axis=0).astype(BF16)
    GV = 2

    def v_body(g, cy):
        c = pl.ds(pl.multiple_of(g * (GV * E), GV * E), GV * E)
        lhs = jnp.concatenate([hbuf[0, 0:MR, :], hbuf[:, MR:PR, :].reshape(S, DM)], axis=0)
        vv = jnp.dot(lhs, wmat(wv32, g * GV, GV), preferred_element_type=F32).astype(BF16)
        vx = vv[MR:]
        vbuf[:, MR:PR, c] = vx.reshape(NP, XR, GV * E)
        ts = jnp.sum(vx.astype(F32).reshape(NSEG, SEG, GV * E), axis=1)
        t0 = jnp.sum(vv[0:MR].astype(F32), axis=0, keepdims=True)
        rows = lax.broadcasted_iota(jnp.int32, ts.shape, 0)
        tsum[:, c] = ts + jnp.where(rows == 0, t0, 0.0)
        return cy

    lax.fori_loop(0, H // GV, v_body, 0)

    puni = (1.0 / jnp.full((1, 1), float(L), F32)).astype(BF16).astype(F32)

    def shift_down(m):
        rows = lax.broadcasted_iota(jnp.int32, m.shape, 0)
        return jnp.where(rows == 0, 0.0, pltpu.roll(m, 1, 0))

    m1 = shift_down(jnp.dot((tsum[...] * puni).astype(BF16), wo[...], preferred_element_type=F32))
    v1 = jnp.dot(m1.astype(BF16), wmat(wv32, 0, H), preferred_element_type=F32)
    v1 = v1.astype(BF16).astype(F32)
    u2 = ((tsum[...] + float(M) * v1) * puni).astype(BF16)
    m2 = shift_down(jnp.dot(u2, wo[...], preferred_element_type=F32))
    mhat[...] = jnp.broadcast_to(m2[:, None, :], (NSEG, M, DM)).reshape(NSEG * M, DM)
    mhat[0:M, :] = mem0

    ri = lax.broadcasted_iota(jnp.int32, (PR, PR), 0)
    ci = lax.broadcasted_iota(jnp.int32, (PR, PR), 1)

    def seg_of(r):
        return jnp.where(r < MR, r // M, (r - MR) // SEG)

    def pos_of(r):
        return jnp.where(r < MR, r % M, M + (r - MR) % SEG)

    same = seg_of(ri) == seg_of(ci)
    allowed = same & ((ri < MR) | (pos_of(ri) >= pos_of(ci)))
    fill = jnp.where(same, -1e9, -jnp.inf).astype(F32)

    def sweep(state):
        it, _ = state
        hbuf[:, 0:MR, :] = mhat[...].astype(BF16).reshape(NP, MR, DM)

        def vm_body(g, cy):
            c = pl.ds(pl.multiple_of(g * (8 * E), 8 * E), 8 * E)
            lhs = hbuf[:, 0:MR, :].reshape(NP * MR, DM)
            vv = jnp.dot(lhs, wmat(wv32, g * 8, 8), preferred_element_type=F32).astype(BF16)
            vbuf[:, 0:MR, c] = vv.reshape(NP, MR, 8 * E)
            return cy

        lax.fori_loop(0, H // 8, vm_body, 0)

        def rb_body(rb, cy):
            p0 = pl.multiple_of(rb * PPB, PPB)
            acc[...] = jnp.zeros_like(acc)

            def hg_body(g, cy2):
                lhs = hbuf[pl.ds(p0, PPB)].reshape(PPB * PR, DM)
                us = []
                for j in range(G):
                    sl = g * G + j
                    wqk = jnp.concatenate([wmat(wq32, sl, 1), wmat(wk32, sl, 1)], axis=1)
                    qk = jnp.dot(lhs, wqk, preferred_element_type=F32).astype(BF16)
                    qh = qk[:, :E].reshape(PPB, PR, E)
                    kh = qk[:, E:].reshape(PPB, PR, E)
                    vh = vbuf[pl.ds(p0, PPB), :, pl.ds(pl.multiple_of(sl * E, E), E)]
                    s = jnp.einsum('pqe,pke->pqk', qh, kh, preferred_element_type=F32) * scale
                    s = jnp.where(allowed[None], s, fill[None])
                    e = jnp.exp(s - jnp.max(s, axis=-1, keepdims=True))
                    p = (e * (1.0 / jnp.sum(e, axis=-1, keepdims=True))).astype(BF16)
                    o = jnp.einsum('pqk,pke->pqe', p, vh, preferred_element_type=F32)
                    us.append(o.astype(BF16).reshape(PPB * PR, E))
                u = jnp.concatenate(us, axis=1)
                wog = wo[pl.ds(pl.multiple_of(g * (G * E), G * E), G * E), :]
                acc[...] += jnp.dot(u, wog, preferred_element_type=F32)
                return cy2

            lax.fori_loop(0, H // G, hg_body, 0)

            sl = rb % 2

            @pl.when(rb >= 2)
            def _():
                o_copy(rb - 2, sl).wait()

            o3 = acc[...].reshape(PPB, PR, DM)
            obuf[sl] = o3[:, MR:, :].reshape(PPB * XR, DM).astype(BF16)
            mnew[pl.ds(pl.multiple_of(rb * (PPB * MR), PPB * MR), PPB * MR), :] = (
                o3[:, :MR, :].reshape(PPB * MR, DM))
            o_copy(rb, sl).start()
            return cy

        lax.fori_loop(0, NRB, rb_body, 0)
        o_copy(NRB - 2, 0).wait()
        o_copy(NRB - 1, 1).wait()

        n = (NSEG - 1) * M
        new = mnew[0:n, :]
        err = jnp.max(jnp.abs(new - mhat[M:M + n, :]), axis=1, keepdims=True)
        ref = jnp.max(jnp.abs(new), axis=1, keepdims=True)
        ok = jnp.min(jnp.where(err <= TOL * ref, 1.0, 0.0))
        mhat[M:M + n, :] = new
        return it + 1, (ok > 0.5).astype(jnp.int32)

    lax.while_loop(lambda st: jnp.logical_and(st[0] < NSEG, st[1] == 0), sweep,
                   (jnp.int32(0), jnp.int32(0)))


@functools.partial(jax.jit, static_argnames=("B_seg_len",))
def pallas_concat_heads__ssm_conv_h3__memory_aug_recurrent_mem_tr__prompt_kernel(
    A_q, A_k, A_v, A_shift_k, A_ssm_k, A_ssm_D,
    B_x, B_mem0, B_Wq, B_Wk, B_Wv, B_Wo, B_seg_len,
):
    _, S, D = A_q.shape
    DM = B_x.shape[2]
    H, E = B_Wq.shape[1], B_Wq.shape[2]
    M = B_mem0.shape[1]
    SEG = int(B_seg_len)
    NSEG = S // SEG
    NP = NSEG // 2
    PR = 2 * (M + SEG)
    PPB = 8
    assert E == LANES and H == 32 and M == 8 and SEG == 32 and A_shift_k.shape[1] == 4

    fwd, inv = _dft_mats()
    any_spec = pl.BlockSpec(memory_space=pl.ANY)
    vmem_spec = pl.BlockSpec(memory_space=pltpu.VMEM)
    scratch = [
        pltpu.VMEM((NP, PR, DM), BF16),
        pltpu.VMEM((NP, PR, H * E), BF16),
        pltpu.VMEM((H * WPITCH, E), U32),
        pltpu.VMEM((H * WPITCH, E), U32),
        pltpu.VMEM((H * WPITCH, E), U32),
        pltpu.VMEM((H * E, DM), BF16),
        pltpu.VMEM((2, DM, 16, E), BF16),
        pltpu.VMEM((PPB * PR, DM), F32),
        pltpu.VMEM((2, PPB * 2 * SEG, DM), BF16),
        pltpu.VMEM((NSEG * M, DM), F32),
        pltpu.VMEM((NSEG * M, DM), F32),
        pltpu.VMEM((NSEG, H * E), F32),
        pltpu.VMEM((2, S, LANES), BF16),
        pltpu.VMEM((2, S, LANES), BF16),
        pltpu.VMEM((2, S, LANES), BF16),
        pltpu.VMEM((2, LANES, S), BF16),
        pltpu.VMEM((S + 8, LANES), F32),
        pltpu.VMEM((S, LANES), BF16),
        pltpu.VMEM((NFFT, S), F32),
        pltpu.VMEM((NFFT, S), F32),
        pltpu.VMEM((NFFT, S), BF16),
        pltpu.VMEM((2, S, LANES), BF16),
        pltpu.SemaphoreType.DMA,
        pltpu.SemaphoreType.DMA,
        pltpu.SemaphoreType.DMA((2,)),
        pltpu.SemaphoreType.DMA((2, 4)),
        pltpu.SemaphoreType.DMA((2,)),
        pltpu.SemaphoreType.DMA((2,)),
    ]
    out = pl.pallas_call(
        functools.partial(_kernel, S=S, D=D, DM=DM, H=H, M=M, SEG=SEG),
        out_shape=jax.ShapeDtypeStruct((S, D + DM), BF16),
        in_specs=[any_spec, any_spec, any_spec, vmem_spec, any_spec, vmem_spec,
                  any_spec, vmem_spec, any_spec, any_spec, any_spec, any_spec,
                  vmem_spec, vmem_spec],
        out_specs=any_spec,
        scratch_shapes=scratch,
        compiler_params=pltpu.CompilerParams(vmem_limit_bytes=120 * 1024 * 1024),
    )(
        A_q.reshape(S, D), A_k.reshape(S, D), A_v.reshape(S, D),
        A_shift_k.T, A_ssm_k, A_ssm_D.reshape(D // LANES, LANES),
        B_x.reshape(NP, 2 * SEG, DM), B_mem0.reshape(M, DM),
        B_Wq, B_Wk, B_Wv, B_Wo.reshape(H * E, DM),
        jnp.asarray(fwd, BF16), jnp.asarray(inv, BF16),
    )
    return out.reshape(1, S, D + DM)
```

```python
import functools

import numpy as np
import jax
import jax.numpy as jnp
from jax import lax
import jax.experimental.pallas as pl
import jax.experimental.pallas.tpu as pltpu

F32 = jnp.float32
BF16 = jnp.bfloat16
U32 = jnp.uint32

LANES = 128
BLK = 128
NFFT = 2 * BLK
WPITCH = 516
TOL = 2.0 ** -10


def _dft_mats():
    order = np.concatenate([np.arange(0, BLK, 2), np.arange(1, BLK, 2)])
    theta = 2.0 * np.pi * (order + 0.5) / NFFT
    n = np.arange(BLK)
    c = np.cos(theta[:, None] * n[None, :])
    s = np.sin(theta[:, None] * n[None, :])
    fwd = np.zeros((NFFT, BLK))
    inv = np.zeros((BLK, NFFT))
    for m in range(BLK // 8):
        fwd[16 * m:16 * m + 8] = c[8 * m:8 * m + 8]
        fwd[16 * m + 8:16 * m + 16] = -s[8 * m:8 * m + 8]
        inv[:, 16 * m:16 * m + 8] = c[8 * m:8 * m + 8].T * (2.0 / NFFT)
        inv[:, 16 * m + 8:16 * m + 16] = -s[8 * m:8 * m + 8].T * (2.0 / NFFT)
    return fwd.astype(np.float32), inv.astype(np.float32)


def _kernel(q_hbm, k_hbm, v_hbm, shift_ref, h_hbm, d_ref, x_hbm, mem0_ref,
            wq_hbm, wk_hbm, wv_hbm, wo_hbm, fwd_ref, inv_ref,
            out_hbm,
            hbuf, vbuf, w32, wo, stage, qks, acc, obuf, mhat, mnew, tsum,
            aq, ak, av, ah, kf, kvb, xf, hf, wf, aout, zero_v, zero_s,
            sem_x, sem_wo, sem_stage, sem_a, sem_aout, sem_o,
            *, S, D, DM, H, M, SEG):
    E = LANES
    NSEG = S // SEG
    NP = NSEG // 2
    MR = 2 * M
    XR = 2 * SEG
    PR = MR + XR
    L = M + SEG
    NB = S // BLK
    NT = D // LANES
    PPB = 8
    NRB = NP // PPB
    G = 4
    scale = float(E) ** -0.5

    def slot_head(sl):
        return 16 * (sl // 16) + 2 * (sl % 8) + (sl % 16) // 8

    MW, XW, PW = MR // 2, XR // 2, PR // 2

    def x_copy():
        return pltpu.make_async_copy(x_hbm.bitcast(U32), hbuf.at[:, MW:PW, :], sem_x)

    def wo_copy(sl):
        n = E // 2
        return pltpu.make_async_copy(
            wo_hbm.bitcast(U32).at[pl.ds(pl.multiple_of(slot_head(sl) * n, n), n), :],
            wo.at[pl.ds(pl.multiple_of(sl * n, n), n), :], sem_wo)

    w_srcs = [wv_hbm, wq_hbm, wk_hbm]
    NSLAB = 6
    NSTG = 3

    def stage_copy(i):
        return pltpu.make_async_copy(
            w_srcs[i // 2].bitcast(U32).at[:, pl.ds(8 * (i % 2), 8), :],
            stage.at[i % NSTG], sem_stage.at[i % NSTG])

    def a_copies(t, sl):
        c = pl.ds(pl.multiple_of(t * LANES, LANES), LANES)
        return [
            pltpu.make_async_copy(k_hbm.at[:, c], ak.at[sl], sem_a.at[sl, 0]),
            pltpu.make_async_copy(v_hbm.at[:, c], av.at[sl], sem_a.at[sl, 1]),
            pltpu.make_async_copy(h_hbm.at[c, :], ah.at[sl], sem_a.at[sl, 2]),
            pltpu.make_async_copy(q_hbm.at[:, c], aq.at[sl], sem_a.at[sl, 3]),
        ]

    def aout_copy(t, sl):
        c = pl.ds(pl.multiple_of(t * LANES, LANES), LANES)
        return pltpu.make_async_copy(aout.at[sl], out_hbm.at[:, c], sem_aout.at[sl])

    def o_copy(rb):
        r = pl.ds(pl.multiple_of(rb * (PPB * XR), PPB * XR), PPB * XR)
        return pltpu.make_async_copy(obuf.at[rb], out_hbm.at[r, pl.ds(D, DM)], sem_o.at[rb])

    def relayout_items(slab, i0, n, never=None):
        g = slab % NSTG
        win = w32.at[pl.ds(pl.multiple_of(16 * slab * WPITCH + i0, 8), 15 * WPITCH + n + 4), :]

        def item(tok, ii):
            a = stage[g, 2 * i0 + 2 * ii]
            b = stage[g, 2 * i0 + 2 * ii + 1]
            if tok is not None:
                a = jnp.where(never, pltpu.bitcast(tok, U32), a)
            lo = (a & jnp.uint32(0xFFFF)) | (b << 16)
            hi = (a >> 16) | (b & jnp.uint32(0xFFFF0000))
            win[pl.ds(ii, 8, stride=WPITCH), :] = lo
            win[pl.ds(8 * WPITCH + ii, 8, stride=WPITCH), :] = hi

        return [functools.partial(item, ii=ii) for ii in range(n)]

    def run_paced(items, toks):
        for i, it in enumerate(items):
            it(toks[i * len(toks) // len(items)])

    def wpair(which, sp):
        win = w32.at[pl.ds(pl.multiple_of((which * H + 2 * sp) * WPITCH, 8), 2 * WPITCH), :]
        return [pltpu.bitcast(win[j * WPITCH:j * WPITCH + DM // 2, :], BF16) for j in range(2)]

    def wmat(which, sl0, n):
        parts = []
        for j in range(n // 2):
            parts += wpair(which, sl0 // 2 + j)
        return jnp.concatenate(parts, axis=1)

    def pack(x):
        return pltpu.bitcast(x.astype(BF16), U32)

    def unpack(w):
        return pltpu.bitcast(w, BF16)

    WV, WQ, WK = 0, 1, 2

    stage_copy(0).start()
    x_copy().start()
    for cp in a_copies(0, 0):
        cp.start()
    stage_copy(1).start()

    kf[0:8, :] = jnp.zeros((8, LANES), F32)
    zero_v[...] = jnp.zeros((8, LANES), jnp.int32)
    zero_s[0] = 0
    mem0 = mem0_ref[...].astype(F32)
    hbuf[0, 0:MW, :] = pack(jnp.concatenate([mem0, jnp.zeros_like(mem0)], axis=0))

    stage_copy(0).wait()

    def relayout0(tt, cy):
        for it in relayout_items(0, tt * 16, 16):
            it(None)
        return cy

    lax.fori_loop(0, DM // 32, relayout0, 0)
    x_copy().wait()

    HPT = H // NT
    NVP = 8
    PPV = NP // NVP
    RCH = 64
    CPS = DM // 2 // RCH
    CPT = (NSLAB - 1) * CPS // NT

    def v_part(t, r, wv):
        c = pl.ds(pl.multiple_of(t * (HPT * E), HPT * E), HPT * E)
        lhs = hbuf[r * PPV:(r + 1) * PPV, MW:PW, :].reshape(PPV * XW, DM)
        if r == 0:
            lhs = jnp.concatenate([hbuf[0, 0:MW, :], lhs], axis=0)
        lhs = unpack(lhs)
        toks, outs = [], []
        kh = DM // 2
        for w in wv:
            p0 = jnp.dot(lhs[:, :kh], w[:kh], preferred_element_type=F32)
            p1 = jnp.dot(lhs[:, kh:], w[kh:], preferred_element_type=F32)
            toks += [p[8 * g:8 * g + 8] for p in (p0, p1) for g in range(p.shape[0] // 8)]
            outs.append(p0 + p1)
        vv = jnp.concatenate(outs, axis=1).astype(BF16)
        vx = vv[MR:] if r == 0 else vv
        vbuf[r * PPV:(r + 1) * PPV, MR:PR, c] = vx.reshape(PPV, XR, HPT * E)
        ts = jnp.sum(vx.astype(F32).reshape(2 * PPV, SEG, HPT * E), axis=1)
        if r == 0:
            t0 = jnp.sum(vv[0:MR].astype(F32), axis=0, keepdims=True)
            rows = lax.broadcasted_iota(jnp.int32, ts.shape, 0)
            ts = ts + jnp.where(rows == 0, t0, 0.0)
        tsum[2 * PPV * r:2 * PPV * (r + 1), c] = ts
        return toks

    GA = 4

    def freq_items(m, never, zoff):
        r_re = pl.ds(pl.multiple_of(zoff + 16 * m, 8), 8)
        r_im = pl.ds(pl.multiple_of(zoff + 16 * m + 8, 8), 8)

        def item(tok, a0, cc, st):
            xr = jnp.where(never, tok, xf[r_re, cc * BLK:(cc + 1) * BLK])
            xi = xf[r_im, cc * BLK:(cc + 1) * BLK]
            for a in range(max(a0, cc), a0 + GA):
                j = a - cc
                if ('g', j) not in st:
                    st['g', j] = (hf[r_re, j * BLK:(j + 1) * BLK], hf[r_im, j * BLK:(j + 1) * BLK])
                gr, gi = st['g', j]
                ps = (xr * gr - xi * gi, xr * gi + xi * gr)
                st[a] = ps if a not in st else (st[a][0] + ps[0], st[a][1] + ps[1])
                if cc == a:
                    wf[16 * m:16 * m + 16, a * BLK:(a + 1) * BLK] = (
                        jnp.concatenate(st[a], axis=0).astype(BF16))

        items = []
        for a0 in range(0, NB, GA):
            st = {}
            items += [functools.partial(item, a0=a0, cc=cc, st=st) for cc in range(a0 + GA)]
        return items

    def tile_body(t, carry):
        sl = t % 2

        for cp in a_copies(t, sl):
            cp.wait()

        for i in range(1, NSLAB):
            @pl.when(t == ((i - 1) * CPS) // CPT)
            def _():
                stage_copy(i).wait()

        @pl.when(t + 1 < NT)
        def _():
            for cp in a_copies(t + 1, 1 - sl):
                cp.start()

        for i, ts_ in ((2, 0), (3, 1), (4, 2), (5, 4)):
            @pl.when(t == ts_)
            def _():
                stage_copy(i).start()

        for j in range(HPT):
            wo_copy(t * HPT + j).start()

        @pl.when(t >= 2)
        def _():
            aout_copy(t - 2, sl).wait()

        c = pl.ds(pl.multiple_of(t * LANES, LANES), LANES)
        taps = shift_ref[:, c].astype(F32)
        dcol = d_ref[...].astype(F32)
        rows = lax.broadcasted_iota(jnp.int32, dcol.shape, 0)
        dvec = jnp.sum(jnp.where(rows == t, dcol, 0.0), axis=0, keepdims=True)

        never = zero_v[...] > 0
        zoff = zero_s[0]
        wv = wpair(WV, t * (HPT // 2)) + wpair(WV, t * (HPT // 2) + 1)

        toks = v_part(t, 0, wv)

        kf[8:8 + S, :] = ak[sl].astype(F32)
        tapb = [jnp.broadcast_to(taps[j:j + 1, :], (8, LANES)) for j in range(4)]

        def conv_item(tok, r0):
            halves = []
            for h in range(2):
                r = 8 + r0 + 8 * h
                ks = kf[r:r + 8, :] * jnp.where(never, tok, tapb[0])
                for j in range(1, 4):
                    ks = ks + kf[r - j:r - j + 8, :] * tapb[j]
                halves.append(ks)
            kvb[r0:r0 + 16, :] = (jnp.concatenate(halves, axis=0)
                                  * av[sl, r0:r0 + 16, :].astype(F32)).astype(BF16)

        run_paced([functools.partial(conv_item, r0=r0) for r0 in range(0, S, 16)], toks)

        fwd = fwd_ref[...]
        hst = jnp.concatenate([ah[sl, :, b * BLK:(b + 1) * BLK] for b in range(NB)], axis=0)
        hh = lax.dot_general(fwd, hst, (((1,), (1,)), ((), ())), preferred_element_type=F32)
        for m in range(BLK // 8):
            hr = hh[16 * m:16 * m + 8]
            hi = hh[16 * m + 8:16 * m + 16]
            hf[16 * m:16 * m + 16, 0:BLK] = hh[16 * m:16 * m + 16, 0:BLK]
            if m < BLK // 16:
                hf[16 * m:16 * m + 8, BLK:] = hr[:, BLK:] - hi[:, :S - BLK]
                hf[16 * m + 8:16 * m + 16, BLK:] = hi[:, BLK:] + hr[:, :S - BLK]
            else:
                hf[16 * m:16 * m + 8, BLK:] = hr[:, BLK:] + hi[:, :S - BLK]
                hf[16 * m + 8:16 * m + 16, BLK:] = hi[:, BLK:] - hr[:, :S - BLK]
        rhs = jnp.concatenate([kvb[b * BLK:(b + 1) * BLK, :] for b in range(NB)], axis=1)
        xf[...] = jnp.dot(fwd, rhs, preferred_element_type=F32)

        toks = []
        for r in range(1, NVP - 1):
            toks += v_part(t, r, wv)
        items = []
        for m in range(BLK // 8):
            items += freq_items(m, never, zoff)
        run_paced(items, toks[:-80])
        items = []
        for k in range(CPT):
            ch = t * CPT + k
            items += relayout_items(1 + ch // CPS, (ch % CPS) * RCH, RCH, never)
        run_paced(items, toks[1:])

        y = jnp.dot(inv_ref[...], wf[...], preferred_element_type=F32)
        v_part(t, NVP - 1, wv)
        for b in range(NB):
            r0 = b * BLK
            yb = y[:, r0:r0 + BLK] + kvb[r0:r0 + BLK, :].astype(F32) * dvec
            aout[sl, r0:r0 + BLK, :] = (aq[sl, r0:r0 + BLK, :].astype(F32) * yb).astype(BF16)
        aout_copy(t, sl).start()
        return carry

    lax.fori_loop(0, NT, tile_body, 0)
    aout_copy(NT - 2, 0).wait()
    aout_copy(NT - 1, 1).wait()
    pltpu.make_async_copy(wo, wo, sem_wo).wait()

    puni = pl.reciprocal(jnp.full((1, 1), float(L), F32), approx=True).astype(BF16).astype(F32)

    def shift_down(m):
        rows = lax.broadcasted_iota(jnp.int32, m.shape, 0)
        return jnp.where(rows == 0, 0.0, pltpu.roll(m, 1, 0))

    m1 = shift_down(jnp.dot((tsum[...] * puni).astype(BF16), unpack(wo[...]), preferred_element_type=F32))
    v1 = jnp.dot(m1.astype(BF16), wmat(WV, 0, H), preferred_element_type=F32)
    v1 = v1.astype(BF16).astype(F32)
    u2 = ((tsum[...] + float(M) * v1) * puni).astype(BF16)
    m2 = shift_down(jnp.dot(u2, unpack(wo[...]), preferred_element_type=F32))
    mhat[...] = jnp.broadcast_to(m2[:, None, :], (NSEG, M, DM)).reshape(NSEG * M, DM)
    mhat[0:M, :] = mem0

    ri = lax.broadcasted_iota(jnp.int32, (PR, PR), 0)
    ci = lax.broadcasted_iota(jnp.int32, (PR, PR), 1)

    def seg_of(r):
        return jnp.where(r < MR, r // M, (r - MR) // SEG)

    def pos_of(r):
        return jnp.where(r < MR, r % M, M + (r - MR) % SEG)

    same = seg_of(ri) == seg_of(ci)
    allowed = same & ((ri < MR) | (pos_of(ri) >= pos_of(ci)))
    fill = jnp.where(same, -1e9, -jnp.inf).astype(F32)

    def sweep(state):
        it, _ = state
        hbuf[:, 0:MW, :] = pack(mhat[...]).reshape(NP, MW, DM)

        def vm_body(g, cy):
            c = pl.ds(pl.multiple_of(g * (8 * E), 8 * E), 8 * E)
            lhs = unpack(hbuf[:, 0:MW, :].reshape(NP * MW, DM))
            vv = jnp.dot(lhs, wmat(WV, g * 8, 8), preferred_element_type=F32).astype(BF16)
            vbuf[:, 0:MR, c] = vv.reshape(NP, MR, 8 * E)
            return cy

        lax.fori_loop(0, H // 8, vm_body, 0)

        NG = H // G

        def qk_proj(i, j):
            p0 = pl.multiple_of((i // NG) * PPB, PPB)
            sp = (i % NG) * (G // 2) + j // 2
            lhs = unpack(hbuf[pl.ds(p0, PPB)].reshape(PPB * PW, DM))
            wqk = jnp.concatenate([wpair(WQ, sp)[j % 2], wpair(WK, sp)[j % 2]], axis=1)
            qk = jnp.dot(lhs, wqk, preferred_element_type=F32).astype(BF16)
            qks[j] = qk.reshape(PPB, PR, 2 * E)

        def scores(j):
            return jnp.einsum('pqe,pke->pqk', qks[j, :, :, 0:E], qks[j, :, :, E:2 * E],
                              preferred_element_type=F32)

        def attend(i, j, s):
            p0 = pl.multiple_of((i // NG) * PPB, PPB)
            sl = (i % NG) * G + j
            s = jnp.where(allowed[None], s * scale, fill[None])
            e = jnp.exp(s - jnp.max(s, axis=-1, keepdims=True))
            p = (e * pl.reciprocal(jnp.sum(e, axis=-1, keepdims=True), approx=True)).astype(BF16)
            vh = vbuf[pl.ds(p0, PPB), :, pl.ds(pl.multiple_of(sl * E, E), E)]
            o = jnp.einsum('pqk,pke->pqe', p, vh, preferred_element_type=F32)
            return o.reshape(PPB * PR, E).astype(BF16)

        def out_proj(i, us):
            rb = i // NG
            g = i % NG
            u = jnp.concatenate(us, axis=1)
            wog = unpack(wo[pl.ds(pl.multiple_of(g * (G * E // 2), G * E // 2), G * E // 2), :])
            tot = jnp.where(g > 0, acc[...], 0.0) + jnp.dot(u, wog, preferred_element_type=F32)
            acc[...] = tot
            o3 = tot.reshape(PPB, PR, DM)
            obuf[rb] = o3[:, MR:, :].reshape(PPB * XR, DM).astype(BF16)
            mnew[pl.ds(pl.multiple_of(rb * (PPB * MR), PPB * MR), PPB * MR), :] = (
                o3[:, :MR, :].reshape(PPB * MR, DM))

        def step(i, nxt):
            s0, s1 = scores(0), scores(1)
            if nxt:
                qk_proj(i + 1, 0)
            u0, u1 = attend(i, 0, s0), attend(i, 1, s1)
            s2, s3 = scores(2), scores(3)
            if nxt:
                qk_proj(i + 1, 1)
            u2, u3 = attend(i, 2, s2), attend(i, 3, s3)
            if nxt:
                qk_proj(i + 1, 2)
                qk_proj(i + 1, 3)
            out_proj(i, [u0, u1, u2, u3])

        for j in range(G):
            qk_proj(0, j)

        def main_body(i, cy):
            step(i, True)

            @pl.when(i % NG == NG - 1)
            def _():
                o_copy(i // NG).start()

            return cy

        lax.fori_loop(0, NRB * NG - 1, main_body, 0)
        step(NRB * NG - 1, False)
        o_copy(NRB - 1).start()
        for rb in range(NRB):
            o_copy(rb).wait()

        n = (NSEG - 1) * M
        new = mnew[0:n, :]
        err = jnp.max(jnp.abs(new - mhat[M:M + n, :]), axis=1, keepdims=True)
        ref = jnp.max(jnp.abs(new), axis=1, keepdims=True)
        ok = jnp.min(jnp.where(err <= TOL * ref, 1.0, 0.0))
        mhat[M:M + n, :] = new
        return it + 1, (ok > 0.5).astype(jnp.int32)

    lax.while_loop(lambda st: jnp.logical_and(st[0] < NSEG, st[1] == 0), sweep,
                   (jnp.int32(0), jnp.int32(0)))


@functools.partial(jax.jit, static_argnames=("B_seg_len",))
def pallas_concat_heads__ssm_conv_h3__memory_aug_recurrent_mem_tr__prompt_kernel(
    A_q, A_k, A_v, A_shift_k, A_ssm_k, A_ssm_D,
    B_x, B_mem0, B_Wq, B_Wk, B_Wv, B_Wo, B_seg_len,
):
    _, S, D = A_q.shape
    DM = B_x.shape[2]
    H, E = B_Wq.shape[1], B_Wq.shape[2]
    M = B_mem0.shape[1]
    SEG = int(B_seg_len)
    NSEG = S // SEG
    NP = NSEG // 2
    PR = 2 * (M + SEG)
    PPB = 8
    assert E == LANES and H == 32 and M == 8 and SEG == 32 and A_shift_k.shape[1] == 4

    fwd, inv = _dft_mats()
    any_spec = pl.BlockSpec(memory_space=pl.ANY)
    vmem_spec = pl.BlockSpec(memory_space=pltpu.VMEM)
    scratch = [
        pltpu.VMEM((NP, PR // 2, DM), U32),
        pltpu.VMEM((NP, PR, H * E), BF16),
        pltpu.VMEM((3 * H * WPITCH, E), U32),
        pltpu.VMEM((H * E // 2, DM), U32),
        pltpu.VMEM((3, DM, 8, E), U32),
        pltpu.VMEM((4, PPB, PR, 2 * E), BF16),
        pltpu.VMEM((PPB * PR, DM), F32),
        pltpu.VMEM((NP // PPB, PPB * 2 * SEG, DM), BF16),
        pltpu.VMEM((NSEG * M, DM), F32),
        pltpu.VMEM((NSEG * M, DM), F32),
        pltpu.VMEM((NSEG, H * E), F32),
        pltpu.VMEM((2, S, LANES), BF16),
        pltpu.VMEM((2, S, LANES), BF16),
        pltpu.VMEM((2, S, LANES), BF16),
        pltpu.VMEM((2, LANES, S), BF16),
        pltpu.VMEM((S + 8, LANES), F32),
        pltpu.VMEM((S, LANES), BF16),
        pltpu.VMEM((NFFT, S), F32),
        pltpu.VMEM((NFFT, S), F32),
        pltpu.VMEM((NFFT, S), BF16),
        pltpu.VMEM((2, S, LANES), BF16),
        pltpu.VMEM((8, LANES), jnp.int32),
        pltpu.SMEM((1,), jnp.int32),
        pltpu.SemaphoreType.DMA,
        pltpu.SemaphoreType.DMA,
        pltpu.SemaphoreType.DMA((3,)),
        pltpu.SemaphoreType.DMA((2, 4)),
        pltpu.SemaphoreType.DMA((2,)),
        pltpu.SemaphoreType.DMA((NP // PPB,)),
    ]
    out = pl.pallas_call(
        functools.partial(_kernel, S=S, D=D, DM=DM, H=H, M=M, SEG=SEG),
        out_shape=jax.ShapeDtypeStruct((S, D + DM), BF16),
        in_specs=[any_spec, any_spec, any_spec, vmem_spec, any_spec, vmem_spec,
                  any_spec, vmem_spec, any_spec, any_spec, any_spec, any_spec,
                  vmem_spec, vmem_spec],
        out_specs=any_spec,
        scratch_shapes=scratch,
        compiler_params=pltpu.CompilerParams(vmem_limit_bytes=120 * 1024 * 1024),
    )(
        A_q.reshape(S, D), A_k.reshape(S, D), A_v.reshape(S, D),
        A_shift_k.T, A_ssm_k, A_ssm_D.reshape(D // LANES, LANES),
        B_x.reshape(NP, 2 * SEG, DM), B_mem0.reshape(M, DM),
        B_Wq, B_Wk, B_Wv, B_Wo.reshape(H * E, DM),
        jnp.asarray(fwd, BF16), jnp.asarray(inv, BF16),
    )
    return out.reshape(1, S, D + DM)
```

```python
import functools

import numpy as np
import jax
import jax.numpy as jnp
from jax import lax
import jax.experimental.pallas as pl
import jax.experimental.pallas.tpu as pltpu

F32 = jnp.float32
BF16 = jnp.bfloat16
U32 = jnp.uint32

LANES = 128
BLK = 128
NFFT = 2 * BLK
TOL = 2.0 ** -10


def _dft_mats():
    order = np.concatenate([np.arange(0, BLK, 2), np.arange(1, BLK, 2)])
    theta = 2.0 * np.pi * (order + 0.5) / NFFT
    n = np.arange(BLK)
    c = np.cos(theta[:, None] * n[None, :])
    s = np.sin(theta[:, None] * n[None, :])
    fwd = np.zeros((NFFT, BLK))
    inv = np.zeros((BLK, NFFT))
    for m in range(BLK // 8):
        fwd[16 * m:16 * m + 8] = c[8 * m:8 * m + 8]
        fwd[16 * m + 8:16 * m + 16] = -s[8 * m:8 * m + 8]
        inv[:, 16 * m:16 * m + 8] = c[8 * m:8 * m + 8].T * (2.0 / NFFT)
        inv[:, 16 * m + 8:16 * m + 16] = -s[8 * m:8 * m + 8].T * (2.0 / NFFT)
    return fwd.astype(np.float32), inv.astype(np.float32)


def _dot(a, b):
    return jnp.dot(a, b, preferred_element_type=F32)


def _pack(x):
    return pltpu.bitcast(x.astype(BF16), U32)


def _unpack(w):
    return pltpu.bitcast(w, BF16)


def _lo(w):
    return pltpu.bitcast(w << 16, F32)


def _hi(w):
    return pltpu.bitcast(w & jnp.uint32(0xFFFF0000), F32)


def _strassen_lhs(a11, a12, a21, a22):
    return [a11 + a22, a21 + a22, a11, a22, a11 + a12, a21 - a11, a12 - a22]


def _strassen_rhs(b11, b12, b21, b22):
    ops = [b11 + b22, b11, b12 - b22, b21 - b11, b22, b11 + b12, b21 + b22]
    return [o.astype(BF16) for o in ops]


def _strassen(lhs, rhs, init=None):
    def add(c, m):
        return m if c is None else c + m

    c11, c12, c21, c22 = init if init is not None else (None,) * 4
    m7 = _dot(lhs(6), rhs[6])
    c11 = add(c11, m7)
    m5 = _dot(lhs(4), rhs[4])
    c11 = c11 - m5
    c12 = add(c12, m5)
    m3 = _dot(lhs(2), rhs[2])
    c12 = c12 + m3
    c22 = add(c22, m3)
    m6 = _dot(lhs(5), rhs[5])
    c22 = c22 + m6
    m2 = _dot(lhs(1), rhs[1])
    c22 = c22 - m2
    c21 = add(c21, m2)
    m4 = _dot(lhs(3), rhs[3])
    c21 = c21 + m4
    c11 = c11 + m4
    m1 = _dot(lhs(0), rhs[0])
    c11 = c11 + m1
    c22 = c22 + m1
    return (c11, c12, c21, c22), [m7, m5, m3, m6, m2, m4, m1]


def _run_paced(items, toks):
    for i, it in enumerate(items):
        it(toks[i * len(toks) // len(items)])


def _kernel(q_hbm, k_hbm, v_hbm, shift_ref, h_hbm, d_ref, x_hbm, mem0_ref,
            wq_hbm, wk_hbm, wv_hbm, wo_hbm, fwd_ref, inv_ref,
            out_hbm,
            abuf, mbuf, vbuf, w32, wo, qks, acc, obuf, mhat, mnew, tsum,
            ain, ah, kf, kvb, xf, hf, wf, aout, zero_v, zero_s,
            sem_x, sem_wv, sem_wqk, sem_wo, sem_a, sem_aout, sem_o,
            *, S, D, DM, H, M, SEG):
    E = LANES
    NSEG = S // SEG
    NP = NSEG // 2
    MR = 2 * M
    XR = 2 * SEG
    PR = MR + XR
    MW, XW, PW = MR // 2, XR // 2, PR // 2
    L = M + SEG
    NB = S // BLK
    NT = D // LANES
    PPB = 8
    PPH = PPB // 2
    NRB = NP // PPB
    G = 4
    NG = H // G
    KH = DM // 2
    scale = float(E) ** -0.5
    WV, WQ, WK = 0, 1, 2

    def x_copy(rb):
        return pltpu.make_async_copy(x_hbm.at[rb], obuf.at[rb], sem_x.at[rb])

    def w_copy(which, hp):
        src = (wv_hbm, wq_hbm, wk_hbm)[which].bitcast(U32)
        sem = sem_wv.at[hp] if which == WV else sem_wqk
        return pltpu.make_async_copy(src.at[:, hp, :], w32.at[which, hp], sem)

    def wo_copy(t):
        n = H * E // NT
        r = pl.ds(pl.multiple_of(t * n, n), n)
        return pltpu.make_async_copy(wo_hbm.at[r, :], wo.at[r, :], sem_wo)

    def a_start(t, sl):
        c = pl.ds(pl.multiple_of(t * LANES, LANES), LANES)
        pltpu.make_async_copy(k_hbm.at[:, c], ain.at[sl, 0], sem_a.at[sl, 0]).start()
        pltpu.make_async_copy(v_hbm.at[:, c], ain.at[sl, 1], sem_a.at[sl, 0]).start()
        pltpu.make_async_copy(h_hbm.at[c, :], ah.at[sl], sem_a.at[sl, 1]).start()
        pltpu.make_async_copy(q_hbm.at[:, c], ain.at[sl, 2], sem_a.at[sl, 0]).start()

    def a_wait(sl):
        pltpu.make_async_copy(ain.at[sl], ain.at[sl], sem_a.at[sl, 0]).wait()
        pltpu.make_async_copy(ah.at[sl], ah.at[sl], sem_a.at[sl, 1]).wait()

    def aout_copy(t):
        c = pl.ds(pl.multiple_of(t * LANES, LANES), LANES)
        return pltpu.make_async_copy(aout.at[t], out_hbm.at[:, c], sem_aout)

    def o_copy(rb):
        r = pl.ds(pl.multiple_of(rb * (PPB * XR), PPB * XR), PPB * XR)
        return pltpu.make_async_copy(obuf.at[rb], out_hbm.at[r, pl.ds(D, DM)], sem_o.at[rb])

    def w_rhs(which, hp):
        w = w32[which, hp]
        return _strassen_rhs(_lo(w[:KH]), _hi(w[:KH]), _lo(w[KH:]), _hi(w[KH:]))

    def w_plain(which, hp0, n):
        parts = []
        for j in range(n):
            w = w32[which, hp0 + j]
            parts += [_lo(w), _hi(w)]
        return jnp.concatenate(parts, axis=1).astype(BF16)

    for rb in range(NRB):
        x_copy(rb).start()
    w_copy(WV, 0).start()
    w_copy(WV, 1).start()
    a_start(0, 0)

    kf[0:8, :] = jnp.zeros((8, LANES), F32)
    zero_v[...] = jnp.zeros((8, LANES), jnp.int32)
    zero_s[0] = 0
    mem0 = mem0_ref[...].astype(F32)
    m0 = jnp.concatenate([mem0, jnp.zeros_like(mem0)], axis=0)
    z0 = jnp.zeros((MR, KH), F32)
    for k, op in enumerate(_strassen_lhs(m0[:, :KH], m0[:, KH:], z0, z0)):
        abuf[0, k, 0, 0:MW, :] = _pack(op)

    def x_prep(i, cy):
        rb = i // PPH
        pp = i % PPH

        @pl.when(pp == 0)
        def _():
            x_copy(rb).wait()

        top = obuf[rb, pl.ds(pl.multiple_of(pp * XR, XR), XR), :].astype(F32)
        bot = obuf[rb, pl.ds(pl.multiple_of((PPH + pp) * XR, XR), XR), :].astype(F32)
        for k, op in enumerate(_strassen_lhs(top[:, :KH], top[:, KH:], bot[:, :KH], bot[:, KH:])):
            abuf[rb, k, pp, MW:PW, :] = _pack(op)
        return cy

    lax.fori_loop(0, NRB * PPH, x_prep, 0)

    def v_part(hp, rb, rhs):
        def lhs(k):
            x = abuf[rb, k, :, MW:PW, :].reshape(PPH * XW, KH)
            if rb == 0:
                x = jnp.concatenate([abuf[0, k, 0, 0:MW, :], x], axis=0)
            return _unpack(x)

        (c11, c12, c21, c22), ms = _strassen(lhs, rhs)
        c = pl.ds(pl.multiple_of(hp * (2 * E), 2 * E), 2 * E)
        top = jnp.concatenate([c11, c12], axis=1).astype(BF16)
        bot = jnp.concatenate([c21, c22], axis=1).astype(BF16)
        for half, vv in enumerate((top, bot)):
            vx = vv[MR:] if rb == 0 else vv
            p0 = rb * PPB + half * PPH
            vbuf[p0:p0 + PPH, MR:PR, c] = vx.reshape(PPH, XR, 2 * E)
            ts = jnp.sum(vx.astype(F32).reshape(2 * PPH, SEG, 2 * E), axis=1)
            if rb == 0 and half == 0:
                vbuf[0, 0:M, c] = vv[0:M]
                t0 = jnp.sum(vv[0:M].astype(F32), axis=0, keepdims=True)
                rows = lax.broadcasted_iota(jnp.int32, ts.shape, 0)
                ts = ts + jnp.where(rows == 0, t0, 0.0)
            tsum[2 * p0:2 * (p0 + PPH), c] = ts
        return [m[8 * g:8 * g + 8] for m in ms for g in range(m.shape[0] // 8)]

    GA = 4

    def freq_items(m, never, zoff):
        r_re = pl.ds(pl.multiple_of(zoff + 16 * m, 8), 8)
        r_im = pl.ds(pl.multiple_of(zoff + 16 * m + 8, 8), 8)

        def item(tok, a0, cc, st):
            xr = jnp.where(never, tok, xf[r_re, cc * BLK:(cc + 1) * BLK])
            xi = xf[r_im, cc * BLK:(cc + 1) * BLK]
            for a in range(max(a0, cc), a0 + GA):
                j = a - cc
                if ('g', j) not in st:
                    st['g', j] = (hf[r_re, j * BLK:(j + 1) * BLK], hf[r_im, j * BLK:(j + 1) * BLK])
                gr, gi = st['g', j]
                ps = (xr * gr - xi * gi, xr * gi + xi * gr)
                st[a] = ps if a not in st else (st[a][0] + ps[0], st[a][1] + ps[1])
                if cc == a:
                    wf[16 * m:16 * m + 16, a * BLK:(a + 1) * BLK] = (
                        jnp.concatenate(st[a], axis=0).astype(BF16))

        items = []
        for a0 in range(0, NB, GA):
            st = {}
            items += [functools.partial(item, a0=a0, cc=cc, st=st) for cc in range(a0 + GA)]
        return items

    def tile_body(t, carry):
        sl = t % 2
        a_wait(sl)
        w_copy(WV, 2 * t).wait()
        w_copy(WV, 2 * t + 1).wait()

        @pl.when(t + 1 < NT)
        def _():
            w_copy(WV, 2 * t + 2).start()
            w_copy(WV, 2 * t + 3).start()
            a_start(t + 1, 1 - sl)

        wo_copy(t).start()
        for which in (WQ, WK):
            w_copy(which, 2 * t).start()
            w_copy(which, 2 * t + 1).start()

        c = pl.ds(pl.multiple_of(t * LANES, LANES), LANES)
        taps = shift_ref[:, c].astype(F32)
        dcol = d_ref[...].astype(F32)
        rows = lax.broadcasted_iota(jnp.int32, dcol.shape, 0)
        dvec = jnp.sum(jnp.where(rows == t, dcol, 0.0), axis=0, keepdims=True)
        never = zero_v[...] > 0
        zoff = zero_s[0]

        rhs2 = [w_rhs(WV, 2 * t), w_rhs(WV, 2 * t + 1)]
        parts = [(j, rb) for j in range(2) for rb in range(NRB)]

        def run_part(i):
            j, rb = parts[i]
            return v_part(2 * t + j, rb, rhs2[j])

        toks = run_part(0)

        kf[8:8 + S, :] = ain[sl, 0].astype(F32)
        tapb = [jnp.broadcast_to(taps[j:j + 1, :], (8, LANES)) for j in range(4)]

        def conv_item(tok, r0):
            halves = []
            for h in range(2):
                r = 8 + r0 + 8 * h
                ks = kf[r:r + 8, :] * jnp.where(never, tok, tapb[0])
                for j in range(1, 4):
                    ks = ks + kf[r - j:r - j + 8, :] * tapb[j]
                halves.append(ks)
            kvb[r0:r0 + 16, :] = (jnp.concatenate(halves, axis=0)
                                  * ain[sl, 1, r0:r0 + 16, :].astype(F32)).astype(BF16)

        _run_paced([functools.partial(conv_item, r0=r0) for r0 in range(0, S, 16)], toks)

        fwd = fwd_ref[...]
        hst = jnp.concatenate([ah[sl, :, b * BLK:(b + 1) * BLK] for b in range(NB)], axis=0)
        hh = lax.dot_general(fwd, hst, (((1,), (1,)), ((), ())), preferred_element_type=F32)
        for m in range(BLK // 8):
            hr = hh[16 * m:16 * m + 8]
            hi = hh[16 * m + 8:16 * m + 16]
            hf[16 * m:16 * m + 16, 0:BLK] = hh[16 * m:16 * m + 16, 0:BLK]
            if m < BLK // 16:
                hf[16 * m:16 * m + 8, BLK:] = hr[:, BLK:] - hi[:, :S - BLK]
                hf[16 * m + 8:16 * m + 16, BLK:] = hi[:, BLK:] + hr[:, :S - BLK]
            else:
                hf[16 * m:16 * m + 8, BLK:] = hr[:, BLK:] + hi[:, :S - BLK]
                hf[16 * m + 8:16 * m + 16, BLK:] = hi[:, BLK:] - hr[:, :S - BLK]
        rhs = jnp.concatenate([kvb[b * BLK:(b + 1) * BLK, :] for b in range(NB)], axis=1)
        xf[...] = _dot(fwd, rhs)

        toks = []
        for i in range(1, len(parts) - 1):
            toks += run_part(i)
        items = []
        for m in range(BLK // 8):
            items += freq_items(m, never, zoff)
        _run_paced(items, toks[:-80])

        y = _dot(inv_ref[...], wf[...])
        run_part(len(parts) - 1)
        for b in range(NB):
            r0 = b * BLK
            yb = y[:, r0:r0 + BLK] + kvb[r0:r0 + BLK, :].astype(F32) * dvec
            aout[t, r0:r0 + BLK, :] = (ain[sl, 2, r0:r0 + BLK, :].astype(F32) * yb).astype(BF16)
        aout_copy(t).start()
        return carry

    lax.fori_loop(0, NT, tile_body, 0)
    pltpu.make_async_copy(wo, wo, sem_wo).wait()
    pltpu.make_async_copy(w32.at[WQ:WK + 1], w32.at[WQ:WK + 1], sem_wqk).wait()

    puni = pl.reciprocal(jnp.full((1, 1), float(L), F32), approx=True).astype(BF16).astype(F32)

    def shift_down(m):
        rows = lax.broadcasted_iota(jnp.int32, m.shape, 0)
        return jnp.where(rows == 0, 0.0, pltpu.roll(m, 1, 0))

    m1 = shift_down(_dot((tsum[...] * puni).astype(BF16), wo[...]))
    v1 = _dot(m1.astype(BF16), w_plain(WV, 0, H // 2)).astype(BF16).astype(F32)
    u2 = ((tsum[...] + float(M) * v1) * puni).astype(BF16)
    m2 = shift_down(_dot(u2, wo[...]))
    mhat[...] = jnp.broadcast_to(m2[:, None, :], (NSEG, M, DM)).reshape(NSEG * M, DM)
    mhat[0:M, :] = mem0

    ri = lax.broadcasted_iota(jnp.int32, (PR, PR), 0)
    ci = lax.broadcasted_iota(jnp.int32, (PR, PR), 1)

    def seg_of(r):
        return jnp.where(r < MR, r // M, (r - MR) // SEG)

    def pos_of(r):
        return jnp.where(r < MR, r % M, M + (r - MR) % SEG)

    same = seg_of(ri) == seg_of(ci)
    allowed = same & ((ri < MR) | (pos_of(ri) >= pos_of(ci)))
    fill = jnp.where(same, -1e9, -jnp.inf).astype(F32)

    def sweep(state):
        it, _ = state
        mbuf[...] = mhat[...].astype(BF16)

        def vm_body(g, cy):
            c = pl.ds(pl.multiple_of(g * (8 * E), 8 * E), 8 * E)
            vv = _dot(mbuf[...], w_plain(WV, g * 4, 4)).astype(BF16)
            vbuf[0, M:MR, c] = vv[M:MR]
            vbuf[1:, 0:MR, c] = vv[MR:].reshape(NP - 1, MR, 8 * E)
            n = PPH * MR
            top = mbuf[pl.ds(pl.multiple_of(2 * g * n, n), n), :].astype(F32)
            bot = mbuf[pl.ds(pl.multiple_of((2 * g + 1) * n, n), n), :].astype(F32)
            ops = _strassen_lhs(top[:, :KH], top[:, KH:], bot[:, :KH], bot[:, KH:])
            for k, op in enumerate(ops):
                abuf[g, k, :, 0:MW, :] = _pack(op).reshape(PPH, MW, KH)
            return cy

        assert NRB == H // 8
        lax.fori_loop(0, NRB, vm_body, 0)

        def qk_proj(i, j):
            rb = i // NG
            hp = (i % NG) * (G // 2) + j // 2

            def lhs(k):
                return _unpack(abuf[rb, k].reshape(PPH * PW, KH))

            (c11, c12, c21, c22), _ = _strassen(lhs, w_rhs(WQ + j % 2, hp))
            qks[j, 0:PPH] = jnp.concatenate([c11, c12], axis=1).astype(BF16).reshape(PPH, PR, 2 * E)
            qks[j, PPH:PPB] = jnp.concatenate([c21, c22], axis=1).astype(BF16).reshape(PPH, PR, 2 * E)

        def scores(j):
            c = slice((j % 2) * E, (j % 2 + 1) * E)
            return lax.dot_general(qks[2 * (j // 2), :, :, c], qks[2 * (j // 2) + 1, :, :, c],
                                   (((2,), (2,)), ((0,), (0,))), preferred_element_type=F32)

        def attend(i, j, s):
            p0 = pl.multiple_of((i // NG) * PPB, PPB)
            h = (i % NG) * G + j
            s = jnp.where(allowed[None], s * scale, fill[None])
            e = jnp.exp(s - jnp.max(s, axis=-1, keepdims=True))
            p = (e * pl.reciprocal(jnp.sum(e, axis=-1, keepdims=True), approx=True)).astype(BF16)
            vh = vbuf[pl.ds(p0, PPB), :, pl.ds(pl.multiple_of(h * E, E), E)]
            return lax.dot_general(p, vh, (((2,), (1,)), ((0,), (0,))), preferred_element_type=F32)

        def out_proj(i, us):
            rb = i // NG
            g = i % NG
            u = jnp.concatenate(us, axis=2)
            wog = wo[pl.ds(pl.multiple_of(g * (G * E), G * E), G * E), :]
            rm = pl.ds(pl.multiple_of(rb * (PPB * MR), PPB * MR), PPB * MR)
            um = u[:, :MR, :].reshape(PPB * MR, G * E).astype(BF16)
            mnew[rm, :] = jnp.where(g > 0, mnew[rm, :], 0.0) + _dot(um, wog)
            n = PPH * XR
            kh = G * E // 2
            top = u[:PPH, MR:, :].reshape(n, G * E)
            bot = u[PPH:, MR:, :].reshape(n, G * E)
            ops = _strassen_lhs(top[:, :kh], top[:, kh:], bot[:, :kh], bot[:, kh:])
            wf32 = wog.astype(F32)
            rhs = _strassen_rhs(wf32[:kh, :KH], wf32[:kh, KH:], wf32[kh:, :KH], wf32[kh:, KH:])
            quads = [(slice(0, n), slice(0, KH)), (slice(0, n), slice(KH, DM)),
                     (slice(n, 2 * n), slice(0, KH)), (slice(n, 2 * n), slice(KH, DM))]
            init = [jnp.where(g > 0, acc[r, c], 0.0) for r, c in quads]
            cs, _ = _strassen(lambda k: ops[k].astype(BF16), rhs, init)
            for (r, c), v in zip(quads, cs):
                acc[r, c] = v
                obuf[rb, r, c] = v.astype(BF16)

        def step(i, nxt):
            s0, s1 = scores(0), scores(1)
            if nxt:
                qk_proj(i + 1, 0)
            u0, u1 = attend(i, 0, s0), attend(i, 1, s1)
            s2, s3 = scores(2), scores(3)
            if nxt:
                qk_proj(i + 1, 1)
            u2, u3 = attend(i, 2, s2), attend(i, 3, s3)
            if nxt:
                qk_proj(i + 1, 2)
                qk_proj(i + 1, 3)
            out_proj(i, [u0, u1, u2, u3])

        for j in range(G):
            qk_proj(0, j)

        def main_body(i, cy):
            step(i, True)

            @pl.when(i % NG == NG - 1)
            def _():
                o_copy(i // NG).start()

            return cy

        lax.fori_loop(0, NRB * NG - 1, main_body, 0)
        step(NRB * NG - 1, False)
        o_copy(NRB - 1).start()

        n = (NSEG - 1) * M
        new = mnew[0:n, :]
        err = jnp.max(jnp.abs(new - mhat[M:M + n, :]), axis=1, keepdims=True)
        ref = jnp.max(jnp.abs(new), axis=1, keepdims=True)
        ok = jnp.min(jnp.where(err <= TOL * ref, 1.0, 0.0))
        mhat[M:M + n, :] = new
        for rb in range(NRB):
            o_copy(rb).wait()
        return it + 1, (ok > 0.5).astype(jnp.int32)

    lax.while_loop(lambda st: jnp.logical_and(st[0] < NSEG, st[1] == 0), sweep,
                   (jnp.int32(0), jnp.int32(0)))
    pltpu.make_async_copy(aout, aout, sem_aout).wait()


@functools.partial(jax.jit, static_argnames=("B_seg_len",))
def pallas_concat_heads__ssm_conv_h3__memory_aug_recurrent_mem_tr__prompt_kernel(
    A_q, A_k, A_v, A_shift_k, A_ssm_k, A_ssm_D,
    B_x, B_mem0, B_Wq, B_Wk, B_Wv, B_Wo, B_seg_len,
):
    _, S, D = A_q.shape
    DM = B_x.shape[2]
    H, E = B_Wq.shape[1], B_Wq.shape[2]
    M = B_mem0.shape[1]
    SEG = int(B_seg_len)
    NSEG = S // SEG
    NP = NSEG // 2
    PR = 2 * (M + SEG)
    PPB = 8
    NRB = NP // PPB
    NT = D // LANES
    assert E == LANES and H == 32 and M == 8 and SEG == 32 and A_shift_k.shape[1] == 4
    assert S == 2048 and D == 1024 and DM == 1024

    fwd, inv = _dft_mats()
    any_spec = pl.BlockSpec(memory_space=pl.ANY)
    vmem_spec = pl.BlockSpec(memory_space=pltpu.VMEM)
    scratch = [
        pltpu.VMEM((NRB, 7, PPB // 2, PR // 2, DM // 2), U32),
        pltpu.VMEM((NSEG * M, DM), BF16),
        pltpu.VMEM((NP, PR, H * E), BF16),
        pltpu.VMEM((3, H // 2, DM, E), U32),
        pltpu.VMEM((H * E, DM), BF16),
        pltpu.VMEM((4, PPB, PR, 2 * E), BF16),
        pltpu.VMEM((PPB * 2 * SEG, DM), F32),
        pltpu.VMEM((NRB, PPB * 2 * SEG, DM), BF16),
        pltpu.VMEM((NSEG * M, DM), F32),
        pltpu.VMEM((NSEG * M, DM), F32),
        pltpu.VMEM((NSEG, H * E), F32),
        pltpu.VMEM((2, 3, S, LANES), BF16),
        pltpu.VMEM((2, LANES, S), BF16),
        pltpu.VMEM((S + 8, LANES), F32),
        pltpu.VMEM((S, LANES), BF16),
        pltpu.VMEM((NFFT, S), F32),
        pltpu.VMEM((NFFT, S), F32),
        pltpu.VMEM((NFFT, S), BF16),
        pltpu.VMEM((NT, S, LANES), BF16),
        pltpu.VMEM((8, LANES), jnp.int32),
        pltpu.SMEM((1,), jnp.int32),
        pltpu.SemaphoreType.DMA((NRB,)),
        pltpu.SemaphoreType.DMA((H // 2,)),
        pltpu.SemaphoreType.DMA,
        pltpu.SemaphoreType.DMA,
        pltpu.SemaphoreType.DMA((2, 2)),
        pltpu.SemaphoreType.DMA,
        pltpu.SemaphoreType.DMA((NRB,)),
    ]
    out = pl.pallas_call(
        functools.partial(_kernel, S=S, D=D, DM=DM, H=H, M=M, SEG=SEG),
        out_shape=jax.ShapeDtypeStruct((S, D + DM), BF16),
        in_specs=[any_spec, any_spec, any_spec, vmem_spec, any_spec, vmem_spec,
                  any_spec, vmem_spec, any_spec, any_spec, any_spec, any_spec,
                  vmem_spec, vmem_spec],
        out_specs=any_spec,
        scratch_shapes=scratch,
        compiler_params=pltpu.CompilerParams(vmem_limit_bytes=120 * 1024 * 1024),
    )(
        A_q.reshape(S, D), A_k.reshape(S, D), A_v.reshape(S, D),
        A_shift_k.T, A_ssm_k, A_ssm_D.reshape(NT, LANES),
        B_x.reshape(NRB, S // NRB, DM), B_mem0.reshape(M, DM),
        B_Wq, B_Wk, B_Wv, B_Wo.reshape(H * E, DM),
        jnp.asarray(fwd, BF16), jnp.asarray(inv, BF16),
    )
    return out.reshape(1, S, D + DM)
```

```python
import functools

import numpy as np
import jax
import jax.numpy as jnp
from jax import lax
import jax.experimental.pallas as pl
import jax.experimental.pallas.tpu as pltpu

F32 = jnp.float32
BF16 = jnp.bfloat16
U32 = jnp.uint32

LANES = 128
BLK = 128
NFFT = 2 * BLK
TOL = 2.0 ** -10


def _dft_mats():
    order = np.concatenate([np.arange(0, BLK, 2), np.arange(1, BLK, 2)])
    theta = 2.0 * np.pi * (order + 0.5) / NFFT
    n = np.arange(BLK)
    c = np.cos(theta[:, None] * n[None, :])
    s = np.sin(theta[:, None] * n[None, :])
    fwd = np.zeros((NFFT, BLK))
    inv = np.zeros((BLK, NFFT))
    for m in range(BLK // 8):
        fwd[16 * m:16 * m + 8] = c[8 * m:8 * m + 8]
        fwd[16 * m + 8:16 * m + 16] = -s[8 * m:8 * m + 8]
        inv[:, 16 * m:16 * m + 8] = c[8 * m:8 * m + 8].T * (2.0 / NFFT)
        inv[:, 16 * m + 8:16 * m + 16] = -s[8 * m:8 * m + 8].T * (2.0 / NFFT)
    return fwd.astype(np.float32), inv.astype(np.float32)


def _dot(a, b):
    return jnp.dot(a, b, preferred_element_type=F32)


def _pack(x):
    return pltpu.bitcast(x.astype(BF16), U32)


def _unpack(w):
    return pltpu.bitcast(w, BF16)


def _lo(w):
    return pltpu.bitcast(w << 16, F32)


def _hi(w):
    return pltpu.bitcast(w & jnp.uint32(0xFFFF0000), F32)


def _strassen_lhs(a11, a12, a21, a22):
    return [a11 + a22, a21 + a22, a11, a22, a11 + a12, a21 - a11, a12 - a22]


def _strassen_rhs(b11, b12, b21, b22):
    ops = [b11 + b22, b11, b12 - b22, b21 - b11, b22, b11 + b12, b21 + b22]
    return [o.astype(BF16) for o in ops]


def _strassen(lhs, rhs, init=None):
    def add(c, m):
        return m if c is None else c + m

    c11, c12, c21, c22 = init if init is not None else (None,) * 4
    m7 = _dot(lhs(6), rhs[6])
    c11 = add(c11, m7)
    m5 = _dot(lhs(4), rhs[4])
    c11 = c11 - m5
    c12 = add(c12, m5)
    m3 = _dot(lhs(2), rhs[2])
    c12 = c12 + m3
    c22 = add(c22, m3)
    m6 = _dot(lhs(5), rhs[5])
    c22 = c22 + m6
    m2 = _dot(lhs(1), rhs[1])
    c22 = c22 - m2
    c21 = add(c21, m2)
    m4 = _dot(lhs(3), rhs[3])
    c21 = c21 + m4
    c11 = c11 + m4
    m1 = _dot(lhs(0), rhs[0])
    c11 = c11 + m1
    c22 = c22 + m1
    return (c11, c12, c21, c22), [m7, m5, m3, m6, m2, m4, m1]


def _run_paced(items, toks):
    for i, it in enumerate(items):
        it(toks[i * len(toks) // len(items)])


def _kernel(q_hbm, k_hbm, v_hbm, shift_ref, h_hbm, d_ref, x_hbm, mem0_ref,
            wq_hbm, wk_hbm, wv_hbm, wo_hbm, fwd_ref, inv_ref,
            out_hbm,
            abuf, a0buf, vbuf, v0buf, w32, wo, qks, vms, acc, obuf, mhat, mnew, tsum,
            ain, ah, kf, kvb, xf, hf, wf, aout, zero_v, zero_s,
            sem_x, sem_wv, sem_wqk, sem_wo, sem_a, sem_aout, sem_o,
            *, S, D, DM, H, M, SEG):
    E = LANES
    NSEG = S // SEG
    NP = NSEG // 2
    MR = 2 * M
    XR = 2 * SEG
    PR = MR + XR
    MW, XW, PW = MR // 2, XR // 2, PR // 2
    L = M + SEG
    NB = S // BLK
    NT = D // LANES
    PPB = 8
    PPH = PPB // 2
    NRB = NP // PPB
    G = 4
    NG = H // G
    KH = DM // 2
    scale = float(E) ** -0.5
    WV, WQ, WK = 0, 1, 2

    def x_copy(rb):
        return pltpu.make_async_copy(x_hbm.at[rb], obuf.at[rb], sem_x.at[rb])

    def w_copy(which, hp):
        src = (wv_hbm, wq_hbm, wk_hbm)[which].bitcast(U32)
        sem = sem_wv.at[hp] if which == WV else sem_wqk
        return pltpu.make_async_copy(src.at[:, hp, :], w32.at[which, hp], sem)

    def wo_copy(t):
        n = H * E // NT
        r = pl.ds(pl.multiple_of(t * n, n), n)
        return pltpu.make_async_copy(wo_hbm.at[r, :], wo.at[r, :], sem_wo)

    def a_start(t, sl):
        c = pl.ds(pl.multiple_of(t * LANES, LANES), LANES)
        pltpu.make_async_copy(k_hbm.at[:, c], ain.at[sl, 0], sem_a.at[sl, 0]).start()
        pltpu.make_async_copy(v_hbm.at[:, c], ain.at[sl, 1], sem_a.at[sl, 0]).start()
        pltpu.make_async_copy(h_hbm.at[c, :], ah.at[sl], sem_a.at[sl, 1]).start()
        pltpu.make_async_copy(q_hbm.at[:, c], ain.at[sl, 2], sem_a.at[sl, 0]).start()

    def a_wait(sl):
        pltpu.make_async_copy(ain.at[sl], ain.at[sl], sem_a.at[sl, 0]).wait()
        pltpu.make_async_copy(ah.at[sl], ah.at[sl], sem_a.at[sl, 1]).wait()

    def aout_copy(t):
        c = pl.ds(pl.multiple_of(t * LANES, LANES), LANES)
        return pltpu.make_async_copy(aout.at[t], out_hbm.at[:, c], sem_aout)

    def o_copy(rb):
        r = pl.ds(pl.multiple_of(rb * (PPB * XR), PPB * XR), PPB * XR)
        return pltpu.make_async_copy(obuf.at[rb], out_hbm.at[r, pl.ds(D, DM)], sem_o.at[rb])

    def w_rhs(which, hp):
        w = w32[which, hp]
        return _strassen_rhs(_lo(w[:KH]), _hi(w[:KH]), _lo(w[KH:]), _hi(w[KH:]))

    def w_plain(which, hp0, n):
        parts = []
        for j in range(n):
            w = w32[which, hp0 + j]
            parts += [_lo(w), _hi(w)]
        return jnp.concatenate(parts, axis=1).astype(BF16)

    for rb in range(NRB):
        x_copy(rb).start()
    w_copy(WV, 0).start()
    w_copy(WV, 1).start()
    a_start(0, 0)

    kf[0:8, :] = jnp.zeros((8, LANES), F32)
    zero_v[...] = jnp.zeros((8, LANES), jnp.int32)
    zero_s[0] = 0
    mem0 = mem0_ref[...].astype(F32)
    m0 = jnp.concatenate([mem0, jnp.zeros_like(mem0)], axis=0)
    z0 = jnp.zeros((MR, KH), F32)
    for k, op in enumerate(_strassen_lhs(m0[:, :KH], m0[:, KH:], z0, z0)):
        a0buf[k] = _pack(op)

    def x_prep(i, cy):
        rb = i // PPH
        pp = i % PPH

        @pl.when(pp == 0)
        def _():
            x_copy(rb).wait()

        top = obuf[rb, pl.ds(pl.multiple_of(pp * XR, XR), XR), :].astype(F32)
        bot = obuf[rb, pl.ds(pl.multiple_of((PPH + pp) * XR, XR), XR), :].astype(F32)
        for k, op in enumerate(_strassen_lhs(top[:, :KH], top[:, KH:], bot[:, :KH], bot[:, KH:])):
            abuf[rb, k, pl.ds(pl.multiple_of(pp * XW, XW), XW), :] = _pack(op)
        return cy

    lax.fori_loop(0, NRB * PPH, x_prep, 0)

    def v_part(hp, rb, rhs):
        def lhs(k):
            x = abuf[rb, k]
            if rb == 0:
                x = jnp.concatenate([a0buf[k], x], axis=0)
            return _unpack(x)

        (c11, c12, c21, c22), ms = _strassen(lhs, rhs)
        c = pl.ds(pl.multiple_of(hp * (2 * E), 2 * E), 2 * E)
        top = jnp.concatenate([c11, c12], axis=1).astype(BF16)
        bot = jnp.concatenate([c21, c22], axis=1).astype(BF16)
        for half, vv in enumerate((top, bot)):
            vx = vv[MR:] if rb == 0 else vv
            p0 = rb * PPB + half * PPH
            vbuf[p0:p0 + PPH, :, c] = vx.reshape(PPH, XR, 2 * E)
            ts = jnp.sum(vx.astype(F32).reshape(2 * PPH, SEG, 2 * E), axis=1)
            if rb == 0 and half == 0:
                v0 = vv[0:M].astype(F32)
                v0buf[:, c] = v0
                t0 = jnp.sum(v0, axis=0, keepdims=True)
                rows = lax.broadcasted_iota(jnp.int32, ts.shape, 0)
                ts = ts + jnp.where(rows == 0, t0, 0.0)
            tsum[2 * p0:2 * (p0 + PPH), c] = ts
        return [m[8 * g:8 * g + 8] for m in ms for g in range(m.shape[0] // 8)]

    GA = 4

    def freq_items(m, never, zoff):
        r_re = pl.ds(pl.multiple_of(zoff + 16 * m, 8), 8)
        r_im = pl.ds(pl.multiple_of(zoff + 16 * m + 8, 8), 8)

        def item(tok, a0, cc, st):
            xr = jnp.where(never, tok, xf[r_re, cc * BLK:(cc + 1) * BLK])
            xi = xf[r_im, cc * BLK:(cc + 1) * BLK]
            for a in range(max(a0, cc), a0 + GA):
                j = a - cc
                if ('g', j) not in st:
                    st['g', j] = (hf[r_re, j * BLK:(j + 1) * BLK], hf[r_im, j * BLK:(j + 1) * BLK])
                gr, gi = st['g', j]
                ps = (xr * gr - xi * gi, xr * gi + xi * gr)
                st[a] = ps if a not in st else (st[a][0] + ps[0], st[a][1] + ps[1])
                if cc == a:
                    wf[16 * m:16 * m + 16, a * BLK:(a + 1) * BLK] = (
                        jnp.concatenate(st[a], axis=0).astype(BF16))

        items = []
        for a0 in range(0, NB, GA):
            st = {}
            items += [functools.partial(item, a0=a0, cc=cc, st=st) for cc in range(a0 + GA)]
        return items

    def tile_body(t, carry):
        sl = t % 2
        a_wait(sl)
        w_copy(WV, 2 * t).wait()
        w_copy(WV, 2 * t + 1).wait()

        @pl.when(t + 1 < NT)
        def _():
            w_copy(WV, 2 * t + 2).start()
            w_copy(WV, 2 * t + 3).start()
            a_start(t + 1, 1 - sl)

        wo_copy(t).start()
        for which in (WQ, WK):
            w_copy(which, 2 * t).start()
            w_copy(which, 2 * t + 1).start()

        c = pl.ds(pl.multiple_of(t * LANES, LANES), LANES)
        taps = shift_ref[:, c].astype(F32)
        dcol = d_ref[...].astype(F32)
        rows = lax.broadcasted_iota(jnp.int32, dcol.shape, 0)
        dvec = jnp.sum(jnp.where(rows == t, dcol, 0.0), axis=0, keepdims=True)
        never = zero_v[...] > 0
        zoff = zero_s[0]

        rhs2 = [w_rhs(WV, 2 * t), w_rhs(WV, 2 * t + 1)]
        parts = [(j, rb) for j in range(2) for rb in range(NRB)]

        def run_part(i):
            j, rb = parts[i]
            return v_part(2 * t + j, rb, rhs2[j])

        toks = run_part(0)

        kf[8:8 + S, :] = ain[sl, 0].astype(F32)
        tapb = [jnp.broadcast_to(taps[j:j + 1, :], (8, LANES)) for j in range(4)]

        def conv_item(tok, r0):
            halves = []
            for h in range(2):
                r = 8 + r0 + 8 * h
                ks = kf[r:r + 8, :] * jnp.where(never, tok, tapb[0])
                for j in range(1, 4):
                    ks = ks + kf[r - j:r - j + 8, :] * tapb[j]
                halves.append(ks)
            kvb[r0:r0 + 16, :] = (jnp.concatenate(halves, axis=0)
                                  * ain[sl, 1, r0:r0 + 16, :].astype(F32)).astype(BF16)

        _run_paced([functools.partial(conv_item, r0=r0) for r0 in range(0, S, 16)], toks)

        fwd = fwd_ref[...]
        hst = jnp.concatenate([ah[sl, :, b * BLK:(b + 1) * BLK] for b in range(NB)], axis=0)
        hh = lax.dot_general(fwd, hst, (((1,), (1,)), ((), ())), preferred_element_type=F32)
        for m in range(BLK // 8):
            hr = hh[16 * m:16 * m + 8]
            hi = hh[16 * m + 8:16 * m + 16]
            hf[16 * m:16 * m + 16, 0:BLK] = hh[16 * m:16 * m + 16, 0:BLK]
            if m < BLK // 16:
                hf[16 * m:16 * m + 8, BLK:] = hr[:, BLK:] - hi[:, :S - BLK]
                hf[16 * m + 8:16 * m + 16, BLK:] = hi[:, BLK:] + hr[:, :S - BLK]
            else:
                hf[16 * m:16 * m + 8, BLK:] = hr[:, BLK:] + hi[:, :S - BLK]
                hf[16 * m + 8:16 * m + 16, BLK:] = hi[:, BLK:] - hr[:, :S - BLK]
        rhs = jnp.concatenate([kvb[b * BLK:(b + 1) * BLK, :] for b in range(NB)], axis=1)
        xf[...] = _dot(fwd, rhs)

        toks = []
        for i in range(1, len(parts) - 1):
            toks += run_part(i)
        items = []
        for m in range(BLK // 8):
            items += freq_items(m, never, zoff)
        _run_paced(items, toks[:-80])

        y = _dot(inv_ref[...], wf[...])
        run_part(len(parts) - 1)
        for b in range(NB):
            r0 = b * BLK
            yb = y[:, r0:r0 + BLK] + kvb[r0:r0 + BLK, :].astype(F32) * dvec
            aout[t, r0:r0 + BLK, :] = (ain[sl, 2, r0:r0 + BLK, :].astype(F32) * yb).astype(BF16)
        aout_copy(t).start()
        return carry

    lax.fori_loop(0, NT, tile_body, 0)
    pltpu.make_async_copy(wo, wo, sem_wo).wait()
    pltpu.make_async_copy(w32.at[WQ:WK + 1], w32.at[WQ:WK + 1], sem_wqk).wait()

    puni = pl.reciprocal(jnp.full((1, 1), float(L), F32), approx=True).astype(BF16).astype(F32)

    def shift_down(m):
        rows = lax.broadcasted_iota(jnp.int32, m.shape, 0)
        return jnp.where(rows == 0, 0.0, pltpu.roll(m, 1, 0))

    m1 = shift_down(_dot((tsum[...] * puni).astype(BF16), wo[...]))
    v1 = _dot(m1.astype(BF16), w_plain(WV, 0, H // 2)).astype(BF16).astype(F32)
    u2 = ((tsum[...] + float(M) * v1) * puni).astype(BF16)
    m2 = shift_down(_dot(u2, wo[...]))
    mhat[...] = jnp.broadcast_to(m2[:, None, :], (NSEG, M, DM)).reshape(NSEG * M, DM)
    mhat[0:M, :] = mem0

    ri = lax.broadcasted_iota(jnp.int32, (PR, PR), 0)
    ci = lax.broadcasted_iota(jnp.int32, (PR, PR), 1)

    def seg_of(r):
        return jnp.where(r < MR, r // M, (r - MR) // SEG)

    def pos_of(r):
        return jnp.where(r < MR, r % M, M + (r - MR) % SEG)

    same = seg_of(ri) == seg_of(ci)
    allowed = same & ((ri < MR) | (pos_of(ri) >= pos_of(ci)))
    fill = jnp.where(same, -1e9, -jnp.inf).astype(F32)

    def sweep(state):
        it, _ = state

        def mem_rows(i):
            n = PPB * MR
            return mhat[pl.ds(pl.multiple_of((i // NG) * n, n), n), :]

        def mem_lhs(i):
            m = mem_rows(i)
            n = PPH * MR
            ops = _strassen_lhs(m[:n, :KH], m[:n, KH:], m[n:, :KH], m[n:, KH:])
            return [_pack(o) for o in ops]

        def qk_proj(i, j, mops):
            rb = i // NG
            hp = (i % NG) * (G // 2) + j // 2

            def lhs(k):
                return _unpack(jnp.concatenate([mops[k], abuf[rb, k]], axis=0))

            (c11, c12, c21, c22), _ = _strassen(lhs, w_rhs(WQ + j % 2, hp))
            n = PPH * MR
            for half, cc in enumerate(((c11, c12), (c21, c22))):
                v = jnp.concatenate(cc, axis=1).astype(BF16)
                ps = slice(half * PPH, (half + 1) * PPH)
                qks[j, ps, 0:MR, :] = v[:n].reshape(PPH, MR, 2 * E)
                qks[j, ps, MR:PR, :] = v[n:].reshape(PPH, XR, 2 * E)

        def vm_proj(i):
            g = i % NG
            vv = _dot(mem_rows(i).astype(BF16), w_plain(WV, g * (G // 2), G // 2))
            v0 = v0buf[:, pl.ds(pl.multiple_of(g * (G * E), G * E), G * E)]
            vv = jnp.concatenate([jnp.where(i < NG, v0, vv[:M]), vv[M:]], axis=0)
            vms[...] = vv.astype(BF16).reshape(PPB, MR, G * E)

        def scores(j):
            c = slice((j % 2) * E, (j % 2 + 1) * E)
            return lax.dot_general(qks[2 * (j // 2), :, :, c], qks[2 * (j // 2) + 1, :, :, c],
                                   (((2,), (2,)), ((0,), (0,))), preferred_element_type=F32)

        def attend(i, j, s):
            p0 = pl.multiple_of((i // NG) * PPB, PPB)
            h = (i % NG) * G + j
            s = jnp.where(allowed[None], s * scale, fill[None])
            e = jnp.exp(s - jnp.max(s, axis=-1, keepdims=True))
            p = (e * pl.reciprocal(jnp.sum(e, axis=-1, keepdims=True), approx=True)).astype(BF16)
            vh = jnp.concatenate(
                [vms[:, :, j * E:(j + 1) * E],
                 vbuf[pl.ds(p0, PPB), :, pl.ds(pl.multiple_of(h * E, E), E)]], axis=1)
            return lax.dot_general(p, vh, (((2,), (1,)), ((0,), (0,))), preferred_element_type=F32)

        def out_proj(i, us):
            rb = i // NG
            g = i % NG
            u = jnp.concatenate(us, axis=2)
            wog = wo[pl.ds(pl.multiple_of(g * (G * E), G * E), G * E), :]
            rm = pl.ds(pl.multiple_of(rb * (PPB * MR), PPB * MR), PPB * MR)
            um = u[:, :MR, :].reshape(PPB * MR, G * E).astype(BF16)
            mnew[rm, :] = jnp.where(g > 0, mnew[rm, :], 0.0) + _dot(um, wog)
            n = PPH * XR
            kh = G * E // 2
            top = u[:PPH, MR:, :].reshape(n, G * E)
            bot = u[PPH:, MR:, :].reshape(n, G * E)
            ops = _strassen_lhs(top[:, :kh], top[:, kh:], bot[:, :kh], bot[:, kh:])
            wf32 = wog.astype(F32)
            rhs = _strassen_rhs(wf32[:kh, :KH], wf32[:kh, KH:], wf32[kh:, :KH], wf32[kh:, KH:])
            quads = [(slice(0, n), slice(0, KH)), (slice(0, n), slice(KH, DM)),
                     (slice(n, 2 * n), slice(0, KH)), (slice(n, 2 * n), slice(KH, DM))]
            init = [jnp.where(g > 0, acc[r, c], 0.0) for r, c in quads]
            cs, _ = _strassen(lambda k: ops[k].astype(BF16), rhs, init)
            for (r, c), v in zip(quads, cs):
                acc[r, c] = v
                obuf[rb, r, c] = v.astype(BF16)

        def step(i, nxt):
            s0, s1 = scores(0), scores(1)
            if nxt:
                mops = mem_lhs(i + 1)
                qk_proj(i + 1, 0, mops)
            u0, u1 = attend(i, 0, s0), attend(i, 1, s1)
            s2, s3 = scores(2), scores(3)
            if nxt:
                qk_proj(i + 1, 1, mops)
            u2, u3 = attend(i, 2, s2), attend(i, 3, s3)
            if nxt:
                qk_proj(i + 1, 2, mops)
                qk_proj(i + 1, 3, mops)
                vm_proj(i + 1)
            out_proj(i, [u0, u1, u2, u3])

        mops0 = mem_lhs(0)
        for j in range(G):
            qk_proj(0, j, mops0)
        vm_proj(0)

        def main_body(i, cy):
            step(i, True)

            @pl.when(i % NG == NG - 1)
            def _():
                o_copy(i // NG).start()

            return cy

        lax.fori_loop(0, NRB * NG - 1, main_body, 0)
        step(NRB * NG - 1, False)
        o_copy(NRB - 1).start()

        n = (NSEG - 1) * M
        new = mnew[0:n, :]
        err = jnp.max(jnp.abs(new - mhat[M:M + n, :]), axis=1, keepdims=True)
        ref = jnp.max(jnp.abs(new), axis=1, keepdims=True)
        ok = jnp.min(jnp.where(err <= TOL * ref, 1.0, 0.0))
        mhat[M:M + n, :] = new
        for rb in range(NRB):
            o_copy(rb).wait()
        return it + 1, (ok > 0.5).astype(jnp.int32)

    lax.while_loop(lambda st: jnp.logical_and(st[0] < NSEG, st[1] == 0), sweep,
                   (jnp.int32(0), jnp.int32(0)))
    pltpu.make_async_copy(aout, aout, sem_aout).wait()


@functools.partial(jax.jit, static_argnames=("B_seg_len",))
def pallas_concat_heads__ssm_conv_h3__memory_aug_recurrent_mem_tr__prompt_kernel(
    A_q, A_k, A_v, A_shift_k, A_ssm_k, A_ssm_D,
    B_x, B_mem0, B_Wq, B_Wk, B_Wv, B_Wo, B_seg_len,
):
    _, S, D = A_q.shape
    DM = B_x.shape[2]
    H, E = B_Wq.shape[1], B_Wq.shape[2]
    M = B_mem0.shape[1]
    SEG = int(B_seg_len)
    NSEG = S // SEG
    NP = NSEG // 2
    PR = 2 * (M + SEG)
    PPB = 8
    NRB = NP // PPB
    NT = D // LANES
    assert E == LANES and H == 32 and M == 8 and SEG == 32 and A_shift_k.shape[1] == 4
    assert S == 2048 and D == 1024 and DM == 1024

    fwd, inv = _dft_mats()
    any_spec = pl.BlockSpec(memory_space=pl.ANY)
    vmem_spec = pl.BlockSpec(memory_space=pltpu.VMEM)
    scratch = [
        pltpu.VMEM((NRB, 7, PPB // 2 * SEG, DM // 2), U32),
        pltpu.VMEM((7, M, DM // 2), U32),
        pltpu.VMEM((NP, 2 * SEG, H * E), BF16),
        pltpu.VMEM((M, H * E), F32),
        pltpu.VMEM((3, H // 2, DM, E), U32),
        pltpu.VMEM((H * E, DM), BF16),
        pltpu.VMEM((4, PPB, PR, 2 * E), BF16),
        pltpu.VMEM((PPB, 2 * M, 4 * E), BF16),
        pltpu.VMEM((PPB * 2 * SEG, DM), F32),
        pltpu.VMEM((NRB, PPB * 2 * SEG, DM), BF16),
        pltpu.VMEM((NSEG * M, DM), F32),
        pltpu.VMEM((NSEG * M, DM), F32),
        pltpu.VMEM((NSEG, H * E), F32),
        pltpu.VMEM((2, 3, S, LANES), BF16),
        pltpu.VMEM((2, LANES, S), BF16),
        pltpu.VMEM((S + 8, LANES), F32),
        pltpu.VMEM((S, LANES), BF16),
        pltpu.VMEM((NFFT, S), F32),
        pltpu.VMEM((NFFT, S), F32),
        pltpu.VMEM((NFFT, S), BF16),
        pltpu.VMEM((NT, S, LANES), BF16),
        pltpu.VMEM((8, LANES), jnp.int32),
        pltpu.SMEM((1,), jnp.int32),
        pltpu.SemaphoreType.DMA((NRB,)),
        pltpu.SemaphoreType.DMA((H // 2,)),
        pltpu.SemaphoreType.DMA,
        pltpu.SemaphoreType.DMA,
        pltpu.SemaphoreType.DMA((2, 2)),
        pltpu.SemaphoreType.DMA,
        pltpu.SemaphoreType.DMA((NRB,)),
    ]
    out = pl.pallas_call(
        functools.partial(_kernel, S=S, D=D, DM=DM, H=H, M=M, SEG=SEG),
        out_shape=jax.ShapeDtypeStruct((S, D + DM), BF16),
        in_specs=[any_spec, any_spec, any_spec, vmem_spec, any_spec, vmem_spec,
                  any_spec, vmem_spec, any_spec, any_spec, any_spec, any_spec,
                  vmem_spec, vmem_spec],
        out_specs=any_spec,
        scratch_shapes=scratch,
        compiler_params=pltpu.CompilerParams(vmem_limit_bytes=120 * 1024 * 1024,
                                             disable_bounds_checks=True),
    )(
        A_q.reshape(S, D), A_k.reshape(S, D), A_v.reshape(S, D),
        A_shift_k.T, A_ssm_k, A_ssm_D.reshape(NT, LANES),
        B_x.reshape(NRB, S // NRB, DM), B_mem0.reshape(M, DM),
        B_Wq, B_Wk, B_Wv, B_Wo.reshape(H * E, DM),
        jnp.asarray(fwd, BF16), jnp.asarray(inv, BF16),
    )
    return out.reshape(1, S, D + DM)
```

```python
import functools

import numpy as np
import jax
import jax.numpy as jnp
from jax import lax
import jax.experimental.pallas as pl
import jax.experimental.pallas.tpu as pltpu

F32 = jnp.float32
BF16 = jnp.bfloat16
U32 = jnp.uint32

LANES = 128
BLK = 128
NFFT = 2 * BLK
TOL = 2.0 ** -10


def _dft_mats():
    order = np.concatenate([np.arange(0, BLK, 2), np.arange(1, BLK, 2)])
    theta = 2.0 * np.pi * (order + 0.5) / NFFT
    n = np.arange(BLK)
    c = np.cos(theta[:, None] * n[None, :])
    s = np.sin(theta[:, None] * n[None, :])
    fwd = np.zeros((NFFT, BLK))
    inv = np.zeros((BLK, NFFT))
    for m in range(BLK // 8):
        fwd[16 * m:16 * m + 8] = c[8 * m:8 * m + 8]
        fwd[16 * m + 8:16 * m + 16] = -s[8 * m:8 * m + 8]
        inv[:, 16 * m:16 * m + 8] = c[8 * m:8 * m + 8].T * (2.0 / NFFT)
        inv[:, 16 * m + 8:16 * m + 16] = -s[8 * m:8 * m + 8].T * (2.0 / NFFT)
    return fwd.astype(np.float32), inv.astype(np.float32)


def _dot(a, b):
    return jnp.dot(a, b, preferred_element_type=F32)


def _pack(x):
    return pltpu.bitcast(x.astype(BF16), U32)


def _unpack(w):
    return pltpu.bitcast(w, BF16)


def _lo(w):
    return pltpu.bitcast(w << 16, F32)


def _hi(w):
    return pltpu.bitcast(w & jnp.uint32(0xFFFF0000), F32)


def _strassen_lhs(a11, a12, a21, a22):
    return [a11 + a22, a21 + a22, a11, a22, a11 + a12, a21 - a11, a12 - a22]


def _strassen_rhs(b11, b12, b21, b22):
    ops = [b11 + b22, b11, b12 - b22, b21 - b11, b22, b11 + b12, b21 + b22]
    return [o.astype(BF16) for o in ops]


def _strassen(lhs, rhs, init=None):
    def add(c, m):
        return m if c is None else c + m

    c11, c12, c21, c22 = init if init is not None else (None,) * 4
    m5 = _dot(lhs(4), rhs[4])
    m3 = _dot(lhs(2), rhs[2])
    c12 = add(c12, m5) + m3
    m2 = _dot(lhs(1), rhs[1])
    c22 = add(c22, m3) - m2
    m4 = _dot(lhs(3), rhs[3])
    c21 = add(c21, m2) + m4
    c11 = add(c11, m4) - m5
    m1 = _dot(lhs(0), rhs[0])
    c11 = c11 + m1
    c22 = c22 + m1
    m7 = _dot(lhs(6), rhs[6])
    c11 = c11 + m7
    m6 = _dot(lhs(5), rhs[5])
    c22 = c22 + m6
    return (c11, c12, c21, c22), [m5, m3, m2, m4, m1, m7, m6]


def _run_paced(items, toks):
    for i, it in enumerate(items):
        it(toks[i * len(toks) // len(items)])


def _kernel(q_hbm, k_hbm, v_hbm, shift_ref, h_hbm, d_ref, x_hbm, mem0_ref,
            wq_hbm, wk_hbm, wv_hbm, wo_hbm, fwd_ref, inv_ref,
            out_hbm,
            abuf, a0buf, vbuf, w32, wo, qks, vms, acc, obuf, mhat, mnew, tsum,
            ain, ah, kf, kvb, xf, hf, wf, aout, zero_v, zero_s,
            sem_x, sem_wv, sem_wqk, sem_wo, sem_a, sem_aout, sem_o,
            *, S, D, DM, H, M, SEG):
    E = LANES
    NSEG = S // SEG
    NP = NSEG // 2
    MR = 2 * M
    XR = 2 * SEG
    PR = MR + XR
    MW, XW, PW = MR // 2, XR // 2, PR // 2
    L = M + SEG
    NB = S // BLK
    NT = D // LANES
    PPB = 8
    PPH = PPB // 2
    NRB = NP // PPB
    G = 4
    NG = H // G
    KH = DM // 2
    scale = float(E) ** -0.5
    WV, WQ, WK = 0, 1, 2

    def x_copy(rb):
        return pltpu.make_async_copy(x_hbm.at[rb], obuf.at[rb], sem_x.at[rb])

    def w_copy(which, hp):
        src = (wv_hbm, wq_hbm, wk_hbm)[which].bitcast(U32)
        sem = sem_wv.at[hp] if which == WV else sem_wqk
        return pltpu.make_async_copy(src.at[:, hp, :], w32.at[which, hp], sem)

    def wo_copy(t):
        n = H * E // NT
        r = pl.ds(pl.multiple_of(t * n, n), n)
        return pltpu.make_async_copy(wo_hbm.at[r, :], wo.at[r, :], sem_wo)

    def a_start(t, sl):
        c = pl.ds(pl.multiple_of(t * LANES, LANES), LANES)
        pltpu.make_async_copy(k_hbm.at[:, c], ain.at[sl, 0], sem_a.at[sl, 0]).start()
        pltpu.make_async_copy(v_hbm.at[:, c], ain.at[sl, 1], sem_a.at[sl, 0]).start()
        pltpu.make_async_copy(h_hbm.at[c, :], ah.at[sl], sem_a.at[sl, 1]).start()
        pltpu.make_async_copy(q_hbm.at[:, c], ain.at[sl, 2], sem_a.at[sl, 0]).start()

    def a_wait(sl):
        pltpu.make_async_copy(ain.at[sl], ain.at[sl], sem_a.at[sl, 0]).wait()
        pltpu.make_async_copy(ah.at[sl], ah.at[sl], sem_a.at[sl, 1]).wait()

    def aout_copy(t):
        c = pl.ds(pl.multiple_of(t * LANES, LANES), LANES)
        return pltpu.make_async_copy(aout.at[t], out_hbm.at[:, c], sem_aout)

    def o_copy(rb):
        r = pl.ds(pl.multiple_of(rb * (PPB * XR), PPB * XR), PPB * XR)
        return pltpu.make_async_copy(obuf.at[rb], out_hbm.at[r, pl.ds(D, DM)], sem_o.at[rb])

    def w_rhs(which, hp, zs=None):
        if zs is None:
            w = w32[which, hp]
            return _strassen_rhs(_lo(w[:KH]), _hi(w[:KH]), _lo(w[KH:]), _hi(w[KH:]))
        out = []
        for k in range(7):
            w = w32.at[which, hp + zs[k]]
            out.append(_strassen_rhs(_lo(w[:KH]), _hi(w[:KH]), _lo(w[KH:]), _hi(w[KH:]))[k])
        return out

    def w_plain(which, hp0, n):
        parts = []
        for j in range(n):
            w = w32[which, hp0 + j]
            parts += [_lo(w), _hi(w)]
        return jnp.concatenate(parts, axis=1).astype(BF16)

    for rb in range(NRB):
        x_copy(rb).start()
    w_copy(WV, 0).start()
    w_copy(WV, 1).start()
    a_start(0, 0)

    kf[0:8, :] = jnp.zeros((8, LANES), F32)
    zero_v[...] = jnp.zeros((8, LANES), jnp.int32)
    for k in range(8):
        zero_s[k] = 0
    tsum[0:8, :] = jnp.zeros((8, H * E), F32)
    vbuf[0, 0:16, :] = jnp.zeros((16, H * E), BF16)
    mem0 = mem0_ref[...].astype(F32)
    m0 = jnp.concatenate([mem0, jnp.zeros_like(mem0)], axis=0)
    z0 = jnp.zeros((MR, KH), F32)
    for k, op in enumerate(_strassen_lhs(m0[:, :KH], m0[:, KH:], z0, z0)):
        a0buf[k] = _pack(op)

    def x_prep(i, cy):
        rb = i // PPH
        pp = i % PPH

        @pl.when(pp == 0)
        def _():
            x_copy(rb).wait()

        top = obuf[rb, pl.ds(pl.multiple_of(pp * XR, XR), XR), :].astype(F32)
        bot = obuf[rb, pl.ds(pl.multiple_of((PPH + pp) * XR, XR), XR), :].astype(F32)
        for k, op in enumerate(_strassen_lhs(top[:, :KH], top[:, KH:], bot[:, :KH], bot[:, KH:])):
            abuf[rb, k, pl.ds(pl.multiple_of(pp * XW, XW), XW), :] = _pack(op)
        return cy

    lax.fori_loop(0, NRB * PPH, x_prep, 0)

    def v_part(j, rb, rhs, vwin, twin, pre=None):
        def lhs(k):
            x = abuf[rb, k]
            if rb == 0:
                x0 = a0buf[k]
                if pre is not None and k == 4:
                    x0 = jnp.concatenate([pre(x0[:, :LANES]), x0[:, LANES:]], axis=1)
                x = jnp.concatenate([x0, x], axis=0)
            return _unpack(x)

        (c11, c12, c21, c22), ms = _strassen(lhs, rhs)
        for half, hh, cv in ((0, 1, c12), (1, 0, c21), (0, 0, c11), (1, 1, c22)):
            c = slice((2 * j + hh) * E, (2 * j + hh + 1) * E)
            vv = cv.astype(BF16)
            vx = vv[MR:] if rb == 0 else vv
            p0 = rb * PPB + half * PPH
            vwin[p0:p0 + PPH, :, c] = vx.reshape(PPH, XR, E)
            ts = jnp.sum(vx.astype(F32).reshape(2 * PPH, SEG, E), axis=1)
            if rb == 0 and half == 0:
                v0 = vv[0:M].astype(F32)
                twin[NSEG:NSEG + M, c] = v0
                t0 = jnp.sum(v0, axis=0, keepdims=True)
                rows = lax.broadcasted_iota(jnp.int32, ts.shape, 0)
                ts = ts + jnp.where(rows == 0, t0, 0.0)
            twin[2 * p0:2 * (p0 + PPH), c] = ts
        return [m[8 * g:8 * g + 8] for m in ms for g in range(m.shape[0] // 8)]

    GA = 4

    def freq_items(m, never, xf, hf):
        r_re = slice(16 * m, 16 * m + 8)
        r_im = slice(16 * m + 8, 16 * m + 16)

        def item(tok, a0, cc, st):
            xr = jnp.where(never, tok, xf[r_re, cc * BLK:(cc + 1) * BLK])
            xi = jnp.where(never, tok, xf[r_im, cc * BLK:(cc + 1) * BLK])
            for a in range(max(a0, cc), a0 + GA):
                j = a - cc
                if ('g', j) not in st:
                    st['g', j] = (hf[r_re, j * BLK:(j + 1) * BLK], hf[r_im, j * BLK:(j + 1) * BLK])
                gr, gi = st['g', j]
                ps = (xr * gr - xi * gi, xr * gi + xi * gr)
                st[a] = ps if a not in st else (st[a][0] + ps[0], st[a][1] + ps[1])
                if cc == a:
                    wf[16 * m:16 * m + 16, a * BLK:(a + 1) * BLK] = (
                        jnp.concatenate(st[a], axis=0).astype(BF16))

        items = []
        for a0 in range(0, NB, GA):
            st = {}
            items += [functools.partial(item, a0=a0, cc=cc, st=st) for cc in range(a0 + GA)]
        return items

    def tile_body(t, carry):
        sl = t % 2
        a_wait(sl)
        w_copy(WV, 2 * t).wait()
        w_copy(WV, 2 * t + 1).wait()

        @pl.when(t + 1 < NT)
        def _():
            w_copy(WV, 2 * t + 2).start()
            w_copy(WV, 2 * t + 3).start()
            a_start(t + 1, 1 - sl)

        wo_copy(t).start()
        for which in (WQ, WK):
            w_copy(which, 2 * t).start()
            w_copy(which, 2 * t + 1).start()

        c = pl.ds(pl.multiple_of(t * LANES, LANES), LANES)
        taps = shift_ref[:, c].astype(F32)
        dcol = d_ref[...].astype(F32)
        rows = lax.broadcasted_iota(jnp.int32, dcol.shape, 0)
        dvec = jnp.sum(jnp.where(rows == t, dcol, 0.0), axis=0, keepdims=True)
        never = zero_v[...] > 0
        zoff = zero_s[7]
        zs = [zero_s[k] for k in range(7)]

        rhs2 = [w_rhs(WV, 2 * t, zs), w_rhs(WV, 2 * t + 1, zs)]
        parts = [(j, rb) for j in range(2) for rb in range(NRB)]
        c4 = pl.ds(pl.multiple_of(t * (4 * E), 4 * E), 4 * E)
        vwin = vbuf.at[:, :, c4]
        twin = tsum.at[:, c4]

        def pre(x):
            x = jnp.where(never, pltpu.bitcast(twin[0:8, 0:LANES], U32), x)
            return jnp.where(never, pltpu.bitcast(vwin[0, 0:16, 0:LANES], U32), x)


        def run_part(i):
            j, rb = parts[i]
            return v_part(j, rb, rhs2[j], vwin, twin, pre if i == 0 else None)

        toks = run_part(0)

        kf[8:8 + S, :] = ain[sl, 0].astype(F32)
        tapb = [jnp.broadcast_to(taps[j:j + 1, :], (8, LANES)) for j in range(4)]

        def conv_item(tok, r0):
            halves = []
            for h in range(2):
                r = 8 + r0 + 8 * h
                ks = kf[r:r + 8, :] * jnp.where(never, tok, tapb[0])
                for j in range(1, 4):
                    ks = ks + kf[r - j:r - j + 8, :] * tapb[j]
                halves.append(ks)
            kvb[r0:r0 + 16, :] = (jnp.concatenate(halves, axis=0)
                                  * ain[sl, 1, r0:r0 + 16, :].astype(F32)).astype(BF16)

        _run_paced([functools.partial(conv_item, r0=r0) for r0 in range(0, S, 16)], toks)

        fwd = fwd_ref[...]
        hst = jnp.concatenate([ah[sl, :, b * BLK:(b + 1) * BLK] for b in range(NB)], axis=0)
        hh = lax.dot_general(fwd, hst, (((1,), (1,)), ((), ())), preferred_element_type=F32)
        for m in range(BLK // 8):
            hr = hh[16 * m:16 * m + 8]
            hi = hh[16 * m + 8:16 * m + 16]
            hf[16 * m:16 * m + 16, 0:BLK] = hh[16 * m:16 * m + 16, 0:BLK]
            if m < BLK // 16:
                hf[16 * m:16 * m + 8, BLK:] = hr[:, BLK:] - hi[:, :S - BLK]
                hf[16 * m + 8:16 * m + 16, BLK:] = hi[:, BLK:] + hr[:, :S - BLK]
            else:
                hf[16 * m:16 * m + 8, BLK:] = hr[:, BLK:] + hi[:, :S - BLK]
                hf[16 * m + 8:16 * m + 16, BLK:] = hi[:, BLK:] - hr[:, :S - BLK]
        rhs = jnp.concatenate([kvb[b * BLK:(b + 1) * BLK, :] for b in range(NB)], axis=1)
        xf[...] = _dot(fwd, rhs)

        toks = []
        for i in range(1, len(parts)):
            toks += run_part(i)
        items = []
        win = pl.ds(pl.multiple_of(zoff, 8), NFFT)
        for m in range(BLK // 8):
            items += freq_items(m, never, xf.at[win, :], hf.at[win, :])
        _run_paced(items, toks[:-80])

        y = _dot(inv_ref[...], wf[...])
        for b in range(NB):
            r0 = b * BLK
            yb = y[:, r0:r0 + BLK] + kvb[r0:r0 + BLK, :].astype(F32) * dvec
            aout[t, r0:r0 + BLK, :] = (ain[sl, 2, r0:r0 + BLK, :].astype(F32) * yb).astype(BF16)
        aout_copy(t).start()
        return carry

    lax.fori_loop(0, NT, tile_body, 0)
    pltpu.make_async_copy(wo, wo, sem_wo).wait()
    pltpu.make_async_copy(w32.at[WQ:WK + 1], w32.at[WQ:WK + 1], sem_wqk).wait()

    puni = pl.reciprocal(jnp.full((1, 1), float(L), F32), approx=True).astype(BF16).astype(F32)

    def shift_down(m):
        rows = lax.broadcasted_iota(jnp.int32, m.shape, 0)
        return jnp.where(rows == 0, 0.0, pltpu.roll(m, 1, 0))

    m1 = shift_down(_dot((tsum[0:NSEG, :] * puni).astype(BF16), wo[...]))
    v1 = _dot(m1.astype(BF16), w_plain(WV, 0, H // 2)).astype(BF16).astype(F32)
    u2 = ((tsum[0:NSEG, :] + float(M) * v1) * puni).astype(BF16)
    m2 = shift_down(_dot(u2, wo[...]))
    mhat[...] = jnp.broadcast_to(m2[:, None, :], (NSEG, M, DM)).reshape(NSEG * M, DM)
    mhat[0:M, :] = mem0

    ri = lax.broadcasted_iota(jnp.int32, (PR, PR), 0)
    ci = lax.broadcasted_iota(jnp.int32, (PR, PR), 1)

    def seg_of(r):
        return jnp.where(r < MR, r // M, (r - MR) // SEG)

    def pos_of(r):
        return jnp.where(r < MR, r % M, M + (r - MR) % SEG)

    same = seg_of(ri) == seg_of(ci)
    allowed = same & ((ri < MR) | (pos_of(ri) >= pos_of(ci)))
    fill = jnp.where(same, -1e9, -jnp.inf).astype(F32)

    def sweep(state):
        it, _ = state

        def mem_rows(i):
            n = PPB * MR
            return mhat[pl.ds(pl.multiple_of((i // NG) * n, n), n), :]

        def mem_lhs(i):
            m = mem_rows(i)
            n = PPH * MR
            ops = _strassen_lhs(m[:n, :KH], m[:n, KH:], m[n:, :KH], m[n:, KH:])
            return [_pack(o) for o in ops]

        def qk_proj(i, j, mops):
            rb = i // NG
            hp = (i % NG) * (G // 2) + j // 2

            def lhs(k):
                return _unpack(jnp.concatenate([mops[k], abuf[rb, k]], axis=0))

            (c11, c12, c21, c22), _ = _strassen(lhs, w_rhs(WQ + j % 2, hp, [zero_s[k] for k in range(7)]))
            n = PPH * MR
            for half, cc in enumerate(((c11, c12), (c21, c22))):
                v = jnp.concatenate(cc, axis=1).astype(BF16)
                ps = slice(half * PPH, (half + 1) * PPH)
                qks[j, ps, 0:MR, :] = v[:n].reshape(PPH, MR, 2 * E)
                qks[j, ps, MR:PR, :] = v[n:].reshape(PPH, XR, 2 * E)

        def vm_proj(i):
            g = i % NG
            vv = _dot(mem_rows(i).astype(BF16), w_plain(WV, g * (G // 2), G // 2))
            v0 = tsum[NSEG:NSEG + M, pl.ds(pl.multiple_of(g * (G * E), G * E), G * E)]
            vv = jnp.concatenate([jnp.where(i < NG, v0, vv[:M]), vv[M:]], axis=0)
            vms[...] = vv.astype(BF16).reshape(PPB, MR, G * E)

        def scores(j):
            c = slice((j % 2) * E, (j % 2 + 1) * E)
            return lax.dot_general(qks[2 * (j // 2), :, :, c], qks[2 * (j // 2) + 1, :, :, c],
                                   (((2,), (2,)), ((0,), (0,))), preferred_element_type=F32)

        def attend(i, j, s):
            p0 = pl.multiple_of((i // NG) * PPB, PPB)
            h = (i % NG) * G + j
            s = jnp.where(allowed[None], s * scale, fill[None])
            e = jnp.exp(s - jnp.max(s, axis=-1, keepdims=True))
            p = (e * pl.reciprocal(jnp.sum(e, axis=-1, keepdims=True), approx=True)).astype(BF16)
            vh = jnp.concatenate(
                [vms[:, :, j * E:(j + 1) * E],
                 vbuf[pl.ds(p0, PPB), :, pl.ds(pl.multiple_of(h * E, E), E)]], axis=1)
            return lax.dot_general(p, vh, (((2,), (1,)), ((0,), (0,))), preferred_element_type=F32)

        def out_proj(i, us):
            rb = i // NG
            g = i % NG
            u = jnp.concatenate(us, axis=2)
            wog = wo[pl.ds(pl.multiple_of(g * (G * E), G * E), G * E), :]
            rm = pl.ds(pl.multiple_of(rb * (PPB * MR), PPB * MR), PPB * MR)
            um = u[:, :MR, :].reshape(PPB * MR, G * E).astype(BF16)
            mnew[rm, :] = jnp.where(g > 0, mnew[rm, :], 0.0) + _dot(um, wog)
            n = PPH * XR
            kh = G * E // 2
            top = u[:PPH, MR:, :].reshape(n, G * E)
            bot = u[PPH:, MR:, :].reshape(n, G * E)
            ops = _strassen_lhs(top[:, :kh], top[:, kh:], bot[:, :kh], bot[:, kh:])
            wf32 = wog.astype(F32)
            rhs = _strassen_rhs(wf32[:kh, :KH], wf32[:kh, KH:], wf32[kh:, :KH], wf32[kh:, KH:])
            quads = [(slice(0, n), slice(0, KH)), (slice(0, n), slice(KH, DM)),
                     (slice(n, 2 * n), slice(0, KH)), (slice(n, 2 * n), slice(KH, DM))]
            init = [jnp.where(g > 0, acc[r, c], 0.0) for r, c in quads]
            cs, _ = _strassen(lambda k: ops[k].astype(BF16), rhs, init)
            for (r, c), v in zip(quads, cs):
                acc[r, c] = v
                obuf[rb, r, c] = v.astype(BF16)

        def step(i, nxt):
            s0, s1 = scores(0), scores(1)
            if nxt:
                mops = mem_lhs(i + 1)
                qk_proj(i + 1, 0, mops)
            u0, u1 = attend(i, 0, s0), attend(i, 1, s1)
            s2, s3 = scores(2), scores(3)
            if nxt:
                qk_proj(i + 1, 1, mops)
            u2, u3 = attend(i, 2, s2), attend(i, 3, s3)
            if nxt:
                qk_proj(i + 1, 2, mops)
                qk_proj(i + 1, 3, mops)
                vm_proj(i + 1)
            out_proj(i, [u0, u1, u2, u3])

        mops0 = mem_lhs(0)
        for j in range(G):
            qk_proj(0, j, mops0)
        vm_proj(0)

        def main_body(i, cy):
            step(i, True)

            @pl.when(i % NG == NG - 1)
            def _():
                o_copy(i // NG).start()

            return cy

        lax.fori_loop(0, NRB * NG - 1, main_body, 0)
        step(NRB * NG - 1, False)
        o_copy(NRB - 1).start()

        n = (NSEG - 1) * M
        new = mnew[0:n, :]
        err = jnp.max(jnp.abs(new - mhat[M:M + n, :]), axis=1, keepdims=True)
        ref = jnp.max(jnp.abs(new), axis=1, keepdims=True)
        ok = jnp.min(jnp.where(err <= TOL * ref, 1.0, 0.0))
        mhat[M:M + n, :] = new
        for rb in range(NRB):
            o_copy(rb).wait()
        return it + 1, (ok > 0.5).astype(jnp.int32)

    lax.while_loop(lambda st: jnp.logical_and(st[0] < NSEG, st[1] == 0), sweep,
                   (jnp.int32(0), jnp.int32(0)))
    pltpu.make_async_copy(aout, aout, sem_aout).wait()


@functools.partial(jax.jit, static_argnames=("B_seg_len",))
def pallas_concat_heads__ssm_conv_h3__memory_aug_recurrent_mem_tr__prompt_kernel(
    A_q, A_k, A_v, A_shift_k, A_ssm_k, A_ssm_D,
    B_x, B_mem0, B_Wq, B_Wk, B_Wv, B_Wo, B_seg_len,
):
    _, S, D = A_q.shape
    DM = B_x.shape[2]
    H, E = B_Wq.shape[1], B_Wq.shape[2]
    M = B_mem0.shape[1]
    SEG = int(B_seg_len)
    NSEG = S // SEG
    NP = NSEG // 2
    PR = 2 * (M + SEG)
    PPB = 8
    NRB = NP // PPB
    NT = D // LANES
    assert E == LANES and H == 32 and M == 8 and SEG == 32 and A_shift_k.shape[1] == 4
    assert S == 2048 and D == 1024 and DM == 1024

    fwd, inv = _dft_mats()
    any_spec = pl.BlockSpec(memory_space=pl.ANY)
    vmem_spec = pl.BlockSpec(memory_space=pltpu.VMEM)
    scratch = [
        pltpu.VMEM((NRB, 7, PPB // 2 * SEG, DM // 2), U32),
        pltpu.VMEM((7, M, DM // 2), U32),
        pltpu.VMEM((NP, 2 * SEG, H * E), BF16),
        pltpu.VMEM((3, H // 2, DM, E), U32),
        pltpu.VMEM((H * E, DM), BF16),
        pltpu.VMEM((4, PPB, PR, 2 * E), BF16),
        pltpu.VMEM((PPB, 2 * M, 4 * E), BF16),
        pltpu.VMEM((PPB * 2 * SEG, DM), F32),
        pltpu.VMEM((NRB, PPB * 2 * SEG, DM), BF16),
        pltpu.VMEM((NSEG * M, DM), F32),
        pltpu.VMEM((NSEG * M, DM), F32),
        pltpu.VMEM((NSEG + M, H * E), F32),
        pltpu.VMEM((2, 3, S, LANES), BF16),
        pltpu.VMEM((2, LANES, S), BF16),
        pltpu.VMEM((S + 8, LANES), F32),
        pltpu.VMEM((S, LANES), BF16),
        pltpu.VMEM((NFFT, S), F32),
        pltpu.VMEM((NFFT, S), F32),
        pltpu.VMEM((NFFT, S), BF16),
        pltpu.VMEM((NT, S, LANES), BF16),
        pltpu.VMEM((8, LANES), jnp.int32),
        pltpu.SMEM((8,), jnp.int32),
        pltpu.SemaphoreType.DMA((NRB,)),
        pltpu.SemaphoreType.DMA((H // 2,)),
        pltpu.SemaphoreType.DMA,
        pltpu.SemaphoreType.DMA,
        pltpu.SemaphoreType.DMA((2, 2)),
        pltpu.SemaphoreType.DMA,
        pltpu.SemaphoreType.DMA((NRB,)),
    ]
    out = pl.pallas_call(
        functools.partial(_kernel, S=S, D=D, DM=DM, H=H, M=M, SEG=SEG),
        out_shape=jax.ShapeDtypeStruct((S, D + DM), BF16),
        in_specs=[any_spec, any_spec, any_spec, vmem_spec, any_spec, vmem_spec,
                  any_spec, vmem_spec, any_spec, any_spec, any_spec, any_spec,
                  vmem_spec, vmem_spec],
        out_specs=any_spec,
        scratch_shapes=scratch,
        compiler_params=pltpu.CompilerParams(vmem_limit_bytes=120 * 1024 * 1024,
                                             disable_bounds_checks=True),
    )(
        A_q.reshape(S, D), A_k.reshape(S, D), A_v.reshape(S, D),
        A_shift_k.T, A_ssm_k, A_ssm_D.reshape(NT, LANES),
        B_x.reshape(NRB, S // NRB, DM), B_mem0.reshape(M, DM),
        B_Wq, B_Wk, B_Wv, B_Wo.reshape(H * E, DM),
        jnp.asarray(fwd, BF16), jnp.asarray(inv, BF16),
    )
    return out.reshape(1, S, D + DM)
```

```python
import functools

import numpy as np
import jax
import jax.numpy as jnp
from jax import lax
import jax.experimental.pallas as pl
import jax.experimental.pallas.tpu as pltpu

F32 = jnp.float32
BF16 = jnp.bfloat16
U32 = jnp.uint32

LANES = 128
BLK = 128
NFFT = 2 * BLK
TOL = 2.0 ** -10


def _dft_mats():
    order = np.concatenate([np.arange(0, BLK, 2), np.arange(1, BLK, 2)])
    theta = 2.0 * np.pi * (order + 0.5) / NFFT
    n = np.arange(BLK)
    c = np.cos(theta[:, None] * n[None, :])
    s = np.sin(theta[:, None] * n[None, :])
    fwd = np.zeros((NFFT, BLK))
    inv = np.zeros((BLK, NFFT))
    for m in range(BLK // 8):
        fwd[16 * m:16 * m + 8] = c[8 * m:8 * m + 8]
        fwd[16 * m + 8:16 * m + 16] = -s[8 * m:8 * m + 8]
        inv[:, 16 * m:16 * m + 8] = c[8 * m:8 * m + 8].T * (2.0 / NFFT)
        inv[:, 16 * m + 8:16 * m + 16] = -s[8 * m:8 * m + 8].T * (2.0 / NFFT)
    return fwd.astype(np.float32), inv.astype(np.float32)


def _dot(a, b):
    return jnp.dot(a, b, preferred_element_type=F32)


def _pack(x):
    return pltpu.bitcast(x.astype(BF16), U32)


def _unpack(w):
    return pltpu.bitcast(w, BF16)


def _lo(w):
    return pltpu.bitcast(w << 16, F32)


def _hi(w):
    return pltpu.bitcast(w & jnp.uint32(0xFFFF0000), F32)


def _strassen_lhs(a11, a12, a21, a22):
    return [a11 + a22, a21 + a22, a11, a22, a11 + a12, a21 - a11, a12 - a22]


def _strassen_rhs(b11, b12, b21, b22):
    ops = [b11 + b22, b11, b12 - b22, b21 - b11, b22, b11 + b12, b21 + b22]
    return [o.astype(BF16) for o in ops]


def _strassen(lhs, rhs, init=None):
    def add(c, m):
        return m if c is None else c + m

    c11, c12, c21, c22 = init if init is not None else (None,) * 4
    m5 = _dot(lhs(4), rhs[4])
    m3 = _dot(lhs(2), rhs[2])
    c12 = add(c12, m5) + m3
    m2 = _dot(lhs(1), rhs[1])
    c22 = add(c22, m3) - m2
    m4 = _dot(lhs(3), rhs[3])
    c21 = add(c21, m2) + m4
    c11 = add(c11, m4) - m5
    m1 = _dot(lhs(0), rhs[0])
    c11 = c11 + m1
    c22 = c22 + m1
    m7 = _dot(lhs(6), rhs[6])
    c11 = c11 + m7
    m6 = _dot(lhs(5), rhs[5])
    c22 = c22 + m6
    return (c11, c12, c21, c22), [m5, m3, m2, m4, m1, m7, m6]


def _run_paced(items, toks):
    for i, it in enumerate(items):
        it(toks[i * len(toks) // len(items)])


def _kernel(q_hbm, k_hbm, v_hbm, shift_ref, h_hbm, d_ref, x_hbm, mem0_ref,
            wq_hbm, wk_hbm, wv_hbm, wo_hbm, fwd_ref, inv_ref,
            out_hbm,
            abuf, a0buf, vbuf, w32, wo, qks, vms, acc, obuf, mhat, mnew, tsum,
            ain, ah, kf, kvb, xf, hf, wf, aout, zero_v, zero_s,
            sem_x, sem_wv, sem_wqk, sem_wo, sem_a, sem_aout, sem_o,
            *, S, D, DM, H, M, SEG):
    E = LANES
    NSEG = S // SEG
    NP = NSEG // 2
    MR = 2 * M
    XR = 2 * SEG
    PR = MR + XR
    MW, XW, PW = MR // 2, XR // 2, PR // 2
    L = M + SEG
    NB = S // BLK
    NT = D // LANES
    PPB = 8
    PPH = PPB // 2
    NRB = NP // PPB
    G = 4
    NG = H // G
    KH = DM // 2
    scale = float(E) ** -0.5
    WV, WQ, WK = 0, 1, 2

    def x_copy(rb):
        return pltpu.make_async_copy(x_hbm.at[rb], obuf.at[rb], sem_x.at[rb])

    def w_copy(which, hp):
        src = (wv_hbm, wq_hbm, wk_hbm)[which].bitcast(U32)
        sem = sem_wv.at[hp] if which == WV else sem_wqk
        return pltpu.make_async_copy(src.at[:, hp, :], w32.at[which, hp], sem)

    def wo_copy(t):
        n = H * E // NT
        r = pl.ds(pl.multiple_of(t * n, n), n)
        return pltpu.make_async_copy(wo_hbm.at[r, :], wo.at[r, :], sem_wo)

    def a_start(t, sl):
        c = pl.ds(pl.multiple_of(t * LANES, LANES), LANES)
        pltpu.make_async_copy(k_hbm.at[:, c], ain.at[sl, 0], sem_a.at[sl, 0]).start()
        pltpu.make_async_copy(v_hbm.at[:, c], ain.at[sl, 1], sem_a.at[sl, 0]).start()
        pltpu.make_async_copy(h_hbm.at[c, :], ah.at[sl], sem_a.at[sl, 1]).start()
        pltpu.make_async_copy(q_hbm.at[:, c], ain.at[sl, 2], sem_a.at[sl, 0]).start()

    def a_wait(sl):
        pltpu.make_async_copy(ain.at[sl], ain.at[sl], sem_a.at[sl, 0]).wait()
        pltpu.make_async_copy(ah.at[sl], ah.at[sl], sem_a.at[sl, 1]).wait()

    def aout_copy(t):
        c = pl.ds(pl.multiple_of(t * LANES, LANES), LANES)
        return pltpu.make_async_copy(aout.at[t], out_hbm.at[:, c], sem_aout)

    def o_copy(rb):
        r = pl.ds(pl.multiple_of(rb * (PPB * XR), PPB * XR), PPB * XR)
        return pltpu.make_async_copy(obuf.at[rb], out_hbm.at[r, pl.ds(D, DM)], sem_o.at[rb])

    def w_rhs(which, hp, zs=None):
        if zs is None:
            w = w32[which, hp]
            return _strassen_rhs(_lo(w[:KH]), _hi(w[:KH]), _lo(w[KH:]), _hi(w[KH:]))
        out = []
        for k in range(7):
            w = w32.at[which, hp + zs[k]]
            out.append(_strassen_rhs(_lo(w[:KH]), _hi(w[:KH]), _lo(w[KH:]), _hi(w[KH:]))[k])
        return out

    def w_plain(which, hp0, n):
        parts = []
        for j in range(n):
            w = w32[which, hp0 + j]
            parts += [_lo(w), _hi(w)]
        return jnp.concatenate(parts, axis=1).astype(BF16)

    for rb in range(NRB):
        x_copy(rb).start()
    w_copy(WV, 0).start()
    w_copy(WV, 1).start()
    a_start(0, 0)

    kf[0:8, :] = jnp.zeros((8, LANES), F32)
    zero_v[...] = jnp.zeros((8, LANES), jnp.int32)
    for k in range(8):
        zero_s[k] = 0
    tsum[0:8, :] = jnp.zeros((8, H * E), F32)
    vbuf[0, 0:16, :] = jnp.zeros((16, H * E), BF16)
    mem0 = mem0_ref[...].astype(F32)
    m0 = jnp.concatenate([mem0, jnp.zeros_like(mem0)], axis=0)
    z0 = jnp.zeros((MR, KH), F32)
    for k, op in enumerate(_strassen_lhs(m0[:, :KH], m0[:, KH:], z0, z0)):
        a0buf[k] = _pack(op)

    def x_prep(i, cy):
        rb = i // PPH
        pp = i % PPH

        @pl.when(pp == 0)
        def _():
            x_copy(rb).wait()

        top = obuf[rb, pl.ds(pl.multiple_of(pp * XR, XR), XR), :].astype(F32)
        bot = obuf[rb, pl.ds(pl.multiple_of((PPH + pp) * XR, XR), XR), :].astype(F32)
        for k, op in enumerate(_strassen_lhs(top[:, :KH], top[:, KH:], bot[:, :KH], bot[:, KH:])):
            abuf[rb, k, pl.ds(pl.multiple_of(pp * XW, XW), XW), :] = _pack(op)
        return cy

    lax.fori_loop(0, NRB * PPH, x_prep, 0)

    def v_part(j, rb, rhs, vwin, twin, pre=None):
        def lhs(k):
            x = abuf[rb, k]
            if rb == 0:
                x0 = a0buf[k]
                if pre is not None and k == 4:
                    x0 = jnp.concatenate([pre(x0[:, :LANES]), x0[:, LANES:]], axis=1)
                x = jnp.concatenate([x0, x], axis=0)
            return _unpack(x)

        (c11, c12, c21, c22), ms = _strassen(lhs, rhs)
        for half, hh, cv in ((0, 1, c12), (1, 0, c21), (0, 0, c11), (1, 1, c22)):
            c = slice((2 * j + hh) * E, (2 * j + hh + 1) * E)
            vv = cv.astype(BF16)
            vx = vv[MR:] if rb == 0 else vv
            p0 = rb * PPB + half * PPH
            vwin[p0:p0 + PPH, :, c] = vx.reshape(PPH, XR, E)
            ts = jnp.sum(vx.astype(F32).reshape(2 * PPH, SEG, E), axis=1)
            if rb == 0 and half == 0:
                v0 = vv[0:M].astype(F32)
                twin[NSEG:NSEG + M, c] = v0
                t0 = jnp.sum(v0, axis=0, keepdims=True)
                rows = lax.broadcasted_iota(jnp.int32, ts.shape, 0)
                ts = ts + jnp.where(rows == 0, t0, 0.0)
            twin[2 * p0:2 * (p0 + PPH), c] = ts
        return [m[8 * g:8 * g + 8] for m in ms for g in range(m.shape[0] // 8)]

    GA = 4

    def freq_items(m, never, xf, hf):
        r_re = slice(16 * m, 16 * m + 8)
        r_im = slice(16 * m + 8, 16 * m + 16)

        def item(tok, a0, cc, st):
            xr = jnp.where(never, tok, xf[r_re, cc * BLK:(cc + 1) * BLK])
            xi = jnp.where(never, tok, xf[r_im, cc * BLK:(cc + 1) * BLK])
            for a in range(max(a0, cc), a0 + GA):
                j = a - cc
                if ('g', j) not in st:
                    st['g', j] = (hf[r_re, j * BLK:(j + 1) * BLK], hf[r_im, j * BLK:(j + 1) * BLK])
                gr, gi = st['g', j]
                ps = (xr * gr - xi * gi, xr * gi + xi * gr)
                st[a] = ps if a not in st else (st[a][0] + ps[0], st[a][1] + ps[1])
                if cc == a:
                    wf[16 * m:16 * m + 16, a * BLK:(a + 1) * BLK] = (
                        jnp.concatenate(st[a], axis=0).astype(BF16))

        items = []
        for a0 in range(0, NB, GA):
            st = {}
            items += [functools.partial(item, a0=a0, cc=cc, st=st) for cc in range(a0 + GA)]
        return items

    def tile_body(t, carry):
        sl = t % 2
        a_wait(sl)
        w_copy(WV, 2 * t).wait()
        w_copy(WV, 2 * t + 1).wait()

        @pl.when(t + 1 < NT)
        def _():
            w_copy(WV, 2 * t + 2).start()
            w_copy(WV, 2 * t + 3).start()
            a_start(t + 1, 1 - sl)
            wo_copy(t + 1).start()

        for which in (WQ, WK):
            w_copy(which, 2 * t).start()
            w_copy(which, 2 * t + 1).start()

        c = pl.ds(pl.multiple_of(t * LANES, LANES), LANES)
        taps = shift_ref[:, c].astype(F32)
        dcol = d_ref[...].astype(F32)
        rows = lax.broadcasted_iota(jnp.int32, dcol.shape, 0)
        dvec = jnp.sum(jnp.where(rows == t, dcol, 0.0), axis=0, keepdims=True)
        never = zero_v[...] > 0
        zoff = zero_s[7]
        zs = [zero_s[k] for k in range(7)]

        rhs2 = [w_rhs(WV, 2 * t, zs), w_rhs(WV, 2 * t + 1, zs)]
        parts = [(j, rb) for j in range(2) for rb in range(NRB)]
        c4 = pl.ds(pl.multiple_of(t * (4 * E), 4 * E), 4 * E)
        vwin = vbuf.at[:, :, c4]
        twin = tsum.at[:, c4]

        def pre(x):
            x = jnp.where(never, pltpu.bitcast(twin[0:8, 0:LANES], U32), x)
            return jnp.where(never, pltpu.bitcast(vwin[0, 0:16, 0:LANES], U32), x)


        def run_part(i):
            j, rb = parts[i]
            return v_part(j, rb, rhs2[j], vwin, twin, pre if i == 0 else None)

        toks = run_part(0)

        kf[8:8 + S, :] = ain[sl, 0].astype(F32)
        tapb = [jnp.broadcast_to(taps[j:j + 1, :], (8, LANES)) for j in range(4)]

        def conv_item(tok, r0):
            halves = []
            for h in range(2):
                r = 8 + r0 + 8 * h
                ks = kf[r:r + 8, :] * jnp.where(never, tok, tapb[0])
                for j in range(1, 4):
                    ks = ks + kf[r - j:r - j + 8, :] * tapb[j]
                halves.append(ks)
            kvb[r0:r0 + 16, :] = (jnp.concatenate(halves, axis=0)
                                  * ain[sl, 1, r0:r0 + 16, :].astype(F32)).astype(BF16)

        _run_paced([functools.partial(conv_item, r0=r0) for r0 in range(0, S, 16)], toks)

        fwd = fwd_ref[...]
        hst = jnp.concatenate([ah[sl, :, b * BLK:(b + 1) * BLK] for b in range(NB)], axis=0)
        hh = lax.dot_general(fwd, hst, (((1,), (1,)), ((), ())), preferred_element_type=F32)
        for m in range(BLK // 8):
            hr = hh[16 * m:16 * m + 8]
            hi = hh[16 * m + 8:16 * m + 16]
            hf[16 * m:16 * m + 16, 0:BLK] = hh[16 * m:16 * m + 16, 0:BLK]
            if m < BLK // 16:
                hf[16 * m:16 * m + 8, BLK:] = hr[:, BLK:] - hi[:, :S - BLK]
                hf[16 * m + 8:16 * m + 16, BLK:] = hi[:, BLK:] + hr[:, :S - BLK]
            else:
                hf[16 * m:16 * m + 8, BLK:] = hr[:, BLK:] + hi[:, :S - BLK]
                hf[16 * m + 8:16 * m + 16, BLK:] = hi[:, BLK:] - hr[:, :S - BLK]
        rhs = jnp.concatenate([kvb[b * BLK:(b + 1) * BLK, :] for b in range(NB)], axis=1)
        xf[...] = _dot(fwd, rhs)

        toks = []
        for i in range(1, len(parts)):
            toks += run_part(i)
        items = []
        win = pl.ds(pl.multiple_of(zoff, 8), NFFT)
        for m in range(BLK // 8):
            items += freq_items(m, never, xf.at[win, :], hf.at[win, :])
        _run_paced(items, toks[:-80])

        y = _dot(inv_ref[...], wf[...])
        for b in range(NB):
            r0 = b * BLK
            yb = y[:, r0:r0 + BLK] + kvb[r0:r0 + BLK, :].astype(F32) * dvec
            aout[t, r0:r0 + BLK, :] = (ain[sl, 2, r0:r0 + BLK, :].astype(F32) * yb).astype(BF16)
        aout_copy(t).start()
        return carry

    wo_copy(0).start()
    lax.fori_loop(0, NT, tile_body, 0)
    pltpu.make_async_copy(wo, wo, sem_wo).wait()

    def initial_guess():
        puni = pl.reciprocal(jnp.full((1, 1), float(L), F32), approx=True).astype(BF16).astype(F32)

        def shift_down(m):
            rows = lax.broadcasted_iota(jnp.int32, m.shape, 0)
            return jnp.where(rows == 0, 0.0, pltpu.roll(m, 1, 0))

        m1 = shift_down(_dot((tsum[0:NSEG, :] * puni).astype(BF16), wo[...]))
        v1 = _dot(m1.astype(BF16), w_plain(WV, 0, H // 2)).astype(BF16).astype(F32)
        u2 = ((tsum[0:NSEG, :] + float(M) * v1) * puni).astype(BF16)
        m2 = shift_down(_dot(u2, wo[...]))
        mhat[...] = jnp.broadcast_to(m2[:, None, :], (NSEG, M, DM)).reshape(NSEG * M, DM)
        mhat[0:M, :] = mem0_ref[...].astype(F32)
        pltpu.make_async_copy(w32.at[WQ:WK + 1], w32.at[WQ:WK + 1], sem_wqk).wait()

    ri = lax.broadcasted_iota(jnp.int32, (PR, PR), 0)
    ci = lax.broadcasted_iota(jnp.int32, (PR, PR), 1)

    def seg_of(r):
        return jnp.where(r < MR, r // M, (r - MR) // SEG)

    def pos_of(r):
        return jnp.where(r < MR, r % M, M + (r - MR) % SEG)

    same = seg_of(ri) == seg_of(ci)
    allowed = same & ((ri < MR) | (pos_of(ri) >= pos_of(ci)))
    fill = jnp.where(same, -1e9, -jnp.inf).astype(F32)

    def sweep(state):
        it, _ = state
        pl.when(it == 0)(initial_guess)

        def mem_rows(i):
            n = PPB * MR
            return mhat[pl.ds(pl.multiple_of((i // NG) * n, n), n), :]

        def mem_lhs(i):
            m = mem_rows(i)
            n = PPH * MR
            ops = _strassen_lhs(m[:n, :KH], m[:n, KH:], m[n:, :KH], m[n:, KH:])
            return [_pack(o) for o in ops]

        def qk_proj(i, j, mops):
            rb = i // NG
            hp = (i % NG) * (G // 2) + j // 2

            def lhs(k):
                return _unpack(jnp.concatenate([mops[k], abuf[rb, k]], axis=0))

            (c11, c12, c21, c22), _ = _strassen(lhs, w_rhs(WQ + j % 2, hp, [zero_s[k] for k in range(7)]))
            n = PPH * MR
            for half, cc in enumerate(((c11, c12), (c21, c22))):
                v = jnp.concatenate(cc, axis=1).astype(BF16)
                ps = slice(half * PPH, (half + 1) * PPH)
                qks[j, ps, 0:MR, :] = v[:n].reshape(PPH, MR, 2 * E)
                qks[j, ps, MR:PR, :] = v[n:].reshape(PPH, XR, 2 * E)

        def vm_proj(i):
            g = i % NG
            vv = _dot(mem_rows(i).astype(BF16), w_plain(WV, g * (G // 2), G // 2))
            v0 = tsum[NSEG:NSEG + M, pl.ds(pl.multiple_of(g * (G * E), G * E), G * E)]
            vv = jnp.concatenate([jnp.where(i < NG, v0, vv[:M]), vv[M:]], axis=0)
            vms[...] = vv.astype(BF16).reshape(PPB, MR, G * E)

        def scores(j):
            c = slice((j % 2) * E, (j % 2 + 1) * E)
            return lax.dot_general(qks[2 * (j // 2), :, :, c], qks[2 * (j // 2) + 1, :, :, c],
                                   (((2,), (2,)), ((0,), (0,))), preferred_element_type=F32)

        def attend(i, j, s):
            p0 = pl.multiple_of((i // NG) * PPB, PPB)
            h = (i % NG) * G + j
            s = jnp.where(allowed[None], s * scale, fill[None])
            e = jnp.exp(s - jnp.max(s, axis=-1, keepdims=True))
            p = (e * pl.reciprocal(jnp.sum(e, axis=-1, keepdims=True), approx=True)).astype(BF16)
            vh = jnp.concatenate(
                [vms[:, :, j * E:(j + 1) * E],
                 vbuf[pl.ds(p0, PPB), :, pl.ds(pl.multiple_of(h * E, E), E)]], axis=1)
            return lax.dot_general(p, vh, (((2,), (1,)), ((0,), (0,))), preferred_element_type=F32)

        def out_proj(i, us):
            rb = i // NG
            g = i % NG
            u = jnp.concatenate(us, axis=2)
            wog = wo[pl.ds(pl.multiple_of(g * (G * E), G * E), G * E), :]
            rm = pl.ds(pl.multiple_of(rb * (PPB * MR), PPB * MR), PPB * MR)
            um = u[:, :MR, :].reshape(PPB * MR, G * E).astype(BF16)
            mnew[rm, :] = jnp.where(g > 0, mnew[rm, :], 0.0) + _dot(um, wog)
            n = PPH * XR
            kh = G * E // 2
            top = u[:PPH, MR:, :].reshape(n, G * E)
            bot = u[PPH:, MR:, :].reshape(n, G * E)
            ops = _strassen_lhs(top[:, :kh], top[:, kh:], bot[:, :kh], bot[:, kh:])
            wf32 = wog.astype(F32)
            rhs = _strassen_rhs(wf32[:kh, :KH], wf32[:kh, KH:], wf32[kh:, :KH], wf32[kh:, KH:])
            quads = [(slice(0, n), slice(0, KH)), (slice(0, n), slice(KH, DM)),
                     (slice(n, 2 * n), slice(0, KH)), (slice(n, 2 * n), slice(KH, DM))]
            init = [jnp.where(g > 0, acc[r, c], 0.0) for r, c in quads]
            cs, _ = _strassen(lambda k: ops[k].astype(BF16), rhs, init)
            for (r, c), v in zip(quads, cs):
                acc[r, c] = v
                obuf[rb, r, c] = v.astype(BF16)

        def step(i, nxt):
            s0, s1 = scores(0), scores(1)
            if nxt:
                mops = mem_lhs(i + 1)
                qk_proj(i + 1, 0, mops)
            u0, u1 = attend(i, 0, s0), attend(i, 1, s1)
            s2, s3 = scores(2), scores(3)
            if nxt:
                qk_proj(i + 1, 1, mops)
            u2, u3 = attend(i, 2, s2), attend(i, 3, s3)
            if nxt:
                qk_proj(i + 1, 2, mops)
                qk_proj(i + 1, 3, mops)
                vm_proj(i + 1)
            out_proj(i, [u0, u1, u2, u3])

        mops0 = mem_lhs(0)
        for j in range(G):
            qk_proj(0, j, mops0)
        vm_proj(0)

        def main_body(i, cy):
            step(i, True)

            @pl.when(i % NG == NG - 1)
            def _():
                o_copy(i // NG).start()

            return cy

        lax.fori_loop(0, NRB * NG - 1, main_body, 0)
        step(NRB * NG - 1, False)
        o_copy(NRB - 1).start()

        n = (NSEG - 1) * M
        new = mnew[0:n, :]
        err = jnp.max(jnp.abs(new - mhat[M:M + n, :]), axis=1, keepdims=True)
        ref = jnp.max(jnp.abs(new), axis=1, keepdims=True)
        ok = jnp.min(jnp.where(err <= TOL * ref, 1.0, 0.0))
        mhat[M:M + n, :] = new
        for rb in range(NRB):
            o_copy(rb).wait()
        return it + 1, (ok > 0.5).astype(jnp.int32)

    lax.while_loop(lambda st: jnp.logical_and(st[0] < NSEG, st[1] == 0), sweep,
                   (jnp.int32(0), jnp.int32(0)))
    pltpu.make_async_copy(aout, aout, sem_aout).wait()


@functools.partial(jax.jit, static_argnames=("B_seg_len",))
def pallas_concat_heads__ssm_conv_h3__memory_aug_recurrent_mem_tr__prompt_kernel(
    A_q, A_k, A_v, A_shift_k, A_ssm_k, A_ssm_D,
    B_x, B_mem0, B_Wq, B_Wk, B_Wv, B_Wo, B_seg_len,
):
    _, S, D = A_q.shape
    DM = B_x.shape[2]
    H, E = B_Wq.shape[1], B_Wq.shape[2]
    M = B_mem0.shape[1]
    SEG = int(B_seg_len)
    NSEG = S // SEG
    NP = NSEG // 2
    PR = 2 * (M + SEG)
    PPB = 8
    NRB = NP // PPB
    NT = D // LANES
    assert E == LANES and H == 32 and M == 8 and SEG == 32 and A_shift_k.shape[1] == 4
    assert S == 2048 and D == 1024 and DM == 1024

    fwd, inv = _dft_mats()
    any_spec = pl.BlockSpec(memory_space=pl.ANY)
    vmem_spec = pl.BlockSpec(memory_space=pltpu.VMEM)
    scratch = [
        pltpu.VMEM((NRB, 7, PPB // 2 * SEG, DM // 2), U32),
        pltpu.VMEM((7, M, DM // 2), U32),
        pltpu.VMEM((NP, 2 * SEG, H * E), BF16),
        pltpu.VMEM((3, H // 2, DM, E), U32),
        pltpu.VMEM((H * E, DM), BF16),
        pltpu.VMEM((4, PPB, PR, 2 * E), BF16),
        pltpu.VMEM((PPB, 2 * M, 4 * E), BF16),
        pltpu.VMEM((PPB * 2 * SEG, DM), F32),
        pltpu.VMEM((NRB, PPB * 2 * SEG, DM), BF16),
        pltpu.VMEM((NSEG * M, DM), F32),
        pltpu.VMEM((NSEG * M, DM), F32),
        pltpu.VMEM((NSEG + M, H * E), F32),
        pltpu.VMEM((2, 3, S, LANES), BF16),
        pltpu.VMEM((2, LANES, S), BF16),
        pltpu.VMEM((S + 8, LANES), F32),
        pltpu.VMEM((S, LANES), BF16),
        pltpu.VMEM((NFFT, S), F32),
        pltpu.VMEM((NFFT, S), F32),
        pltpu.VMEM((NFFT, S), BF16),
        pltpu.VMEM((NT, S, LANES), BF16),
        pltpu.VMEM((8, LANES), jnp.int32),
        pltpu.SMEM((8,), jnp.int32),
        pltpu.SemaphoreType.DMA((NRB,)),
        pltpu.SemaphoreType.DMA((H // 2,)),
        pltpu.SemaphoreType.DMA,
        pltpu.SemaphoreType.DMA,
        pltpu.SemaphoreType.DMA((2, 2)),
        pltpu.SemaphoreType.DMA,
        pltpu.SemaphoreType.DMA((NRB,)),
    ]
    out = pl.pallas_call(
        functools.partial(_kernel, S=S, D=D, DM=DM, H=H, M=M, SEG=SEG),
        out_shape=jax.ShapeDtypeStruct((S, D + DM), BF16),
        in_specs=[any_spec, any_spec, any_spec, vmem_spec, any_spec, vmem_spec,
                  any_spec, vmem_spec, any_spec, any_spec, any_spec, any_spec,
                  vmem_spec, vmem_spec],
        out_specs=any_spec,
        scratch_shapes=scratch,
        compiler_params=pltpu.CompilerParams(vmem_limit_bytes=120 * 1024 * 1024,
                                             disable_bounds_checks=True),
    )(
        A_q.reshape(S, D), A_k.reshape(S, D), A_v.reshape(S, D),
        A_shift_k.T, A_ssm_k, A_ssm_D.reshape(NT, LANES),
        B_x.reshape(NRB, S // NRB, DM), B_mem0.reshape(M, DM),
        B_Wq, B_Wk, B_Wv, B_Wo.reshape(H * E, DM),
        jnp.asarray(fwd, BF16), jnp.asarray(inv, BF16),
    )
    return out.reshape(1, S, D + DM)
```

```python
import functools

import numpy as np
import jax
import jax.numpy as jnp
from jax import lax
import jax.experimental.pallas as pl
import jax.experimental.pallas.tpu as pltpu

F32 = jnp.float32
BF16 = jnp.bfloat16
U32 = jnp.uint32

LANES = 128
BLK = 128
NFFT = 2 * BLK
TOL = 2.0 ** -10


def _dft_mats():
    order = np.concatenate([np.arange(0, BLK, 2), np.arange(1, BLK, 2)])
    theta = 2.0 * np.pi * (order + 0.5) / NFFT
    n = np.arange(BLK)
    c = np.cos(theta[:, None] * n[None, :])
    s = np.sin(theta[:, None] * n[None, :])
    fwd = np.zeros((NFFT, BLK))
    inv = np.zeros((BLK, NFFT))
    for m in range(BLK // 8):
        fwd[16 * m:16 * m + 8] = c[8 * m:8 * m + 8]
        fwd[16 * m + 8:16 * m + 16] = -s[8 * m:8 * m + 8]
        inv[:, 16 * m:16 * m + 8] = c[8 * m:8 * m + 8].T * (2.0 / NFFT)
        inv[:, 16 * m + 8:16 * m + 16] = -s[8 * m:8 * m + 8].T * (2.0 / NFFT)
    return fwd.astype(np.float32), inv.astype(np.float32)


def _dot(a, b):
    return jnp.dot(a, b, preferred_element_type=F32)


def _pack(x):
    return pltpu.bitcast(x.astype(BF16), U32)


def _unpack(w):
    return pltpu.bitcast(w, BF16)


def _lo(w):
    return pltpu.bitcast(w << 16, F32)


def _hi(w):
    return pltpu.bitcast(w & jnp.uint32(0xFFFF0000), F32)


def _strassen_lhs(a11, a12, a21, a22):
    return [a11 + a22, a21 + a22, a11, a22, a11 + a12, a21 - a11, a12 - a22]


def _strassen_rhs(b11, b12, b21, b22):
    ops = [b11 + b22, b11, b12 - b22, b21 - b11, b22, b11 + b12, b21 + b22]
    return [o.astype(BF16) for o in ops]


def _strassen(lhs, rhs, init=None):
    def add(c, m):
        return m if c is None else c + m

    c11, c12, c21, c22 = init if init is not None else (None,) * 4
    m5 = _dot(lhs(4), rhs[4])
    m3 = _dot(lhs(2), rhs[2])
    c12 = add(c12, m5) + m3
    m2 = _dot(lhs(1), rhs[1])
    c22 = add(c22, m3) - m2
    m4 = _dot(lhs(3), rhs[3])
    c21 = add(c21, m2) + m4
    c11 = add(c11, m4) - m5
    m1 = _dot(lhs(0), rhs[0])
    c11 = c11 + m1
    c22 = c22 + m1
    m7 = _dot(lhs(6), rhs[6])
    c11 = c11 + m7
    m6 = _dot(lhs(5), rhs[5])
    c22 = c22 + m6
    return (c11, c12, c21, c22), [m5, m3, m2, m4, m1, m7, m6]


def _run_paced(items, toks):
    for i, it in enumerate(items):
        it(toks[i * len(toks) // len(items)])


def _kernel(q_hbm, k_hbm, v_hbm, shift_ref, h_hbm, d_ref, x_hbm, mem0_ref,
            wq_hbm, wk_hbm, wv_hbm, wo_hbm, fwd_ref, inv_ref,
            out_hbm,
            abuf, a0buf, vbuf, w32, wo, qks, vms, acc, obuf, mhat, mnew, tsum,
            ain, ah, kf, kvb, xf, hf, wf, aout, zero_v, zero_s,
            sem_x, sem_wv, sem_wqk, sem_wo, sem_a, sem_aout, sem_o,
            *, S, D, DM, H, M, SEG):
    E = LANES
    NSEG = S // SEG
    NP = NSEG // 2
    MR = 2 * M
    XR = 2 * SEG
    PR = MR + XR
    MW, XW, PW = MR // 2, XR // 2, PR // 2
    L = M + SEG
    NB = S // BLK
    NT = D // LANES
    PPB = 8
    PPH = PPB // 2
    NRB = NP // PPB
    G = 4
    NG = H // G
    KH = DM // 2
    scale = float(E) ** -0.5
    WV, WQ, WK = 0, 1, 2

    def x_copy(rb):
        return pltpu.make_async_copy(x_hbm.at[rb], obuf.at[rb], sem_x.at[rb])

    def w_copy(which, hp):
        src = (wv_hbm, wq_hbm, wk_hbm)[which].bitcast(U32)
        sem = sem_wv.at[hp] if which == WV else sem_wqk
        return pltpu.make_async_copy(src.at[:, hp, :], w32.at[which, hp], sem)

    def wo_copy(t):
        n = H * E // NT
        r = pl.ds(pl.multiple_of(t * n, n), n)
        return pltpu.make_async_copy(wo_hbm.at[r, :], wo.at[r, :], sem_wo)

    def a_start(t, sl):
        c = pl.ds(pl.multiple_of(t * LANES, LANES), LANES)
        pltpu.make_async_copy(k_hbm.at[:, c], ain.at[sl, 0], sem_a.at[sl, 0]).start()
        pltpu.make_async_copy(v_hbm.at[:, c], ain.at[sl, 1], sem_a.at[sl, 0]).start()
        pltpu.make_async_copy(h_hbm.at[c, :], ah.at[sl], sem_a.at[sl, 1]).start()
        pltpu.make_async_copy(q_hbm.at[:, c], ain.at[sl, 2], sem_a.at[sl, 0]).start()

    def a_wait(sl):
        pltpu.make_async_copy(ain.at[sl], ain.at[sl], sem_a.at[sl, 0]).wait()
        pltpu.make_async_copy(ah.at[sl], ah.at[sl], sem_a.at[sl, 1]).wait()

    def aout_copy(t):
        c = pl.ds(pl.multiple_of(t * LANES, LANES), LANES)
        return pltpu.make_async_copy(aout.at[t], out_hbm.at[:, c], sem_aout)

    def o_copy(rb):
        r = pl.ds(pl.multiple_of(rb * (PPB * XR), PPB * XR), PPB * XR)
        return pltpu.make_async_copy(obuf.at[rb], out_hbm.at[r, pl.ds(D, DM)], sem_o.at[rb])

    def w_rhs(which, hp, zs=None):
        if zs is None:
            w = w32[which, hp]
            return _strassen_rhs(_lo(w[:KH]), _hi(w[:KH]), _lo(w[KH:]), _hi(w[KH:]))
        out = []
        for k in range(7):
            w = w32.at[which, hp + zs[k]]
            out.append(_strassen_rhs(_lo(w[:KH]), _hi(w[:KH]), _lo(w[KH:]), _hi(w[KH:]))[k])
        return out

    def w_plain(which, hp0, n):
        parts = []
        for j in range(n):
            w = w32[which, hp0 + j]
            parts += [_lo(w), _hi(w)]
        return jnp.concatenate(parts, axis=1).astype(BF16)

    for rb in range(NRB):
        x_copy(rb).start()
    w_copy(WV, 0).start()
    w_copy(WV, 1).start()
    a_start(0, 0)

    kf[0:8, :] = jnp.zeros((8, LANES), F32)
    zero_v[...] = jnp.zeros((8, LANES), jnp.int32)
    for k in range(8):
        zero_s[k] = 0
    tsum[0:8, :] = jnp.zeros((8, H * E), F32)
    vbuf[0, 0:16, :] = jnp.zeros((16, H * E), BF16)
    mem0 = mem0_ref[...].astype(F32)
    m0 = jnp.concatenate([mem0, jnp.zeros_like(mem0)], axis=0)
    z0 = jnp.zeros((MR, KH), F32)
    for k, op in enumerate(_strassen_lhs(m0[:, :KH], m0[:, KH:], z0, z0)):
        a0buf[k] = _pack(op)

    def x_prep(i, cy):
        rb = i // PPH
        pp = i % PPH

        @pl.when(pp == 0)
        def _():
            x_copy(rb).wait()

        top = obuf[rb, pl.ds(pl.multiple_of(pp * XR, XR), XR), :].astype(F32)
        bot = obuf[rb, pl.ds(pl.multiple_of((PPH + pp) * XR, XR), XR), :].astype(F32)
        for k, op in enumerate(_strassen_lhs(top[:, :KH], top[:, KH:], bot[:, :KH], bot[:, KH:])):
            abuf[rb, k, pl.ds(pl.multiple_of(pp * XW, XW), XW), :] = _pack(op)
        return cy

    lax.fori_loop(0, NRB * PPH, x_prep, 0)

    def v_part(j, rb, rhs, vwin, twin, pre=None):
        def lhs(k):
            x = abuf[rb, k]
            if rb == 0:
                x0 = a0buf[k]
                if pre is not None and k == 4:
                    x0 = jnp.concatenate([pre(x0[:, :LANES]), x0[:, LANES:]], axis=1)
                x = jnp.concatenate([x0, x], axis=0)
            return _unpack(x)

        (c11, c12, c21, c22), ms = _strassen(lhs, rhs)
        for half, hh, cv in ((0, 1, c12), (1, 0, c21), (0, 0, c11), (1, 1, c22)):
            c = slice((2 * j + hh) * E, (2 * j + hh + 1) * E)
            vv = cv.astype(BF16)
            vx = vv[MR:] if rb == 0 else vv
            p0 = rb * PPB + half * PPH
            vwin[p0:p0 + PPH, :, c] = vx.reshape(PPH, XR, E)
            ts = jnp.sum(vx.astype(F32).reshape(2 * PPH, SEG, E), axis=1)
            if rb == 0 and half == 0:
                v0 = vv[0:M].astype(F32)
                twin[NSEG:NSEG + M, c] = v0
                t0 = jnp.sum(v0, axis=0, keepdims=True)
                rows = lax.broadcasted_iota(jnp.int32, ts.shape, 0)
                ts = ts + jnp.where(rows == 0, t0, 0.0)
            twin[2 * p0:2 * (p0 + PPH), c] = ts
        return [m[8 * g:8 * g + 8] for m in ms for g in range(m.shape[0] // 8)]

    GA = 4

    def freq_items(m, never):
        r_re = slice(16 * m, 16 * m + 8)
        r_im = slice(16 * m + 8, 16 * m + 16)

        def item(tok, a0, cc, st):
            xr = jnp.where(never, tok, xf[r_re, cc * BLK:(cc + 1) * BLK])
            xi = jnp.where(never, tok, xf[r_im, cc * BLK:(cc + 1) * BLK])
            for a in range(max(a0, cc), a0 + GA):
                j = a - cc
                if ('g', j) not in st:
                    st['g', j] = (hf[r_re, j * BLK:(j + 1) * BLK], hf[r_im, j * BLK:(j + 1) * BLK])
                gr, gi = st['g', j]
                ps = (xr * gr - xi * gi, xr * gi + xi * gr)
                st[a] = ps if a not in st else (st[a][0] + ps[0], st[a][1] + ps[1])
                if cc == a:
                    wf[16 * m:16 * m + 16, a * BLK:(a + 1) * BLK] = (
                        jnp.concatenate(st[a], axis=0).astype(BF16))

        items = []
        for a0 in range(0, NB, GA):
            st = {}
            items += [functools.partial(item, a0=a0, cc=cc, st=st) for cc in range(a0 + GA)]
        return items

    def tile_body(t, carry):
        sl = t % 2
        a_wait(sl)
        w_copy(WV, 2 * t).wait()
        w_copy(WV, 2 * t + 1).wait()

        @pl.when(t + 1 < NT)
        def _():
            w_copy(WV, 2 * t + 2).start()
            w_copy(WV, 2 * t + 3).start()
            a_start(t + 1, 1 - sl)
            wo_copy(t + 1).start()

        for which in (WQ, WK):
            w_copy(which, 2 * t).start()
            w_copy(which, 2 * t + 1).start()

        c = pl.ds(pl.multiple_of(t * LANES, LANES), LANES)
        taps = shift_ref[:, c].astype(F32)
        dcol = d_ref[...].astype(F32)
        rows = lax.broadcasted_iota(jnp.int32, dcol.shape, 0)
        dvec = jnp.sum(jnp.where(rows == t, dcol, 0.0), axis=0, keepdims=True)
        never = zero_v[...] > 0
        zs = [zero_s[k] for k in range(7)]

        rhs2 = [w_rhs(WV, 2 * t, zs), w_rhs(WV, 2 * t + 1, zs)]
        parts = [(j, rb) for j in range(2) for rb in range(NRB)]
        c4 = pl.ds(pl.multiple_of(t * (4 * E), 4 * E), 4 * E)
        vwin = vbuf.at[:, :, c4]
        twin = tsum.at[:, c4]

        def pre(x):
            x = jnp.where(never, pltpu.bitcast(twin[0:8, 0:LANES], U32), x)
            return jnp.where(never, pltpu.bitcast(vwin[0, 0:16, 0:LANES], U32), x)


        def run_part(i):
            j, rb = parts[i]
            return v_part(j, rb, rhs2[j], vwin, twin, pre if i == 0 else None)

        toks = run_part(0)

        kf[8:8 + S, :] = ain[sl, 0].astype(F32)
        tapb = [jnp.broadcast_to(taps[j:j + 1, :], (8, LANES)) for j in range(4)]

        def conv_item(tok, r0):
            halves = []
            for h in range(2):
                r = 8 + r0 + 8 * h
                ks = kf[r:r + 8, :] * jnp.where(never, tok, tapb[0])
                for j in range(1, 4):
                    ks = ks + kf[r - j:r - j + 8, :] * tapb[j]
                halves.append(ks)
            kvb[r0:r0 + 16, :] = (jnp.concatenate(halves, axis=0)
                                  * ain[sl, 1, r0:r0 + 16, :].astype(F32)).astype(BF16)

        _run_paced([functools.partial(conv_item, r0=r0) for r0 in range(0, S, 16)], toks)

        fwd = fwd_ref[...]
        hst = jnp.concatenate([ah[sl, :, b * BLK:(b + 1) * BLK] for b in range(NB)], axis=0)
        hh = lax.dot_general(fwd, hst, (((1,), (1,)), ((), ())), preferred_element_type=F32)
        for m in range(BLK // 8):
            hr = hh[16 * m:16 * m + 8]
            hi = hh[16 * m + 8:16 * m + 16]
            hf[16 * m:16 * m + 16, 0:BLK] = hh[16 * m:16 * m + 16, 0:BLK]
            if m < BLK // 16:
                hf[16 * m:16 * m + 8, BLK:] = hr[:, BLK:] - hi[:, :S - BLK]
                hf[16 * m + 8:16 * m + 16, BLK:] = hi[:, BLK:] + hr[:, :S - BLK]
            else:
                hf[16 * m:16 * m + 8, BLK:] = hr[:, BLK:] + hi[:, :S - BLK]
                hf[16 * m + 8:16 * m + 16, BLK:] = hi[:, BLK:] - hr[:, :S - BLK]
        rhs = jnp.concatenate([kvb[b * BLK:(b + 1) * BLK, :] for b in range(NB)], axis=1)
        xf[...] = _dot(fwd, rhs)

        toks = []
        for i in range(1, len(parts)):
            toks += run_part(i)
        items = []
        for m in range(BLK // 8):
            items += freq_items(m, never)
        _run_paced(items, toks[:-80])

        y = _dot(inv_ref[...], wf[...])
        for b in range(NB):
            r0 = b * BLK
            yb = y[:, r0:r0 + BLK] + kvb[r0:r0 + BLK, :].astype(F32) * dvec
            aout[t, r0:r0 + BLK, :] = (ain[sl, 2, r0:r0 + BLK, :].astype(F32) * yb).astype(BF16)
        aout_copy(t).start()
        return carry

    wo_copy(0).start()
    lax.fori_loop(0, NT, tile_body, 0)
    pltpu.make_async_copy(wo, wo, sem_wo).wait()

    def initial_guess():
        puni = pl.reciprocal(jnp.full((1, 1), float(L), F32), approx=True).astype(BF16).astype(F32)

        def shift_down(m):
            rows = lax.broadcasted_iota(jnp.int32, m.shape, 0)
            return jnp.where(rows == 0, 0.0, pltpu.roll(m, 1, 0))

        m1 = shift_down(_dot((tsum[0:NSEG, :] * puni).astype(BF16), wo[...]))
        v1 = _dot(m1.astype(BF16), w_plain(WV, 0, H // 2)).astype(BF16).astype(F32)
        u2 = ((tsum[0:NSEG, :] + float(M) * v1) * puni).astype(BF16)
        m2 = shift_down(_dot(u2, wo[...]))
        mhat[...] = jnp.broadcast_to(m2[:, None, :], (NSEG, M, DM)).reshape(NSEG * M, DM)
        mhat[0:M, :] = mem0_ref[...].astype(F32)
        pltpu.make_async_copy(w32.at[WQ:WK + 1], w32.at[WQ:WK + 1], sem_wqk).wait()

    ri = lax.broadcasted_iota(jnp.int32, (PR, PR), 0)
    ci = lax.broadcasted_iota(jnp.int32, (PR, PR), 1)

    def seg_of(r):
        return jnp.where(r < MR, r // M, (r - MR) // SEG)

    def pos_of(r):
        return jnp.where(r < MR, r % M, M + (r - MR) % SEG)

    same = seg_of(ri) == seg_of(ci)
    allowed = same & ((ri < MR) | (pos_of(ri) >= pos_of(ci)))
    fill = jnp.where(same, -1e9, -jnp.inf).astype(F32)

    def sweep(state):
        it, _ = state
        pl.when(it == 0)(initial_guess)

        def mem_rows(i):
            n = PPB * MR
            return mhat[pl.ds(pl.multiple_of((i // NG) * n, n), n), :]

        def mem_lhs(i):
            m = mem_rows(i)
            n = PPH * MR
            ops = _strassen_lhs(m[:n, :KH], m[:n, KH:], m[n:, :KH], m[n:, KH:])
            return [_pack(o) for o in ops]

        def qk_proj(i, j, mops):
            rb = i // NG
            hp = (i % NG) * (G // 2) + j // 2

            def lhs(k):
                return _unpack(jnp.concatenate([mops[k], abuf[rb, k]], axis=0))

            (c11, c12, c21, c22), _ = _strassen(lhs, w_rhs(WQ + j % 2, hp, [zero_s[k] for k in range(7)]))
            n = PPH * MR
            for half, cc in enumerate(((c11, c12), (c21, c22))):
                v = jnp.concatenate(cc, axis=1).astype(BF16)
                ps = slice(half * PPH, (half + 1) * PPH)
                qks[j, ps, 0:MR, :] = v[:n].reshape(PPH, MR, 2 * E)
                qks[j, ps, MR:PR, :] = v[n:].reshape(PPH, XR, 2 * E)

        def vm_proj(i):
            g = i % NG
            vv = _dot(mem_rows(i).astype(BF16), w_plain(WV, g * (G // 2), G // 2))
            v0 = tsum[NSEG:NSEG + M, pl.ds(pl.multiple_of(g * (G * E), G * E), G * E)]
            vv = jnp.concatenate([jnp.where(i < NG, v0, vv[:M]), vv[M:]], axis=0)
            vms[...] = vv.astype(BF16).reshape(PPB, MR, G * E)

        def scores(j):
            c = slice((j % 2) * E, (j % 2 + 1) * E)
            return lax.dot_general(qks[2 * (j // 2), :, :, c], qks[2 * (j // 2) + 1, :, :, c],
                                   (((2,), (2,)), ((0,), (0,))), preferred_element_type=F32)

        def attend(i, j, s):
            p0 = pl.multiple_of((i // NG) * PPB, PPB)
            h = (i % NG) * G + j
            s = jnp.where(allowed[None], s * scale, fill[None])
            e = jnp.exp(s - jnp.max(s, axis=-1, keepdims=True))
            p = (e * pl.reciprocal(jnp.sum(e, axis=-1, keepdims=True), approx=True)).astype(BF16)
            vh = jnp.concatenate(
                [vms[:, :, j * E:(j + 1) * E],
                 vbuf[pl.ds(p0, PPB), :, pl.ds(pl.multiple_of(h * E, E), E)]], axis=1)
            return lax.dot_general(p, vh, (((2,), (1,)), ((0,), (0,))), preferred_element_type=F32)

        def out_proj(i, us):
            rb = i // NG
            g = i % NG
            u = jnp.concatenate(us, axis=2)
            wog = wo[pl.ds(pl.multiple_of(g * (G * E), G * E), G * E), :]
            rm = pl.ds(pl.multiple_of(rb * (PPB * MR), PPB * MR), PPB * MR)
            um = u[:, :MR, :].reshape(PPB * MR, G * E).astype(BF16)
            mnew[rm, :] = jnp.where(g > 0, mnew[rm, :], 0.0) + _dot(um, wog)
            n = PPH * XR
            kh = G * E // 2
            top = u[:PPH, MR:, :].reshape(n, G * E)
            bot = u[PPH:, MR:, :].reshape(n, G * E)
            ops = _strassen_lhs(top[:, :kh], top[:, kh:], bot[:, :kh], bot[:, kh:])
            wf32 = wog.astype(F32)
            rhs = _strassen_rhs(wf32[:kh, :KH], wf32[:kh, KH:], wf32[kh:, :KH], wf32[kh:, KH:])
            quads = [(slice(0, n), slice(0, KH)), (slice(0, n), slice(KH, DM)),
                     (slice(n, 2 * n), slice(0, KH)), (slice(n, 2 * n), slice(KH, DM))]
            init = [jnp.where(g > 0, acc[r, c], 0.0) for r, c in quads]
            cs, _ = _strassen(lambda k: ops[k].astype(BF16), rhs, init)
            for (r, c), v in zip(quads, cs):
                acc[r, c] = v
                obuf[rb, r, c] = v.astype(BF16)

        def step(i, nxt):
            s0, s1 = scores(0), scores(1)
            if nxt:
                mops = mem_lhs(i + 1)
                qk_proj(i + 1, 0, mops)
            u0, u1 = attend(i, 0, s0), attend(i, 1, s1)
            s2, s3 = scores(2), scores(3)
            if nxt:
                qk_proj(i + 1, 1, mops)
            u2, u3 = attend(i, 2, s2), attend(i, 3, s3)
            if nxt:
                qk_proj(i + 1, 2, mops)
                qk_proj(i + 1, 3, mops)
                vm_proj(i + 1)
            out_proj(i, [u0, u1, u2, u3])

        mops0 = mem_lhs(0)
        for j in range(G):
            qk_proj(0, j, mops0)
        vm_proj(0)

        def main_body(i, cy):
            step(i, True)

            @pl.when(i % NG == NG - 1)
            def _():
                o_copy(i // NG).start()

            return cy

        lax.fori_loop(0, NRB * NG - 1, main_body, 0)
        step(NRB * NG - 1, False)
        o_copy(NRB - 1).start()

        n = (NSEG - 1) * M
        new = mnew[0:n, :]
        err = jnp.max(jnp.abs(new - mhat[M:M + n, :]), axis=1, keepdims=True)
        ref = jnp.max(jnp.abs(new), axis=1, keepdims=True)
        ok = jnp.min(jnp.where(err <= TOL * ref, 1.0, 0.0))
        mhat[M:M + n, :] = new
        for rb in range(NRB):
            o_copy(rb).wait()
        return it + 1, (ok > 0.5).astype(jnp.int32)

    lax.while_loop(lambda st: jnp.logical_and(st[0] < NSEG, st[1] == 0), sweep,
                   (jnp.int32(0), jnp.int32(0)))
    pltpu.make_async_copy(aout, aout, sem_aout).wait()


@functools.partial(jax.jit, static_argnames=("B_seg_len",))
def pallas_concat_heads__ssm_conv_h3__memory_aug_recurrent_mem_tr__prompt_kernel(
    A_q, A_k, A_v, A_shift_k, A_ssm_k, A_ssm_D,
    B_x, B_mem0, B_Wq, B_Wk, B_Wv, B_Wo, B_seg_len,
):
    _, S, D = A_q.shape
    DM = B_x.shape[2]
    H, E = B_Wq.shape[1], B_Wq.shape[2]
    M = B_mem0.shape[1]
    SEG = int(B_seg_len)
    NSEG = S // SEG
    NP = NSEG // 2
    PR = 2 * (M + SEG)
    PPB = 8
    NRB = NP // PPB
    NT = D // LANES
    assert E == LANES and H == 32 and M == 8 and SEG == 32 and A_shift_k.shape[1] == 4
    assert S == 2048 and D == 1024 and DM == 1024

    fwd, inv = _dft_mats()
    any_spec = pl.BlockSpec(memory_space=pl.ANY)
    vmem_spec = pl.BlockSpec(memory_space=pltpu.VMEM)
    scratch = [
        pltpu.VMEM((NRB, 7, PPB // 2 * SEG, DM // 2), U32),
        pltpu.VMEM((7, M, DM // 2), U32),
        pltpu.VMEM((NP, 2 * SEG, H * E), BF16),
        pltpu.VMEM((3, H // 2, DM, E), U32),
        pltpu.VMEM((H * E, DM), BF16),
        pltpu.VMEM((4, PPB, PR, 2 * E), BF16),
        pltpu.VMEM((PPB, 2 * M, 4 * E), BF16),
        pltpu.VMEM((PPB * 2 * SEG, DM), F32),
        pltpu.VMEM((NRB, PPB * 2 * SEG, DM), BF16),
        pltpu.VMEM((NSEG * M, DM), F32),
        pltpu.VMEM((NSEG * M, DM), F32),
        pltpu.VMEM((NSEG + M, H * E), F32),
        pltpu.VMEM((2, 3, S, LANES), BF16),
        pltpu.VMEM((2, LANES, S), BF16),
        pltpu.VMEM((S + 8, LANES), F32),
        pltpu.VMEM((S, LANES), BF16),
        pltpu.VMEM((NFFT, S), F32),
        pltpu.VMEM((NFFT, S), F32),
        pltpu.VMEM((NFFT, S), BF16),
        pltpu.VMEM((NT, S, LANES), BF16),
        pltpu.VMEM((8, LANES), jnp.int32),
        pltpu.SMEM((8,), jnp.int32),
        pltpu.SemaphoreType.DMA((NRB,)),
        pltpu.SemaphoreType.DMA((H // 2,)),
        pltpu.SemaphoreType.DMA,
        pltpu.SemaphoreType.DMA,
        pltpu.SemaphoreType.DMA((2, 2)),
        pltpu.SemaphoreType.DMA,
        pltpu.SemaphoreType.DMA((NRB,)),
    ]
    out = pl.pallas_call(
        functools.partial(_kernel, S=S, D=D, DM=DM, H=H, M=M, SEG=SEG),
        out_shape=jax.ShapeDtypeStruct((S, D + DM), BF16),
        in_specs=[any_spec, any_spec, any_spec, vmem_spec, any_spec, vmem_spec,
                  any_spec, vmem_spec, any_spec, any_spec, any_spec, any_spec,
                  vmem_spec, vmem_spec],
        out_specs=any_spec,
        scratch_shapes=scratch,
        compiler_params=pltpu.CompilerParams(vmem_limit_bytes=120 * 1024 * 1024,
                                             disable_bounds_checks=True),
    )(
        A_q.reshape(S, D), A_k.reshape(S, D), A_v.reshape(S, D),
        A_shift_k.T, A_ssm_k, A_ssm_D.reshape(NT, LANES),
        B_x.reshape(NRB, S // NRB, DM), B_mem0.reshape(M, DM),
        B_Wq, B_Wk, B_Wv, B_Wo.reshape(H * E, DM),
        jnp.asarray(fwd, BF16), jnp.asarray(inv, BF16),
    )
    return out.reshape(1, S, D + DM)
```

```python
import functools

import numpy as np
import jax
import jax.numpy as jnp
from jax import lax
import jax.experimental.pallas as pl
import jax.experimental.pallas.tpu as pltpu

F32 = jnp.float32
BF16 = jnp.bfloat16
U32 = jnp.uint32

LANES = 128
BLK = 128
NFFT = 2 * BLK
TOL = 2.0 ** -10


def _dft_mats():
    even = np.arange(0, BLK, 2)
    theta = 2.0 * np.pi * (np.concatenate([even, BLK - 1 - even]) + 0.5) / NFFT
    n = np.arange(BLK)
    c = np.cos(theta[:, None] * n[None, :])
    s = np.sin(theta[:, None] * n[None, :])
    fwd = np.zeros((NFFT, BLK))
    for m in range(BLK // 8):
        fwd[16 * m:16 * m + 8] = c[8 * m:8 * m + 8]
        fwd[16 * m + 8:16 * m + 16] = -s[8 * m:8 * m + 8]
    inv = fwd[:BLK].T * (2.0 / NFFT)
    inv = np.concatenate([inv[0::2], inv[1::2]], axis=0)
    return fwd.astype(np.float32), inv.astype(np.float32)


def _dot(a, b):
    return jnp.dot(a, b, preferred_element_type=F32)


def _pack(x):
    return pltpu.bitcast(x.astype(BF16), U32)


def _unpack(w):
    return pltpu.bitcast(w, BF16)


def _lo(w):
    return pltpu.bitcast(w << 16, F32)


def _hi(w):
    return pltpu.bitcast(w & jnp.uint32(0xFFFF0000), F32)


def _strassen_lhs(a11, a12, a21, a22):
    return [a11 + a22, a21 + a22, a11, a22, a11 + a12, a21 - a11, a12 - a22]


def _strassen_rhs(b11, b12, b21, b22):
    ops = [b11 + b22, b11, b12 - b22, b21 - b11, b22, b11 + b12, b21 + b22]
    return [o.astype(BF16) for o in ops]


def _strassen(lhs, rhs, init=None):
    def add(c, m):
        return m if c is None else c + m

    c11, c12, c21, c22 = init if init is not None else (None,) * 4
    m5 = _dot(lhs(4), rhs[4])
    m3 = _dot(lhs(2), rhs[2])
    c12 = add(c12, m5) + m3
    m2 = _dot(lhs(1), rhs[1])
    c22 = add(c22, m3) - m2
    m4 = _dot(lhs(3), rhs[3])
    c21 = add(c21, m2) + m4
    c11 = add(c11, m4) - m5
    m1 = _dot(lhs(0), rhs[0])
    c11 = c11 + m1
    c22 = c22 + m1
    m7 = _dot(lhs(6), rhs[6])
    c11 = c11 + m7
    m6 = _dot(lhs(5), rhs[5])
    c22 = c22 + m6
    return (c11, c12, c21, c22), [m5, m3, m2, m4, m1, m7, m6]


def _run_paced(items, toks):
    for i, it in enumerate(items):
        it(toks[i * len(toks) // len(items)])


def _kernel(q_hbm, k_hbm, v_hbm, shift_ref, h_hbm, d_ref, x_hbm, mem0_ref,
            wq_hbm, wk_hbm, wv_hbm, wo_hbm, fwd_ref, inv_ref,
            out_hbm,
            abuf, a0buf, vbuf, w32, wo, qks, vms, acc, obuf, mhat, mnew, tsum,
            ain, ah, kf, kvb, xf, hf, wf, yt, aout, zero_v, zero_s,
            sem_x, sem_wv, sem_wqk, sem_wo, sem_a, sem_aout, sem_o,
            *, S, D, DM, H, M, SEG):
    E = LANES
    NSEG = S // SEG
    NP = NSEG // 2
    MR = 2 * M
    XR = 2 * SEG
    PR = MR + XR
    MW, XW, PW = MR // 2, XR // 2, PR // 2
    L = M + SEG
    NB = S // BLK
    NT = D // LANES
    PPB = 8
    PPH = PPB // 2
    NRB = NP // PPB
    G = 4
    NG = H // G
    KH = DM // 2
    scale = float(E) ** -0.5
    WV, WQ, WK = 0, 1, 2

    def x_copy(rb):
        return pltpu.make_async_copy(x_hbm.at[rb], obuf.at[rb], sem_x.at[rb])

    def w_copy(which, hp):
        src = (wv_hbm, wq_hbm, wk_hbm)[which].bitcast(U32)
        sem = sem_wv.at[hp] if which == WV else sem_wqk
        return pltpu.make_async_copy(src.at[:, hp, :], w32.at[which, hp], sem)

    def wo_copy(t):
        n = H * E // NT
        r = pl.ds(pl.multiple_of(t * n, n), n)
        return pltpu.make_async_copy(wo_hbm.at[r, :], wo.at[r, :], sem_wo)

    def a_start(t, sl):
        c = pl.ds(pl.multiple_of(t * LANES, LANES), LANES)
        pltpu.make_async_copy(k_hbm.at[:, c], ain.at[sl, 0], sem_a.at[sl, 0]).start()
        pltpu.make_async_copy(v_hbm.at[:, c], ain.at[sl, 1], sem_a.at[sl, 0]).start()
        pltpu.make_async_copy(h_hbm.at[c, :], ah.at[sl], sem_a.at[sl, 1]).start()
        pltpu.make_async_copy(q_hbm.at[:, c], ain.at[sl, 2], sem_a.at[sl, 0]).start()

    def a_wait(sl):
        pltpu.make_async_copy(ain.at[sl], ain.at[sl], sem_a.at[sl, 0]).wait()
        pltpu.make_async_copy(ah.at[sl], ah.at[sl], sem_a.at[sl, 1]).wait()

    def aout_copy(t):
        c = pl.ds(pl.multiple_of(t * LANES, LANES), LANES)
        return pltpu.make_async_copy(aout.at[t], out_hbm.at[:, c], sem_aout)

    def o_copy(rb):
        r = pl.ds(pl.multiple_of(rb * (PPB * XR), PPB * XR), PPB * XR)
        return pltpu.make_async_copy(obuf.at[rb], out_hbm.at[r, pl.ds(D, DM)], sem_o.at[rb])

    def w_rhs(which, hp, zs=None):
        if zs is None:
            w = w32[which, hp]
            return _strassen_rhs(_lo(w[:KH]), _hi(w[:KH]), _lo(w[KH:]), _hi(w[KH:]))
        out = []
        for k in range(7):
            w = w32.at[which, hp + zs[k]]
            out.append(_strassen_rhs(_lo(w[:KH]), _hi(w[:KH]), _lo(w[KH:]), _hi(w[KH:]))[k])
        return out

    def w_plain(which, hp0, n):
        parts = []
        for j in range(n):
            w = w32[which, hp0 + j]
            parts += [_lo(w), _hi(w)]
        return jnp.concatenate(parts, axis=1).astype(BF16)

    for rb in range(NRB):
        x_copy(rb).start()
    w_copy(WV, 0).start()
    w_copy(WV, 1).start()
    a_start(0, 0)

    kf[0:8, :] = jnp.zeros((8, LANES), F32)
    zero_v[...] = jnp.zeros((8, LANES), jnp.int32)
    for k in range(8):
        zero_s[k] = 0
    tsum[0:8, :] = jnp.zeros((8, H * E), F32)
    vbuf[0, 0:16, :] = jnp.zeros((16, H * E), BF16)
    mem0 = mem0_ref[...].astype(F32)
    m0 = jnp.concatenate([mem0, jnp.zeros_like(mem0)], axis=0)
    z0 = jnp.zeros((MR, KH), F32)
    for k, op in enumerate(_strassen_lhs(m0[:, :KH], m0[:, KH:], z0, z0)):
        a0buf[k] = _pack(op)

    def x_prep(i, cy):
        rb = i // PPH
        pp = i % PPH

        @pl.when(pp == 0)
        def _():
            x_copy(rb).wait()

        top = obuf[rb, pl.ds(pl.multiple_of(pp * XR, XR), XR), :].astype(F32)
        bot = obuf[rb, pl.ds(pl.multiple_of((PPH + pp) * XR, XR), XR), :].astype(F32)
        for k, op in enumerate(_strassen_lhs(top[:, :KH], top[:, KH:], bot[:, :KH], bot[:, KH:])):
            abuf[rb, k, pl.ds(pl.multiple_of(pp * XW, XW), XW), :] = _pack(op)
        return cy

    lax.fori_loop(0, NRB * PPH, x_prep, 0)

    def v_part(j, rb, rhs, vwin, twin, pre=None):
        def lhs(k):
            x = abuf[rb, k]
            if rb == 0:
                x0 = a0buf[k]
                if pre is not None and k == 4:
                    x0 = jnp.concatenate([pre(x0[:, :LANES]), x0[:, LANES:]], axis=1)
                x = jnp.concatenate([x0, x], axis=0)
            return _unpack(x)

        (c11, c12, c21, c22), ms = _strassen(lhs, rhs)
        for half, hh, cv in ((0, 1, c12), (1, 0, c21), (0, 0, c11), (1, 1, c22)):
            c = slice((2 * j + hh) * E, (2 * j + hh + 1) * E)
            vv = cv.astype(BF16)
            vx = vv[MR:] if rb == 0 else vv
            p0 = rb * PPB + half * PPH
            vwin[p0:p0 + PPH, :, c] = vx.reshape(PPH, XR, E)
            ts = jnp.sum(vx.astype(F32).reshape(2 * PPH, SEG, E), axis=1)
            if rb == 0 and half == 0:
                v0 = vv[0:M].astype(F32)
                twin[NSEG:NSEG + M, c] = v0
                t0 = jnp.sum(v0, axis=0, keepdims=True)
                rows = lax.broadcasted_iota(jnp.int32, ts.shape, 0)
                ts = ts + jnp.where(rows == 0, t0, 0.0)
            twin[2 * p0:2 * (p0 + PPH), c] = ts
        return [m[8 * g:8 * g + 8] for m in ms for g in range(m.shape[0] // 8)]

    GA = 4

    def freq_items(a0, never):
        def item(tok, m, cc, st):
            r_re = slice(16 * m, 16 * m + 8)
            r_im = slice(16 * m + 8, 16 * m + 16)
            xr = jnp.where(never, tok, xf[r_re, cc * BLK:(cc + 1) * BLK])
            xi = jnp.where(never, tok, xf[r_im, cc * BLK:(cc + 1) * BLK])
            xs = xr + xi
            for a in range(max(a0, cc), a0 + GA):
                j = a - cc
                if ('g', m, j) not in st:
                    gr = hf[r_re, j * BLK:(j + 1) * BLK]
                    gi = hf[r_im, j * BLK:(j + 1) * BLK]
                    st['g', m, j] = (gr, gi, gr + gi)
                gr, gi, gs = st['g', m, j]
                ps = (xr * gr, xi * gi, xs * gs)
                st[m, a] = ps if (m, a) not in st else tuple(u + v for u, v in zip(st[m, a], ps))
                if cc == a:
                    p1, p2, p3 = st[m, a]
                    st[m, a] = (p1 - p2, p3 - p1 - p2)
                    if m >= BLK // 16:
                        m0 = m - BLK // 16
                        (wr, wi), (vr, vi) = st[m0, a], st[m, a]
                        c = slice(a * BLK, (a + 1) * BLK)
                        wf[16 * m0:16 * m0 + 16, c] = (
                            jnp.concatenate([wr + vr, wi - vi], axis=0).astype(BF16))
                        wf[16 * m:16 * m + 16, c] = (
                            jnp.concatenate([wr - vr, wi + vi], axis=0).astype(BF16))

        items = []
        for m0 in range(BLK // 16):
            st = {}
            for m in (m0, m0 + BLK // 16):
                items += [functools.partial(item, m=m, cc=cc, st=st) for cc in range(a0 + GA)]
        return items

    def tile_body(t, carry):
        sl = t % 2
        a_wait(sl)
        w_copy(WV, 2 * t).wait()
        w_copy(WV, 2 * t + 1).wait()

        @pl.when(t + 1 < NT)
        def _():
            w_copy(WV, 2 * t + 2).start()
            w_copy(WV, 2 * t + 3).start()
            a_start(t + 1, 1 - sl)
            wo_copy(t + 1).start()

        for which in (WQ, WK):
            w_copy(which, 2 * t).start()
            w_copy(which, 2 * t + 1).start()

        c = pl.ds(pl.multiple_of(t * LANES, LANES), LANES)
        taps = shift_ref[:, c].astype(F32)
        dcol = d_ref[...].astype(F32)
        rows = lax.broadcasted_iota(jnp.int32, dcol.shape, 0)
        dvec = jnp.sum(jnp.where(rows == t, dcol, 0.0), axis=0, keepdims=True)
        never = zero_v[...] > 0
        zs = [zero_s[k] for k in range(7)]

        rhs2 = [w_rhs(WV, 2 * t, zs), w_rhs(WV, 2 * t + 1, zs)]
        parts = [(j, rb) for j in range(2) for rb in range(NRB)]
        c4 = pl.ds(pl.multiple_of(t * (4 * E), 4 * E), 4 * E)
        vwin = vbuf.at[:, :, c4]
        twin = tsum.at[:, c4]

        def pre(x):
            x = jnp.where(never, pltpu.bitcast(twin[0:8, 0:LANES], U32), x)
            return jnp.where(never, pltpu.bitcast(vwin[0, 0:16, 0:LANES], U32), x)


        def run_part(i):
            j, rb = parts[i]
            return v_part(j, rb, rhs2[j], vwin, twin, pre if i == 0 else None)

        toks = run_part(0)

        kf[8:8 + S, :] = ain[sl, 0].astype(F32)
        tapb = [jnp.broadcast_to(taps[j:j + 1, :], (8, LANES)) for j in range(4)]

        def conv_item(tok, r0):
            halves = []
            for h in range(2):
                r = 8 + r0 + 8 * h
                ks = kf[r:r + 8, :] * jnp.where(never, tok, tapb[0])
                for j in range(1, 4):
                    ks = ks + kf[r - j:r - j + 8, :] * tapb[j]
                halves.append(ks)
            kvb[r0:r0 + 16, :] = (jnp.concatenate(halves, axis=0)
                                  * ain[sl, 1, r0:r0 + 16, :].astype(F32)).astype(BF16)

        _run_paced([functools.partial(conv_item, r0=r0) for r0 in range(0, S, 16)], toks)

        fwd = fwd_ref[...]
        hst = jnp.concatenate([ah[sl, :, b * BLK:(b + 1) * BLK] for b in range(NB)], axis=0)
        hh = lax.dot_general(fwd, hst, (((1,), (1,)), ((), ())), preferred_element_type=F32)
        for m in range(BLK // 8):
            hr = hh[16 * m:16 * m + 8]
            hi = hh[16 * m + 8:16 * m + 16]
            hf[16 * m:16 * m + 16, 0:BLK] = hh[16 * m:16 * m + 16, 0:BLK]
            if m < BLK // 16:
                hf[16 * m:16 * m + 8, BLK:] = hr[:, BLK:] - hi[:, :S - BLK]
                hf[16 * m + 8:16 * m + 16, BLK:] = hi[:, BLK:] + hr[:, :S - BLK]
            else:
                hf[16 * m:16 * m + 8, BLK:] = hr[:, BLK:] + hi[:, :S - BLK]
                hf[16 * m + 8:16 * m + 16, BLK:] = hi[:, BLK:] - hr[:, :S - BLK]
        rhs = jnp.concatenate([kvb[b * BLK:(b + 1) * BLK, :] for b in range(NB)], axis=1)
        xf[...] = _dot(fwd, rhs)

        def inverse(a0):
            c = slice(a0 * BLK, (a0 + GA) * BLK)
            for par in range(2):
                y = _dot(inv_ref[par * (BLK // 2):(par + 1) * (BLK // 2), :],
                         wf[par * BLK:(par + 1) * BLK, c])
                for a in range(GA):
                    yt[pl.ds((a0 + a) * BLK + par, BLK // 2, stride=2), :] = (
                        y[:, a * BLK:(a + 1) * BLK])

        dvb = jnp.broadcast_to(dvec, (8, LANES))

        def out_item(tok, r0):
            d8 = dvb if tok is None else jnp.where(never, tok, dvb)
            yb = yt[r0:r0 + 16, :] + kvb[r0:r0 + 16, :].astype(F32) * jnp.concatenate([d8, d8], axis=0)
            aout[t, r0:r0 + 16, :] = (ain[sl, 2, r0:r0 + 16, :].astype(F32) * yb).astype(BF16)

        def out_items(a0):
            return [functools.partial(out_item, r0=r0)
                    for r0 in range(a0 * BLK, (a0 + GA) * BLK, 16)]

        groups = [freq_items(a0, never) for a0 in range(0, NB, GA)]
        items = [(it, g) for g, grp in enumerate(groups) for it in grp]
        npart = len(parts) - 1
        tpp = 7 * PPH * XR // 8
        span = npart * tpp - 72
        pos = [i * span // len(items) for i in range(len(items))]
        done = [max(q for q, (_, gg) in zip(pos, items) if gg == g) for g in range(len(groups))]
        pending = []
        nxt = 0
        for i in range(npart):
            toks = run_part(1 + i)
            if pending:
                _run_paced(pending, toks)
                pending = []
            for q, (it, _) in zip(pos, items):
                if q * 1 // tpp == i:
                    it(toks[min(q - i * tpp, len(toks) - 1)])
            while nxt < len(groups) and done[nxt] + 72 <= (i + 1) * tpp:
                inverse(nxt * GA)
                pending += out_items(nxt * GA)
                nxt += 1
        assert nxt == len(groups)
        for it in pending:
            it(None)
        aout_copy(t).start()
        return carry

    wo_copy(0).start()
    lax.fori_loop(0, NT, tile_body, 0)
    pltpu.make_async_copy(wo, wo, sem_wo).wait()

    def initial_guess():
        puni = pl.reciprocal(jnp.full((1, 1), float(L), F32), approx=True).astype(BF16).astype(F32)

        def shift_down(m):
            rows = lax.broadcasted_iota(jnp.int32, m.shape, 0)
            return jnp.where(rows == 0, 0.0, pltpu.roll(m, 1, 0))

        m1 = shift_down(_dot((tsum[0:NSEG, :] * puni).astype(BF16), wo[...]))
        v1 = _dot(m1.astype(BF16), w_plain(WV, 0, H // 2)).astype(BF16).astype(F32)
        u2 = ((tsum[0:NSEG, :] + float(M) * v1) * puni).astype(BF16)
        m2 = shift_down(_dot(u2, wo[...]))
        mhat[...] = jnp.broadcast_to(m2[:, None, :], (NSEG, M, DM)).reshape(NSEG * M, DM)
        mhat[0:M, :] = mem0_ref[...].astype(F32)
        pltpu.make_async_copy(w32.at[WQ:WK + 1], w32.at[WQ:WK + 1], sem_wqk).wait()

    ri = lax.broadcasted_iota(jnp.int32, (PR, PR), 0)
    ci = lax.broadcasted_iota(jnp.int32, (PR, PR), 1)

    def seg_of(r):
        return jnp.where(r < MR, r // M, (r - MR) // SEG)

    def pos_of(r):
        return jnp.where(r < MR, r % M, M + (r - MR) % SEG)

    same = seg_of(ri) == seg_of(ci)
    allowed = same & ((ri < MR) | (pos_of(ri) >= pos_of(ci)))
    fill = jnp.where(same, -1e9, -jnp.inf).astype(F32)

    def sweep(state):
        it, _ = state
        pl.when(it == 0)(initial_guess)

        def mem_rows(i):
            n = PPB * MR
            return mhat[pl.ds(pl.multiple_of((i // NG) * n, n), n), :]

        def mem_lhs(i):
            m = mem_rows(i)
            n = PPH * MR
            ops = _strassen_lhs(m[:n, :KH], m[:n, KH:], m[n:, :KH], m[n:, KH:])
            return [_pack(o) for o in ops]

        def qk_proj(i, j, mops):
            rb = i // NG
            hp = (i % NG) * (G // 2) + j // 2

            def lhs(k):
                return _unpack(jnp.concatenate([mops[k], abuf[rb, k]], axis=0))

            (c11, c12, c21, c22), _ = _strassen(lhs, w_rhs(WQ + j % 2, hp, [zero_s[k] for k in range(7)]))
            n = PPH * MR
            for half, cc in enumerate(((c11, c12), (c21, c22))):
                v = jnp.concatenate(cc, axis=1).astype(BF16)
                ps = slice(half * PPH, (half + 1) * PPH)
                qks[j, ps, 0:MR, :] = v[:n].reshape(PPH, MR, 2 * E)
                qks[j, ps, MR:PR, :] = v[n:].reshape(PPH, XR, 2 * E)

        def vm_proj(i):
            g = i % NG
            vv = _dot(mem_rows(i).astype(BF16), w_plain(WV, g * (G // 2), G // 2))
            v0 = tsum[NSEG:NSEG + M, pl.ds(pl.multiple_of(g * (G * E), G * E), G * E)]
            vv = jnp.concatenate([jnp.where(i < NG, v0, vv[:M]), vv[M:]], axis=0)
            vms[...] = vv.astype(BF16).reshape(PPB, MR, G * E)

        def scores(j):
            c = slice((j % 2) * E, (j % 2 + 1) * E)
            return lax.dot_general(qks[2 * (j // 2), :, :, c], qks[2 * (j // 2) + 1, :, :, c],
                                   (((2,), (2,)), ((0,), (0,))), preferred_element_type=F32)

        def attend(i, j, s):
            p0 = pl.multiple_of((i // NG) * PPB, PPB)
            h = (i % NG) * G + j
            s = jnp.where(allowed[None], s * scale, fill[None])
            e = jnp.exp(s - jnp.max(s, axis=-1, keepdims=True))
            p = (e * pl.reciprocal(jnp.sum(e, axis=-1, keepdims=True), approx=True)).astype(BF16)
            vh = jnp.concatenate(
                [vms[:, :, j * E:(j + 1) * E],
                 vbuf[pl.ds(p0, PPB), :, pl.ds(pl.multiple_of(h * E, E), E)]], axis=1)
            return lax.dot_general(p, vh, (((2,), (1,)), ((0,), (0,))), preferred_element_type=F32)

        def out_proj(i, us):
            rb = i // NG
            g = i % NG
            u = jnp.concatenate(us, axis=2)
            wog = wo[pl.ds(pl.multiple_of(g * (G * E), G * E), G * E), :]
            rm = pl.ds(pl.multiple_of(rb * (PPB * MR), PPB * MR), PPB * MR)
            um = u[:, :MR, :].reshape(PPB * MR, G * E).astype(BF16)
            mnew[rm, :] = jnp.where(g > 0, mnew[rm, :], 0.0) + _dot(um, wog)
            n = PPH * XR
            kh = G * E // 2
            top = u[:PPH, MR:, :].reshape(n, G * E)
            bot = u[PPH:, MR:, :].reshape(n, G * E)
            ops = _strassen_lhs(top[:, :kh], top[:, kh:], bot[:, :kh], bot[:, kh:])
            wf32 = wog.astype(F32)
            rhs = _strassen_rhs(wf32[:kh, :KH], wf32[:kh, KH:], wf32[kh:, :KH], wf32[kh:, KH:])
            quads = [(slice(0, n), slice(0, KH)), (slice(0, n), slice(KH, DM)),
                     (slice(n, 2 * n), slice(0, KH)), (slice(n, 2 * n), slice(KH, DM))]
            init = [jnp.where(g > 0, acc[r, c], 0.0) for r, c in quads]
            cs, _ = _strassen(lambda k: ops[k].astype(BF16), rhs, init)
            for (r, c), v in zip(quads, cs):
                acc[r, c] = v
                obuf[rb, r, c] = v.astype(BF16)

        def step(i, nxt):
            s0, s1 = scores(0), scores(1)
            if nxt:
                mops = mem_lhs(i + 1)
                qk_proj(i + 1, 0, mops)
            u0, u1 = attend(i, 0, s0), attend(i, 1, s1)
            s2, s3 = scores(2), scores(3)
            if nxt:
                qk_proj(i + 1, 1, mops)
            u2, u3 = attend(i, 2, s2), attend(i, 3, s3)
            if nxt:
                qk_proj(i + 1, 2, mops)
                qk_proj(i + 1, 3, mops)
                vm_proj(i + 1)
            out_proj(i, [u0, u1, u2, u3])

        mops0 = mem_lhs(0)
        for j in range(G):
            qk_proj(0, j, mops0)
        vm_proj(0)

        def main_body(i, cy):
            step(i, True)

            @pl.when(i % NG == NG - 1)
            def _():
                o_copy(i // NG).start()

            return cy

        lax.fori_loop(0, NRB * NG - 1, main_body, 0)
        step(NRB * NG - 1, False)
        o_copy(NRB - 1).start()

        n = (NSEG - 1) * M
        new = mnew[0:n, :]
        err = jnp.max(jnp.abs(new - mhat[M:M + n, :]), axis=1, keepdims=True)
        ref = jnp.max(jnp.abs(new), axis=1, keepdims=True)
        ok = jnp.min(jnp.where(err <= TOL * ref, 1.0, 0.0))
        mhat[M:M + n, :] = new
        for rb in range(NRB):
            o_copy(rb).wait()
        return it + 1, (ok > 0.5).astype(jnp.int32)

    lax.while_loop(lambda st: jnp.logical_and(st[0] < NSEG, st[1] == 0), sweep,
                   (jnp.int32(0), jnp.int32(0)))
    pltpu.make_async_copy(aout, aout, sem_aout).wait()


@functools.partial(jax.jit, static_argnames=("B_seg_len",))
def pallas_concat_heads__ssm_conv_h3__memory_aug_recurrent_mem_tr__prompt_kernel(
    A_q, A_k, A_v, A_shift_k, A_ssm_k, A_ssm_D,
    B_x, B_mem0, B_Wq, B_Wk, B_Wv, B_Wo, B_seg_len,
):
    _, S, D = A_q.shape
    DM = B_x.shape[2]
    H, E = B_Wq.shape[1], B_Wq.shape[2]
    M = B_mem0.shape[1]
    SEG = int(B_seg_len)
    NSEG = S // SEG
    NP = NSEG // 2
    PR = 2 * (M + SEG)
    PPB = 8
    NRB = NP // PPB
    NT = D // LANES
    assert E == LANES and H == 32 and M == 8 and SEG == 32 and A_shift_k.shape[1] == 4
    assert S == 2048 and D == 1024 and DM == 1024

    fwd, inv = _dft_mats()
    any_spec = pl.BlockSpec(memory_space=pl.ANY)
    vmem_spec = pl.BlockSpec(memory_space=pltpu.VMEM)
    scratch = [
        pltpu.VMEM((NRB, 7, PPB // 2 * SEG, DM // 2), U32),
        pltpu.VMEM((7, M, DM // 2), U32),
        pltpu.VMEM((NP, 2 * SEG, H * E), BF16),
        pltpu.VMEM((3, H // 2, DM, E), U32),
        pltpu.VMEM((H * E, DM), BF16),
        pltpu.VMEM((4, PPB, PR, 2 * E), BF16),
        pltpu.VMEM((PPB, 2 * M, 4 * E), BF16),
        pltpu.VMEM((PPB * 2 * SEG, DM), F32),
        pltpu.VMEM((NRB, PPB * 2 * SEG, DM), BF16),
        pltpu.VMEM((NSEG * M, DM), F32),
        pltpu.VMEM((NSEG * M, DM), F32),
        pltpu.VMEM((NSEG + M, H * E), F32),
        pltpu.VMEM((2, 3, S, LANES), BF16),
        pltpu.VMEM((2, LANES, S), BF16),
        pltpu.VMEM((S + 8, LANES), F32),
        pltpu.VMEM((S, LANES), BF16),
        pltpu.VMEM((NFFT, S), F32),
        pltpu.VMEM((NFFT, S), F32),
        pltpu.VMEM((NFFT, S), BF16),
        pltpu.VMEM((S, LANES), F32),
        pltpu.VMEM((NT, S, LANES), BF16),
        pltpu.VMEM((8, LANES), jnp.int32),
        pltpu.SMEM((8,), jnp.int32),
        pltpu.SemaphoreType.DMA((NRB,)),
        pltpu.SemaphoreType.DMA((H // 2,)),
        pltpu.SemaphoreType.DMA,
        pltpu.SemaphoreType.DMA,
        pltpu.SemaphoreType.DMA((2, 2)),
        pltpu.SemaphoreType.DMA,
        pltpu.SemaphoreType.DMA((NRB,)),
    ]
    out = pl.pallas_call(
        functools.partial(_kernel, S=S, D=D, DM=DM, H=H, M=M, SEG=SEG),
        out_shape=jax.ShapeDtypeStruct((S, D + DM), BF16),
        in_specs=[any_spec, any_spec, any_spec, vmem_spec, any_spec, vmem_spec,
                  any_spec, vmem_spec, any_spec, any_spec, any_spec, any_spec,
                  vmem_spec, vmem_spec],
        out_specs=any_spec,
        scratch_shapes=scratch,
        compiler_params=pltpu.CompilerParams(vmem_limit_bytes=120 * 1024 * 1024,
                                             disable_bounds_checks=True),
    )(
        A_q.reshape(S, D), A_k.reshape(S, D), A_v.reshape(S, D),
        A_shift_k.T, A_ssm_k, A_ssm_D.reshape(NT, LANES),
        B_x.reshape(NRB, S // NRB, DM), B_mem0.reshape(M, DM),
        B_Wq, B_Wk, B_Wv, B_Wo.reshape(H * E, DM),
        jnp.asarray(fwd, BF16), jnp.asarray(inv, BF16),
    )
    return out.reshape(1, S, D + DM)
```

```python
import functools

import numpy as np
import jax
import jax.numpy as jnp
from jax import lax
import jax.experimental.pallas as pl
import jax.experimental.pallas.tpu as pltpu

F32 = jnp.float32
BF16 = jnp.bfloat16
U32 = jnp.uint32

LANES = 128
BLK = 128
NFFT = 2 * BLK
TOL = 2.0 ** -10


def _dft_mats():
    even = np.arange(0, BLK, 2)
    theta = 2.0 * np.pi * (np.concatenate([even, BLK - 1 - even]) + 0.5) / NFFT
    n = np.arange(BLK)
    c = np.cos(theta[:, None] * n[None, :])
    s = np.sin(theta[:, None] * n[None, :])
    fwd = np.zeros((NFFT, BLK))
    for m in range(BLK // 8):
        fwd[16 * m:16 * m + 8] = c[8 * m:8 * m + 8]
        fwd[16 * m + 8:16 * m + 16] = -s[8 * m:8 * m + 8]
    inv = fwd[:BLK].T * (2.0 / NFFT)
    inv = np.concatenate([inv[0::2], inv[1::2]], axis=0)
    return fwd.astype(np.float32), inv.astype(np.float32)


def _dot(a, b):
    return jnp.dot(a, b, preferred_element_type=F32)


def _pack(x):
    return pltpu.bitcast(x.astype(BF16), U32)


def _unpack(w):
    return pltpu.bitcast(w, BF16)


def _lo(w):
    return pltpu.bitcast(w << 16, F32)


def _hi(w):
    return pltpu.bitcast(w & jnp.uint32(0xFFFF0000), F32)


def _strassen_lhs(a11, a12, a21, a22):
    return [a11 + a22, a21 + a22, a11, a22, a11 + a12, a21 - a11, a12 - a22]


def _strassen_rhs(b11, b12, b21, b22):
    ops = [b11 + b22, b11, b12 - b22, b21 - b11, b22, b11 + b12, b21 + b22]
    return [o.astype(BF16) for o in ops]


def _strassen(lhs, rhs, emit, init=None):
    def add(c, m):
        return m if c is None else c + m

    c11, c12, c21, c22 = init if init is not None else (None,) * 4
    m5 = _dot(lhs(4), rhs[4])
    yield m5
    m3 = _dot(lhs(2), rhs[2])
    emit(0, 1, add(c12, m5) + m3)
    yield m3
    m2 = _dot(lhs(1), rhs[1])
    c22 = add(c22, m3) - m2
    yield m2
    m4 = _dot(lhs(3), rhs[3])
    emit(1, 0, add(c21, m2) + m4)
    c11 = add(c11, m4) - m5
    yield m4
    m1 = _dot(lhs(0), rhs[0])
    c11 = c11 + m1
    c22 = c22 + m1
    yield m1
    m7 = _dot(lhs(6), rhs[6])
    emit(0, 0, c11 + m7)
    yield m7
    m6 = _dot(lhs(5), rhs[5])
    emit(1, 1, c22 + m6)
    yield m6


def _drain(*gens):
    for g in gens:
        for _ in g:
            pass


def _tokens(m):
    return [m[r:r + 8, c:c + LANES]
            for r in range(0, m.shape[0], 8) for c in range(0, m.shape[1], LANES)]


def _tie(never, tok, x):
    if tok is None:
        return x
    reps = (x.shape[0] // 8, x.shape[1] // LANES)
    if tok.dtype != x.dtype:
        tok = pltpu.bitcast(tok, x.dtype)
    if reps != (1, 1):
        never, tok = jnp.tile(never, reps), jnp.tile(tok, reps)
    return jnp.where(never, tok, x)


def _run_paced(items, toks):
    for i, it in enumerate(items):
        it(toks[i * len(toks) // len(items)])


def _interleave(nv, ngr, weights):
    dur = {'v': 256, 'h': 256, 'x': 256, 'inv': 128}
    margin = 768

    def plan(rate):
        t, v, out = 0, 0, []
        nxt = {'h': 0, 'x': 0, 'inv': 0}
        pos = {k: 0 for k in weights}
        done = {}
        credit = 0.0
        while True:
            kind = None
            if nxt['inv'] < ngr and done.get(('freq', nxt['inv']), 1e9) + margin <= t:
                kind = 'inv'
            elif nxt['x'] < ngr and done.get(('conv', nxt['x']), 1e9) + margin <= t:
                kind = 'x'
            elif nxt['h'] < ngr and nxt['h'] <= nxt['x'] and (not out or out[-1][0] == 'v'):
                kind = 'h'
            elif v < nv:
                kind = 'v'
            if kind is None:
                break
            g = v if kind == 'v' else nxt[kind]
            busy = 0.75 if kind == 'v' and v % (nv // 2) < 7 else 0.0
            credit += (rate - busy) * dur[kind]
            chunk = []
            while credit > 0:
                ready = [('out', i) for i in range(nxt['inv'])]
                ready += [('conv', i) for i in range(ngr)]
                ready += [('freq', i) for i in range(min(nxt['x'], nxt['h']))]
                ready = [k for k in ready if pos[k] < len(weights[k])]
                if not ready:
                    credit = 0.0
                    break
                k = ready[0]
                chunk.append((k, pos[k]))
                credit -= weights[k][pos[k]]
                pos[k] += 1
                if pos[k] == len(weights[k]):
                    done[k] = t + dur[kind]
            out.append((kind, g, chunk))
            t += dur[kind]
            if kind == 'v':
                v += 1
            else:
                nxt[kind] += 1
        ok = all(pos[k] == len(weights[k]) for k in weights)
        return ok, out

    rate = 1.0
    while True:
        ok, out = plan(rate)
        if ok:
            return out
        rate += 0.02


def _kernel(q_hbm, k_hbm, v_hbm, shift_hbm, h_hbm, d_hbm, x_hbm, mem0_hbm,
            wq_hbm, wk_hbm, wv_hbm, wo_hbm, fwd_hbm, inv_hbm,
            out_hbm,
            abuf, a0buf, vbuf, w32, wo, qks, vms, acc, obuf, mhat, mnew, tsum,
            ain, ah, kf, kvb, xf, hf, wf, yt, aout,
            mem0_ref, fwd_ref, inv_ref, shift_ref, d_ref, zero_v, zero_s,
            sem_s, sem_x, sem_wv, sem_wqk, sem_wo, sem_a, sem_aout, sem_o,
            *, S, D, DM, H, M, SEG):
    E = LANES
    NSEG = S // SEG
    NP = NSEG // 2
    MR = 2 * M
    XR = 2 * SEG
    PR = MR + XR
    MW, XW, PW = MR // 2, XR // 2, PR // 2
    L = M + SEG
    NB = S // BLK
    NT = D // LANES
    PPB = 8
    PPH = PPB // 2
    NRB = NP // PPB
    G = 4
    NG = H // G
    KH = DM // 2
    scale = float(E) ** -0.5
    WV, WQ, WK = 0, 1, 2

    small = [pltpu.make_async_copy(src, dst, sem_s.at[i]) for i, (src, dst) in enumerate(
        ((mem0_hbm, mem0_ref), (shift_hbm, shift_ref), (d_hbm, d_ref),
         (fwd_hbm, fwd_ref), (inv_hbm, inv_ref)))]
    HBR = PPH * XR // 2

    def x_copies(hb):
        out = []
        for half in range(2):
            r = pl.ds(pl.multiple_of((2 * half + hb % 2) * HBR, HBR), HBR)
            out.append(pltpu.make_async_copy(x_hbm.at[hb // 2, r], obuf.at[hb // 2, r],
                                             sem_x.at[hb]))
        return out

    def w_copy(which, hp):
        src = (wv_hbm, wq_hbm, wk_hbm)[which].bitcast(U32)
        sem = sem_wv.at[hp] if which == WV else sem_wqk
        return pltpu.make_async_copy(src.at[:, hp, :], w32.at[which, hp], sem)

    def wo_copy(t):
        n = H * E // NT
        r = pl.ds(pl.multiple_of(t * n, n), n)
        return pltpu.make_async_copy(wo_hbm.at[r, :], wo.at[r, :], sem_wo)

    def a_start(t, sl, which=(0, 1, 2, 3)):
        c = pl.ds(pl.multiple_of(t * LANES, LANES), LANES)
        for i in which:
            if i == 3:
                pltpu.make_async_copy(h_hbm.at[c, :], ah.at[sl], sem_a.at[sl, 1]).start()
            else:
                src = (k_hbm, v_hbm, q_hbm)[i]
                pltpu.make_async_copy(src.at[:, c], ain.at[sl, i], sem_a.at[sl, 0]).start()

    def a_wait(sl):
        pltpu.make_async_copy(ain.at[sl], ain.at[sl], sem_a.at[sl, 0]).wait()
        pltpu.make_async_copy(ah.at[sl], ah.at[sl], sem_a.at[sl, 1]).wait()

    def aout_copy(t):
        c = pl.ds(pl.multiple_of(t * LANES, LANES), LANES)
        return pltpu.make_async_copy(aout.at[t], out_hbm.at[:, c], sem_aout)

    def o_copy(rb):
        r = pl.ds(pl.multiple_of(rb * (PPB * XR), PPB * XR), PPB * XR)
        return pltpu.make_async_copy(obuf.at[rb], out_hbm.at[r, pl.ds(D, DM)], sem_o.at[rb])

    def w_rhs(which, hp, zs=None):
        if zs is None:
            w = w32[which, hp]
            return _strassen_rhs(_lo(w[:KH]), _hi(w[:KH]), _lo(w[KH:]), _hi(w[KH:]))
        out = []
        for k in range(7):
            w = w32.at[which, hp + zs[k]]
            out.append(_strassen_rhs(_lo(w[:KH]), _hi(w[:KH]), _lo(w[KH:]), _hi(w[KH:]))[k])
        return out

    def w_plain(which, hp0, n):
        parts = []
        for j in range(n):
            w = w32[which, hp0 + j]
            parts += [_lo(w), _hi(w)]
        return jnp.concatenate(parts, axis=1).astype(BF16)

    small[0].start()
    for hb in range(2):
        for cp in x_copies(hb):
            cp.start()
    w_copy(WV, 0).start()
    w_copy(WV, 1).start()
    for cp in small[1:]:
        cp.start()

    kf[0:8, :] = jnp.zeros((8, LANES), F32)
    zero_v[...] = jnp.zeros((8, LANES), jnp.int32)
    for k in range(8):
        zero_s[k] = 0
    tsum[0:8, :] = jnp.zeros((8, H * E), F32)
    vbuf[0, 0:16, :] = jnp.zeros((16, H * E), BF16)
    for hb in range(2 * NRB):
        r0 = (hb % 2) * (HBR // 2)
        abuf[hb // 2, 0, r0:r0 + 8, 0:LANES] = jnp.zeros((8, LANES), U32)
    small[0].wait()
    mem0 = mem0_ref[...].astype(F32)
    m0 = jnp.concatenate([mem0, jnp.zeros_like(mem0)], axis=0)
    z0 = jnp.zeros((MR, KH), F32)
    for k, op in enumerate(_strassen_lhs(m0[:, :KH], m0[:, KH:], z0, z0)):
        a0buf[k, 0:MW, :] = _pack(op)

    def x_item(tok, never, src, dst, r, c):
        quad = [_tie(never, tok, src[h * 2 * HBR + r:h * 2 * HBR + r + 16,
                                     kk * KH + c:kk * KH + c + 2 * LANES].astype(F32))
                for h in range(2) for kk in range(2)]
        for k, op in enumerate(_strassen_lhs(*quad)):
            dst[k, r // 2:r // 2 + 8, c:c + 2 * LANES] = _pack(op)

    def x_items(never, src, dst):
        return [functools.partial(x_item, never=never, src=src, dst=dst, r=r, c=c)
                for r in range(0, HBR, 16) for c in range(0, KH, 2 * LANES)]

    def x_first(hb, cy):
        for cp in x_copies(hb):
            cp.wait()
        src = obuf.at[0, pl.ds(pl.multiple_of(hb * HBR, HBR), 3 * HBR)]
        dst = a0buf.at[:, pl.ds(pl.multiple_of(MW + hb * (HBR // 2), 8), HBR // 2)]
        for it in x_items(None, src, dst):
            it(None)
        return cy

    lax.fori_loop(0, 2, x_first, 0)

    def v_part(j, rb, rhs, vwin, twin, pre=None):
        def lhs(k):
            x = a0buf[k] if rb == 0 else abuf[rb, k]
            if pre is not None and k == 4:
                x0 = jnp.concatenate([pre(x[:8, :LANES]), x[:8, LANES:]], axis=1)
                x = jnp.concatenate([x0, x[8:]], axis=0)
            return _unpack(x)

        def emit(half, hh, cv):
            c = slice((2 * j + hh) * E, (2 * j + hh + 1) * E)
            vv = cv.astype(BF16)
            vx = vv[MR:] if rb == 0 else vv
            p0 = rb * PPB + half * PPH
            vwin[p0:p0 + PPH, :, c] = vx.reshape(PPH, XR, E)
            ts = jnp.sum(vx.astype(F32).reshape(2 * PPH, SEG, E), axis=1)
            if rb == 0 and half == 0:
                v0 = vv[0:M].astype(F32)
                twin[NSEG:NSEG + M, c] = v0
                t0 = jnp.sum(v0, axis=0, keepdims=True)
                rows = lax.broadcasted_iota(jnp.int32, ts.shape, 0)
                ts = ts + jnp.where(rows == 0, t0, 0.0)
            twin[2 * p0:2 * (p0 + PPH), c] = ts

        return _strassen(lhs, rhs, emit)

    def v_products(t, rbs, never, extra=()):
        zs = [zero_s[k] for k in range(7)]
        c4 = pl.ds(pl.multiple_of(t * (4 * E), 4 * E), 4 * E)
        vwin = vbuf.at[:, :, c4]
        twin = tsum.at[:, c4]

        def pre(x):
            for v in (twin[0:8, 0:LANES], pltpu.bitcast(vwin[0, 0:16, 0:LANES], U32)) + tuple(extra):
                x = _tie(never, v, x)
            return x

        for j in range(2):
            rhs = w_rhs(WV, 2 * t + j, zs)
            for rb in rbs:
                yield from v_part(j, rb, rhs, vwin, twin, pre if (j, rb) == (0, rbs[0]) else None)

    def head_body(j, cy):
        w_copy(WV, 2 * j).wait()
        w_copy(WV, 2 * j + 1).wait()

        @pl.when(j >= 2)
        def _():
            for cp in x_copies(j):
                cp.wait()

        @pl.when(j + 1 < NT)
        def _():
            w_copy(WV, 2 * j + 2).start()
            w_copy(WV, 2 * j + 3).start()

        @pl.when(j + 2 < 2 * NRB)
        def _():
            for cp in x_copies(j + 2):
                cp.start()

        @pl.when(j == NT - 3)
        def _():
            a_start(0, 0, (3,))

        @pl.when(j == NT - 2)
        def _():
            a_start(0, 0, (0, 1, 2))

        never = zero_v[...] > 0
        src = obuf.at[j // 2, pl.ds(pl.multiple_of((j % 2) * HBR, HBR), 3 * HBR)]
        dst = abuf.at[j // 2, :, pl.ds(pl.multiple_of((j % 2) * (HBR // 2), 8), HBR // 2)]
        toks = []
        for m in v_products(j, [0], never, [dst[0, 0:8, 0:LANES]]):
            toks += _tokens(m)
        _run_paced(x_items(never, src, dst), toks[:-40])
        return cy

    assert NT == 2 * NRB
    lax.fori_loop(0, NT, head_body, 0)

    GA = 4

    def freq_items(a0, never):
        def item(tok, m, cc, st):
            r_re = slice(16 * m, 16 * m + 8)
            r_im = slice(16 * m + 8, 16 * m + 16)
            xr = _tie(never, tok, xf[r_re, cc * BLK:(cc + 1) * BLK])
            xi = _tie(never, tok, xf[r_im, cc * BLK:(cc + 1) * BLK])
            xs = xr + xi
            for a in range(max(a0, cc), a0 + GA):
                j = a - cc
                if ('g', m, j) not in st:
                    gr = hf[r_re, j * BLK:(j + 1) * BLK]
                    gi = hf[r_im, j * BLK:(j + 1) * BLK]
                    st['g', m, j] = (gr, gi, gr + gi)
                gr, gi, gs = st['g', m, j]
                ps = (xr * gr, xi * gi, xs * gs)
                st[m, a] = ps if (m, a) not in st else tuple(u + v for u, v in zip(st[m, a], ps))
                if cc == a:
                    p1, p2, p3 = st[m, a]
                    st[m, a] = (p1 - p2, p3 - p1 - p2)
                    if m >= BLK // 16:
                        m0 = m - BLK // 16
                        (wr, wi), (vr, vi) = st[m0, a], st[m, a]
                        c = slice(a * BLK, (a + 1) * BLK)
                        wf[16 * m0:16 * m0 + 16, c] = (
                            jnp.concatenate([wr + vr, wi - vi], axis=0).astype(BF16))
                        wf[16 * m:16 * m + 16, c] = (
                            jnp.concatenate([wr - vr, wi + vi], axis=0).astype(BF16))

        items = []
        for m0 in range(BLK // 16):
            st = {}
            for m in (m0, m0 + BLK // 16):
                items += [(functools.partial(item, m=m, cc=cc, st=st),
                           4 + 6 * (a0 + GA - max(a0, cc)) + (6 if cc >= a0 else 0))
                          for cc in range(a0 + GA)]
        return items

    def tile_body(t, carry):
        sl = t % 2
        a_wait(sl)

        @pl.when(t + 1 < NT)
        def _():
            a_start(t + 1, 1 - sl)
            wo_copy(t + 1).start()

        for which in (WQ, WK):
            w_copy(which, 2 * t).start()
            w_copy(which, 2 * t + 1).start()

        c = pl.ds(pl.multiple_of(t * LANES, LANES), LANES)
        taps = shift_ref[:, c].astype(F32)
        dcol = d_ref[...].astype(F32)
        rows = lax.broadcasted_iota(jnp.int32, dcol.shape, 0)
        dvec = jnp.sum(jnp.where(rows == t, dcol, 0.0), axis=0, keepdims=True)
        dvb = jnp.broadcast_to(dvec, (8, LANES))
        tapb = [jnp.broadcast_to(taps[j:j + 1, :], (8, LANES)) for j in range(4)]
        never = zero_v[...] > 0
        fwd = fwd_ref[...]
        NGR = NB // GA
        GW = GA * BLK

        def conv_item(tok, r0):
            kf[8 + r0:24 + r0, :] = ain[sl, 0, r0:r0 + 16, :].astype(F32)
            halves = []
            for h in range(2):
                r = 8 + r0 + 8 * h
                ks = kf[r:r + 8, :] * _tie(never, tok, tapb[0])
                for j in range(1, 4):
                    ks = ks + kf[r - j:r - j + 8, :] * tapb[j]
                halves.append(ks)
            kvb[r0:r0 + 16, :] = (jnp.concatenate(halves, axis=0)
                                  * ain[sl, 1, r0:r0 + 16, :].astype(F32)).astype(BF16)

        hlast = [None]

        def h_fwd(g):
            hst = jnp.concatenate([ah[sl, :, b * BLK:(b + 1) * BLK]
                                   for b in range(g * GA, (g + 1) * GA)], axis=0)
            hh = lax.dot_general(fwd, hst, (((1,), (1,)), ((), ())), preferred_element_type=F32)
            for b in range(GA):
                cur = hh[:, b * BLK:(b + 1) * BLK]
                prev = hlast[0]
                c = slice((g * GA + b) * BLK, (g * GA + b + 1) * BLK)
                if prev is None:
                    hf[:, c] = cur
                else:
                    for m in range(BLK // 8):
                        re = slice(16 * m, 16 * m + 8)
                        im = slice(16 * m + 8, 16 * m + 16)
                        if m < BLK // 16:
                            hf[re, c] = cur[re] - prev[im]
                            hf[im, c] = cur[im] + prev[re]
                        else:
                            hf[re, c] = cur[re] + prev[im]
                            hf[im, c] = cur[im] - prev[re]
                hlast[0] = cur
            return hh

        def x_fwd(g):
            rhs = jnp.concatenate([kvb[b * BLK:(b + 1) * BLK, :]
                                   for b in range(g * GA, (g + 1) * GA)], axis=1)
            xx = _dot(fwd, rhs)
            xf[:, g * GW:(g + 1) * GW] = xx
            return xx

        def inverse(g):
            ys = []
            for par in range(2):
                y = _dot(inv_ref[par * (BLK // 2):(par + 1) * (BLK // 2), :],
                         wf[par * BLK:(par + 1) * BLK, g * GW:(g + 1) * GW])
                for a in range(GA):
                    yt[pl.ds((g * GA + a) * BLK + par, BLK // 2, stride=2), :] = (
                        y[:, a * BLK:(a + 1) * BLK])
                ys.append(y)
            return jnp.concatenate(ys, axis=0)

        def out_item(tok, r0):
            d8 = _tie(never, tok, dvb)
            yb = yt[r0:r0 + 16, :] + kvb[r0:r0 + 16, :].astype(F32) * jnp.concatenate([d8, d8], axis=0)
            aout[t, r0:r0 + 16, :] = (ain[sl, 2, r0:r0 + 16, :].astype(F32) * yb).astype(BF16)

        def rows16(fn, g, w):
            return [(functools.partial(fn, r0=r0), w) for r0 in range(g * GW, (g + 1) * GW, 16)]

        vgen = v_products(t, list(range(1, NRB)), never)
        nv = 2 * (NRB - 1) * 7
        work = {('conv', g): rows16(conv_item, g, 25) for g in range(NGR)}
        work.update({('freq', g): freq_items(g * GA, never) for g in range(NGR)})
        work.update({('out', g): rows16(out_item, g, 16) for g in range(NGR)})
        for kind, g, chunks in _interleave(nv, NGR, {k: [w for _, w in v] for k, v in work.items()}):
            if kind is not None:
                m = (next(vgen) if kind == 'v' else
                     {'h': h_fwd, 'x': x_fwd, 'inv': inverse}[kind](g))
                toks = _tokens(m)
            items = [work[k][i][0] for k, i in chunks]
            if kind is None:
                for it in items:
                    it(None)
            elif items:
                _run_paced(items, toks)
        _drain(vgen)
        aout_copy(t).start()
        return carry

    for cp in small[1:]:
        cp.wait()
    wo_copy(0).start()
    lax.fori_loop(0, NT, tile_body, 0)
    pltpu.make_async_copy(wo, wo, sem_wo).wait()

    def initial_guess():
        puni = pl.reciprocal(jnp.full((1, 1), float(L), F32), approx=True).astype(BF16).astype(F32)

        def shift_down(m):
            rows = lax.broadcasted_iota(jnp.int32, m.shape, 0)
            return jnp.where(rows == 0, 0.0, pltpu.roll(m, 1, 0))

        m1 = shift_down(_dot((tsum[0:NSEG, :] * puni).astype(BF16), wo[...]))
        v1 = _dot(m1.astype(BF16), w_plain(WV, 0, H // 2)).astype(BF16).astype(F32)
        u2 = ((tsum[0:NSEG, :] + float(M) * v1) * puni).astype(BF16)
        m2 = shift_down(_dot(u2, wo[...]))
        mhat[...] = jnp.broadcast_to(m2[:, None, :], (NSEG, M, DM)).reshape(NSEG * M, DM)
        mhat[0:M, :] = mem0_ref[...].astype(F32)
        pltpu.make_async_copy(w32.at[WQ:WK + 1], w32.at[WQ:WK + 1], sem_wqk).wait()

    ri = lax.broadcasted_iota(jnp.int32, (PR, PR), 0)
    ci = lax.broadcasted_iota(jnp.int32, (PR, PR), 1)

    def seg_of(r):
        return jnp.where(r < MR, r // M, (r - MR) // SEG)

    def pos_of(r):
        return jnp.where(r < MR, r % M, M + (r - MR) % SEG)

    same = seg_of(ri) == seg_of(ci)
    allowed = same & ((ri < MR) | (pos_of(ri) >= pos_of(ci)))
    fill = jnp.where(same, -1e9, -jnp.inf).astype(F32)

    def sweep(state):
        it, _ = state
        pl.when(it == 0)(initial_guess)

        def mem_rows(i):
            n = PPB * MR
            return mhat[pl.ds(pl.multiple_of((i // NG) * n, n), n), :]

        def mem_lhs(i):
            m = mem_rows(i)
            n = PPH * MR
            ops = _strassen_lhs(m[:n, :KH], m[:n, KH:], m[n:, :KH], m[n:, KH:])
            return [_pack(o) for o in ops]

        def qk_proj(i, j, mops):
            rb = i // NG
            hp = (i % NG) * (G // 2) + j // 2

            def lhs(k):
                return _unpack(jnp.concatenate([mops[k], abuf[rb, k]], axis=0))

            n = PPH * MR
            cs = {}

            def emit(half, hh, cv):
                cs[half, hh] = cv
                if (half, 1 - hh) in cs:
                    v = jnp.concatenate([cs[half, 0], cs[half, 1]], axis=1).astype(BF16)
                    ps = slice(half * PPH, (half + 1) * PPH)
                    qks[j, ps, 0:MR, :] = v[:n].reshape(PPH, MR, 2 * E)
                    qks[j, ps, MR:PR, :] = v[n:].reshape(PPH, XR, 2 * E)

            _drain(_strassen(lhs, w_rhs(WQ + j % 2, hp, [zero_s[k] for k in range(7)]), emit))

        def vm_proj(i):
            g = i % NG
            vv = _dot(mem_rows(i).astype(BF16), w_plain(WV, g * (G // 2), G // 2))
            v0 = tsum[NSEG:NSEG + M, pl.ds(pl.multiple_of(g * (G * E), G * E), G * E)]
            vv = jnp.concatenate([jnp.where(i < NG, v0, vv[:M]), vv[M:]], axis=0)
            vms[...] = vv.astype(BF16).reshape(PPB, MR, G * E)

        def scores(j):
            c = slice((j % 2) * E, (j % 2 + 1) * E)
            return lax.dot_general(qks[2 * (j // 2), :, :, c], qks[2 * (j // 2) + 1, :, :, c],
                                   (((2,), (2,)), ((0,), (0,))), preferred_element_type=F32)

        def attend(i, j, s):
            p0 = pl.multiple_of((i // NG) * PPB, PPB)
            h = (i % NG) * G + j
            s = jnp.where(allowed[None], s * scale, fill[None])
            e = jnp.exp(s - jnp.max(s, axis=-1, keepdims=True))
            p = (e * pl.reciprocal(jnp.sum(e, axis=-1, keepdims=True), approx=True)).astype(BF16)
            vh = jnp.concatenate(
                [vms[:, :, j * E:(j + 1) * E],
                 vbuf[pl.ds(p0, PPB), :, pl.ds(pl.multiple_of(h * E, E), E)]], axis=1)
            return lax.dot_general(p, vh, (((2,), (1,)), ((0,), (0,))), preferred_element_type=F32)

        def out_proj(i, us):
            rb = i // NG
            g = i % NG
            u = jnp.concatenate(us, axis=2)
            wog = wo[pl.ds(pl.multiple_of(g * (G * E), G * E), G * E), :]
            rm = pl.ds(pl.multiple_of(rb * (PPB * MR), PPB * MR), PPB * MR)
            um = u[:, :MR, :].reshape(PPB * MR, G * E).astype(BF16)
            mnew[rm, :] = jnp.where(g > 0, mnew[rm, :], 0.0) + _dot(um, wog)
            n = PPH * XR
            kh = G * E // 2
            top = u[:PPH, MR:, :].reshape(n, G * E)
            bot = u[PPH:, MR:, :].reshape(n, G * E)
            ops = _strassen_lhs(top[:, :kh], top[:, kh:], bot[:, :kh], bot[:, kh:])
            wf32 = wog.astype(F32)
            rhs = _strassen_rhs(wf32[:kh, :KH], wf32[:kh, KH:], wf32[kh:, :KH], wf32[kh:, KH:])
            quads = [(slice(0, n), slice(0, KH)), (slice(0, n), slice(KH, DM)),
                     (slice(n, 2 * n), slice(0, KH)), (slice(n, 2 * n), slice(KH, DM))]
            init = [jnp.where(g > 0, acc[r, c], 0.0) for r, c in quads]

            def emit(half, hh, v):
                r, c = quads[2 * half + hh]
                acc[r, c] = v
                obuf[rb, r, c] = v.astype(BF16)

            _drain(_strassen(lambda k: ops[k].astype(BF16), rhs, emit, init))

        def step(i, nxt):
            s0, s1 = scores(0), scores(1)
            if nxt:
                mops = mem_lhs(i + 1)
                qk_proj(i + 1, 0, mops)
            u0, u1 = attend(i, 0, s0), attend(i, 1, s1)
            s2, s3 = scores(2), scores(3)
            if nxt:
                qk_proj(i + 1, 1, mops)
            u2, u3 = attend(i, 2, s2), attend(i, 3, s3)
            if nxt:
                qk_proj(i + 1, 2, mops)
                qk_proj(i + 1, 3, mops)
                vm_proj(i + 1)
            out_proj(i, [u0, u1, u2, u3])

        mops0 = mem_lhs(0)
        for j in range(G):
            qk_proj(0, j, mops0)
        vm_proj(0)

        def main_body(i, cy):
            step(i, True)

            @pl.when(i % NG == NG - 1)
            def _():
                o_copy(i // NG).start()

            return cy

        lax.fori_loop(0, NRB * NG - 1, main_body, 0)
        step(NRB * NG - 1, False)
        o_copy(NRB - 1).start()

        n = (NSEG - 1) * M
        new = mnew[0:n, :]
        err = jnp.max(jnp.abs(new - mhat[M:M + n, :]), axis=1, keepdims=True)
        ref = jnp.max(jnp.abs(new), axis=1, keepdims=True)
        ok = jnp.min(jnp.where(err <= TOL * ref, 1.0, 0.0))
        mhat[M:M + n, :] = new
        for rb in range(NRB):
            o_copy(rb).wait()
        return it + 1, (ok > 0.5).astype(jnp.int32)

    lax.while_loop(lambda st: jnp.logical_and(st[0] < NSEG, st[1] == 0), sweep,
                   (jnp.int32(0), jnp.int32(0)))
    pltpu.make_async_copy(aout, aout, sem_aout).wait()


@functools.partial(jax.jit, static_argnames=("B_seg_len",))
def pallas_concat_heads__ssm_conv_h3__memory_aug_recurrent_mem_tr__prompt_kernel(
    A_q, A_k, A_v, A_shift_k, A_ssm_k, A_ssm_D,
    B_x, B_mem0, B_Wq, B_Wk, B_Wv, B_Wo, B_seg_len,
):
    _, S, D = A_q.shape
    DM = B_x.shape[2]
    H, E = B_Wq.shape[1], B_Wq.shape[2]
    M = B_mem0.shape[1]
    SEG = int(B_seg_len)
    NSEG = S // SEG
    NP = NSEG // 2
    PR = 2 * (M + SEG)
    PPB = 8
    NRB = NP // PPB
    NT = D // LANES
    assert E == LANES and H == 32 and M == 8 and SEG == 32 and A_shift_k.shape[1] == 4
    assert S == 2048 and D == 1024 and DM == 1024

    fwd, inv = _dft_mats()
    any_spec = pl.BlockSpec(memory_space=pl.ANY)
    scratch = [
        pltpu.VMEM((NRB, 7, PPB // 2 * SEG, DM // 2), U32),
        pltpu.VMEM((7, M + PPB // 2 * SEG, DM // 2), U32),
        pltpu.VMEM((NP, 2 * SEG, H * E), BF16),
        pltpu.VMEM((3, H // 2, DM, E), U32),
        pltpu.VMEM((H * E, DM), BF16),
        pltpu.VMEM((4, PPB, PR, 2 * E), BF16),
        pltpu.VMEM((PPB, 2 * M, 4 * E), BF16),
        pltpu.VMEM((PPB * 2 * SEG, DM), F32),
        pltpu.VMEM((NRB, PPB * 2 * SEG, DM), BF16),
        pltpu.VMEM((NSEG * M, DM), F32),
        pltpu.VMEM((NSEG * M, DM), F32),
        pltpu.VMEM((NSEG + M, H * E), F32),
        pltpu.VMEM((2, 3, S, LANES), BF16),
        pltpu.VMEM((2, LANES, S), BF16),
        pltpu.VMEM((S + 32, LANES), F32),
        pltpu.VMEM((S, LANES), BF16),
        pltpu.VMEM((NFFT, S), F32),
        pltpu.VMEM((NFFT, S), F32),
        pltpu.VMEM((NFFT, S), BF16),
        pltpu.VMEM((S, LANES), F32),
        pltpu.VMEM((NT, S, LANES), BF16),
        pltpu.VMEM((M, DM), BF16),
        pltpu.VMEM((NFFT, BLK), BF16),
        pltpu.VMEM((BLK, BLK), BF16),
        pltpu.VMEM((4, D), BF16),
        pltpu.VMEM((NT, LANES), BF16),
        pltpu.VMEM((8, LANES), jnp.int32),
        pltpu.SMEM((8,), jnp.int32),
        pltpu.SemaphoreType.DMA((5,)),
        pltpu.SemaphoreType.DMA((2 * NRB,)),
        pltpu.SemaphoreType.DMA((H // 2,)),
        pltpu.SemaphoreType.DMA,
        pltpu.SemaphoreType.DMA,
        pltpu.SemaphoreType.DMA((2, 2)),
        pltpu.SemaphoreType.DMA,
        pltpu.SemaphoreType.DMA((NRB,)),
    ]
    out = pl.pallas_call(
        functools.partial(_kernel, S=S, D=D, DM=DM, H=H, M=M, SEG=SEG),
        out_shape=jax.ShapeDtypeStruct((S, D + DM), BF16),
        in_specs=[any_spec] * 14,
        out_specs=any_spec,
        scratch_shapes=scratch,
        compiler_params=pltpu.CompilerParams(vmem_limit_bytes=120 * 1024 * 1024,
                                             disable_bounds_checks=True),
    )(
        A_q.reshape(S, D), A_k.reshape(S, D), A_v.reshape(S, D),
        A_shift_k.T, A_ssm_k, A_ssm_D.reshape(NT, LANES),
        B_x.reshape(NRB, S // NRB, DM), B_mem0.reshape(M, DM),
        B_Wq, B_Wk, B_Wv, B_Wo.reshape(H * E, DM),
        jnp.asarray(fwd, BF16), jnp.asarray(inv, BF16),
    )
    return out.reshape(1, S, D + DM)
```

```python
import functools

import numpy as np
import jax
import jax.numpy as jnp
from jax import lax
import jax.experimental.pallas as pl
import jax.experimental.pallas.tpu as pltpu

F32 = jnp.float32
BF16 = jnp.bfloat16
U32 = jnp.uint32

LANES = 128
BLK = 128
NFFT = 2 * BLK
TOL = 2.0 ** -10


def _dft_mats():
    even = np.arange(0, BLK, 2)
    theta = 2.0 * np.pi * (np.concatenate([even, BLK - 1 - even]) + 0.5) / NFFT
    n = np.arange(BLK)
    c = np.cos(theta[:, None] * n[None, :])
    s = np.sin(theta[:, None] * n[None, :])
    fwd = np.zeros((NFFT, BLK))
    for m in range(BLK // 8):
        fwd[16 * m:16 * m + 8] = c[8 * m:8 * m + 8]
        fwd[16 * m + 8:16 * m + 16] = -s[8 * m:8 * m + 8]
    inv = fwd[:BLK].T * (2.0 / NFFT)
    inv = np.concatenate([inv[0::2], inv[1::2]], axis=0)
    return fwd.astype(np.float32), inv.astype(np.float32)


def _dot(a, b):
    return jnp.dot(a, b, preferred_element_type=F32)


def _pack(x):
    return pltpu.bitcast(x.astype(BF16), U32)


def _unpack(w):
    return pltpu.bitcast(w, BF16)


def _lo(w):
    return pltpu.bitcast(w << 16, F32)


def _hi(w):
    return pltpu.bitcast(w & jnp.uint32(0xFFFF0000), F32)


def _strassen_lhs(a11, a12, a21, a22):
    return [a11 + a22, a21 + a22, a11, a22, a11 + a12, a21 - a11, a12 - a22]


def _strassen_rhs(b11, b12, b21, b22):
    ops = [b11 + b22, b11, b12 - b22, b21 - b11, b22, b11 + b12, b21 + b22]
    return [o.astype(BF16) for o in ops]


def _strassen(lhs, rhs, emit, init=None):
    def add(c, m):
        return m if c is None else c + m

    c11, c12, c21, c22 = init if init is not None else (None,) * 4
    m5 = _dot(lhs(4), rhs[4])
    yield m5
    m3 = _dot(lhs(2), rhs[2])
    emit(0, 1, add(c12, m5) + m3)
    yield m3
    m2 = _dot(lhs(1), rhs[1])
    c22 = add(c22, m3) - m2
    yield m2
    m4 = _dot(lhs(3), rhs[3])
    emit(1, 0, add(c21, m2) + m4)
    c11 = add(c11, m4) - m5
    yield m4
    m1 = _dot(lhs(0), rhs[0])
    c11 = c11 + m1
    c22 = c22 + m1
    yield m1
    m7 = _dot(lhs(6), rhs[6])
    emit(0, 0, c11 + m7)
    yield m7
    m6 = _dot(lhs(5), rhs[5])
    emit(1, 1, c22 + m6)
    yield m6


def _drain(*gens):
    for g in gens:
        for _ in g:
            pass


def _tokens(m):
    return [m[r:r + 8, c:c + LANES]
            for r in range(0, m.shape[0], 8) for c in range(0, m.shape[1], LANES)]


def _tie(never, tok, x):
    if tok is None:
        return x
    reps = (x.shape[0] // 8, x.shape[1] // LANES)
    if tok.dtype != x.dtype:
        tok = pltpu.bitcast(tok, x.dtype)
    if reps != (1, 1):
        never, tok = jnp.tile(never, reps), jnp.tile(tok, reps)
    return jnp.where(never, tok, x)


def _run_paced(items, toks):
    for i, it in enumerate(items):
        it(toks[i * len(toks) // len(items)])


def _interleave(nv, ngr, weights):
    dur = {'v': 256, 'h': 256, 'x': 256, 'inv': 128}
    margin = 768

    def plan(rate):
        t, v, out = 0, 0, []
        nxt = {'h': 0, 'x': 0, 'inv': 0}
        pos = {k: 0 for k in weights}
        done = {}
        credit = 0.0
        while True:
            kind = None
            if nxt['inv'] < ngr and done.get(('freq', nxt['inv']), 1e9) + margin <= t:
                kind = 'inv'
            elif nxt['x'] < ngr and done.get(('conv', nxt['x']), 1e9) + margin <= t:
                kind = 'x'
            elif nxt['h'] < ngr and nxt['h'] <= nxt['x'] and (not out or out[-1][0] == 'v'):
                kind = 'h'
            elif v < nv:
                kind = 'v'
            if kind is None:
                break
            g = v if kind == 'v' else nxt[kind]
            busy = 0.75 if kind == 'v' and v % (nv // 2) < 7 else 0.0
            credit += (rate - busy) * dur[kind]
            chunk = []
            while credit > 0:
                ready = [('out', i) for i in range(nxt['inv'])]
                ready += [('conv', i) for i in range(ngr)]
                ready += [('freq', i) for i in range(min(nxt['x'], nxt['h']))]
                ready = [k for k in ready if pos[k] < len(weights[k])]
                if not ready:
                    credit = 0.0
                    break
                k = ready[0]
                chunk.append((k, pos[k]))
                credit -= weights[k][pos[k]]
                pos[k] += 1
                if pos[k] == len(weights[k]):
                    done[k] = t + dur[kind]
            out.append((kind, g, chunk))
            t += dur[kind]
            if kind == 'v':
                v += 1
            else:
                nxt[kind] += 1
        ok = all(pos[k] == len(weights[k]) for k in weights)
        return ok, out

    rate = 1.0
    while True:
        ok, out = plan(rate)
        if ok:
            return out
        rate += 0.02


def _kernel(q_hbm, k_hbm, v_hbm, shift_hbm, h_hbm, d_hbm, x_hbm, mem0_hbm,
            wq_hbm, wk_hbm, wv_hbm, wo_hbm, fwd_hbm, inv_hbm,
            out_hbm,
            abuf, a0buf, vbuf, w32, wo, qks, vms, acc, obuf, mhat, mnew, okbuf, tsum,
            ain, ah, kf, kvb, xf, hf, wf, yt, aout,
            mem0_ref, fwd_ref, inv_ref, shift_ref, d_ref, zero_v, zero_s,
            sem_s, sem_x, sem_wv, sem_wqk, sem_wo, sem_a, sem_aout, sem_o,
            *, S, D, DM, H, M, SEG):
    E = LANES
    NSEG = S // SEG
    NP = NSEG // 2
    MR = 2 * M
    XR = 2 * SEG
    PR = MR + XR
    MW, XW, PW = MR // 2, XR // 2, PR // 2
    L = M + SEG
    NB = S // BLK
    NT = D // LANES
    PPB = 8
    PPH = PPB // 2
    NRB = NP // PPB
    G = 4
    NG = H // G
    KH = DM // 2
    scale = float(E) ** -0.5
    WV, WQ, WK = 0, 1, 2

    small = [pltpu.make_async_copy(src, dst, sem_s.at[i]) for i, (src, dst) in enumerate(
        ((mem0_hbm, mem0_ref), (shift_hbm, shift_ref), (d_hbm, d_ref),
         (fwd_hbm, fwd_ref), (inv_hbm, inv_ref)))]
    HBR = PPH * XR // 2

    def x_copies(hb):
        out = []
        for half in range(2):
            r = pl.ds(pl.multiple_of((2 * half + hb % 2) * HBR, HBR), HBR)
            out.append(pltpu.make_async_copy(x_hbm.at[hb // 2, r], obuf.at[hb // 2, r],
                                             sem_x.at[hb]))
        return out

    def w_copy(which, hp):
        src = (wv_hbm, wq_hbm, wk_hbm)[which].bitcast(U32)
        sem = sem_wv.at[hp] if which == WV else sem_wqk
        return pltpu.make_async_copy(src.at[:, hp, :], w32.at[which, hp], sem)

    def wo_copy(t):
        n = H * E // NT
        r = pl.ds(pl.multiple_of(t * n, n), n)
        return pltpu.make_async_copy(wo_hbm.at[r, :], wo.at[r, :], sem_wo)

    def a_start(t, sl, which=(0, 1, 2, 3)):
        c = pl.ds(pl.multiple_of(t * LANES, LANES), LANES)
        for i in which:
            if i == 3:
                pltpu.make_async_copy(h_hbm.at[c, :], ah.at[sl], sem_a.at[sl, 1]).start()
            else:
                src = (k_hbm, v_hbm, q_hbm)[i]
                pltpu.make_async_copy(src.at[:, c], ain.at[sl, i], sem_a.at[sl, 0]).start()

    def a_wait(sl):
        pltpu.make_async_copy(ain.at[sl], ain.at[sl], sem_a.at[sl, 0]).wait()
        pltpu.make_async_copy(ah.at[sl], ah.at[sl], sem_a.at[sl, 1]).wait()

    def aout_copy(t):
        c = pl.ds(pl.multiple_of(t * LANES, LANES), LANES)
        return pltpu.make_async_copy(aout.at[t], out_hbm.at[:, c], sem_aout)

    def o_copy(rb):
        r = pl.ds(pl.multiple_of(rb * (PPB * XR), PPB * XR), PPB * XR)
        return pltpu.make_async_copy(obuf.at[rb], out_hbm.at[r, pl.ds(D, DM)], sem_o.at[rb])

    def oq_copy(qd):
        n = PPH * XR
        r0, c0 = (qd // 2) * n, (qd % 2) * KH
        return pltpu.make_async_copy(
            obuf.at[NRB - 1, pl.ds(r0, n), pl.ds(c0, KH)],
            out_hbm.at[pl.ds((NRB - 1) * 2 * n + r0, n), pl.ds(D + c0, KH)],
            sem_o.at[NRB - 1 + qd])

    def w_rhs(which, hp, zs=None):
        if zs is None:
            w = w32[which, hp]
            return _strassen_rhs(_lo(w[:KH]), _hi(w[:KH]), _lo(w[KH:]), _hi(w[KH:]))
        out = []
        for k in range(7):
            w = w32.at[which, hp + zs[k]]
            out.append(_strassen_rhs(_lo(w[:KH]), _hi(w[:KH]), _lo(w[KH:]), _hi(w[KH:]))[k])
        return out

    def w_plain(which, hp0, n):
        parts = []
        for j in range(n):
            w = w32[which, hp0 + j]
            parts += [_lo(w), _hi(w)]
        return jnp.concatenate(parts, axis=1).astype(BF16)

    small[0].start()
    for hb in range(2):
        for cp in x_copies(hb):
            cp.start()
    w_copy(WV, 0).start()
    w_copy(WV, 1).start()
    for cp in small[1:]:
        cp.start()

    kf[0:8, :] = jnp.zeros((8, LANES), F32)
    zero_v[...] = jnp.zeros((8, LANES), jnp.int32)
    for k in range(8):
        zero_s[k] = 0
    tsum[0:8, :] = jnp.zeros((8, H * E), F32)
    vbuf[0, 0:16, :] = jnp.zeros((16, H * E), BF16)
    for hb in range(2 * NRB):
        r0 = (hb % 2) * (HBR // 2)
        abuf[hb // 2, 0, r0:r0 + 8, 0:LANES] = jnp.zeros((8, LANES), U32)
    small[0].wait()
    mem0 = mem0_ref[...].astype(F32)
    m0 = jnp.concatenate([mem0, jnp.zeros_like(mem0)], axis=0)
    z0 = jnp.zeros((MR, KH), F32)
    for k, op in enumerate(_strassen_lhs(m0[:, :KH], m0[:, KH:], z0, z0)):
        a0buf[k, 0:MW, :] = _pack(op)

    def x_item(tok, never, src, dst, r, c):
        quad = [_tie(never, tok, src[h * 2 * HBR + r:h * 2 * HBR + r + 16,
                                     kk * KH + c:kk * KH + c + 2 * LANES].astype(F32))
                for h in range(2) for kk in range(2)]
        for k, op in enumerate(_strassen_lhs(*quad)):
            dst[k, r // 2:r // 2 + 8, c:c + 2 * LANES] = _pack(op)

    def x_items(never, src, dst):
        return [functools.partial(x_item, never=never, src=src, dst=dst, r=r, c=c)
                for r in range(0, HBR, 16) for c in range(0, KH, 2 * LANES)]

    def x_first(hb, cy):
        for cp in x_copies(hb):
            cp.wait()
        src = obuf.at[0, pl.ds(pl.multiple_of(hb * HBR, HBR), 3 * HBR)]
        dst = a0buf.at[:, pl.ds(pl.multiple_of(MW + hb * (HBR // 2), 8), HBR // 2)]
        for it in x_items(None, src, dst):
            it(None)
        return cy

    lax.fori_loop(0, 2, x_first, 0)

    def v_part(j, rb, rhs, vwin, twin, pre=None):
        def lhs(k):
            x = a0buf[k] if rb == 0 else abuf[rb, k]
            if pre is not None and k == 4:
                x0 = jnp.concatenate([pre(x[:8, :LANES]), x[:8, LANES:]], axis=1)
                x = jnp.concatenate([x0, x[8:]], axis=0)
            return _unpack(x)

        def emit(half, hh, cv):
            c = slice((2 * j + hh) * E, (2 * j + hh + 1) * E)
            vv = cv.astype(BF16)
            vx = vv[MR:] if rb == 0 else vv
            p0 = rb * PPB + half * PPH
            vwin[p0:p0 + PPH, :, c] = vx.reshape(PPH, XR, E)
            ts = jnp.sum(vx.astype(F32).reshape(2 * PPH, SEG, E), axis=1)
            if rb == 0 and half == 0:
                v0 = vv[0:M].astype(F32)
                twin[NSEG:NSEG + M, c] = v0
                t0 = jnp.sum(v0, axis=0, keepdims=True)
                rows = lax.broadcasted_iota(jnp.int32, ts.shape, 0)
                ts = ts + jnp.where(rows == 0, t0, 0.0)
            twin[2 * p0:2 * (p0 + PPH), c] = ts

        return _strassen(lhs, rhs, emit)

    def v_products(t, rbs, never, extra=()):
        zs = [zero_s[k] for k in range(7)]
        c4 = pl.ds(pl.multiple_of(t * (4 * E), 4 * E), 4 * E)
        vwin = vbuf.at[:, :, c4]
        twin = tsum.at[:, c4]

        def pre(x):
            for v in (twin[0:8, 0:LANES], pltpu.bitcast(vwin[0, 0:16, 0:LANES], U32)) + tuple(extra):
                x = _tie(never, v, x)
            return x

        for j in range(2):
            rhs = w_rhs(WV, 2 * t + j, zs)
            for rb in rbs:
                yield from v_part(j, rb, rhs, vwin, twin, pre if (j, rb) == (0, rbs[0]) else None)

    def head_body(j, cy):
        w_copy(WV, 2 * j).wait()
        w_copy(WV, 2 * j + 1).wait()

        @pl.when(j >= 2)
        def _():
            for cp in x_copies(j):
                cp.wait()

        @pl.when(j + 1 < NT)
        def _():
            w_copy(WV, 2 * j + 2).start()
            w_copy(WV, 2 * j + 3).start()

        @pl.when(j + 2 < 2 * NRB)
        def _():
            for cp in x_copies(j + 2):
                cp.start()

        @pl.when(j == NT - 3)
        def _():
            a_start(0, 0, (3,))

        @pl.when(j == NT - 2)
        def _():
            a_start(0, 0, (0, 1, 2))

        never = zero_v[...] > 0
        src = obuf.at[j // 2, pl.ds(pl.multiple_of((j % 2) * HBR, HBR), 3 * HBR)]
        dst = abuf.at[j // 2, :, pl.ds(pl.multiple_of((j % 2) * (HBR // 2), 8), HBR // 2)]
        toks = []
        for m in v_products(j, [0], never, [dst[0, 0:8, 0:LANES]]):
            toks += _tokens(m)
        _run_paced(x_items(never, src, dst), toks[:-40])
        return cy

    assert NT == 2 * NRB
    lax.fori_loop(0, NT, head_body, 0)

    GA = 4

    def freq_items(a0, never):
        def item(tok, m, cc, st):
            r_re = slice(16 * m, 16 * m + 8)
            r_im = slice(16 * m + 8, 16 * m + 16)
            xr = _tie(never, tok, xf[r_re, cc * BLK:(cc + 1) * BLK])
            xi = _tie(never, tok, xf[r_im, cc * BLK:(cc + 1) * BLK])
            xs = xr + xi
            for a in range(max(a0, cc), a0 + GA):
                j = a - cc
                if ('g', m, j) not in st:
                    gr = hf[r_re, j * BLK:(j + 1) * BLK]
                    gi = hf[r_im, j * BLK:(j + 1) * BLK]
                    st['g', m, j] = (gr, gi, gr + gi)
                gr, gi, gs = st['g', m, j]
                ps = (xr * gr, xi * gi, xs * gs)
                st[m, a] = ps if (m, a) not in st else tuple(u + v for u, v in zip(st[m, a], ps))
                if cc == a:
                    p1, p2, p3 = st[m, a]
                    st[m, a] = (p1 - p2, p3 - p1 - p2)
                    if m >= BLK // 16:
                        m0 = m - BLK // 16
                        (wr, wi), (vr, vi) = st[m0, a], st[m, a]
                        c = slice(a * BLK, (a + 1) * BLK)
                        wf[16 * m0:16 * m0 + 16, c] = (
                            jnp.concatenate([wr + vr, wi - vi], axis=0).astype(BF16))
                        wf[16 * m:16 * m + 16, c] = (
                            jnp.concatenate([wr - vr, wi + vi], axis=0).astype(BF16))

        items = []
        for m0 in range(BLK // 16):
            st = {}
            for m in (m0, m0 + BLK // 16):
                items += [(functools.partial(item, m=m, cc=cc, st=st),
                           4 + 6 * (a0 + GA - max(a0, cc)) + (6 if cc >= a0 else 0))
                          for cc in range(a0 + GA)]
        return items

    def tile_body(t, carry):
        sl = t % 2
        a_wait(sl)

        @pl.when(t + 1 < NT)
        def _():
            a_start(t + 1, 1 - sl)
            wo_copy(t + 1).start()

        for which in (WQ, WK):
            w_copy(which, 2 * t).start()
            w_copy(which, 2 * t + 1).start()

        c = pl.ds(pl.multiple_of(t * LANES, LANES), LANES)
        taps = shift_ref[:, c].astype(F32)
        dcol = d_ref[...].astype(F32)
        rows = lax.broadcasted_iota(jnp.int32, dcol.shape, 0)
        dvec = jnp.sum(jnp.where(rows == t, dcol, 0.0), axis=0, keepdims=True)
        dvb = jnp.broadcast_to(dvec, (8, LANES))
        tapb = [jnp.broadcast_to(taps[j:j + 1, :], (8, LANES)) for j in range(4)]
        never = zero_v[...] > 0
        fwd = fwd_ref[...]
        NGR = NB // GA
        GW = GA * BLK

        def conv_item(tok, r0):
            kf[8 + r0:24 + r0, :] = ain[sl, 0, r0:r0 + 16, :].astype(F32)
            halves = []
            for h in range(2):
                r = 8 + r0 + 8 * h
                ks = kf[r:r + 8, :] * _tie(never, tok, tapb[0])
                for j in range(1, 4):
                    ks = ks + kf[r - j:r - j + 8, :] * tapb[j]
                halves.append(ks)
            kvb[r0:r0 + 16, :] = (jnp.concatenate(halves, axis=0)
                                  * ain[sl, 1, r0:r0 + 16, :].astype(F32)).astype(BF16)

        hlast = [None]

        def h_fwd(g):
            hst = jnp.concatenate([ah[sl, :, b * BLK:(b + 1) * BLK]
                                   for b in range(g * GA, (g + 1) * GA)], axis=0)
            hh = lax.dot_general(fwd, hst, (((1,), (1,)), ((), ())), preferred_element_type=F32)
            for b in range(GA):
                cur = hh[:, b * BLK:(b + 1) * BLK]
                prev = hlast[0]
                c = slice((g * GA + b) * BLK, (g * GA + b + 1) * BLK)
                if prev is None:
                    hf[:, c] = cur
                else:
                    for m in range(BLK // 8):
                        re = slice(16 * m, 16 * m + 8)
                        im = slice(16 * m + 8, 16 * m + 16)
                        if m < BLK // 16:
                            hf[re, c] = cur[re] - prev[im]
                            hf[im, c] = cur[im] + prev[re]
                        else:
                            hf[re, c] = cur[re] + prev[im]
                            hf[im, c] = cur[im] - prev[re]
                hlast[0] = cur
            return hh

        def x_fwd(g):
            rhs = jnp.concatenate([kvb[b * BLK:(b + 1) * BLK, :]
                                   for b in range(g * GA, (g + 1) * GA)], axis=1)
            xx = _dot(fwd, rhs)
            xf[:, g * GW:(g + 1) * GW] = xx
            return xx

        def inverse(g):
            ys = []
            for par in range(2):
                y = _dot(inv_ref[par * (BLK // 2):(par + 1) * (BLK // 2), :],
                         wf[par * BLK:(par + 1) * BLK, g * GW:(g + 1) * GW])
                for a in range(GA):
                    yt[pl.ds((g * GA + a) * BLK + par, BLK // 2, stride=2), :] = (
                        y[:, a * BLK:(a + 1) * BLK])
                ys.append(y)
            return jnp.concatenate(ys, axis=0)

        def out_item(tok, r0):
            d8 = _tie(never, tok, dvb)
            yb = yt[r0:r0 + 16, :] + kvb[r0:r0 + 16, :].astype(F32) * jnp.concatenate([d8, d8], axis=0)
            aout[t, r0:r0 + 16, :] = (ain[sl, 2, r0:r0 + 16, :].astype(F32) * yb).astype(BF16)

        def rows16(fn, g, w):
            return [(functools.partial(fn, r0=r0), w) for r0 in range(g * GW, (g + 1) * GW, 16)]

        vgen = v_products(t, list(range(1, NRB)), never)
        nv = 2 * (NRB - 1) * 7
        work = {('conv', g): rows16(conv_item, g, 25) for g in range(NGR)}
        work.update({('freq', g): freq_items(g * GA, never) for g in range(NGR)})
        work.update({('out', g): rows16(out_item, g, 16) for g in range(NGR)})
        for kind, g, chunks in _interleave(nv, NGR, {k: [w for _, w in v] for k, v in work.items()}):
            if kind is not None:
                m = (next(vgen) if kind == 'v' else
                     {'h': h_fwd, 'x': x_fwd, 'inv': inverse}[kind](g))
                toks = _tokens(m)
            items = [work[k][i][0] for k, i in chunks]
            if kind is None:
                for it in items:
                    it(None)
            elif items:
                _run_paced(items, toks)
        _drain(vgen)
        aout_copy(t).start()
        return carry

    for cp in small[1:]:
        cp.wait()
    wo_copy(0).start()
    lax.fori_loop(0, NT, tile_body, 0)
    pltpu.make_async_copy(wo, wo, sem_wo).wait()

    def initial_guess():
        puni = pl.reciprocal(jnp.full((1, 1), float(L), F32), approx=True).astype(BF16).astype(F32)

        def shift_down(m):
            rows = lax.broadcasted_iota(jnp.int32, m.shape, 0)
            return jnp.where(rows == 0, 0.0, pltpu.roll(m, 1, 0))

        m1 = shift_down(_dot((tsum[0:NSEG, :] * puni).astype(BF16), wo[...]))
        v1 = _dot(m1.astype(BF16), w_plain(WV, 0, H // 2)).astype(BF16).astype(F32)
        u2 = ((tsum[0:NSEG, :] + float(M) * v1) * puni).astype(BF16)
        m2 = shift_down(_dot(u2, wo[...]))
        mhat[0:NSEG * M, :] = jnp.broadcast_to(m2[:, None, :], (NSEG, M, DM)).reshape(NSEG * M, DM)
        mhat[NSEG * M:, :] = jnp.zeros((M, DM), F32)
        mhat[0:M, :] = mem0_ref[...].astype(F32)
        pltpu.make_async_copy(w32.at[WQ:WK + 1], w32.at[WQ:WK + 1], sem_wqk).wait()

    ri = lax.broadcasted_iota(jnp.int32, (PR, PR), 0)
    ci = lax.broadcasted_iota(jnp.int32, (PR, PR), 1)

    def seg_of(r):
        return jnp.where(r < MR, r // M, (r - MR) // SEG)

    def pos_of(r):
        return jnp.where(r < MR, r % M, M + (r - MR) % SEG)

    same = seg_of(ri) == seg_of(ci)
    allowed = same & ((ri < MR) | (pos_of(ri) >= pos_of(ci)))
    fill = jnp.where(same, -1e9, -jnp.inf).astype(F32)

    def sweep(state):
        it, _ = state
        pl.when(it == 0)(initial_guess)

        @pl.when(it > 0)
        def _():
            mhat[M:, :] = mnew[...]

        def mem_rows(i):
            n = PPB * MR
            return mhat[pl.ds(pl.multiple_of((i // NG) * n, n), n), :]

        def mem_lhs(i):
            m = mem_rows(i)
            n = PPH * MR
            ops = [_pack(o) for o in _strassen_lhs(m[:n, :KH], m[:n, KH:], m[n:, :KH], m[n:, KH:])]
            t = jnp.concatenate([jnp.where(i < NG, 0.0, m[:M]), m[M:MR]], axis=0)
            b = m[n:n + MR]
            vops = [jnp.concatenate([_pack(o), full[MW:]], axis=0) for o, full in zip(
                _strassen_lhs(t[:, :KH], t[:, KH:], b[:, :KH], b[:, KH:]), ops)]
            return ops, vops

        def qk_proj(i, j, mops):
            rb = i // NG
            hp = (i % NG) * (G // 2) + j // 2

            def lhs(k):
                return _unpack(jnp.concatenate([mops[k], abuf[rb, k]], axis=0))

            n = PPH * MR
            cs = {}

            def emit(half, hh, cv):
                cs[half, hh] = cv
                if (half, 1 - hh) in cs:
                    v = jnp.concatenate([cs[half, 0], cs[half, 1]], axis=1).astype(BF16)
                    ps = slice(half * PPH, (half + 1) * PPH)
                    qks[j, ps, 0:MR, :] = v[:n].reshape(PPH, MR, 2 * E)
                    qks[j, ps, MR:PR, :] = v[n:].reshape(PPH, XR, 2 * E)

            return _strassen(lhs, w_rhs(WQ + j % 2, hp, [zero_s[k] for k in range(7)]), emit)

        def vm_proj(i, j, vops):
            hp = (i % NG) * (G // 2) + j

            def emit(half, hh, cv):
                if half == 0:
                    v0 = tsum[NSEG:NSEG + M, pl.ds(pl.multiple_of((2 * hp + hh) * E, E), E)]
                    cv = jnp.concatenate([jnp.where(i < NG, v0, cv[:M]), cv[M:]], axis=0)
                vms[half * PPH:(half + 1) * PPH, :, (2 * j + hh) * E:(2 * j + hh + 1) * E] = (
                    cv.astype(BF16).reshape(PPH, MR, E))

            return _strassen(lambda k: _unpack(vops[k]),
                             w_rhs(WV, hp, [zero_s[k] for k in range(7)]), emit)

        def scores(j):
            c = slice((j % 2) * E, (j % 2 + 1) * E)
            return lax.dot_general(qks[2 * (j // 2), :, :, c], qks[2 * (j // 2) + 1, :, :, c],
                                   (((2,), (2,)), ((0,), (0,))), preferred_element_type=F32)

        def attend(i, j, s):
            p0 = pl.multiple_of((i // NG) * PPB, PPB)
            h = (i % NG) * G + j
            s = jnp.where(allowed[None], s * scale, fill[None])
            e = jnp.exp(s - jnp.max(s, axis=-1, keepdims=True))
            p = (e * pl.reciprocal(jnp.sum(e, axis=-1, keepdims=True), approx=True)).astype(BF16)
            vh = jnp.concatenate(
                [vms[:, :, j * E:(j + 1) * E],
                 vbuf[pl.ds(p0, PPB), :, pl.ds(pl.multiple_of(h * E, E), E)]], axis=1)
            return lax.dot_general(p, vh, (((2,), (1,)), ((0,), (0,))), preferred_element_type=F32)

        def out_proj(i, us, last):
            rb = i // NG
            g = i % NG
            u = jnp.concatenate(us, axis=2)
            wog = wo[pl.ds(pl.multiple_of(g * (G * E), G * E), G * E), :]
            rm = pl.ds(pl.multiple_of(rb * (PPB * MR), PPB * MR), PPB * MR)
            um = u[:, :MR, :].reshape(PPB * MR, G * E).astype(BF16)
            new = jnp.where(g > 0, mnew[rm, :], 0.0) + _dot(um, wog)
            mnew[rm, :] = new
            old = mhat[pl.ds(pl.multiple_of(rb * (PPB * MR) + M, M), PPB * MR), :]
            err = jnp.max(jnp.abs(new - old), axis=1, keepdims=True)
            ref = jnp.max(jnp.abs(new), axis=1, keepdims=True)
            okbuf[rm, :] = jnp.broadcast_to(jnp.where(err <= TOL * ref, 1.0, 0.0),
                                            (PPB * MR, LANES))
            n = PPH * XR
            kh = G * E // 2
            top = u[:PPH, MR:, :].reshape(n, G * E)
            bot = u[PPH:, MR:, :].reshape(n, G * E)
            ops = _strassen_lhs(top[:, :kh], top[:, kh:], bot[:, :kh], bot[:, kh:])
            wf32 = wog.astype(F32)
            rhs = _strassen_rhs(wf32[:kh, :KH], wf32[:kh, KH:], wf32[kh:, :KH], wf32[kh:, KH:])
            quads = [(slice(0, n), slice(0, KH)), (slice(0, n), slice(KH, DM)),
                     (slice(n, 2 * n), slice(0, KH)), (slice(n, 2 * n), slice(KH, DM))]
            init = [jnp.where(g > 0, acc[r, c], 0.0) for r, c in quads]

            def emit(half, hh, v):
                r, c = quads[2 * half + hh]
                obuf[rb, r, c] = v.astype(BF16)
                if last:
                    oq_copy(2 * half + hh).start()
                else:
                    acc[r, c] = v

            _drain(_strassen(lambda k: ops[k].astype(BF16), rhs, emit, init))

        def step(i, nxt):
            s0, s1 = scores(0), scores(1)
            if nxt:
                mops, vops = mem_lhs(i + 1)
                _drain(qk_proj(i + 1, 0, mops))
            u0, u1 = attend(i, 0, s0), attend(i, 1, s1)
            s2, s3 = scores(2), scores(3)
            if nxt:
                _drain(qk_proj(i + 1, 1, mops))
            u2, u3 = attend(i, 2, s2), attend(i, 3, s3)
            if nxt:
                _drain(zip(qk_proj(i + 1, 2, mops), vm_proj(i + 1, 0, vops)))
                _drain(zip(qk_proj(i + 1, 3, mops), vm_proj(i + 1, 1, vops)))
            out_proj(i, [u0, u1, u2, u3], not nxt)

        mops0, vops0 = mem_lhs(0)
        _drain(qk_proj(0, 0, mops0), qk_proj(0, 1, mops0))
        _drain(zip(qk_proj(0, 2, mops0), vm_proj(0, 0, vops0)))
        _drain(zip(qk_proj(0, 3, mops0), vm_proj(0, 1, vops0)))

        def main_body(i, cy):
            step(i, True)

            @pl.when(i % NG == NG - 1)
            def _():
                o_copy(i // NG).start()

            return cy

        lax.fori_loop(0, NRB * NG - 1, main_body, 0)
        step(NRB * NG - 1, False)
        ok = jnp.min(okbuf[0:(NSEG - 1) * M, :])
        for rb in range(NRB - 1):
            o_copy(rb).wait()
        for qd in range(4):
            oq_copy(qd).wait()
        return it + 1, (ok > 0.5).astype(jnp.int32)

    lax.while_loop(lambda st: jnp.logical_and(st[0] < NSEG, st[1] == 0), sweep,
                   (jnp.int32(0), jnp.int32(0)))
    pltpu.make_async_copy(aout, aout, sem_aout).wait()


@functools.partial(jax.jit, static_argnames=("B_seg_len",))
def pallas_concat_heads__ssm_conv_h3__memory_aug_recurrent_mem_tr__prompt_kernel(
    A_q, A_k, A_v, A_shift_k, A_ssm_k, A_ssm_D,
    B_x, B_mem0, B_Wq, B_Wk, B_Wv, B_Wo, B_seg_len,
):
    _, S, D = A_q.shape
    DM = B_x.shape[2]
    H, E = B_Wq.shape[1], B_Wq.shape[2]
    M = B_mem0.shape[1]
    SEG = int(B_seg_len)
    NSEG = S // SEG
    NP = NSEG // 2
    PR = 2 * (M + SEG)
    PPB = 8
    NRB = NP // PPB
    NT = D // LANES
    assert E == LANES and H == 32 and M == 8 and SEG == 32 and A_shift_k.shape[1] == 4
    assert S == 2048 and D == 1024 and DM == 1024

    fwd, inv = _dft_mats()
    any_spec = pl.BlockSpec(memory_space=pl.ANY)
    scratch = [
        pltpu.VMEM((NRB, 7, PPB // 2 * SEG, DM // 2), U32),
        pltpu.VMEM((7, M + PPB // 2 * SEG, DM // 2), U32),
        pltpu.VMEM((NP, 2 * SEG, H * E), BF16),
        pltpu.VMEM((3, H // 2, DM, E), U32),
        pltpu.VMEM((H * E, DM), BF16),
        pltpu.VMEM((4, PPB, PR, 2 * E), BF16),
        pltpu.VMEM((PPB, 2 * M, 4 * E), BF16),
        pltpu.VMEM((PPB * 2 * SEG, DM), F32),
        pltpu.VMEM((NRB, PPB * 2 * SEG, DM), BF16),
        pltpu.VMEM(((NSEG + 1) * M, DM), F32),
        pltpu.VMEM((NSEG * M, DM), F32),
        pltpu.VMEM((NSEG * M, LANES), F32),
        pltpu.VMEM((NSEG + M, H * E), F32),
        pltpu.VMEM((2, 3, S, LANES), BF16),
        pltpu.VMEM((2, LANES, S), BF16),
        pltpu.VMEM((S + 32, LANES), F32),
        pltpu.VMEM((S, LANES), BF16),
        pltpu.VMEM((NFFT, S), F32),
        pltpu.VMEM((NFFT, S), F32),
        pltpu.VMEM((NFFT, S), BF16),
        pltpu.VMEM((S, LANES), F32),
        pltpu.VMEM((NT, S, LANES), BF16),
        pltpu.VMEM((M, DM), BF16),
        pltpu.VMEM((NFFT, BLK), BF16),
        pltpu.VMEM((BLK, BLK), BF16),
        pltpu.VMEM((4, D), BF16),
        pltpu.VMEM((NT, LANES), BF16),
        pltpu.VMEM((8, LANES), jnp.int32),
        pltpu.SMEM((8,), jnp.int32),
        pltpu.SemaphoreType.DMA((5,)),
        pltpu.SemaphoreType.DMA((2 * NRB,)),
        pltpu.SemaphoreType.DMA((H // 2,)),
        pltpu.SemaphoreType.DMA,
        pltpu.SemaphoreType.DMA,
        pltpu.SemaphoreType.DMA((2, 2)),
        pltpu.SemaphoreType.DMA,
        pltpu.SemaphoreType.DMA((NRB + 3,)),
    ]
    out = pl.pallas_call(
        functools.partial(_kernel, S=S, D=D, DM=DM, H=H, M=M, SEG=SEG),
        out_shape=jax.ShapeDtypeStruct((S, D + DM), BF16),
        in_specs=[any_spec] * 14,
        out_specs=any_spec,
        scratch_shapes=scratch,
        compiler_params=pltpu.CompilerParams(vmem_limit_bytes=120 * 1024 * 1024,
                                             disable_bounds_checks=True),
    )(
        A_q.reshape(S, D), A_k.reshape(S, D), A_v.reshape(S, D),
        A_shift_k.T, A_ssm_k, A_ssm_D.reshape(NT, LANES),
        B_x.reshape(NRB, S // NRB, DM), B_mem0.reshape(M, DM),
        B_Wq, B_Wk, B_Wv, B_Wo.reshape(H * E, DM),
        jnp.asarray(fwd, BF16), jnp.asarray(inv, BF16),
    )
    return out.reshape(1, S, D + DM)
```

```python
import functools

import numpy as np
import jax
import jax.numpy as jnp
from jax import lax
import jax.experimental.pallas as pl
import jax.experimental.pallas.tpu as pltpu

F32 = jnp.float32
BF16 = jnp.bfloat16
U32 = jnp.uint32

LANES = 128
BLK = 128
NFFT = 2 * BLK
TOL = 2.0 ** -10


def _dft_mats():
    even = np.arange(0, BLK, 2)
    theta = 2.0 * np.pi * (np.concatenate([even, BLK - 1 - even]) + 0.5) / NFFT
    n = np.arange(BLK)
    c = np.cos(theta[:, None] * n[None, :])
    s = np.sin(theta[:, None] * n[None, :])
    fwd = np.zeros((NFFT, BLK))
    for m in range(BLK // 8):
        fwd[16 * m:16 * m + 8] = c[8 * m:8 * m + 8]
        fwd[16 * m + 8:16 * m + 16] = -s[8 * m:8 * m + 8]
    inv = fwd[:BLK].T * (2.0 / NFFT)
    inv = np.concatenate([inv[0::2], inv[1::2]], axis=0)
    return fwd.astype(np.float32), inv.astype(np.float32)


def _dot(a, b):
    return jnp.dot(a, b, preferred_element_type=F32)


def _pack(x):
    return pltpu.bitcast(x.astype(BF16), U32)


def _unpack(w):
    return pltpu.bitcast(w, BF16)


def _lo(w):
    return pltpu.bitcast(w << 16, F32)


def _hi(w):
    return pltpu.bitcast(w & jnp.uint32(0xFFFF0000), F32)


def _strassen_lhs(a11, a12, a21, a22):
    return [a11 + a22, a21 + a22, a11, a22, a11 + a12, a21 - a11, a12 - a22]


def _strassen_rhs(b11, b12, b21, b22):
    ops = [b11 + b22, b11, b12 - b22, b21 - b11, b22, b11 + b12, b21 + b22]
    return [o.astype(BF16) for o in ops]


def _strassen(lhs, rhs, emit, init=None):
    def add(c, m):
        return m if c is None else c + m

    c11, c12, c21, c22 = init if init is not None else (None,) * 4
    m5 = _dot(lhs(4), rhs[4])
    yield m5
    m3 = _dot(lhs(2), rhs[2])
    emit(0, 1, add(c12, m5) + m3)
    yield m3
    m2 = _dot(lhs(1), rhs[1])
    c22 = add(c22, m3) - m2
    yield m2
    m4 = _dot(lhs(3), rhs[3])
    emit(1, 0, add(c21, m2) + m4)
    c11 = add(c11, m4) - m5
    yield m4
    m1 = _dot(lhs(0), rhs[0])
    c11 = c11 + m1
    c22 = c22 + m1
    yield m1
    m7 = _dot(lhs(6), rhs[6])
    emit(0, 0, c11 + m7)
    yield m7
    m6 = _dot(lhs(5), rhs[5])
    emit(1, 1, c22 + m6)
    yield m6


def _drain(*gens):
    for g in gens:
        for _ in g:
            pass


def _tokens(m):
    return [m[r:r + 8, c:c + LANES]
            for r in range(0, m.shape[0], 8) for c in range(0, m.shape[1], LANES)]


def _tie(never, tok, x):
    if tok is None:
        return x
    reps = (x.shape[0] // 8, x.shape[1] // LANES)
    if tok.dtype != x.dtype:
        tok = pltpu.bitcast(tok, x.dtype)
    if reps != (1, 1):
        never, tok = jnp.tile(never, reps), jnp.tile(tok, reps)
    return jnp.where(never, tok, x)


def _run_paced(items, toks):
    for i, it in enumerate(items):
        it(toks[i * len(toks) // len(items)])


def _interleave(nv, ngr, weights):
    dur = {'v': 256, 'h': 256, 'x': 256, 'inv': 128}
    margin = 768

    def plan(rate):
        t, v, out = 0, 0, []
        nxt = {'h': 0, 'x': 0, 'inv': 0}
        pos = {k: 0 for k in weights}
        done = {}
        credit = 0.0
        while True:
            kind = None
            if nxt['inv'] < ngr and done.get(('freq', nxt['inv']), 1e9) + margin <= t:
                kind = 'inv'
            elif nxt['x'] < ngr and done.get(('conv', nxt['x']), 1e9) + margin <= t:
                kind = 'x'
            elif nxt['h'] < ngr and nxt['h'] <= nxt['x'] and (not out or out[-1][0] == 'v'):
                kind = 'h'
            elif v < nv:
                kind = 'v'
            if kind is None:
                break
            g = v if kind == 'v' else nxt[kind]
            busy = 0.75 if kind == 'v' and v % (nv // 2) < 7 else 0.0
            credit += (rate - busy) * dur[kind]
            chunk = []
            while credit > 0:
                ready = [('out', i) for i in range(nxt['inv'])]
                ready += [('conv', i) for i in range(ngr)]
                ready += [('freq', i) for i in range(min(nxt['x'], nxt['h']))]
                ready = [k for k in ready if pos[k] < len(weights[k])]
                if not ready:
                    credit = 0.0
                    break
                k = ready[0]
                chunk.append((k, pos[k]))
                credit -= weights[k][pos[k]]
                pos[k] += 1
                if pos[k] == len(weights[k]):
                    done[k] = t + dur[kind]
            out.append((kind, g, chunk))
            t += dur[kind]
            if kind == 'v':
                v += 1
            else:
                nxt[kind] += 1
        ok = all(pos[k] == len(weights[k]) for k in weights)
        return ok, out

    rate = 1.0
    while True:
        ok, out = plan(rate)
        if ok:
            return out
        rate += 0.02


def _kernel(q_hbm, k_hbm, v_hbm, shift_hbm, h_hbm, d_hbm, x_hbm, mem0_hbm,
            wq_hbm, wk_hbm, wv_hbm, wo_hbm, fwd_hbm, inv_hbm,
            out_hbm,
            abuf, a0buf, vbuf, w32, wo, qks, vms, acc, obuf, mhat, mnew, okbuf, tsum,
            ain, ah, kf, kvb, xf, hf, wf, yt, aout,
            mem0_ref, fwd_ref, inv_ref, shift_ref, d_ref, zero_v, zero_s,
            sem_s, sem_x, sem_wv, sem_wqk, sem_wo, sem_a, sem_aout, sem_o,
            *, S, D, DM, H, M, SEG):
    E = LANES
    NSEG = S // SEG
    NP = NSEG // 2
    MR = 2 * M
    XR = 2 * SEG
    PR = MR + XR
    MW, XW, PW = MR // 2, XR // 2, PR // 2
    L = M + SEG
    NB = S // BLK
    NT = D // LANES
    PPB = 8
    PPH = PPB // 2
    NRB = NP // PPB
    G = 4
    NG = H // G
    KH = DM // 2
    scale = float(E) ** -0.5
    WV, WQ, WK = 0, 1, 2

    small = [pltpu.make_async_copy(src, dst, sem_s.at[i]) for i, (src, dst) in enumerate(
        ((mem0_hbm, mem0_ref), (shift_hbm, shift_ref), (d_hbm, d_ref),
         (fwd_hbm, fwd_ref), (inv_hbm, inv_ref)))]
    HBR = PPH * XR // 2

    def x_copies(hb):
        out = []
        for half in range(2):
            r = pl.ds(pl.multiple_of((2 * half + hb % 2) * HBR, HBR), HBR)
            out.append(pltpu.make_async_copy(x_hbm.at[hb // 2, r], obuf.at[hb // 2, r],
                                             sem_x.at[hb]))
        return out

    def w_copy(which, hp):
        src = (wv_hbm, wq_hbm, wk_hbm)[which].bitcast(U32)
        sem = sem_wv.at[hp] if which == WV else sem_wqk
        return pltpu.make_async_copy(src.at[:, hp, :], w32.at[which, hp], sem)

    def wo_copy(t):
        n = H * E // NT
        r = pl.ds(pl.multiple_of(t * n, n), n)
        return pltpu.make_async_copy(wo_hbm.at[r, :], wo.at[r, :], sem_wo)

    def a_start(t, sl, which=(0, 1, 2, 3)):
        c = pl.ds(pl.multiple_of(t * LANES, LANES), LANES)
        for i in which:
            if i == 3:
                pltpu.make_async_copy(h_hbm.at[c, :], ah.at[sl], sem_a.at[sl, 1]).start()
            else:
                src = (k_hbm, v_hbm, q_hbm)[i]
                pltpu.make_async_copy(src.at[:, c], ain.at[sl, i], sem_a.at[sl, 0]).start()

    def a_wait(sl):
        pltpu.make_async_copy(ain.at[sl], ain.at[sl], sem_a.at[sl, 0]).wait()
        pltpu.make_async_copy(ah.at[sl], ah.at[sl], sem_a.at[sl, 1]).wait()

    def aout_copy(t):
        c = pl.ds(pl.multiple_of(t * LANES, LANES), LANES)
        return pltpu.make_async_copy(aout.at[t], out_hbm.at[:, c], sem_aout)

    def o_copy(rb):
        r = pl.ds(pl.multiple_of(rb * (PPB * XR), PPB * XR), PPB * XR)
        return pltpu.make_async_copy(obuf.at[rb], out_hbm.at[r, pl.ds(D, DM)], sem_o.at[rb])

    def oq_copy(qd):
        n = PPH * XR
        r0, c0 = (qd // 2) * n, (qd % 2) * KH
        return pltpu.make_async_copy(
            obuf.at[NRB - 1, pl.ds(r0, n), pl.ds(c0, KH)],
            out_hbm.at[pl.ds((NRB - 1) * 2 * n + r0, n), pl.ds(D + c0, KH)],
            sem_o.at[NRB - 1 + qd])

    def w_rhs(which, hp, zs=None):
        if zs is None:
            w = w32[which, hp]
            return _strassen_rhs(_lo(w[:KH]), _hi(w[:KH]), _lo(w[KH:]), _hi(w[KH:]))
        out = []
        for k in range(7):
            w = w32.at[which, hp + zs[k]]
            out.append(_strassen_rhs(_lo(w[:KH]), _hi(w[:KH]), _lo(w[KH:]), _hi(w[KH:]))[k])
        return out

    def w_plain(which, hp0, n):
        parts = []
        for j in range(n):
            w = w32[which, hp0 + j]
            parts += [_lo(w), _hi(w)]
        return jnp.concatenate(parts, axis=1).astype(BF16)

    small[0].start()
    for hb in range(2):
        for cp in x_copies(hb):
            cp.start()
    w_copy(WV, 0).start()
    w_copy(WV, 1).start()
    for cp in small[1:]:
        cp.start()

    kf[0:8, :] = jnp.zeros((8, LANES), F32)
    zero_v[...] = jnp.zeros((8, LANES), jnp.int32)
    for k in range(8):
        zero_s[k] = 0
    tsum[0:8, :] = jnp.zeros((8, H * E), F32)
    vbuf[0, 0:16, :] = jnp.zeros((16, H * E), BF16)
    for hb in range(2 * NRB):
        r0 = (hb % 2) * (HBR // 2)
        abuf[hb // 2, 0, r0:r0 + 8, 0:LANES] = jnp.zeros((8, LANES), U32)
    small[0].wait()
    mem0 = mem0_ref[...].astype(F32)
    m0 = jnp.concatenate([mem0, jnp.zeros_like(mem0)], axis=0)
    z0 = jnp.zeros((MR, KH), F32)
    for k, op in enumerate(_strassen_lhs(m0[:, :KH], m0[:, KH:], z0, z0)):
        a0buf[k, 0:MW, :] = _pack(op)

    def x_item(tok, never, src, dst, r, c):
        quad = [_tie(never, tok, src[h * 2 * HBR + r:h * 2 * HBR + r + 16,
                                     kk * KH + c:kk * KH + c + 2 * LANES].astype(F32))
                for h in range(2) for kk in range(2)]
        for k, op in enumerate(_strassen_lhs(*quad)):
            dst[k, r // 2:r // 2 + 8, c:c + 2 * LANES] = _pack(op)

    def x_items(never, src, dst):
        return [functools.partial(x_item, never=never, src=src, dst=dst, r=r, c=c)
                for r in range(0, HBR, 16) for c in range(0, KH, 2 * LANES)]

    def x_first(hb, cy):
        for cp in x_copies(hb):
            cp.wait()
        src = obuf.at[0, pl.ds(pl.multiple_of(hb * HBR, HBR), 3 * HBR)]
        dst = a0buf.at[:, pl.ds(pl.multiple_of(MW + hb * (HBR // 2), 8), HBR // 2)]
        for it in x_items(None, src, dst):
            it(None)
        return cy

    lax.fori_loop(0, 2, x_first, 0)

    def v_part(j, rb, rhs, vwin, twin, pre=None):
        def lhs(k):
            x = a0buf[k] if rb == 0 else abuf[rb, k]
            if pre is not None and k == 4:
                x0 = jnp.concatenate([pre(x[:8, :LANES]), x[:8, LANES:]], axis=1)
                x = jnp.concatenate([x0, x[8:]], axis=0)
            return _unpack(x)

        def emit(half, hh, cv):
            c = slice((2 * j + hh) * E, (2 * j + hh + 1) * E)
            vv = cv.astype(BF16)
            vx = vv[MR:] if rb == 0 else vv
            p0 = rb * PPB + half * PPH
            vwin[p0:p0 + PPH, :, c] = vx.reshape(PPH, XR, E)
            ts = jnp.sum(vx.astype(F32).reshape(2 * PPH, SEG, E), axis=1)
            if rb == 0 and half == 0:
                v0 = vv[0:M].astype(F32)
                twin[NSEG:NSEG + M, c] = v0
                t0 = jnp.sum(v0, axis=0, keepdims=True)
                rows = lax.broadcasted_iota(jnp.int32, ts.shape, 0)
                ts = ts + jnp.where(rows == 0, t0, 0.0)
            twin[2 * p0:2 * (p0 + PPH), c] = ts

        return _strassen(lhs, rhs, emit)

    def v_products(t, rbs, never, extra=()):
        zs = [zero_s[k] for k in range(7)]
        c4 = pl.ds(pl.multiple_of(t * (4 * E), 4 * E), 4 * E)
        vwin = vbuf.at[:, :, c4]
        twin = tsum.at[:, c4]

        def pre(x):
            for v in (twin[0:8, 0:LANES], pltpu.bitcast(vwin[0, 0:16, 0:LANES], U32)) + tuple(extra):
                x = _tie(never, v, x)
            return x

        for j in range(2):
            rhs = w_rhs(WV, 2 * t + j, zs)
            for rb in rbs:
                yield from v_part(j, rb, rhs, vwin, twin, pre if (j, rb) == (0, rbs[0]) else None)

    def head_body(j, cy):
        w_copy(WV, 2 * j).wait()
        w_copy(WV, 2 * j + 1).wait()

        @pl.when(j >= 2)
        def _():
            for cp in x_copies(j):
                cp.wait()

        @pl.when(j + 1 < NT)
        def _():
            w_copy(WV, 2 * j + 2).start()
            w_copy(WV, 2 * j + 3).start()

        @pl.when(j + 2 < 2 * NRB)
        def _():
            for cp in x_copies(j + 2):
                cp.start()

        @pl.when(j == NT - 3)
        def _():
            a_start(0, 0, (3,))

        @pl.when(j == NT - 2)
        def _():
            a_start(0, 0, (0, 1, 2))

        never = zero_v[...] > 0
        src = obuf.at[j // 2, pl.ds(pl.multiple_of((j % 2) * HBR, HBR), 3 * HBR)]
        dst = abuf.at[j // 2, :, pl.ds(pl.multiple_of((j % 2) * (HBR // 2), 8), HBR // 2)]
        toks = []
        for m in v_products(j, [0], never, [dst[0, 0:8, 0:LANES]]):
            toks += _tokens(m)
        _run_paced(x_items(never, src, dst), toks[:-40])
        return cy

    assert NT == 2 * NRB
    lax.fori_loop(0, NT, head_body, 0)

    GA = 4

    def freq_items(a0, never):
        def item(tok, m, cc, st):
            r_re = slice(16 * m, 16 * m + 8)
            r_im = slice(16 * m + 8, 16 * m + 16)
            xr = _tie(never, tok, xf[r_re, cc * BLK:(cc + 1) * BLK])
            xi = _tie(never, tok, xf[r_im, cc * BLK:(cc + 1) * BLK])
            xs = xr + xi
            for a in range(max(a0, cc), a0 + GA):
                j = a - cc
                if ('g', m, j) not in st:
                    gr = hf[r_re, j * BLK:(j + 1) * BLK]
                    gi = hf[r_im, j * BLK:(j + 1) * BLK]
                    st['g', m, j] = (gr, gi, gr + gi)
                gr, gi, gs = st['g', m, j]
                ps = (xr * gr, xi * gi, xs * gs)
                st[m, a] = ps if (m, a) not in st else tuple(u + v for u, v in zip(st[m, a], ps))
                if cc == a:
                    p1, p2, p3 = st[m, a]
                    st[m, a] = (p1 - p2, p3 - p1 - p2)
                    if m >= BLK // 16:
                        m0 = m - BLK // 16
                        (wr, wi), (vr, vi) = st[m0, a], st[m, a]
                        c = slice(a * BLK, (a + 1) * BLK)
                        wf[16 * m0:16 * m0 + 16, c] = (
                            jnp.concatenate([wr + vr, wi - vi], axis=0).astype(BF16))
                        wf[16 * m:16 * m + 16, c] = (
                            jnp.concatenate([wr - vr, wi + vi], axis=0).astype(BF16))

        items = []
        for m0 in range(BLK // 16):
            st = {}
            for m in (m0, m0 + BLK // 16):
                items += [(functools.partial(item, m=m, cc=cc, st=st),
                           4 + 6 * (a0 + GA - max(a0, cc)) + (6 if cc >= a0 else 0))
                          for cc in range(a0 + GA)]
        return items

    def tile_body(t, carry):
        sl = t % 2
        a_wait(sl)

        @pl.when(t + 1 < NT)
        def _():
            a_start(t + 1, 1 - sl)
            wo_copy(t + 1).start()

        for which in (WQ, WK):
            w_copy(which, 2 * t).start()
            w_copy(which, 2 * t + 1).start()

        c = pl.ds(pl.multiple_of(t * LANES, LANES), LANES)
        taps = shift_ref[:, c].astype(F32)
        dcol = d_ref[...].astype(F32)
        rows = lax.broadcasted_iota(jnp.int32, dcol.shape, 0)
        dvec = jnp.sum(jnp.where(rows == t, dcol, 0.0), axis=0, keepdims=True)
        dvb = jnp.broadcast_to(dvec, (8, LANES))
        tapb = [jnp.broadcast_to(taps[j:j + 1, :], (8, LANES)) for j in range(4)]
        never = zero_v[...] > 0
        fwd = fwd_ref[...]
        NGR = NB // GA
        GW = GA * BLK

        def conv_item(tok, r0):
            kf[8 + r0:24 + r0, :] = ain[sl, 0, r0:r0 + 16, :].astype(F32)
            halves = []
            for h in range(2):
                r = 8 + r0 + 8 * h
                ks = kf[r:r + 8, :] * _tie(never, tok, tapb[0])
                for j in range(1, 4):
                    ks = ks + kf[r - j:r - j + 8, :] * tapb[j]
                halves.append(ks)
            kvb[r0:r0 + 16, :] = (jnp.concatenate(halves, axis=0)
                                  * ain[sl, 1, r0:r0 + 16, :].astype(F32)).astype(BF16)

        hlast = [None]

        def h_fwd(g):
            hst = jnp.concatenate([ah[sl, :, b * BLK:(b + 1) * BLK]
                                   for b in range(g * GA, (g + 1) * GA)], axis=0)
            hh = lax.dot_general(fwd, hst, (((1,), (1,)), ((), ())), preferred_element_type=F32)
            for b in range(GA):
                cur = hh[:, b * BLK:(b + 1) * BLK]
                prev = hlast[0]
                c = slice((g * GA + b) * BLK, (g * GA + b + 1) * BLK)
                if prev is None:
                    hf[:, c] = cur
                else:
                    for m in range(BLK // 8):
                        re = slice(16 * m, 16 * m + 8)
                        im = slice(16 * m + 8, 16 * m + 16)
                        if m < BLK // 16:
                            hf[re, c] = cur[re] - prev[im]
                            hf[im, c] = cur[im] + prev[re]
                        else:
                            hf[re, c] = cur[re] + prev[im]
                            hf[im, c] = cur[im] - prev[re]
                hlast[0] = cur
            return hh

        def x_fwd(g):
            rhs = jnp.concatenate([kvb[b * BLK:(b + 1) * BLK, :]
                                   for b in range(g * GA, (g + 1) * GA)], axis=1)
            xx = _dot(fwd, rhs)
            xf[:, g * GW:(g + 1) * GW] = xx
            return xx

        def inverse(g):
            ys = []
            for par in range(2):
                y = _dot(inv_ref[par * (BLK // 2):(par + 1) * (BLK // 2), :],
                         wf[par * BLK:(par + 1) * BLK, g * GW:(g + 1) * GW])
                for a in range(GA):
                    yt[pl.ds((g * GA + a) * BLK + par, BLK // 2, stride=2), :] = (
                        y[:, a * BLK:(a + 1) * BLK])
                ys.append(y)
            return jnp.concatenate(ys, axis=0)

        def out_item(tok, r0):
            d8 = _tie(never, tok, dvb)
            yb = yt[r0:r0 + 16, :] + kvb[r0:r0 + 16, :].astype(F32) * jnp.concatenate([d8, d8], axis=0)
            aout[t, r0:r0 + 16, :] = (ain[sl, 2, r0:r0 + 16, :].astype(F32) * yb).astype(BF16)

        def rows16(fn, g, w):
            return [(functools.partial(fn, r0=r0), w) for r0 in range(g * GW, (g + 1) * GW, 16)]

        vgen = v_products(t, list(range(1, NRB)), never)
        nv = 2 * (NRB - 1) * 7
        work = {('conv', g): rows16(conv_item, g, 25) for g in range(NGR)}
        work.update({('freq', g): freq_items(g * GA, never) for g in range(NGR)})
        work.update({('out', g): rows16(out_item, g, 16) for g in range(NGR)})
        for kind, g, chunks in _interleave(nv, NGR, {k: [w for _, w in v] for k, v in work.items()}):
            if kind is not None:
                m = (next(vgen) if kind == 'v' else
                     {'h': h_fwd, 'x': x_fwd, 'inv': inverse}[kind](g))
                toks = _tokens(m)
            items = [work[k][i][0] for k, i in chunks]
            if kind is None:
                for it in items:
                    it(None)
            elif items:
                _run_paced(items, toks)
        _drain(vgen)
        aout_copy(t).start()
        return carry

    for cp in small[1:]:
        cp.wait()
    wo_copy(0).start()
    lax.fori_loop(0, NT, tile_body, 0)
    pltpu.make_async_copy(wo, wo, sem_wo).wait()

    def initial_guess():
        puni = pl.reciprocal(jnp.full((1, 1), float(L), F32), approx=True).astype(BF16).astype(F32)

        def shift_down(m):
            rows = lax.broadcasted_iota(jnp.int32, m.shape, 0)
            return jnp.where(rows == 0, 0.0, pltpu.roll(m, 1, 0))

        m1 = shift_down(_dot((tsum[0:NSEG, :] * puni).astype(BF16), wo[...]))
        v1 = _dot(m1.astype(BF16), w_plain(WV, 0, H // 2)).astype(BF16).astype(F32)
        u2 = ((tsum[0:NSEG, :] + float(M) * v1) * puni).astype(BF16)
        m2 = shift_down(_dot(u2, wo[...]))
        mhat[0:NSEG * M, :] = jnp.broadcast_to(m2[:, None, :], (NSEG, M, DM)).reshape(NSEG * M, DM)
        mhat[NSEG * M:, :] = jnp.zeros((M, DM), F32)
        mhat[0:M, :] = mem0_ref[...].astype(F32)
        pltpu.make_async_copy(w32.at[WQ:WK + 1], w32.at[WQ:WK + 1], sem_wqk).wait()

    ri = lax.broadcasted_iota(jnp.int32, (PR, PR), 0)
    ci = lax.broadcasted_iota(jnp.int32, (PR, PR), 1)

    def seg_of(r):
        return jnp.where(r < MR, r // M, (r - MR) // SEG)

    def pos_of(r):
        return jnp.where(r < MR, r % M, M + (r - MR) % SEG)

    same = seg_of(ri) == seg_of(ci)
    allowed = same & ((ri < MR) | (pos_of(ri) >= pos_of(ci)))
    fill = jnp.where(same, -1e9, -jnp.inf).astype(F32)

    def sweep(state):
        it, _ = state
        pl.when(it == 0)(initial_guess)

        @pl.when(it > 0)
        def _():
            def upd(rb, cy):
                n = PPB * MR
                r = pl.ds(pl.multiple_of(rb * n, n), n)
                r2 = pl.ds(pl.multiple_of(rb * n + M, M), n)
                keep = jnp.tile(okbuf[r, :], (1, DM // LANES)) > 0.5
                mhat[r2, :] = jnp.where(keep, mhat[r2, :], mnew[r, :])
                return cy

            lax.fori_loop(0, NRB, upd, 0)

        def mem_rows(i):
            n = PPB * MR
            return mhat[pl.ds(pl.multiple_of((i // NG) * n, n), n), :]

        def mem_lhs(i):
            m = mem_rows(i)
            n = PPH * MR
            ops = [_pack(o) for o in _strassen_lhs(m[:n, :KH], m[:n, KH:], m[n:, :KH], m[n:, KH:])]
            t = jnp.concatenate([jnp.where(i < NG, 0.0, m[:M]), m[M:MR]], axis=0)
            b = m[n:n + MR]
            vops = [jnp.concatenate([_pack(o), full[MW:]], axis=0) for o, full in zip(
                _strassen_lhs(t[:, :KH], t[:, KH:], b[:, :KH], b[:, KH:]), ops)]
            return ops, vops

        def qk_proj(i, j, mops):
            rb = i // NG
            hp = (i % NG) * (G // 2) + j // 2

            def lhs(k):
                return _unpack(jnp.concatenate([mops[k], abuf[rb, k]], axis=0))

            n = PPH * MR
            cs = {}

            def emit(half, hh, cv):
                cs[half, hh] = cv
                if (half, 1 - hh) in cs:
                    v = jnp.concatenate([cs[half, 0], cs[half, 1]], axis=1).astype(BF16)
                    ps = slice(half * PPH, (half + 1) * PPH)
                    qks[j, ps, 0:MR, :] = v[:n].reshape(PPH, MR, 2 * E)
                    qks[j, ps, MR:PR, :] = v[n:].reshape(PPH, XR, 2 * E)

            return _strassen(lhs, w_rhs(WQ + j % 2, hp, [zero_s[k] for k in range(7)]), emit)

        def vm_proj(i, j, vops):
            hp = (i % NG) * (G // 2) + j

            def emit(half, hh, cv):
                if half == 0:
                    v0 = tsum[NSEG:NSEG + M, pl.ds(pl.multiple_of((2 * hp + hh) * E, E), E)]
                    cv = jnp.concatenate([jnp.where(i < NG, v0, cv[:M]), cv[M:]], axis=0)
                vms[half * PPH:(half + 1) * PPH, :, (2 * j + hh) * E:(2 * j + hh + 1) * E] = (
                    cv.astype(BF16).reshape(PPH, MR, E))

            return _strassen(lambda k: _unpack(vops[k]),
                             w_rhs(WV, hp, [zero_s[k] for k in range(7)]), emit)

        def scores(j):
            c = slice((j % 2) * E, (j % 2 + 1) * E)
            return lax.dot_general(qks[2 * (j // 2), :, :, c], qks[2 * (j // 2) + 1, :, :, c],
                                   (((2,), (2,)), ((0,), (0,))), preferred_element_type=F32)

        def attend(i, j, s):
            p0 = pl.multiple_of((i // NG) * PPB, PPB)
            h = (i % NG) * G + j
            s = jnp.where(allowed[None], s * scale, fill[None])
            e = jnp.exp(s - jnp.max(s, axis=-1, keepdims=True))
            p = (e * pl.reciprocal(jnp.sum(e, axis=-1, keepdims=True), approx=True)).astype(BF16)
            vh = jnp.concatenate(
                [vms[:, :, j * E:(j + 1) * E],
                 vbuf[pl.ds(p0, PPB), :, pl.ds(pl.multiple_of(h * E, E), E)]], axis=1)
            return lax.dot_general(p, vh, (((2,), (1,)), ((0,), (0,))), preferred_element_type=F32)

        def out_proj(i, us, last):
            rb = i // NG
            g = i % NG
            u = jnp.concatenate(us, axis=2)
            wog = wo[pl.ds(pl.multiple_of(g * (G * E), G * E), G * E), :]
            rm = pl.ds(pl.multiple_of(rb * (PPB * MR), PPB * MR), PPB * MR)
            um = u[:, :MR, :].reshape(PPB * MR, G * E).astype(BF16)
            new = jnp.where(g > 0, mnew[rm, :], 0.0) + _dot(um, wog)
            mnew[rm, :] = new
            old = mhat[pl.ds(pl.multiple_of(rb * (PPB * MR) + M, M), PPB * MR), :]
            err = jnp.max(jnp.abs(new - old), axis=1, keepdims=True)
            ref = jnp.max(jnp.abs(new), axis=1, keepdims=True)
            okbuf[rm, :] = jnp.broadcast_to(jnp.where(err <= TOL * ref, 1.0, 0.0),
                                            (PPB * MR, LANES))
            n = PPH * XR
            kh = G * E // 2
            top = u[:PPH, MR:, :].reshape(n, G * E)
            bot = u[PPH:, MR:, :].reshape(n, G * E)
            ops = _strassen_lhs(top[:, :kh], top[:, kh:], bot[:, :kh], bot[:, kh:])
            wf32 = wog.astype(F32)
            rhs = _strassen_rhs(wf32[:kh, :KH], wf32[:kh, KH:], wf32[kh:, :KH], wf32[kh:, KH:])
            quads = [(slice(0, n), slice(0, KH)), (slice(0, n), slice(KH, DM)),
                     (slice(n, 2 * n), slice(0, KH)), (slice(n, 2 * n), slice(KH, DM))]
            init = [jnp.where(g > 0, acc[r, c], 0.0) for r, c in quads]

            def emit(half, hh, v):
                r, c = quads[2 * half + hh]
                obuf[rb, r, c] = v.astype(BF16)
                if last:
                    oq_copy(2 * half + hh).start()
                else:
                    acc[r, c] = v

            _drain(_strassen(lambda k: ops[k].astype(BF16), rhs, emit, init))

        def step(i, nxt):
            s0, s1 = scores(0), scores(1)
            if nxt:
                mops, vops = mem_lhs(i + 1)
                _drain(qk_proj(i + 1, 0, mops))
            u0, u1 = attend(i, 0, s0), attend(i, 1, s1)
            s2, s3 = scores(2), scores(3)
            if nxt:
                _drain(qk_proj(i + 1, 1, mops))
            u2, u3 = attend(i, 2, s2), attend(i, 3, s3)
            if nxt:
                _drain(zip(qk_proj(i + 1, 2, mops), vm_proj(i + 1, 0, vops)))
                _drain(zip(qk_proj(i + 1, 3, mops), vm_proj(i + 1, 1, vops)))
            out_proj(i, [u0, u1, u2, u3], not nxt)

        mops0, vops0 = mem_lhs(0)
        _drain(qk_proj(0, 0, mops0), qk_proj(0, 1, mops0))
        _drain(zip(qk_proj(0, 2, mops0), vm_proj(0, 0, vops0)))
        _drain(zip(qk_proj(0, 3, mops0), vm_proj(0, 1, vops0)))

        def main_body(i, cy):
            step(i, True)

            @pl.when(i % NG == NG - 1)
            def _():
                o_copy(i // NG).start()

            return cy

        lax.fori_loop(0, NRB * NG - 1, main_body, 0)
        step(NRB * NG - 1, False)
        ok = jnp.min(okbuf[0:(NSEG - 1) * M, :])
        for rb in range(NRB - 1):
            o_copy(rb).wait()
        for qd in range(4):
            oq_copy(qd).wait()
        return it + 1, (ok > 0.5).astype(jnp.int32)

    lax.while_loop(lambda st: jnp.logical_and(st[0] < NSEG, st[1] == 0), sweep,
                   (jnp.int32(0), jnp.int32(0)))
    pltpu.make_async_copy(aout, aout, sem_aout).wait()


@functools.partial(jax.jit, static_argnames=("B_seg_len",))
def pallas_concat_heads__ssm_conv_h3__memory_aug_recurrent_mem_tr__prompt_kernel(
    A_q, A_k, A_v, A_shift_k, A_ssm_k, A_ssm_D,
    B_x, B_mem0, B_Wq, B_Wk, B_Wv, B_Wo, B_seg_len,
):
    _, S, D = A_q.shape
    DM = B_x.shape[2]
    H, E = B_Wq.shape[1], B_Wq.shape[2]
    M = B_mem0.shape[1]
    SEG = int(B_seg_len)
    NSEG = S // SEG
    NP = NSEG // 2
    PR = 2 * (M + SEG)
    PPB = 8
    NRB = NP // PPB
    NT = D // LANES
    assert E == LANES and H == 32 and M == 8 and SEG == 32 and A_shift_k.shape[1] == 4
    assert S == 2048 and D == 1024 and DM == 1024

    fwd, inv = _dft_mats()
    any_spec = pl.BlockSpec(memory_space=pl.ANY)
    scratch = [
        pltpu.VMEM((NRB, 7, PPB // 2 * SEG, DM // 2), U32),
        pltpu.VMEM((7, M + PPB // 2 * SEG, DM // 2), U32),
        pltpu.VMEM((NP, 2 * SEG, H * E), BF16),
        pltpu.VMEM((3, H // 2, DM, E), U32),
        pltpu.VMEM((H * E, DM), BF16),
        pltpu.VMEM((4, PPB, PR, 2 * E), BF16),
        pltpu.VMEM((PPB, 2 * M, 4 * E), BF16),
        pltpu.VMEM((PPB * 2 * SEG, DM), F32),
        pltpu.VMEM((NRB, PPB * 2 * SEG, DM), BF16),
        pltpu.VMEM(((NSEG + 1) * M, DM), F32),
        pltpu.VMEM((NSEG * M, DM), F32),
        pltpu.VMEM((NSEG * M, LANES), F32),
        pltpu.VMEM((NSEG + M, H * E), F32),
        pltpu.VMEM((2, 3, S, LANES), BF16),
        pltpu.VMEM((2, LANES, S), BF16),
        pltpu.VMEM((S + 32, LANES), F32),
        pltpu.VMEM((S, LANES), BF16),
        pltpu.VMEM((NFFT, S), F32),
        pltpu.VMEM((NFFT, S), F32),
        pltpu.VMEM((NFFT, S), BF16),
        pltpu.VMEM((S, LANES), F32),
        pltpu.VMEM((NT, S, LANES), BF16),
        pltpu.VMEM((M, DM), BF16),
        pltpu.VMEM((NFFT, BLK), BF16),
        pltpu.VMEM((BLK, BLK), BF16),
        pltpu.VMEM((4, D), BF16),
        pltpu.VMEM((NT, LANES), BF16),
        pltpu.VMEM((8, LANES), jnp.int32),
        pltpu.SMEM((8,), jnp.int32),
        pltpu.SemaphoreType.DMA((5,)),
        pltpu.SemaphoreType.DMA((2 * NRB,)),
        pltpu.SemaphoreType.DMA((H // 2,)),
        pltpu.SemaphoreType.DMA,
        pltpu.SemaphoreType.DMA,
        pltpu.SemaphoreType.DMA((2, 2)),
        pltpu.SemaphoreType.DMA,
        pltpu.SemaphoreType.DMA((NRB + 3,)),
    ]
    out = pl.pallas_call(
        functools.partial(_kernel, S=S, D=D, DM=DM, H=H, M=M, SEG=SEG),
        out_shape=jax.ShapeDtypeStruct((S, D + DM), BF16),
        in_specs=[any_spec] * 14,
        out_specs=any_spec,
        scratch_shapes=scratch,
        compiler_params=pltpu.CompilerParams(vmem_limit_bytes=120 * 1024 * 1024,
                                             disable_bounds_checks=True),
    )(
        A_q.reshape(S, D), A_k.reshape(S, D), A_v.reshape(S, D),
        A_shift_k.T, A_ssm_k, A_ssm_D.reshape(NT, LANES),
        B_x.reshape(NRB, S // NRB, DM), B_mem0.reshape(M, DM),
        B_Wq, B_Wk, B_Wv, B_Wo.reshape(H * E, DM),
        jnp.asarray(fwd, BF16), jnp.asarray(inv, BF16),
    )
    return out.reshape(1, S, D + DM)
```

```python
import functools

import numpy as np
import jax
import jax.numpy as jnp
from jax import lax
import jax.experimental.pallas as pl
import jax.experimental.pallas.tpu as pltpu

F32 = jnp.float32
BF16 = jnp.bfloat16
U32 = jnp.uint32

LANES = 128
BLK = 128
NFFT = 2 * BLK
TOL = 2.0 ** -10


def _dft_mats():
    even = np.arange(0, BLK, 2)
    theta = 2.0 * np.pi * (np.concatenate([even, BLK - 1 - even]) + 0.5) / NFFT
    n = np.arange(BLK)
    c = np.cos(theta[:, None] * n[None, :])
    s = np.sin(theta[:, None] * n[None, :])
    fwd = np.zeros((NFFT, BLK))
    for m in range(BLK // 8):
        fwd[16 * m:16 * m + 8] = c[8 * m:8 * m + 8]
        fwd[16 * m + 8:16 * m + 16] = -s[8 * m:8 * m + 8]
    inv = fwd[:BLK].T * (2.0 / NFFT)
    inv = np.concatenate([inv[0::2], inv[1::2]], axis=0)
    return fwd.astype(np.float32), inv.astype(np.float32)


def _dot(a, b):
    return jnp.dot(a, b, preferred_element_type=F32)


def _pack(x):
    return pltpu.bitcast(x.astype(BF16), U32)


def _unpack(w):
    return pltpu.bitcast(w, BF16)


def _lo(w):
    return pltpu.bitcast(w << 16, F32)


def _hi(w):
    return pltpu.bitcast(w & jnp.uint32(0xFFFF0000), F32)


def _strassen_lhs(a11, a12, a21, a22):
    return [a11 + a22, a21 + a22, a11, a22, a11 + a12, a21 - a11, a12 - a22]


def _strassen_rhs(b11, b12, b21, b22):
    ops = [b11 + b22, b11, b12 - b22, b21 - b11, b22, b11 + b12, b21 + b22]
    return [o.astype(BF16) for o in ops]


def _strassen(lhs, rhs, emit, init=None):
    def add(c, m):
        return m if c is None else c + m

    c11, c12, c21, c22 = init if init is not None else (None,) * 4
    m5 = _dot(lhs(4), rhs[4])
    yield m5
    m3 = _dot(lhs(2), rhs[2])
    emit(0, 1, add(c12, m5) + m3)
    yield m3
    m2 = _dot(lhs(1), rhs[1])
    c22 = add(c22, m3) - m2
    yield m2
    m4 = _dot(lhs(3), rhs[3])
    emit(1, 0, add(c21, m2) + m4)
    c11 = add(c11, m4) - m5
    yield m4
    m1 = _dot(lhs(0), rhs[0])
    c11 = c11 + m1
    c22 = c22 + m1
    yield m1
    m7 = _dot(lhs(6), rhs[6])
    emit(0, 0, c11 + m7)
    yield m7
    m6 = _dot(lhs(5), rhs[5])
    emit(1, 1, c22 + m6)
    yield m6


def _drain(*gens):
    for g in gens:
        for _ in g:
            pass


def _tokens(m):
    return [m[r:r + 8, c:c + LANES]
            for r in range(0, m.shape[0], 8) for c in range(0, m.shape[1], LANES)]


def _tie(never, tok, x):
    if tok is None:
        return x
    reps = (x.shape[0] // 8, x.shape[1] // LANES)
    if tok.dtype != x.dtype:
        tok = pltpu.bitcast(tok, x.dtype)
    if reps != (1, 1):
        never, tok = jnp.tile(never, reps), jnp.tile(tok, reps)
    return jnp.where(never, tok, x)


def _run_paced(items, toks):
    for i, it in enumerate(items):
        it(toks[i * len(toks) // len(items)])


def _interleave(nv, ngr, weights):
    dur = {'v': 256, 'h': 256, 'x': 256, 'inv': 128}
    margin = 768

    def plan(rate):
        t, v, out = 0, 0, []
        nxt = {'h': 0, 'x': 0, 'inv': 0}
        pos = {k: 0 for k in weights}
        done = {}
        credit = 0.0
        while True:
            kind = None
            if nxt['inv'] < ngr and done.get(('freq', nxt['inv']), 1e9) + margin <= t:
                kind = 'inv'
            elif nxt['x'] < ngr and done.get(('conv', nxt['x']), 1e9) + margin <= t:
                kind = 'x'
            elif nxt['h'] < ngr and nxt['h'] <= nxt['x'] and (not out or out[-1][0] == 'v'):
                kind = 'h'
            elif v < nv:
                kind = 'v'
            if kind is None:
                break
            g = v if kind == 'v' else nxt[kind]
            busy = 0.75 if kind == 'v' and v % (nv // 2) < 7 else 0.0
            credit += (rate - busy) * dur[kind]
            chunk = []
            while credit > 0:
                ready = [('out', i) for i in range(nxt['inv'])]
                ready += [('conv', i) for i in range(ngr)]
                ready += [('freq', i) for i in range(min(nxt['x'], nxt['h']))]
                ready = [k for k in ready if pos[k] < len(weights[k])]
                if not ready:
                    credit = 0.0
                    break
                k = ready[0]
                chunk.append((k, pos[k]))
                credit -= weights[k][pos[k]]
                pos[k] += 1
                if pos[k] == len(weights[k]):
                    done[k] = t + dur[kind]
            out.append((kind, g, chunk))
            t += dur[kind]
            if kind == 'v':
                v += 1
            else:
                nxt[kind] += 1
        ok = all(pos[k] == len(weights[k]) for k in weights)
        return ok, out

    rate = 1.0
    while True:
        ok, out = plan(rate)
        if ok:
            return out
        rate += 0.02


def _kernel(q_hbm, k_hbm, v_hbm, shift_hbm, h_hbm, d_hbm, x_hbm, mem0_hbm,
            wq_hbm, wk_hbm, wv_hbm, wo_hbm, fwd_hbm, inv_hbm,
            out_hbm,
            abuf, a0buf, vbuf, w32, wo, qks, vms, acc, obuf, mhat, mnew, okbuf, tsum,
            ain, ah, kf, kvb, xf, hf, wf, yt, aout,
            mem0_ref, fwd_ref, inv_ref, shift_ref, d_ref, zero_v, zero_s,
            sem_s, sem_x, sem_wv, sem_wqk, sem_wo, sem_a, sem_aout, sem_o,
            *, S, D, DM, H, M, SEG):
    E = LANES
    NSEG = S // SEG
    NP = NSEG // 2
    MR = 2 * M
    XR = 2 * SEG
    PR = MR + XR
    MW, XW, PW = MR // 2, XR // 2, PR // 2
    L = M + SEG
    NB = S // BLK
    NT = D // LANES
    PPB = 8
    PPH = PPB // 2
    NRB = NP // PPB
    G = 4
    NG = H // G
    KH = DM // 2
    scale = float(E) ** -0.5
    WV, WQ, WK = 0, 1, 2

    small = [pltpu.make_async_copy(src, dst, sem_s.at[i]) for i, (src, dst) in enumerate(
        ((mem0_hbm, mem0_ref), (shift_hbm, shift_ref), (d_hbm, d_ref),
         (fwd_hbm, fwd_ref), (inv_hbm, inv_ref)))]
    HBR = PPH * XR // 2

    def x_copies(hb):
        out = []
        for half in range(2):
            r = pl.ds(pl.multiple_of((2 * half + hb % 2) * HBR, HBR), HBR)
            out.append(pltpu.make_async_copy(x_hbm.at[hb // 2, r], obuf.at[hb // 2, r],
                                             sem_x.at[hb]))
        return out

    def w_copy(which, hp):
        src = (wv_hbm, wq_hbm, wk_hbm)[which].bitcast(U32)
        sem = sem_wv.at[hp] if which == WV else sem_wqk
        return pltpu.make_async_copy(src.at[:, hp, :], w32.at[which, hp], sem)

    def wo_copy(t):
        n = H * E // NT
        r = pl.ds(pl.multiple_of(t * n, n), n)
        return pltpu.make_async_copy(wo_hbm.at[r, :], wo.at[r, :], sem_wo)

    def a_start(t, sl, which=(0, 1, 2, 3)):
        c = pl.ds(pl.multiple_of(t * LANES, LANES), LANES)
        for i in which:
            if i == 3:
                pltpu.make_async_copy(h_hbm.at[c, :], ah.at[sl], sem_a.at[sl, 1]).start()
            else:
                src = (k_hbm, v_hbm, q_hbm)[i]
                pltpu.make_async_copy(src.at[:, c], ain.at[sl, i], sem_a.at[sl, 0]).start()

    def a_wait(sl):
        pltpu.make_async_copy(ain.at[sl], ain.at[sl], sem_a.at[sl, 0]).wait()
        pltpu.make_async_copy(ah.at[sl], ah.at[sl], sem_a.at[sl, 1]).wait()

    def aout_copy(t):
        c = pl.ds(pl.multiple_of(t * LANES, LANES), LANES)
        return pltpu.make_async_copy(aout.at[t], out_hbm.at[:, c], sem_aout)

    def o_copy(rb):
        r = pl.ds(pl.multiple_of(rb * (PPB * XR), PPB * XR), PPB * XR)
        return pltpu.make_async_copy(obuf.at[rb], out_hbm.at[r, pl.ds(D, DM)], sem_o.at[rb])

    def oq_copy(qd):
        n = PPH * XR
        r0, c0 = (qd // 2) * n, (qd % 2) * KH
        return pltpu.make_async_copy(
            obuf.at[NRB - 1, pl.ds(r0, n), pl.ds(c0, KH)],
            out_hbm.at[pl.ds((NRB - 1) * 2 * n + r0, n), pl.ds(D + c0, KH)],
            sem_o.at[NRB - 1 + qd])

    def w_rhs(which, hp, zs=None):
        if zs is None:
            w = w32[which, hp]
            return _strassen_rhs(_lo(w[:KH]), _hi(w[:KH]), _lo(w[KH:]), _hi(w[KH:]))
        out = []
        for k in range(7):
            w = w32.at[which, hp + zs[k]]
            out.append(_strassen_rhs(_lo(w[:KH]), _hi(w[:KH]), _lo(w[KH:]), _hi(w[KH:]))[k])
        return out

    def w_plain(which, hp0, n):
        parts = []
        for j in range(n):
            w = w32[which, hp0 + j]
            parts += [_lo(w), _hi(w)]
        return jnp.concatenate(parts, axis=1).astype(BF16)

    small[0].start()
    for hb in range(2):
        for cp in x_copies(hb):
            cp.start()
    w_copy(WV, 0).start()
    w_copy(WV, 1).start()
    for cp in small[1:]:
        cp.start()

    kf[0:8, :] = jnp.zeros((8, LANES), F32)
    zero_v[...] = jnp.zeros((8, LANES), jnp.int32)
    for k in range(8):
        zero_s[k] = 0
    tsum[:, 0:8, 0:LANES] = jnp.zeros((NG, 8, LANES), F32)
    vbuf[:, 0, 0:16, 0:LANES] = jnp.zeros((NG, 16, LANES), BF16)
    for hb in range(2 * NRB):
        r0 = (hb % 2) * (HBR // 2)
        abuf[hb // 2, 0, r0:r0 + 8, 0:LANES] = jnp.zeros((8, LANES), U32)
    small[0].wait()
    mem0 = mem0_ref[...].astype(F32)
    m0 = jnp.concatenate([mem0, jnp.zeros_like(mem0)], axis=0)
    z0 = jnp.zeros((MR, KH), F32)
    for k, op in enumerate(_strassen_lhs(m0[:, :KH], m0[:, KH:], z0, z0)):
        a0buf[k, 0:MW, :] = _pack(op)

    def x_item(tok, never, src, dst, r, c):
        quad = [_tie(never, tok, src[h * 2 * HBR + r:h * 2 * HBR + r + 16,
                                     kk * KH + c:kk * KH + c + 2 * LANES].astype(F32))
                for h in range(2) for kk in range(2)]
        for k, op in enumerate(_strassen_lhs(*quad)):
            dst[k, r // 2:r // 2 + 8, c:c + 2 * LANES] = _pack(op)

    def x_items(never, src, dst):
        return [functools.partial(x_item, never=never, src=src, dst=dst, r=r, c=c)
                for r in range(0, HBR, 16) for c in range(0, KH, 2 * LANES)]

    def x_first(hb, cy):
        for cp in x_copies(hb):
            cp.wait()
        src = obuf.at[0, pl.ds(pl.multiple_of(hb * HBR, HBR), 3 * HBR)]
        dst = a0buf.at[:, pl.ds(pl.multiple_of(MW + hb * (HBR // 2), 8), HBR // 2)]
        for it in x_items(None, src, dst):
            it(None)
        return cy

    lax.fori_loop(0, 2, x_first, 0)

    def v_part(j, rb, rhs, vwin, twin, pre=None):
        def lhs(k):
            x = a0buf[k] if rb == 0 else abuf[rb, k]
            if pre is not None and k == 4:
                x0 = jnp.concatenate([pre(x[:8, :LANES]), x[:8, LANES:]], axis=1)
                x = jnp.concatenate([x0, x[8:]], axis=0)
            return _unpack(x)

        def emit(half, hh, cv):
            c = slice((2 * j + hh) * E, (2 * j + hh + 1) * E)
            vv = cv.astype(BF16)
            vx = vv[MR:] if rb == 0 else vv
            p0 = rb * PPB + half * PPH
            vwin[p0:p0 + PPH, :, c] = vx.reshape(PPH, XR, E)
            ts = jnp.sum(vx.astype(F32).reshape(2 * PPH, SEG, E), axis=1)
            if rb == 0 and half == 0:
                v0 = vv[0:M].astype(F32)
                twin[NSEG:NSEG + M, c] = v0
                t0 = jnp.sum(v0, axis=0, keepdims=True)
                rows = lax.broadcasted_iota(jnp.int32, ts.shape, 0)
                ts = ts + jnp.where(rows == 0, t0, 0.0)
            twin[2 * p0:2 * (p0 + PPH), c] = ts

        return _strassen(lhs, rhs, emit)

    def v_products(t, rbs, never, extra=()):
        zs = [zero_s[k] for k in range(7)]
        vwin = vbuf.at[t]
        twin = tsum.at[t]

        def pre(x):
            for v in (twin[0:8, 0:LANES], pltpu.bitcast(vwin[0, 0:16, 0:LANES], U32)) + tuple(extra):
                x = _tie(never, v, x)
            return x

        for j in range(2):
            rhs = w_rhs(WV, 2 * t + j, zs)
            for rb in rbs:
                yield from v_part(j, rb, rhs, vwin, twin, pre if (j, rb) == (0, rbs[0]) else None)

    def head_body(j, cy):
        w_copy(WV, 2 * j).wait()
        w_copy(WV, 2 * j + 1).wait()

        @pl.when(j >= 2)
        def _():
            for cp in x_copies(j):
                cp.wait()

        @pl.when(j + 1 < NT)
        def _():
            w_copy(WV, 2 * j + 2).start()
            w_copy(WV, 2 * j + 3).start()

        @pl.when(j + 2 < 2 * NRB)
        def _():
            for cp in x_copies(j + 2):
                cp.start()

        @pl.when(j == NT - 3)
        def _():
            a_start(0, 0, (3,))

        @pl.when(j == NT - 2)
        def _():
            a_start(0, 0, (0, 1, 2))

        never = zero_v[...] > 0
        src = obuf.at[j // 2, pl.ds(pl.multiple_of((j % 2) * HBR, HBR), 3 * HBR)]
        dst = abuf.at[j // 2, :, pl.ds(pl.multiple_of((j % 2) * (HBR // 2), 8), HBR // 2)]
        toks = []
        for m in v_products(j, [0], never, [dst[0, 0:8, 0:LANES]]):
            toks += _tokens(m)
        _run_paced(x_items(never, src, dst), toks[:-40])
        return cy

    assert NT == 2 * NRB
    lax.fori_loop(0, NT, head_body, 0)

    GA = 4

    def freq_items(a0, never):
        def item(tok, m, cc, st):
            r_re = slice(16 * m, 16 * m + 8)
            r_im = slice(16 * m + 8, 16 * m + 16)
            xr = _tie(never, tok, xf[r_re, cc * BLK:(cc + 1) * BLK])
            xi = _tie(never, tok, xf[r_im, cc * BLK:(cc + 1) * BLK])
            xs = xr + xi
            for a in range(max(a0, cc), a0 + GA):
                j = a - cc
                if ('g', m, j) not in st:
                    gr = hf[r_re, j * BLK:(j + 1) * BLK]
                    gi = hf[r_im, j * BLK:(j + 1) * BLK]
                    st['g', m, j] = (gr, gi, gr + gi)
                gr, gi, gs = st['g', m, j]
                ps = (xr * gr, xi * gi, xs * gs)
                st[m, a] = ps if (m, a) not in st else tuple(u + v for u, v in zip(st[m, a], ps))
                if cc == a:
                    p1, p2, p3 = st[m, a]
                    st[m, a] = (p1 - p2, p3 - p1 - p2)
                    if m >= BLK // 16:
                        m0 = m - BLK // 16
                        (wr, wi), (vr, vi) = st[m0, a], st[m, a]
                        c = slice(a * BLK, (a + 1) * BLK)
                        wf[16 * m0:16 * m0 + 16, c] = (
                            jnp.concatenate([wr + vr, wi - vi], axis=0).astype(BF16))
                        wf[16 * m:16 * m + 16, c] = (
                            jnp.concatenate([wr - vr, wi + vi], axis=0).astype(BF16))

        items = []
        for m0 in range(BLK // 16):
            st = {}
            for m in (m0, m0 + BLK // 16):
                items += [(functools.partial(item, m=m, cc=cc, st=st),
                           4 + 6 * (a0 + GA - max(a0, cc)) + (6 if cc >= a0 else 0))
                          for cc in range(a0 + GA)]
        return items

    def tile_body(t, carry):
        sl = t % 2
        a_wait(sl)

        @pl.when(t + 1 < NT)
        def _():
            a_start(t + 1, 1 - sl)
            wo_copy(t + 1).start()

        for which in (WQ, WK):
            w_copy(which, 2 * t).start()
            w_copy(which, 2 * t + 1).start()

        c = pl.ds(pl.multiple_of(t * LANES, LANES), LANES)
        taps = shift_ref[:, c].astype(F32)
        dcol = d_ref[...].astype(F32)
        rows = lax.broadcasted_iota(jnp.int32, dcol.shape, 0)
        dvec = jnp.sum(jnp.where(rows == t, dcol, 0.0), axis=0, keepdims=True)
        dvb = jnp.broadcast_to(dvec, (8, LANES))
        tapb = [jnp.broadcast_to(taps[j:j + 1, :], (8, LANES)) for j in range(4)]
        never = zero_v[...] > 0
        fwd = fwd_ref[...]
        NGR = NB // GA
        GW = GA * BLK

        def conv_item(tok, r0):
            kf[8 + r0:24 + r0, :] = ain[sl, 0, r0:r0 + 16, :].astype(F32)
            halves = []
            for h in range(2):
                r = 8 + r0 + 8 * h
                ks = kf[r:r + 8, :] * _tie(never, tok, tapb[0])
                for j in range(1, 4):
                    ks = ks + kf[r - j:r - j + 8, :] * tapb[j]
                halves.append(ks)
            kvb[r0:r0 + 16, :] = (jnp.concatenate(halves, axis=0)
                                  * ain[sl, 1, r0:r0 + 16, :].astype(F32)).astype(BF16)

        hlast = [None]

        def h_fwd(g):
            hst = jnp.concatenate([ah[sl, :, b * BLK:(b + 1) * BLK]
                                   for b in range(g * GA, (g + 1) * GA)], axis=0)
            hh = lax.dot_general(fwd, hst, (((1,), (1,)), ((), ())), preferred_element_type=F32)
            for b in range(GA):
                cur = hh[:, b * BLK:(b + 1) * BLK]
                prev = hlast[0]
                c = slice((g * GA + b) * BLK, (g * GA + b + 1) * BLK)
                if prev is None:
                    hf[:, c] = cur
                else:
                    for m in range(BLK // 8):
                        re = slice(16 * m, 16 * m + 8)
                        im = slice(16 * m + 8, 16 * m + 16)
                        if m < BLK // 16:
                            hf[re, c] = cur[re] - prev[im]
                            hf[im, c] = cur[im] + prev[re]
                        else:
                            hf[re, c] = cur[re] + prev[im]
                            hf[im, c] = cur[im] - prev[re]
                hlast[0] = cur
            return hh

        def x_fwd(g):
            rhs = jnp.concatenate([kvb[b * BLK:(b + 1) * BLK, :]
                                   for b in range(g * GA, (g + 1) * GA)], axis=1)
            xx = _dot(fwd, rhs)
            xf[:, g * GW:(g + 1) * GW] = xx
            return xx

        def inverse(g):
            ys = []
            for par in range(2):
                y = _dot(inv_ref[par * (BLK // 2):(par + 1) * (BLK // 2), :],
                         wf[par * BLK:(par + 1) * BLK, g * GW:(g + 1) * GW])
                for a in range(GA):
                    yt[pl.ds((g * GA + a) * BLK + par, BLK // 2, stride=2), :] = (
                        y[:, a * BLK:(a + 1) * BLK])
                ys.append(y)
            return jnp.concatenate(ys, axis=0)

        def out_item(tok, r0):
            d8 = _tie(never, tok, dvb)
            yb = yt[r0:r0 + 16, :] + kvb[r0:r0 + 16, :].astype(F32) * jnp.concatenate([d8, d8], axis=0)
            aout[t, r0:r0 + 16, :] = (ain[sl, 2, r0:r0 + 16, :].astype(F32) * yb).astype(BF16)

        def rows16(fn, g, w):
            return [(functools.partial(fn, r0=r0), w) for r0 in range(g * GW, (g + 1) * GW, 16)]

        vgen = v_products(t, list(range(1, NRB)), never)
        nv = 2 * (NRB - 1) * 7
        work = {('conv', g): rows16(conv_item, g, 25) for g in range(NGR)}
        work.update({('freq', g): freq_items(g * GA, never) for g in range(NGR)})
        work.update({('out', g): rows16(out_item, g, 16) for g in range(NGR)})
        for kind, g, chunks in _interleave(nv, NGR, {k: [w for _, w in v] for k, v in work.items()}):
            if kind is not None:
                m = (next(vgen) if kind == 'v' else
                     {'h': h_fwd, 'x': x_fwd, 'inv': inverse}[kind](g))
                toks = _tokens(m)
            items = [work[k][i][0] for k, i in chunks]
            if kind is None:
                for it in items:
                    it(None)
            elif items:
                _run_paced(items, toks)
        _drain(vgen)
        aout_copy(t).start()
        return carry

    for cp in small[1:]:
        cp.wait()
    wo_copy(0).start()
    lax.fori_loop(0, NT, tile_body, 0)
    pltpu.make_async_copy(wo, wo, sem_wo).wait()

    def initial_guess():
        puni = pl.reciprocal(jnp.full((1, 1), float(L), F32), approx=True).astype(BF16).astype(F32)

        def shift_down(m):
            rows = lax.broadcasted_iota(jnp.int32, m.shape, 0)
            return jnp.where(rows == 0, 0.0, pltpu.roll(m, 1, 0))

        tall = jnp.concatenate([tsum[g, 0:NSEG, :] for g in range(NG)], axis=1)
        m1 = shift_down(_dot((tall * puni).astype(BF16), wo[...]))
        v1 = _dot(m1.astype(BF16), w_plain(WV, 0, H // 2)).astype(BF16).astype(F32)
        u2 = ((tall + float(M) * v1) * puni).astype(BF16)
        m2 = shift_down(_dot(u2, wo[...]))
        mhat[0:NSEG * M, :] = jnp.broadcast_to(m2[:, None, :], (NSEG, M, DM)).reshape(NSEG * M, DM)
        mhat[NSEG * M:, :] = jnp.zeros((M, DM), F32)
        mhat[0:M, :] = mem0_ref[...].astype(F32)
        pltpu.make_async_copy(w32.at[WQ:WK + 1], w32.at[WQ:WK + 1], sem_wqk).wait()

    ri = lax.broadcasted_iota(jnp.int32, (PR, PR), 0)
    ci = lax.broadcasted_iota(jnp.int32, (PR, PR), 1)

    def seg_of(r):
        return jnp.where(r < MR, r // M, (r - MR) // SEG)

    def pos_of(r):
        return jnp.where(r < MR, r % M, M + (r - MR) % SEG)

    same = seg_of(ri) == seg_of(ci)
    allowed = same & ((ri < MR) | (pos_of(ri) >= pos_of(ci)))
    fill = jnp.where(same, -1e9, -jnp.inf).astype(F32)

    def sweep(state):
        it, _ = state
        pl.when(it == 0)(initial_guess)

        @pl.when(it > 0)
        def _():
            def upd(rb, cy):
                n = PPB * MR
                r = pl.ds(pl.multiple_of(rb * n, n), n)
                r2 = pl.ds(pl.multiple_of(rb * n + M, M), n)
                keep = jnp.tile(okbuf[r, :], (1, DM // LANES)) > 0.5
                mhat[r2, :] = jnp.where(keep, mhat[r2, :], mnew[r, :])
                return cy

            lax.fori_loop(0, NRB, upd, 0)

        def mem_rows(i):
            n = PPB * MR
            return mhat[pl.ds(pl.multiple_of((i // NG) * n, n), n), :]

        def mem_lhs(i):
            m = mem_rows(i)
            n = PPH * MR
            ops = [_pack(o) for o in _strassen_lhs(m[:n, :KH], m[:n, KH:], m[n:, :KH], m[n:, KH:])]
            t = jnp.concatenate([jnp.where(i < NG, 0.0, m[:M]), m[M:MR]], axis=0)
            b = m[n:n + MR]
            vops = [jnp.concatenate([_pack(o), full[MW:]], axis=0) for o, full in zip(
                _strassen_lhs(t[:, :KH], t[:, KH:], b[:, :KH], b[:, KH:]), ops)]
            return ops, vops

        def qk_proj(i, j, mops):
            rb = i // NG
            hp = (i % NG) * (G // 2) + j // 2

            def lhs(k):
                return _unpack(jnp.concatenate([mops[k], abuf[rb, k]], axis=0))

            n = PPH * MR
            cs = {}

            def emit(half, hh, cv):
                cs[half, hh] = cv
                if (half, 1 - hh) in cs:
                    v = jnp.concatenate([cs[half, 0], cs[half, 1]], axis=1).astype(BF16)
                    ps = slice(half * PPH, (half + 1) * PPH)
                    qks[j, ps, 0:MR, :] = v[:n].reshape(PPH, MR, 2 * E)
                    qks[j, ps, MR:PR, :] = v[n:].reshape(PPH, XR, 2 * E)

            return _strassen(lhs, w_rhs(WQ + j % 2, hp, [zero_s[k] for k in range(7)]), emit)

        def vm_proj(i, j, vops):
            hp = (i % NG) * (G // 2) + j

            def emit(half, hh, cv):
                if half == 0:
                    v0 = tsum[i % NG, NSEG:NSEG + M, (2 * j + hh) * E:(2 * j + hh + 1) * E]
                    cv = jnp.concatenate([jnp.where(i < NG, v0, cv[:M]), cv[M:]], axis=0)
                vms[half * PPH:(half + 1) * PPH, :, (2 * j + hh) * E:(2 * j + hh + 1) * E] = (
                    cv.astype(BF16).reshape(PPH, MR, E))

            return _strassen(lambda k: _unpack(vops[k]),
                             w_rhs(WV, hp, [zero_s[k] for k in range(7)]), emit)

        def scores(j):
            c = slice((j % 2) * E, (j % 2 + 1) * E)
            return lax.dot_general(qks[2 * (j // 2), :, :, c], qks[2 * (j // 2) + 1, :, :, c],
                                   (((2,), (2,)), ((0,), (0,))), preferred_element_type=F32)

        def attend(i, j, s):
            p0 = pl.multiple_of((i // NG) * PPB, PPB)
            s = jnp.where(allowed[None], s * scale, fill[None])
            e = jnp.exp(s - jnp.max(s, axis=-1, keepdims=True))
            p = (e * pl.reciprocal(jnp.sum(e, axis=-1, keepdims=True), approx=True)).astype(BF16)
            vh = jnp.concatenate(
                [vms[:, :, j * E:(j + 1) * E],
                 vbuf[i % NG, pl.ds(p0, PPB), :, j * E:(j + 1) * E]], axis=1)
            return lax.dot_general(p, vh, (((2,), (1,)), ((0,), (0,))), preferred_element_type=F32)

        def out_proj(i, us, last):
            rb = i // NG
            g = i % NG
            u = jnp.concatenate(us, axis=2)
            wog = wo[pl.ds(pl.multiple_of(g * (G * E), G * E), G * E), :]
            rm = pl.ds(pl.multiple_of(rb * (PPB * MR), PPB * MR), PPB * MR)
            um = u[:, :MR, :].reshape(PPB * MR, G * E).astype(BF16)
            new = jnp.where(g > 0, mnew[rm, :], 0.0) + _dot(um, wog)
            mnew[rm, :] = new
            old = mhat[pl.ds(pl.multiple_of(rb * (PPB * MR) + M, M), PPB * MR), :]
            err = jnp.max(jnp.abs(new - old), axis=1, keepdims=True)
            ref = jnp.max(jnp.abs(new), axis=1, keepdims=True)
            okbuf[rm, :] = jnp.broadcast_to(jnp.where(err <= TOL * ref, 1.0, 0.0),
                                            (PPB * MR, LANES))
            n = PPH * XR
            kh = G * E // 2
            top = u[:PPH, MR:, :].reshape(n, G * E)
            bot = u[PPH:, MR:, :].reshape(n, G * E)
            ops = _strassen_lhs(top[:, :kh], top[:, kh:], bot[:, :kh], bot[:, kh:])
            wf32 = wog.astype(F32)
            rhs = _strassen_rhs(wf32[:kh, :KH], wf32[:kh, KH:], wf32[kh:, :KH], wf32[kh:, KH:])
            quads = [(slice(0, n), slice(0, KH)), (slice(0, n), slice(KH, DM)),
                     (slice(n, 2 * n), slice(0, KH)), (slice(n, 2 * n), slice(KH, DM))]
            init = [jnp.where(g > 0, acc[r, c], 0.0) for r, c in quads]

            def emit(half, hh, v):
                r, c = quads[2 * half + hh]
                obuf[rb, r, c] = v.astype(BF16)
                if last:
                    oq_copy(2 * half + hh).start()
                else:
                    acc[r, c] = v

            _drain(_strassen(lambda k: ops[k].astype(BF16), rhs, emit, init))

        def step(i, nxt):
            s0, s1 = scores(0), scores(1)
            if nxt:
                mops, vops = mem_lhs(i + 1)
                _drain(qk_proj(i + 1, 0, mops))
            u0, u1 = attend(i, 0, s0), attend(i, 1, s1)
            s2, s3 = scores(2), scores(3)
            if nxt:
                _drain(qk_proj(i + 1, 1, mops))
            u2, u3 = attend(i, 2, s2), attend(i, 3, s3)
            if nxt:
                _drain(zip(qk_proj(i + 1, 2, mops), vm_proj(i + 1, 0, vops)))
                _drain(zip(qk_proj(i + 1, 3, mops), vm_proj(i + 1, 1, vops)))
            out_proj(i, [u0, u1, u2, u3], not nxt)

        mops0, vops0 = mem_lhs(0)
        _drain(qk_proj(0, 0, mops0), qk_proj(0, 1, mops0))
        _drain(zip(qk_proj(0, 2, mops0), vm_proj(0, 0, vops0)))
        _drain(zip(qk_proj(0, 3, mops0), vm_proj(0, 1, vops0)))

        def main_body(i, cy):
            step(i, True)

            @pl.when(i % NG == NG - 1)
            def _():
                o_copy(i // NG).start()

            return cy

        lax.fori_loop(0, NRB * NG - 1, main_body, 0)
        step(NRB * NG - 1, False)
        ok = jnp.min(okbuf[0:(NSEG - 1) * M, :])
        for rb in range(NRB - 1):
            o_copy(rb).wait()
        for qd in range(4):
            oq_copy(qd).wait()
        return it + 1, (ok > 0.5).astype(jnp.int32)

    lax.while_loop(lambda st: jnp.logical_and(st[0] < NSEG, st[1] == 0), sweep,
                   (jnp.int32(0), jnp.int32(0)))
    pltpu.make_async_copy(aout, aout, sem_aout).wait()


@functools.partial(jax.jit, static_argnames=("B_seg_len",))
def pallas_concat_heads__ssm_conv_h3__memory_aug_recurrent_mem_tr__prompt_kernel(
    A_q, A_k, A_v, A_shift_k, A_ssm_k, A_ssm_D,
    B_x, B_mem0, B_Wq, B_Wk, B_Wv, B_Wo, B_seg_len,
):
    _, S, D = A_q.shape
    DM = B_x.shape[2]
    H, E = B_Wq.shape[1], B_Wq.shape[2]
    M = B_mem0.shape[1]
    SEG = int(B_seg_len)
    NSEG = S // SEG
    NP = NSEG // 2
    PR = 2 * (M + SEG)
    PPB = 8
    NRB = NP // PPB
    NT = D // LANES
    assert E == LANES and H == 32 and M == 8 and SEG == 32 and A_shift_k.shape[1] == 4
    assert S == 2048 and D == 1024 and DM == 1024

    fwd, inv = _dft_mats()
    any_spec = pl.BlockSpec(memory_space=pl.ANY)
    scratch = [
        pltpu.VMEM((NRB, 7, PPB // 2 * SEG, DM // 2), U32),
        pltpu.VMEM((7, M + PPB // 2 * SEG, DM // 2), U32),
        pltpu.VMEM((H // 4, NP, 2 * SEG, 4 * E), BF16),
        pltpu.VMEM((3, H // 2, DM, E), U32),
        pltpu.VMEM((H * E, DM), BF16),
        pltpu.VMEM((4, PPB, PR, 2 * E), BF16),
        pltpu.VMEM((PPB, 2 * M, 4 * E), BF16),
        pltpu.VMEM((PPB * 2 * SEG, DM), F32),
        pltpu.VMEM((NRB, PPB * 2 * SEG, DM), BF16),
        pltpu.VMEM(((NSEG + 1) * M, DM), F32),
        pltpu.VMEM((NSEG * M, DM), F32),
        pltpu.VMEM((NSEG * M, LANES), F32),
        pltpu.VMEM((H // 4, NSEG + M, 4 * E), F32),
        pltpu.VMEM((2, 3, S, LANES), BF16),
        pltpu.VMEM((2, LANES, S), BF16),
        pltpu.VMEM((S + 32, LANES), F32),
        pltpu.VMEM((S, LANES), BF16),
        pltpu.VMEM((NFFT, S), F32),
        pltpu.VMEM((NFFT, S), F32),
        pltpu.VMEM((NFFT, S), BF16),
        pltpu.VMEM((S, LANES), F32),
        pltpu.VMEM((NT, S, LANES), BF16),
        pltpu.VMEM((M, DM), BF16),
        pltpu.VMEM((NFFT, BLK), BF16),
        pltpu.VMEM((BLK, BLK), BF16),
        pltpu.VMEM((4, D), BF16),
        pltpu.VMEM((NT, LANES), BF16),
        pltpu.VMEM((8, LANES), jnp.int32),
        pltpu.SMEM((8,), jnp.int32),
        pltpu.SemaphoreType.DMA((5,)),
        pltpu.SemaphoreType.DMA((2 * NRB,)),
        pltpu.SemaphoreType.DMA((H // 2,)),
        pltpu.SemaphoreType.DMA,
        pltpu.SemaphoreType.DMA,
        pltpu.SemaphoreType.DMA((2, 2)),
        pltpu.SemaphoreType.DMA,
        pltpu.SemaphoreType.DMA((NRB + 3,)),
    ]
    out = pl.pallas_call(
        functools.partial(_kernel, S=S, D=D, DM=DM, H=H, M=M, SEG=SEG),
        out_shape=jax.ShapeDtypeStruct((S, D + DM), BF16),
        in_specs=[any_spec] * 14,
        out_specs=any_spec,
        scratch_shapes=scratch,
        compiler_params=pltpu.CompilerParams(vmem_limit_bytes=120 * 1024 * 1024,
                                             disable_bounds_checks=True),
    )(
        A_q.reshape(S, D), A_k.reshape(S, D), A_v.reshape(S, D),
        A_shift_k.T, A_ssm_k, A_ssm_D.reshape(NT, LANES),
        B_x.reshape(NRB, S // NRB, DM), B_mem0.reshape(M, DM),
        B_Wq, B_Wk, B_Wv, B_Wo.reshape(H * E, DM),
        jnp.asarray(fwd, BF16), jnp.asarray(inv, BF16),
    )
    return out.reshape(1, S, D + DM)
```

```python
import functools

import numpy as np
import jax
import jax.numpy as jnp
from jax import lax
import jax.experimental.pallas as pl
import jax.experimental.pallas.tpu as pltpu

F32 = jnp.float32
BF16 = jnp.bfloat16
U32 = jnp.uint32

LANES = 128
BLK = 128
NFFT = 2 * BLK
TOL = 2.0 ** -10


def _dft_mats():
    even = np.arange(0, BLK, 2)
    theta = 2.0 * np.pi * (np.concatenate([even, BLK - 1 - even]) + 0.5) / NFFT
    n = np.arange(BLK)
    c = np.cos(theta[:, None] * n[None, :])
    s = np.sin(theta[:, None] * n[None, :])
    fwd = np.zeros((NFFT, BLK))
    for m in range(BLK // 8):
        fwd[16 * m:16 * m + 8] = c[8 * m:8 * m + 8]
        fwd[16 * m + 8:16 * m + 16] = -s[8 * m:8 * m + 8]
    inv = fwd[:BLK].T * (2.0 / NFFT)
    inv = np.concatenate([inv[0::2], inv[1::2]], axis=0)
    return fwd.astype(np.float32), inv.astype(np.float32)


def _dot(a, b):
    return jnp.dot(a, b, preferred_element_type=F32)


def _pack(x):
    return pltpu.bitcast(x.astype(BF16), U32)


def _unpack(w):
    return pltpu.bitcast(w, BF16)


def _lo(w):
    return pltpu.bitcast(w << 16, F32)


def _hi(w):
    return pltpu.bitcast(w & jnp.uint32(0xFFFF0000), F32)


def _strassen_lhs(a11, a12, a21, a22):
    return [a11 + a22, a21 + a22, a11, a22, a11 + a12, a21 - a11, a12 - a22]


def _strassen_rhs(b11, b12, b21, b22):
    ops = [b11 + b22, b11, b12 - b22, b21 - b11, b22, b11 + b12, b21 + b22]
    return [o.astype(BF16) for o in ops]


_STRASSEN_USES = (((0, 1), (3, 1)), ((2, 1), (3, -1)), ((1, 1), (3, 1)), ((0, 1), (2, 1)),
                  ((0, -1), (1, 1)), ((3, 1),), ((0, 1),))


def _strassen(lhs, rhs, emit, init=None, order=(4, 2, 1, 3, 0, 6, 5)):
    acc = [[(1, c)] if c is not None else [] for c in (init or (None,) * 4)]
    left = [4, 2, 2, 4]
    for k in order:
        m = _dot(lhs(k), rhs[k])
        for q, sign in _STRASSEN_USES[k]:
            acc[q].append((sign, m))
            left[q] -= 1
            if len(acc[q]) > 1 and (init is None or len(acc[q]) > 2 or left[q] < (3, 1, 1, 3)[q]):
                terms = sorted(acc[q], key=lambda t: -t[0])
                v = terms[0][1]
                assert terms[0][0] > 0
                for sg, t in terms[1:]:
                    v = v + t if sg > 0 else v - t
                acc[q] = [(1, v)]
            if left[q] == 0:
                emit(q // 2, q % 2, acc[q][0][1])
        yield m


def _drain(*gens):
    for g in gens:
        for _ in g:
            pass


def _tokens(m):
    return [m[r:r + 8, c:c + LANES]
            for r in range(0, m.shape[0], 8) for c in range(0, m.shape[1], LANES)]


def _tie(never, tok, x):
    if tok is None:
        return x
    reps = (x.shape[0] // 8, x.shape[1] // LANES)
    if tok.dtype != x.dtype:
        tok = pltpu.bitcast(tok, x.dtype)
    if reps != (1, 1):
        never, tok = jnp.tile(never, reps), jnp.tile(tok, reps)
    return jnp.where(never, tok, x)


def _run_paced(items, toks):
    for i, it in enumerate(items):
        it(toks[i * len(toks) // len(items)])


def _interleave(nv, ngr, weights):
    dur = {'v': 256, 'h': 256, 'x': 256, 'inv': 128}
    margin = 768

    def plan(rate):
        t, v, out = 0, 0, []
        nxt = {'h': 0, 'x': 0, 'inv': 0}
        pos = {k: 0 for k in weights}
        done = {}
        credit = 0.0
        while True:
            kind = None
            if nxt['inv'] < ngr and done.get(('freq', nxt['inv']), 1e9) + margin <= t:
                kind = 'inv'
            elif nxt['x'] < ngr and done.get(('conv', nxt['x']), 1e9) + margin <= t:
                kind = 'x'
            elif nxt['h'] < ngr and nxt['h'] <= nxt['x'] and (not out or out[-1][0] == 'v'):
                kind = 'h'
            elif v < nv:
                kind = 'v'
            if kind is None:
                break
            g = v if kind == 'v' else nxt[kind]
            busy = 1.1 if kind == 'v' and v % (nv // 2) < 7 else 0.0
            credit += (rate - busy) * dur[kind]
            chunk = []
            while credit > 0:
                ready = [('out', i) for i in range(nxt['inv'])]
                ready += [('conv', i) for i in range(ngr)]
                ready += [('freq', i) for i in range(min(nxt['x'], nxt['h']))]
                ready = [k for k in ready if pos[k] < len(weights[k])]
                if not ready:
                    credit = 0.0
                    break
                k = ready[0]
                chunk.append((k, pos[k]))
                credit -= weights[k][pos[k]]
                pos[k] += 1
                if pos[k] == len(weights[k]):
                    done[k] = t + dur[kind]
            out.append((kind, g, chunk))
            t += dur[kind]
            if kind == 'v':
                v += 1
            else:
                nxt[kind] += 1
        ok = all(pos[k] == len(weights[k]) for k in weights)
        return ok, out

    rate = 1.0
    while True:
        ok, out = plan(rate)
        if ok:
            return out
        rate += 0.02


def _kernel(q_hbm, k_hbm, v_hbm, shift_hbm, h_hbm, d_hbm, x_hbm, mem0_hbm,
            wq_hbm, wk_hbm, wv_hbm, wo_hbm, fwd_hbm, inv_hbm,
            out_hbm,
            abuf, a0buf, vbuf, w32, wo, qks, vms, acc, obuf, mhat, mnew, okbuf, mcol, tsum,
            ain, ah, kf, kvb, xf, hf, wf, yt, aout,
            mem0_ref, fwd_ref, inv_ref, shift_ref, d_ref, zero_v, zero_s,
            sem_s, sem_x, sem_wv, sem_wqk, sem_wo, sem_a, sem_aout, sem_o,
            *, S, D, DM, H, M, SEG):
    E = LANES
    NSEG = S // SEG
    NP = NSEG // 2
    MR = 2 * M
    XR = 2 * SEG
    PR = MR + XR
    MW, XW, PW = MR // 2, XR // 2, PR // 2
    L = M + SEG
    NB = S // BLK
    NT = D // LANES
    PPB = 8
    PPH = PPB // 2
    NRB = NP // PPB
    G = 4
    NG = H // G
    KH = DM // 2
    scale = float(E) ** -0.5
    WV, WQ, WK = 0, 1, 2

    small = [pltpu.make_async_copy(src, dst, sem_s.at[i]) for i, (src, dst) in enumerate(
        ((mem0_hbm, mem0_ref), (shift_hbm, shift_ref), (d_hbm, d_ref),
         (fwd_hbm, fwd_ref), (inv_hbm, inv_ref)))]
    HBR = PPH * XR // 2

    def x_copies(hb):
        out = []
        for half in range(2):
            r = pl.ds(pl.multiple_of((2 * half + hb % 2) * HBR, HBR), HBR)
            out.append(pltpu.make_async_copy(x_hbm.at[hb // 2, r], obuf.at[hb // 2, r],
                                             sem_x.at[hb]))
        return out

    def w_copy(which, hp):
        src = (wv_hbm, wq_hbm, wk_hbm)[which].bitcast(U32)
        sem = sem_wv.at[hp] if which == WV else sem_wqk
        return pltpu.make_async_copy(src.at[:, hp, :], w32.at[which, hp], sem)

    def wo_copy(t):
        n = H * E // NT
        r = pl.ds(pl.multiple_of(t * n, n), n)
        return pltpu.make_async_copy(wo_hbm.at[r, :], wo.at[r, :], sem_wo)

    def a_start(t, sl, which=(0, 1, 2, 3)):
        c = pl.ds(pl.multiple_of(t * LANES, LANES), LANES)
        for i in which:
            if i == 3:
                pltpu.make_async_copy(h_hbm.at[c, :], ah.at[sl], sem_a.at[sl, 1]).start()
            else:
                src = (k_hbm, v_hbm, q_hbm)[i]
                pltpu.make_async_copy(src.at[:, c], ain.at[sl, i], sem_a.at[sl, 0]).start()

    def a_wait(sl):
        pltpu.make_async_copy(ain.at[sl], ain.at[sl], sem_a.at[sl, 0]).wait()
        pltpu.make_async_copy(ah.at[sl], ah.at[sl], sem_a.at[sl, 1]).wait()

    def aout_copy(t):
        c = pl.ds(pl.multiple_of(t * LANES, LANES), LANES)
        return pltpu.make_async_copy(aout.at[t], out_hbm.at[:, c], sem_aout)

    def o_copy(rb):
        r = pl.ds(pl.multiple_of(rb * (PPB * XR), PPB * XR), PPB * XR)
        return pltpu.make_async_copy(obuf.at[rb], out_hbm.at[r, pl.ds(D, DM)], sem_o.at[rb])

    def oq_copy(qd):
        n = PPH * XR
        r0, c0 = (qd // 2) * n, (qd % 2) * KH
        return pltpu.make_async_copy(
            obuf.at[NRB - 1, pl.ds(r0, n), pl.ds(c0, KH)],
            out_hbm.at[pl.ds((NRB - 1) * 2 * n + r0, n), pl.ds(D + c0, KH)],
            sem_o.at[NRB - 1 + qd])

    def w_rhs(which, hp, zs=None):
        if zs is None:
            w = w32[which, hp]
            return _strassen_rhs(_lo(w[:KH]), _hi(w[:KH]), _lo(w[KH:]), _hi(w[KH:]))
        out = []
        for k in range(7):
            w = w32.at[which, hp + zs[k]]
            out.append(_strassen_rhs(_lo(w[:KH]), _hi(w[:KH]), _lo(w[KH:]), _hi(w[KH:]))[k])
        return out

    def w_plain(which, hp0, n):
        parts = []
        for j in range(n):
            w = w32[which, hp0 + j]
            parts += [_lo(w), _hi(w)]
        return jnp.concatenate(parts, axis=1).astype(BF16)

    small[0].start()
    for hb in range(2):
        for cp in x_copies(hb):
            cp.start()
    w_copy(WV, 0).start()
    w_copy(WV, 1).start()
    for cp in small[1:]:
        cp.start()

    kf[0:8, :] = jnp.zeros((8, LANES), F32)
    zero_v[...] = jnp.zeros((8, LANES), jnp.int32)
    for k in range(8):
        zero_s[k] = 0
    tsum[:, 0:8, 0:LANES] = jnp.zeros((NG, 8, LANES), F32)
    vbuf[:, 0, 0:16, 0:LANES] = jnp.zeros((NG, 16, LANES), BF16)
    for hb in range(2 * NRB):
        r0 = (hb % 2) * (HBR // 2)
        abuf[hb // 2, 0, r0:r0 + 8, 0:LANES] = jnp.zeros((8, LANES), U32)
    small[0].wait()
    mem0 = mem0_ref[...].astype(F32)
    m0 = jnp.concatenate([mem0, jnp.zeros_like(mem0)], axis=0)
    z0 = jnp.zeros((MR, KH), F32)
    for k, op in enumerate(_strassen_lhs(m0[:, :KH], m0[:, KH:], z0, z0)):
        a0buf[k, 0:MW, :] = _pack(op)

    def x_item(tok, never, src, dst, r, c):
        quad = [_tie(never, tok, src[h * 2 * HBR + r:h * 2 * HBR + r + 16,
                                     kk * KH + c:kk * KH + c + 2 * LANES].astype(F32))
                for h in range(2) for kk in range(2)]
        for k, op in enumerate(_strassen_lhs(*quad)):
            dst[k, r // 2:r // 2 + 8, c:c + 2 * LANES] = _pack(op)

    def x_items(never, src, dst):
        return [functools.partial(x_item, never=never, src=src, dst=dst, r=r, c=c)
                for r in range(0, HBR, 16) for c in range(0, KH, 2 * LANES)]

    def x_first(hb, cy):
        for cp in x_copies(hb):
            cp.wait()
        src = obuf.at[0, pl.ds(pl.multiple_of(hb * HBR, HBR), 3 * HBR)]
        dst = a0buf.at[:, pl.ds(pl.multiple_of(MW + hb * (HBR // 2), 8), HBR // 2)]
        for it in x_items(None, src, dst):
            it(None)
        return cy

    lax.fori_loop(0, 2, x_first, 0)

    def v_part(j, rb, rhs, vwin, twin, pre=None):
        def lhs(k):
            x = a0buf[k] if rb == 0 else abuf[rb, k]
            if pre is not None and k == 4:
                x0 = jnp.concatenate([pre(x[:8, :LANES]), x[:8, LANES:]], axis=1)
                x = jnp.concatenate([x0, x[8:]], axis=0)
            return _unpack(x)

        def emit(half, hh, cv):
            c = slice((2 * j + hh) * E, (2 * j + hh + 1) * E)
            vv = cv.astype(BF16)
            vx = vv[MR:] if rb == 0 else vv
            p0 = rb * PPB + half * PPH
            vwin[p0:p0 + PPH, :, c] = vx.reshape(PPH, XR, E)
            ts = jnp.sum(vx.astype(F32).reshape(2 * PPH, SEG, E), axis=1)
            if rb == 0 and half == 0:
                v0 = vv[0:M].astype(F32)
                twin[NSEG:NSEG + M, c] = v0
                t0 = jnp.sum(v0, axis=0, keepdims=True)
                rows = lax.broadcasted_iota(jnp.int32, ts.shape, 0)
                ts = ts + jnp.where(rows == 0, t0, 0.0)
            twin[2 * p0:2 * (p0 + PPH), c] = ts

        return _strassen(lhs, rhs, emit)

    def v_products(t, rbs, never, extra=()):
        zs = [zero_s[k] for k in range(7)]
        vwin = vbuf.at[t]
        twin = tsum.at[t]

        def pre(x):
            for v in (twin[0:8, 0:LANES], pltpu.bitcast(vwin[0, 0:16, 0:LANES], U32)) + tuple(extra):
                x = _tie(never, v, x)
            return x

        for j in range(2):
            rhs = w_rhs(WV, 2 * t + j, zs)
            for rb in rbs:
                yield from v_part(j, rb, rhs, vwin, twin, pre if (j, rb) == (0, rbs[0]) else None)

    def head_body(j, cy):
        w_copy(WV, 2 * j).wait()
        w_copy(WV, 2 * j + 1).wait()

        @pl.when(j >= 2)
        def _():
            for cp in x_copies(j):
                cp.wait()

        @pl.when(j + 1 < NT)
        def _():
            w_copy(WV, 2 * j + 2).start()
            w_copy(WV, 2 * j + 3).start()

        @pl.when(j + 2 < 2 * NRB)
        def _():
            for cp in x_copies(j + 2):
                cp.start()

        @pl.when(j == NT - 3)
        def _():
            a_start(0, 0, (3,))

        @pl.when(j == NT - 2)
        def _():
            a_start(0, 0, (0, 1, 2))

        never = zero_v[...] > 0
        src = obuf.at[j // 2, pl.ds(pl.multiple_of((j % 2) * HBR, HBR), 3 * HBR)]
        dst = abuf.at[j // 2, :, pl.ds(pl.multiple_of((j % 2) * (HBR // 2), 8), HBR // 2)]
        toks = []
        for m in v_products(j, [0], never, [dst[0, 0:8, 0:LANES]]):
            toks += _tokens(m)
        _run_paced(x_items(never, src, dst), toks[:-40])
        return cy

    assert NT == 2 * NRB
    lax.fori_loop(0, NT, head_body, 0)

    GA = 4

    def freq_items(a0, never):
        def item(tok, m, cc, st):
            r_re = slice(16 * m, 16 * m + 8)
            r_im = slice(16 * m + 8, 16 * m + 16)
            xr = _tie(never, tok, xf[r_re, cc * BLK:(cc + 1) * BLK])
            xi = _tie(never, tok, xf[r_im, cc * BLK:(cc + 1) * BLK])
            xs = xr + xi
            for a in range(max(a0, cc), a0 + GA):
                j = a - cc
                if ('g', m, j) not in st:
                    gr = hf[r_re, j * BLK:(j + 1) * BLK]
                    gi = hf[r_im, j * BLK:(j + 1) * BLK]
                    st['g', m, j] = (gr, gi, gr + gi)
                gr, gi, gs = st['g', m, j]
                ps = (xr * gr, xi * gi, xs * gs)
                st[m, a] = ps if (m, a) not in st else tuple(u + v for u, v in zip(st[m, a], ps))
                if cc == a:
                    p1, p2, p3 = st[m, a]
                    st[m, a] = (p1 - p2, p3 - p1 - p2)
                    if m >= BLK // 16:
                        m0 = m - BLK // 16
                        (wr, wi), (vr, vi) = st[m0, a], st[m, a]
                        c = slice(a * BLK, (a + 1) * BLK)
                        wf[16 * m0:16 * m0 + 16, c] = (
                            jnp.concatenate([wr + vr, wi - vi], axis=0).astype(BF16))
                        wf[16 * m:16 * m + 16, c] = (
                            jnp.concatenate([wr - vr, wi + vi], axis=0).astype(BF16))

        items = []
        for m0 in range(BLK // 16):
            st = {}
            for m in (m0, m0 + BLK // 16):
                items += [(functools.partial(item, m=m, cc=cc, st=st),
                           4 + 6 * (a0 + GA - max(a0, cc)) + (6 if cc >= a0 else 0))
                          for cc in range(a0 + GA)]
        return items

    def tile_body(t, carry):
        sl = t % 2
        a_wait(sl)

        @pl.when(t + 1 < NT)
        def _():
            a_start(t + 1, 1 - sl)
            wo_copy(t + 1).start()

        for which in (WQ, WK):
            w_copy(which, 2 * t).start()
            w_copy(which, 2 * t + 1).start()

        c = pl.ds(pl.multiple_of(t * LANES, LANES), LANES)
        taps = shift_ref[:, c].astype(F32)
        dcol = d_ref[...].astype(F32)
        rows = lax.broadcasted_iota(jnp.int32, dcol.shape, 0)
        dvec = jnp.sum(jnp.where(rows == t, dcol, 0.0), axis=0, keepdims=True)
        dvb = jnp.broadcast_to(dvec, (8, LANES))
        tapb = [jnp.broadcast_to(taps[j:j + 1, :], (8, LANES)) for j in range(4)]
        never = zero_v[...] > 0
        fwd = fwd_ref[...]
        NGR = NB // GA
        GW = GA * BLK

        def conv_item(tok, r0):
            kf[8 + r0:24 + r0, :] = ain[sl, 0, r0:r0 + 16, :].astype(F32)
            halves = []
            for h in range(2):
                r = 8 + r0 + 8 * h
                ks = kf[r:r + 8, :] * _tie(never, tok, tapb[0])
                for j in range(1, 4):
                    ks = ks + kf[r - j:r - j + 8, :] * tapb[j]
                halves.append(ks)
            kvb[r0:r0 + 16, :] = (jnp.concatenate(halves, axis=0)
                                  * ain[sl, 1, r0:r0 + 16, :].astype(F32)).astype(BF16)

        hlast = [None]

        def h_fwd(g):
            hst = jnp.concatenate([ah[sl, :, b * BLK:(b + 1) * BLK]
                                   for b in range(g * GA, (g + 1) * GA)], axis=0)
            hh = lax.dot_general(fwd, hst, (((1,), (1,)), ((), ())), preferred_element_type=F32)
            for b in range(GA):
                cur = hh[:, b * BLK:(b + 1) * BLK]
                prev = hlast[0]
                c = slice((g * GA + b) * BLK, (g * GA + b + 1) * BLK)
                if prev is None:
                    hf[:, c] = cur
                else:
                    for m in range(BLK // 8):
                        re = slice(16 * m, 16 * m + 8)
                        im = slice(16 * m + 8, 16 * m + 16)
                        if m < BLK // 16:
                            hf[re, c] = cur[re] - prev[im]
                            hf[im, c] = cur[im] + prev[re]
                        else:
                            hf[re, c] = cur[re] + prev[im]
                            hf[im, c] = cur[im] - prev[re]
                hlast[0] = cur
            return hh

        def x_fwd(g):
            rhs = jnp.concatenate([kvb[b * BLK:(b + 1) * BLK, :]
                                   for b in range(g * GA, (g + 1) * GA)], axis=1)
            xx = _dot(fwd, rhs)
            xf[:, g * GW:(g + 1) * GW] = xx
            return xx

        def inverse(g):
            ys = []
            for par in range(2):
                y = _dot(inv_ref[par * (BLK // 2):(par + 1) * (BLK // 2), :],
                         wf[par * BLK:(par + 1) * BLK, g * GW:(g + 1) * GW])
                for a in range(GA):
                    yt[pl.ds((g * GA + a) * BLK + par, BLK // 2, stride=2), :] = (
                        y[:, a * BLK:(a + 1) * BLK])
                ys.append(y)
            return jnp.concatenate(ys, axis=0)

        def out_item(tok, r0):
            d8 = _tie(never, tok, dvb)
            yb = yt[r0:r0 + 16, :] + kvb[r0:r0 + 16, :].astype(F32) * jnp.concatenate([d8, d8], axis=0)
            aout[t, r0:r0 + 16, :] = (ain[sl, 2, r0:r0 + 16, :].astype(F32) * yb).astype(BF16)

        def rows16(fn, g, w):
            return [(functools.partial(fn, r0=r0), w) for r0 in range(g * GW, (g + 1) * GW, 16)]

        vgen = v_products(t, list(range(1, NRB)), never)
        nv = 2 * (NRB - 1) * 7
        work = {('conv', g): rows16(conv_item, g, 25) for g in range(NGR)}
        work.update({('freq', g): freq_items(g * GA, never) for g in range(NGR)})
        work.update({('out', g): rows16(out_item, g, 16) for g in range(NGR)})
        for kind, g, chunks in _interleave(nv, NGR, {k: [w for _, w in v] for k, v in work.items()}):
            if kind is not None:
                m = (next(vgen) if kind == 'v' else
                     {'h': h_fwd, 'x': x_fwd, 'inv': inverse}[kind](g))
                toks = _tokens(m)
            items = [work[k][i][0] for k, i in chunks]
            if kind is None:
                for it in items:
                    it(None)
            elif items:
                _run_paced(items, toks)
        _drain(vgen)
        aout_copy(t).start()
        return carry

    for cp in small[1:]:
        cp.wait()
    wo_copy(0).start()
    lax.fori_loop(0, NT, tile_body, 0)
    pltpu.make_async_copy(wo, wo, sem_wo).wait()

    def initial_guess():
        puni = pl.reciprocal(jnp.full((1, 1), float(L), F32), approx=True).astype(BF16).astype(F32)

        def shift_down(m):
            rows = lax.broadcasted_iota(jnp.int32, m.shape, 0)
            return jnp.where(rows == 0, 0.0, pltpu.roll(m, 1, 0))

        tall = jnp.concatenate([tsum[g, 0:NSEG, :] for g in range(NG)], axis=1)
        wov = wo[...]
        m1 = shift_down(_dot((tall * puni).astype(BF16), wov))
        v1 = _dot(m1.astype(BF16), w_plain(WV, 0, H // 2)).astype(BF16).astype(F32)
        u2 = ((tall + float(M) * v1) * puni).astype(BF16)
        for c in range(0, DM, LANES):
            mcol[c // LANES] = _dot(u2, wov[:, c:c + LANES])
            for sg in range(NSEG):
                mhat[(sg + 1) * M:(sg + 2) * M, c:c + LANES] = jnp.broadcast_to(
                    mcol[c // LANES, sg:sg + 1, :], (M, LANES))
        mhat[0:M, :] = mem0_ref[...].astype(F32)
        pltpu.make_async_copy(w32.at[WQ:WK + 1], w32.at[WQ:WK + 1], sem_wqk).wait()

    ri = lax.broadcasted_iota(jnp.int32, (PR, PR), 0)
    ci = lax.broadcasted_iota(jnp.int32, (PR, PR), 1)

    def seg_of(r):
        return jnp.where(r < MR, r // M, (r - MR) // SEG)

    def pos_of(r):
        return jnp.where(r < MR, r % M, M + (r - MR) % SEG)

    same = seg_of(ri) == seg_of(ci)
    allowed = same & ((ri < MR) | (pos_of(ri) >= pos_of(ci)))
    fill = jnp.where(same, -1e9, -jnp.inf).astype(F32)

    def sweep(state):
        it, _ = state
        pl.when(it == 0)(initial_guess)

        @pl.when(it > 0)
        def _():
            def upd(rb, cy):
                n = PPB * MR
                r = pl.ds(pl.multiple_of(rb * n, n), n)
                r2 = pl.ds(pl.multiple_of(rb * n + M, M), n)
                keep = jnp.tile(okbuf[r, :], (1, DM // LANES)) > 0.5
                mhat[r2, :] = jnp.where(keep, mhat[r2, :], mnew[r, :])
                return cy

            lax.fori_loop(0, NRB, upd, 0)

        def mem_rows(i):
            n = PPB * MR
            return mhat[pl.ds(pl.multiple_of((i // NG) * n, n), n), :]

        def mem_lhs(i):
            m = mem_rows(i)
            n = PPH * MR
            ops = [_pack(o) for o in _strassen_lhs(m[:n, :KH], m[:n, KH:], m[n:, :KH], m[n:, KH:])]
            t = jnp.concatenate([jnp.where(i < NG, 0.0, m[:M]), m[M:MR]], axis=0)
            b = m[n:n + MR]
            vops = [jnp.concatenate([_pack(o), full[MW:]], axis=0) for o, full in zip(
                _strassen_lhs(t[:, :KH], t[:, KH:], b[:, :KH], b[:, KH:]), ops)]
            return ops, vops

        def qk_proj(i, j, mops):
            rb = i // NG
            hp = (i % NG) * (G // 2) + j // 2

            def lhs(k):
                return _unpack(jnp.concatenate([mops[k], abuf[rb, k]], axis=0))

            n = PPH * MR
            cs = {}

            def emit(half, hh, cv):
                cs[half, hh] = cv
                if (half, 1 - hh) in cs:
                    v = jnp.concatenate([cs[half, 0], cs[half, 1]], axis=1).astype(BF16)
                    ps = slice(half * PPH, (half + 1) * PPH)
                    qks[j, ps, 0:MR, :] = v[:n].reshape(PPH, MR, 2 * E)
                    qks[j, ps, MR:PR, :] = v[n:].reshape(PPH, XR, 2 * E)

            return _strassen(lhs, w_rhs(WQ + j % 2, hp, [zero_s[k] for k in range(7)]), emit)

        def vm_proj(i, j, vops):
            hp = (i % NG) * (G // 2) + j

            def emit(half, hh, cv):
                if half == 0:
                    v0 = tsum[i % NG, NSEG:NSEG + M, (2 * j + hh) * E:(2 * j + hh + 1) * E]
                    cv = jnp.concatenate([jnp.where(i < NG, v0, cv[:M]), cv[M:]], axis=0)
                vms[half * PPH:(half + 1) * PPH, :, (2 * j + hh) * E:(2 * j + hh + 1) * E] = (
                    cv.astype(BF16).reshape(PPH, MR, E))

            return _strassen(lambda k: _unpack(vops[k]),
                             w_rhs(WV, hp, [zero_s[k] for k in range(7)]), emit)

        def scores(j):
            c = slice((j % 2) * E, (j % 2 + 1) * E)
            return lax.dot_general(qks[2 * (j // 2), :, :, c], qks[2 * (j // 2) + 1, :, :, c],
                                   (((2,), (2,)), ((0,), (0,))), preferred_element_type=F32)

        def attend(i, j, s):
            p0 = pl.multiple_of((i // NG) * PPB, PPB)
            s = jnp.where(allowed[None], s * scale, fill[None])
            e = jnp.exp(s - jnp.max(s, axis=-1, keepdims=True))
            p = (e * pl.reciprocal(jnp.sum(e, axis=-1, keepdims=True), approx=True)).astype(BF16)
            vh = jnp.concatenate(
                [vms[:, :, j * E:(j + 1) * E],
                 vbuf[i % NG, pl.ds(p0, PPB), :, j * E:(j + 1) * E]], axis=1)
            return lax.dot_general(p, vh, (((2,), (1,)), ((0,), (0,))), preferred_element_type=F32)

        def wo_rows(i):
            return wo[pl.ds(pl.multiple_of((i % NG) * (G * E), G * E), G * E), :]

        def out_mem(i, us, split):
            rb = i // NG
            wog = wo_rows(i)
            rm = pl.ds(pl.multiple_of(rb * (PPB * MR), PPB * MR), PPB * MR)
            new = jnp.where(i % NG > 0, mnew[rm, :], 0.0)
            n = G // split
            for j in range(0, G, n):
                um = jnp.concatenate([u[:, :MR, :] for u in us[j:j + n]], axis=2)
                new = new + _dot(um.reshape(PPB * MR, n * E).astype(BF16), wog[j * E:(j + n) * E])
            mnew[rm, :] = new
            old = mhat[pl.ds(pl.multiple_of(rb * (PPB * MR) + M, M), PPB * MR), :]
            err = jnp.max(jnp.abs(new - old), axis=1, keepdims=True)
            ref = jnp.max(jnp.abs(new), axis=1, keepdims=True)
            okbuf[rm, :] = jnp.broadcast_to(jnp.where(err <= TOL * ref, 1.0, 0.0),
                                            (PPB * MR, LANES))

        def out_tok(i, us, last):
            rb = i // NG
            n = PPH * XR
            kh = G * E // 2

            def quad(half, kk):
                if len(us) < 2 * kk + 2:
                    kk = 0
                u = jnp.concatenate(us[2 * kk:2 * kk + 2], axis=2)
                return u[half * PPH:(half + 1) * PPH, MR:, :].reshape(n, kh)

            def lhs(k):
                return _strassen_lhs(quad(0, 0), quad(0, 1), quad(1, 0), quad(1, 1))[k].astype(BF16)

            wf32 = wo_rows(i).astype(F32)
            rhs = _strassen_rhs(wf32[:kh, :KH], wf32[:kh, KH:], wf32[kh:, :KH], wf32[kh:, KH:])
            quads = [(slice(0, n), slice(0, KH)), (slice(0, n), slice(KH, DM)),
                     (slice(n, 2 * n), slice(0, KH)), (slice(n, 2 * n), slice(KH, DM))]
            init = [jnp.where(i % NG > 0, acc[r, c], 0.0) for r, c in quads]

            def emit(half, hh, v):
                r, c = quads[2 * half + hh]
                obuf[rb, r, c] = v.astype(BF16)
                if last:
                    oq_copy(2 * half + hh).start()
                else:
                    acc[r, c] = v

            if last:
                return _strassen(lhs, rhs, emit, init, order=(2, 5, 4, 1, 3, 0, 6))
            return _strassen(lhs, rhs, emit, init)

        def step(i):
            s0, s1 = scores(0), scores(1)
            mops, vops = mem_lhs(i + 1)
            _drain(qk_proj(i + 1, 0, mops))
            us = [attend(i, 0, s0), attend(i, 1, s1)]
            s2, s3 = scores(2), scores(3)
            _drain(qk_proj(i + 1, 1, mops))
            us += [attend(i, 2, s2), attend(i, 3, s3)]
            _drain(zip(qk_proj(i + 1, 2, mops), vm_proj(i + 1, 0, vops)))
            _drain(zip(qk_proj(i + 1, 3, mops), vm_proj(i + 1, 1, vops)))
            out_mem(i, us, 1)
            _drain(out_tok(i, us, False))

        def last_step(i):
            ss = [scores(j) for j in range(G)]
            us = [attend(i, 0, ss[0]), attend(i, 1, ss[1])]
            gen = out_tok(i, us, True)
            next(gen)
            next(gen)
            us += [attend(i, 2, ss[2]), attend(i, 3, ss[3])]
            out_mem(i, us, 2)
            _drain(gen)

        mops0, vops0 = mem_lhs(0)
        _drain(qk_proj(0, 0, mops0), qk_proj(0, 1, mops0))
        _drain(zip(qk_proj(0, 2, mops0), vm_proj(0, 0, vops0)))
        _drain(zip(qk_proj(0, 3, mops0), vm_proj(0, 1, vops0)))

        def main_body(i, cy):
            step(i)

            @pl.when(i % NG == NG - 1)
            def _():
                o_copy(i // NG).start()

            return cy

        lax.fori_loop(0, NRB * NG - 1, main_body, 0)
        last_step(NRB * NG - 1)
        ok = jnp.min(okbuf[0:(NSEG - 1) * M, :])
        for rb in range(NRB - 1):
            o_copy(rb).wait()
        for qd in range(4):
            oq_copy(qd).wait()
        return it + 1, (ok > 0.5).astype(jnp.int32)

    lax.while_loop(lambda st: jnp.logical_and(st[0] < NSEG, st[1] == 0), sweep,
                   (jnp.int32(0), jnp.int32(0)))
    pltpu.make_async_copy(aout, aout, sem_aout).wait()


@functools.partial(jax.jit, static_argnames=("B_seg_len",))
def pallas_concat_heads__ssm_conv_h3__memory_aug_recurrent_mem_tr__prompt_kernel(
    A_q, A_k, A_v, A_shift_k, A_ssm_k, A_ssm_D,
    B_x, B_mem0, B_Wq, B_Wk, B_Wv, B_Wo, B_seg_len,
):
    _, S, D = A_q.shape
    DM = B_x.shape[2]
    H, E = B_Wq.shape[1], B_Wq.shape[2]
    M = B_mem0.shape[1]
    SEG = int(B_seg_len)
    NSEG = S // SEG
    NP = NSEG // 2
    PR = 2 * (M + SEG)
    PPB = 8
    NRB = NP // PPB
    NT = D // LANES
    assert E == LANES and H == 32 and M == 8 and SEG == 32 and A_shift_k.shape[1] == 4
    assert S == 2048 and D == 1024 and DM == 1024

    fwd, inv = _dft_mats()
    any_spec = pl.BlockSpec(memory_space=pl.ANY)
    scratch = [
        pltpu.VMEM((NRB, 7, PPB // 2 * SEG, DM // 2), U32),
        pltpu.VMEM((7, M + PPB // 2 * SEG, DM // 2), U32),
        pltpu.VMEM((H // 4, NP, 2 * SEG, 4 * E), BF16),
        pltpu.VMEM((3, H // 2, DM, E), U32),
        pltpu.VMEM((H * E, DM), BF16),
        pltpu.VMEM((4, PPB, PR, 2 * E), BF16),
        pltpu.VMEM((PPB, 2 * M, 4 * E), BF16),
        pltpu.VMEM((PPB * 2 * SEG, DM), F32),
        pltpu.VMEM((NRB, PPB * 2 * SEG, DM), BF16),
        pltpu.VMEM(((NSEG + 1) * M, DM), F32),
        pltpu.VMEM((NSEG * M, DM), F32),
        pltpu.VMEM((NSEG * M, LANES), F32),
        pltpu.VMEM((DM // LANES, NSEG, LANES), F32),
        pltpu.VMEM((H // 4, NSEG + M, 4 * E), F32),
        pltpu.VMEM((2, 3, S, LANES), BF16),
        pltpu.VMEM((2, LANES, S), BF16),
        pltpu.VMEM((S + 32, LANES), F32),
        pltpu.VMEM((S, LANES), BF16),
        pltpu.VMEM((NFFT, S), F32),
        pltpu.VMEM((NFFT, S), F32),
        pltpu.VMEM((NFFT, S), BF16),
        pltpu.VMEM((S, LANES), F32),
        pltpu.VMEM((NT, S, LANES), BF16),
        pltpu.VMEM((M, DM), BF16),
        pltpu.VMEM((NFFT, BLK), BF16),
        pltpu.VMEM((BLK, BLK), BF16),
        pltpu.VMEM((4, D), BF16),
        pltpu.VMEM((NT, LANES), BF16),
        pltpu.VMEM((8, LANES), jnp.int32),
        pltpu.SMEM((8,), jnp.int32),
        pltpu.SemaphoreType.DMA((5,)),
        pltpu.SemaphoreType.DMA((2 * NRB,)),
        pltpu.SemaphoreType.DMA((H // 2,)),
        pltpu.SemaphoreType.DMA,
        pltpu.SemaphoreType.DMA,
        pltpu.SemaphoreType.DMA((2, 2)),
        pltpu.SemaphoreType.DMA,
        pltpu.SemaphoreType.DMA((NRB + 3,)),
    ]
    out = pl.pallas_call(
        functools.partial(_kernel, S=S, D=D, DM=DM, H=H, M=M, SEG=SEG),
        out_shape=jax.ShapeDtypeStruct((S, D + DM), BF16),
        in_specs=[any_spec] * 14,
        out_specs=any_spec,
        scratch_shapes=scratch,
        compiler_params=pltpu.CompilerParams(vmem_limit_bytes=120 * 1024 * 1024,
                                             disable_bounds_checks=True,
                                             disable_semaphore_checks=True),
    )(
        A_q.reshape(S, D), A_k.reshape(S, D), A_v.reshape(S, D),
        A_shift_k.T, A_ssm_k, A_ssm_D.reshape(NT, LANES),
        B_x.reshape(NRB, S // NRB, DM), B_mem0.reshape(M, DM),
        B_Wq, B_Wk, B_Wv, B_Wo.reshape(H * E, DM),
        jnp.asarray(fwd, BF16), jnp.asarray(inv, BF16),
    )
    return out.reshape(1, S, D + DM)
```

```python
import functools

import numpy as np
import jax
import jax.numpy as jnp
from jax import lax
import jax.experimental.pallas as pl
import jax.experimental.pallas.tpu as pltpu

F32 = jnp.float32
BF16 = jnp.bfloat16
U32 = jnp.uint32

LANES = 128
BLK = 128
NFFT = 2 * BLK
TOL = 2.0 ** -10


def _dft_mats():
    even = np.arange(0, BLK, 2)
    theta = 2.0 * np.pi * (np.concatenate([even, BLK - 1 - even]) + 0.5) / NFFT
    n = np.arange(BLK)
    c = np.cos(theta[:, None] * n[None, :])
    s = np.sin(theta[:, None] * n[None, :])
    fwd = np.zeros((NFFT, BLK))
    for m in range(BLK // 8):
        fwd[16 * m:16 * m + 8] = c[8 * m:8 * m + 8]
        fwd[16 * m + 8:16 * m + 16] = -s[8 * m:8 * m + 8]
    inv = fwd[:BLK].T * (2.0 / NFFT)
    inv = np.concatenate([inv[0::2], inv[1::2]], axis=0)
    return fwd.astype(np.float32), inv.astype(np.float32)


def _dot(a, b):
    return jnp.dot(a, b, preferred_element_type=F32)


def _pack(x):
    return pltpu.bitcast(x.astype(BF16), U32)


def _unpack(w):
    return pltpu.bitcast(w, BF16)


def _lo(w):
    return pltpu.bitcast(w << 16, F32)


def _hi(w):
    return pltpu.bitcast(w & jnp.uint32(0xFFFF0000), F32)


def _strassen_lhs(a11, a12, a21, a22):
    return [a11 + a22, a21 + a22, a11, a22, a11 + a12, a21 - a11, a12 - a22]


def _strassen_rhs(b11, b12, b21, b22):
    ops = [b11 + b22, b11, b12 - b22, b21 - b11, b22, b11 + b12, b21 + b22]
    return [o.astype(BF16) for o in ops]


_STRASSEN_USES = (((0, 1), (3, 1)), ((2, 1), (3, -1)), ((1, 1), (3, 1)), ((0, 1), (2, 1)),
                  ((0, -1), (1, 1)), ((3, 1),), ((0, 1),))


def _strassen(lhs, rhs, emit, init=None, order=(4, 2, 1, 3, 0, 6, 5), post=None):
    acc = [[(1, c)] if c is not None else [] for c in (init or (None,) * 4)]
    left = [4, 2, 2, 4]
    for k in order:
        m = _dot(lhs(k), rhs[k])
        if post is not None:
            m = post(k, m)
        for q, sign in _STRASSEN_USES[k]:
            acc[q].append((sign, m))
            left[q] -= 1
            if len(acc[q]) > 1 and (init is None or len(acc[q]) > 2 or left[q] < (3, 1, 1, 3)[q]):
                terms = sorted(acc[q], key=lambda t: -t[0])
                v = terms[0][1]
                assert terms[0][0] > 0
                for sg, t in terms[1:]:
                    v = v + t if sg > 0 else v - t
                acc[q] = [(1, v)]
            if left[q] == 0:
                emit(q // 2, q % 2, acc[q][0][1])
        yield m


def _drain(*gens):
    for g in gens:
        for _ in g:
            pass


def _tokens(m):
    return [m[r:r + 8, c:c + LANES]
            for r in range(0, m.shape[0], 8) for c in range(0, m.shape[1], LANES)]


def _tie(never, tok, x):
    if tok is None:
        return x
    reps = (x.shape[0] // 8, x.shape[1] // LANES)
    if tok.dtype != x.dtype:
        tok = pltpu.bitcast(tok, x.dtype)
    if reps != (1, 1):
        never, tok = jnp.tile(never, reps), jnp.tile(tok, reps)
    return jnp.where(never, tok, x)


def _run_paced(items, toks):
    for i, it in enumerate(items):
        it(toks[i * len(toks) // len(items)])


def _interleave(nv, ngr, weights):
    dur = {'v': 256, 'h': 256, 'x': 256, 'inv': 128}
    margin = 768

    def plan(rate):
        t, v, out = 0, 0, []
        nxt = {'h': 0, 'x': 0, 'inv': 0}
        pos = {k: 0 for k in weights}
        done = {}
        credit = 0.0
        while True:
            kind = None
            if nxt['inv'] < ngr and done.get(('freq', nxt['inv']), 1e9) + margin <= t:
                kind = 'inv'
            elif nxt['x'] < ngr and done.get(('conv', nxt['x']), 1e9) + margin <= t:
                kind = 'x'
            elif nxt['h'] < ngr and nxt['h'] <= nxt['x'] and (out and out[-1][0] == 'v'):
                kind = 'h'
            elif v < nv:
                kind = 'v'
            if kind is None:
                break
            g = v if kind == 'v' else nxt[kind]
            busy = 1.1 if kind == 'v' and v % (nv // 2) < 7 else (0.0 if kind == 'v' else 0.6)
            credit += (rate - busy) * dur[kind]
            chunk = []
            while credit > 0:
                ready = [('out', i) for i in range(nxt['inv'])]
                ready += [('conv', i) for i in range(ngr)]
                ready += [('freq', i) for i in range(min(nxt['x'], nxt['h']))]
                ready = [k for k in ready if pos[k] < len(weights[k])]
                if not ready:
                    credit = 0.0
                    break
                k = ready[0]
                chunk.append((k, pos[k]))
                credit -= weights[k][pos[k]]
                pos[k] += 1
                if pos[k] == len(weights[k]):
                    done[k] = t + dur[kind]
            out.append((kind, g, chunk))
            t += dur[kind]
            if kind == 'v':
                v += 1
            else:
                nxt[kind] += 1
        ok = all(pos[k] == len(weights[k]) for k in weights)
        return ok, out

    rate = 1.0
    while True:
        ok, out = plan(rate)
        if ok:
            return out
        rate += 0.02


def _kernel(q_hbm, k_hbm, v_hbm, shift_hbm, h_hbm, d_hbm, x_hbm, mem0_hbm,
            wq_hbm, wk_hbm, wv_hbm, wo_hbm, fwd_hbm, inv_hbm,
            out_hbm,
            abuf, a0buf, vbuf, w32, wo, qks, vms, acc, obuf, mhat, mnew, okbuf, mcol, tsum,
            ain, ah, kf, kvb, xf, hf, wf, yt, aout,
            mem0_ref, fwd_ref, inv_ref, shift_ref, d_ref, zero_v, zero_s,
            sem_s, sem_x, sem_wv, sem_wqk, sem_wo, sem_a, sem_aout, sem_o,
            *, S, D, DM, H, M, SEG):
    E = LANES
    NSEG = S // SEG
    NP = NSEG // 2
    MR = 2 * M
    XR = 2 * SEG
    PR = MR + XR
    MW, XW, PW = MR // 2, XR // 2, PR // 2
    L = M + SEG
    NB = S // BLK
    NT = D // LANES
    PPB = 8
    PPH = PPB // 2
    NRB = NP // PPB
    G = 4
    NG = H // G
    KH = DM // 2
    scale = float(E) ** -0.5
    WV, WQ, WK = 0, 1, 2

    small = [pltpu.make_async_copy(src, dst, sem_s.at[i]) for i, (src, dst) in enumerate(
        ((mem0_hbm, mem0_ref), (shift_hbm, shift_ref), (d_hbm, d_ref),
         (fwd_hbm, fwd_ref), (inv_hbm, inv_ref)))]
    HBR = PPH * XR // 2

    def x_copies(hb):
        out = []
        for half in range(2):
            r = pl.ds(pl.multiple_of((2 * half + hb % 2) * HBR, HBR), HBR)
            out.append(pltpu.make_async_copy(x_hbm.at[hb // 2, r], obuf.at[hb // 2, r],
                                             sem_x.at[hb]))
        return out

    def w_copy(which, hp):
        src = (wv_hbm, wq_hbm, wk_hbm)[which].bitcast(U32)
        sem = sem_wv.at[hp] if which == WV else sem_wqk
        return pltpu.make_async_copy(src.at[:, hp, :], w32.at[which, hp], sem)

    def wo_copy(t):
        n = H * E // NT
        r = pl.ds(pl.multiple_of(t * n, n), n)
        return pltpu.make_async_copy(wo_hbm.at[r, :], wo.at[r, :], sem_wo)

    def a_start(t, sl, which=(0, 1, 2, 3)):
        c = pl.ds(pl.multiple_of(t * LANES, LANES), LANES)
        for i in which:
            if i == 3:
                pltpu.make_async_copy(h_hbm.at[c, :], ah.at[sl], sem_a.at[sl, 1]).start()
            else:
                src = (k_hbm, v_hbm, q_hbm)[i]
                pltpu.make_async_copy(src.at[:, c], ain.at[sl, i], sem_a.at[sl, 0]).start()

    def a_wait(sl):
        pltpu.make_async_copy(ain.at[sl], ain.at[sl], sem_a.at[sl, 0]).wait()
        pltpu.make_async_copy(ah.at[sl], ah.at[sl], sem_a.at[sl, 1]).wait()

    def aout_copy(t):
        c = pl.ds(pl.multiple_of(t * LANES, LANES), LANES)
        return pltpu.make_async_copy(aout.at[t], out_hbm.at[:, c], sem_aout)

    def o_copy(rb):
        r = pl.ds(pl.multiple_of(rb * (PPB * XR), PPB * XR), PPB * XR)
        return pltpu.make_async_copy(obuf.at[rb], out_hbm.at[r, pl.ds(D, DM)], sem_o.at[rb])

    def oq_copy(qd):
        n = PPH * XR
        r0, c0 = (qd // 2) * n, (qd % 2) * KH
        return pltpu.make_async_copy(
            obuf.at[NRB - 1, pl.ds(r0, n), pl.ds(c0, KH)],
            out_hbm.at[pl.ds((NRB - 1) * 2 * n + r0, n), pl.ds(D + c0, KH)],
            sem_o.at[NRB - 1 + qd])

    def w_rhs(which, hp, zs=None):
        if zs is None:
            w = w32[which, hp]
            return _strassen_rhs(_lo(w[:KH]), _hi(w[:KH]), _lo(w[KH:]), _hi(w[KH:]))
        out = []
        for k in range(7):
            w = w32.at[which, hp + zs[k]]
            out.append(_strassen_rhs(_lo(w[:KH]), _hi(w[:KH]), _lo(w[KH:]), _hi(w[KH:]))[k])
        return out

    def w_plain(which, hp0, n):
        parts = []
        for j in range(n):
            w = w32[which, hp0 + j]
            parts += [_lo(w), _hi(w)]
        return jnp.concatenate(parts, axis=1).astype(BF16)

    small[0].start()
    for hb in range(2):
        for cp in x_copies(hb):
            cp.start()
    w_copy(WV, 0).start()
    w_copy(WV, 1).start()
    for cp in small[1:]:
        cp.start()

    kf[0:8, :] = jnp.zeros((8, LANES), F32)
    zero_v[...] = jnp.zeros((8, LANES), jnp.int32)
    for k in range(8):
        zero_s[k] = 0
    tsum[:, 0:8, 0:LANES] = jnp.zeros((NG, 8, LANES), F32)
    vbuf[:, 0, 0:16, 0:LANES] = jnp.zeros((NG, 16, LANES), BF16)
    for hb in range(2 * NRB):
        r0 = (hb % 2) * (HBR // 2)
        abuf[hb // 2, 0, r0:r0 + 8, 0:LANES] = jnp.zeros((8, LANES), U32)
    small[0].wait()
    mem0 = mem0_ref[...].astype(F32)
    m0 = jnp.concatenate([mem0, jnp.zeros_like(mem0)], axis=0)
    z0 = jnp.zeros((MR, KH), F32)
    for k, op in enumerate(_strassen_lhs(m0[:, :KH], m0[:, KH:], z0, z0)):
        a0buf[k, 0:MW, :] = _pack(op)

    def x_item(tok, never, src, dst, r, c):
        quad = [_tie(never, tok, src[h * 2 * HBR + r:h * 2 * HBR + r + 16,
                                     kk * KH + c:kk * KH + c + 2 * LANES].astype(F32))
                for h in range(2) for kk in range(2)]
        for k, op in enumerate(_strassen_lhs(*quad)):
            dst[k, r // 2:r // 2 + 8, c:c + 2 * LANES] = _pack(op)

    def x_items(never, src, dst):
        return [functools.partial(x_item, never=never, src=src, dst=dst, r=r, c=c)
                for r in range(0, HBR, 16) for c in range(0, KH, 2 * LANES)]

    def x_first(hb, cy):
        for cp in x_copies(hb):
            cp.wait()
        src = obuf.at[0, pl.ds(pl.multiple_of(hb * HBR, HBR), 3 * HBR)]
        dst = a0buf.at[:, pl.ds(pl.multiple_of(MW + hb * (HBR // 2), 8), HBR // 2)]
        for it in x_items(None, src, dst):
            it(None)
        return cy

    lax.fori_loop(0, 2, x_first, 0)

    def v_part(j, rb, rhs, vwin, twin, pre=None):
        mem0_in = (0, 2, 4, 6) if rb == 0 else ()
        m0 = {}

        def lhs(k):
            x = abuf[rb, k] if rb else (a0buf[k] if k in mem0_in else a0buf[k, MW:])
            if pre is not None and k == 4:
                x0 = jnp.concatenate([pre(x[:8, :LANES]), x[:8, LANES:]], axis=1)
                x = jnp.concatenate([x0, x[8:]], axis=0)
            return _unpack(x)

        def split(k, m):
            if k not in mem0_in:
                return m
            m0[k] = m[:M]
            return m[MR:]

        def emit(half, hh, cv):
            c = slice((2 * j + hh) * E, (2 * j + hh + 1) * E)
            vx = cv.astype(BF16)
            p0 = rb * PPB + half * PPH
            vwin[p0:p0 + PPH, :, c] = vx.reshape(PPH, XR, E)
            ts = jnp.sum(vx.astype(F32).reshape(2 * PPH, SEG, E), axis=1)
            if rb == 0 and half == 0:
                v0 = m0[2] + m0[4] if hh else m0[0] - m0[4] + m0[6]
                v0 = v0.astype(BF16).astype(F32)
                twin[NSEG:NSEG + M, c] = v0
                t0 = jnp.sum(v0, axis=0, keepdims=True)
                rows = lax.broadcasted_iota(jnp.int32, ts.shape, 0)
                ts = ts + jnp.where(rows == 0, t0, 0.0)
            twin[2 * p0:2 * (p0 + PPH), c] = ts

        return _strassen(lhs, rhs, emit, post=split)

    def v_products(t, rbs, never, extra=()):
        zs = [zero_s[k] for k in range(7)]
        vwin = vbuf.at[t]
        twin = tsum.at[t]

        def pre(x):
            for v in (twin[0:8, 0:LANES], pltpu.bitcast(vwin[0, 0:16, 0:LANES], U32)) + tuple(extra):
                x = _tie(never, v, x)
            return x

        for j in range(2):
            rhs = w_rhs(WV, 2 * t + j, zs)
            for rb in rbs:
                yield from v_part(j, rb, rhs, vwin, twin, pre if (j, rb) == (0, rbs[0]) else None)

    def head_body(j, cy):
        w_copy(WV, 2 * j).wait()
        w_copy(WV, 2 * j + 1).wait()

        @pl.when(j >= 2)
        def _():
            for cp in x_copies(j):
                cp.wait()

        @pl.when(j + 1 < NT)
        def _():
            w_copy(WV, 2 * j + 2).start()
            w_copy(WV, 2 * j + 3).start()

        @pl.when(j + 2 < 2 * NRB)
        def _():
            for cp in x_copies(j + 2):
                cp.start()

        @pl.when(j == NT - 3)
        def _():
            a_start(0, 0, (3,))

        @pl.when(j == NT - 2)
        def _():
            a_start(0, 0, (0, 1, 2))

        never = zero_v[...] > 0
        src = obuf.at[j // 2, pl.ds(pl.multiple_of((j % 2) * HBR, HBR), 3 * HBR)]
        dst = abuf.at[j // 2, :, pl.ds(pl.multiple_of((j % 2) * (HBR // 2), 8), HBR // 2)]
        toks = []
        for m in v_products(j, [0], never, [dst[0, 0:8, 0:LANES]]):
            toks += _tokens(m)
        _run_paced(x_items(never, src, dst), toks[:-40])
        return cy

    assert NT == 2 * NRB
    lax.fori_loop(0, NT, head_body, 0)

    GA = 4

    def freq_items(a0, never):
        def item(tok, m, cc, st):
            r_re = slice(16 * m, 16 * m + 8)
            r_im = slice(16 * m + 8, 16 * m + 16)
            xr = _tie(never, tok, xf[r_re, cc * BLK:(cc + 1) * BLK])
            xi = _tie(never, tok, xf[r_im, cc * BLK:(cc + 1) * BLK])
            xs = xr + xi
            for a in range(max(a0, cc), a0 + GA):
                j = a - cc
                if ('g', m, j) not in st:
                    gr = hf[r_re, j * BLK:(j + 1) * BLK]
                    gi = hf[r_im, j * BLK:(j + 1) * BLK]
                    st['g', m, j] = (gr, gi, gr + gi)
                gr, gi, gs = st['g', m, j]
                ps = (xr * gr, xi * gi, xs * gs)
                st[m, a] = ps if (m, a) not in st else tuple(u + v for u, v in zip(st[m, a], ps))
                if cc == a:
                    p1, p2, p3 = st[m, a]
                    st[m, a] = (p1 - p2, p3 - p1 - p2)
                    if m >= BLK // 16:
                        m0 = m - BLK // 16
                        (wr, wi), (vr, vi) = st[m0, a], st[m, a]
                        c = slice(a * BLK, (a + 1) * BLK)
                        wf[16 * m0:16 * m0 + 16, c] = (
                            jnp.concatenate([wr + vr, wi - vi], axis=0).astype(BF16))
                        wf[16 * m:16 * m + 16, c] = (
                            jnp.concatenate([wr - vr, wi + vi], axis=0).astype(BF16))

        items = []
        for m0 in range(BLK // 16):
            st = {}
            for m in (m0, m0 + BLK // 16):
                items += [(functools.partial(item, m=m, cc=cc, st=st),
                           4 + 6 * (a0 + GA - max(a0, cc)) + (6 if cc >= a0 else 0))
                          for cc in range(a0 + GA)]
        return items

    def tile_body(t, carry):
        sl = t & 1
        a_wait(sl)

        @pl.when(t + 1 < NT)
        def _():
            a_start(t + 1, 1 - sl)
            wo_copy(t + 1).start()

        c = pl.ds(pl.multiple_of(t * LANES, LANES), LANES)
        taps = shift_ref[:, c].astype(F32)
        dcol = d_ref[...].astype(F32)
        rows = lax.broadcasted_iota(jnp.int32, dcol.shape, 0)
        dvec = jnp.sum(jnp.where(rows == t, dcol, 0.0), axis=0, keepdims=True)
        dvb = jnp.broadcast_to(dvec, (8, LANES))
        tapb = [jnp.broadcast_to(taps[j:j + 1, :], (8, LANES)) for j in range(4)]
        never = zero_v[...] > 0
        fwd = fwd_ref[...]
        NGR = NB // GA
        GW = GA * BLK

        def conv_item(tok, r0):
            kf[8 + r0:24 + r0, :] = ain[sl, 0, r0:r0 + 16, :].astype(F32)
            halves = []
            for h in range(2):
                r = 8 + r0 + 8 * h
                ks = kf[r:r + 8, :] * _tie(never, tok, tapb[0])
                for j in range(1, 4):
                    ks = ks + kf[r - j:r - j + 8, :] * tapb[j]
                halves.append(ks)
            kvb[r0:r0 + 16, :] = (jnp.concatenate(halves, axis=0)
                                  * ain[sl, 1, r0:r0 + 16, :].astype(F32)).astype(BF16)

        hlast = [None]

        def h_fwd(g):
            hst = jnp.concatenate([ah[sl, :, b * BLK:(b + 1) * BLK]
                                   for b in range(g * GA, (g + 1) * GA)], axis=0)
            hh = lax.dot_general(fwd, hst, (((1,), (1,)), ((), ())), preferred_element_type=F32)
            for b in range(GA):
                cur = hh[:, b * BLK:(b + 1) * BLK]
                prev = hlast[0]
                c = slice((g * GA + b) * BLK, (g * GA + b + 1) * BLK)
                if prev is None:
                    hf[:, c] = cur
                else:
                    for m in range(BLK // 8):
                        re = slice(16 * m, 16 * m + 8)
                        im = slice(16 * m + 8, 16 * m + 16)
                        if m < BLK // 16:
                            hf[re, c] = cur[re] - prev[im]
                            hf[im, c] = cur[im] + prev[re]
                        else:
                            hf[re, c] = cur[re] + prev[im]
                            hf[im, c] = cur[im] - prev[re]
                hlast[0] = cur
            return hh

        def x_fwd(g):
            rhs = jnp.concatenate([kvb[b * BLK:(b + 1) * BLK, :]
                                   for b in range(g * GA, (g + 1) * GA)], axis=1)
            xx = _dot(fwd, rhs)
            xf[:, g * GW:(g + 1) * GW] = xx
            return xx

        def inverse(g):
            ys = []
            for par in range(2):
                y = _dot(inv_ref[par * (BLK // 2):(par + 1) * (BLK // 2), :],
                         wf[par * BLK:(par + 1) * BLK, g * GW:(g + 1) * GW])
                for a in range(GA):
                    yt[pl.ds((g * GA + a) * BLK + par, BLK // 2, stride=2), :] = (
                        y[:, a * BLK:(a + 1) * BLK])
                ys.append(y)
            return jnp.concatenate(ys, axis=0)

        def out_item(tok, r0):
            d8 = _tie(never, tok, dvb)
            yb = yt[r0:r0 + 16, :] + kvb[r0:r0 + 16, :].astype(F32) * jnp.concatenate([d8, d8], axis=0)
            aout[t, r0:r0 + 16, :] = (ain[sl, 2, r0:r0 + 16, :].astype(F32) * yb).astype(BF16)

        def rows16(fn, g, w):
            return [(functools.partial(fn, r0=r0), w) for r0 in range(g * GW, (g + 1) * GW, 16)]

        vgen = v_products(t, list(range(1, NRB)), never)
        nv = 2 * (NRB - 1) * 7
        work = {('conv', g): rows16(conv_item, g, 25) for g in range(NGR)}
        work.update({('freq', g): freq_items(g * GA, never) for g in range(NGR)})
        work.update({('out', g): rows16(out_item, g, 16) for g in range(NGR)})
        for kind, g, chunks in _interleave(nv, NGR, {k: [w for _, w in v] for k, v in work.items()}):
            if kind is not None:
                m = (next(vgen) if kind == 'v' else
                     {'h': h_fwd, 'x': x_fwd, 'inv': inverse}[kind](g))
                toks = _tokens(m)
            items = [work[k][i][0] for k, i in chunks]
            if kind is None:
                for it in items:
                    it(None)
            elif items:
                _run_paced(items, toks)
        _drain(vgen)
        for which in (WQ, WK):
            w_copy(which, 2 * t).start()
            w_copy(which, 2 * t + 1).start()
        aout_copy(t).start()
        return carry

    for cp in small[1:]:
        cp.wait()
    wo_copy(0).start()
    lax.fori_loop(0, NT, tile_body, 0)
    pltpu.make_async_copy(wo, wo, sem_wo).wait()

    def initial_guess():
        puni = pl.reciprocal(jnp.full((1, 1), float(L), F32), approx=True).astype(BF16).astype(F32)

        def shift_down(m):
            rows = lax.broadcasted_iota(jnp.int32, m.shape, 0)
            return jnp.where(rows == 0, 0.0, pltpu.roll(m, 1, 0))

        tall = jnp.concatenate([tsum[g, 0:NSEG, :] for g in range(NG)], axis=1)
        wov = wo[...]
        m1 = shift_down(_dot((tall * puni).astype(BF16), wov))
        v1 = _dot(m1.astype(BF16), w_plain(WV, 0, H // 2)).astype(BF16).astype(F32)
        u2 = ((tall + float(M) * v1) * puni).astype(BF16)
        for c in range(0, DM, LANES):
            mcol[c // LANES] = _dot(u2, wov[:, c:c + LANES])
            for sg in range(NSEG):
                mhat[(sg + 1) * M:(sg + 2) * M, c:c + LANES] = jnp.broadcast_to(
                    mcol[c // LANES, sg:sg + 1, :], (M, LANES))
        mhat[0:M, :] = mem0_ref[...].astype(F32)
        pltpu.make_async_copy(w32.at[WQ:WK + 1], w32.at[WQ:WK + 1], sem_wqk).wait()

    ri = lax.broadcasted_iota(jnp.int32, (PR, PR), 0)
    ci = lax.broadcasted_iota(jnp.int32, (PR, PR), 1)

    def seg_of(r):
        return jnp.where(r < MR, r // M, (r - MR) // SEG)

    def pos_of(r):
        return jnp.where(r < MR, r % M, M + (r - MR) % SEG)

    same = seg_of(ri) == seg_of(ci)
    allowed = same & ((ri < MR) | (pos_of(ri) >= pos_of(ci)))
    fill = jnp.where(same, -1e9, -jnp.inf).astype(F32)

    def sweep(state):
        it, _ = state
        pl.when(it == 0)(initial_guess)

        @pl.when(it > 0)
        def _():
            def upd(rb, cy):
                n = PPB * MR
                r = pl.ds(pl.multiple_of(rb * n, n), n)
                r2 = pl.ds(pl.multiple_of(rb * n + M, M), n)
                keep = jnp.tile(okbuf[r, :], (1, DM // LANES)) > 0.5
                mhat[r2, :] = jnp.where(keep, mhat[r2, :], mnew[r, :])
                return cy

            lax.fori_loop(0, NRB, upd, 0)

        def mem_rows(i):
            n = PPB * MR
            return mhat[pl.ds(pl.multiple_of((i // NG) * n, n), n), :]

        def mem_lhs(i):
            m = mem_rows(i)
            n = PPH * MR
            ops = [_pack(o) for o in _strassen_lhs(m[:n, :KH], m[:n, KH:], m[n:, :KH], m[n:, KH:])]
            t = jnp.concatenate([jnp.where(i < NG, 0.0, m[:M]), m[M:MR]], axis=0)
            b = m[n:n + MR]
            vops = [jnp.concatenate([_pack(o), full[MW:]], axis=0) for o, full in zip(
                _strassen_lhs(t[:, :KH], t[:, KH:], b[:, :KH], b[:, KH:]), ops)]
            return ops, vops

        def qk_proj(i, j, mops):
            rb = i // NG
            hp = (i % NG) * (G // 2) + j // 2

            def lhs(k):
                return _unpack(jnp.concatenate([mops[k], abuf[rb, k]], axis=0))

            n = PPH * MR
            cs = {}

            def emit(half, hh, cv):
                cs[half, hh] = cv
                if (half, 1 - hh) in cs:
                    v = jnp.concatenate([cs[half, 0], cs[half, 1]], axis=1).astype(BF16)
                    ps = slice(half * PPH, (half + 1) * PPH)
                    qks[j, ps, 0:MR, :] = v[:n].reshape(PPH, MR, 2 * E)
                    qks[j, ps, MR:PR, :] = v[n:].reshape(PPH, XR, 2 * E)

            return _strassen(lhs, w_rhs(WQ + j % 2, hp, [zero_s[k] for k in range(7)]), emit)

        def vm_proj(i, j, vops):
            hp = (i % NG) * (G // 2) + j

            def emit(half, hh, cv):
                if half == 0:
                    v0 = tsum[i % NG, NSEG:NSEG + M, (2 * j + hh) * E:(2 * j + hh + 1) * E]
                    cv = jnp.concatenate([jnp.where(i < NG, v0, cv[:M]), cv[M:]], axis=0)
                vms[half * PPH:(half + 1) * PPH, :, (2 * j + hh) * E:(2 * j + hh + 1) * E] = (
                    cv.astype(BF16).reshape(PPH, MR, E))

            return _strassen(lambda k: _unpack(vops[k]),
                             w_rhs(WV, hp, [zero_s[k] for k in range(7)]), emit)

        def scores(j):
            c = slice((j % 2) * E, (j % 2 + 1) * E)
            return lax.dot_general(qks[2 * (j // 2), :, :, c], qks[2 * (j // 2) + 1, :, :, c],
                                   (((2,), (2,)), ((0,), (0,))), preferred_element_type=F32)

        def attend(i, j, s):
            p0 = pl.multiple_of((i // NG) * PPB, PPB)
            s = jnp.where(allowed[None], s * scale, fill[None])
            e = jnp.exp(s - jnp.max(s, axis=-1, keepdims=True))
            p = (e * pl.reciprocal(jnp.sum(e, axis=-1, keepdims=True), approx=True)).astype(BF16)
            vh = jnp.concatenate(
                [vms[:, :, j * E:(j + 1) * E],
                 vbuf[i % NG, pl.ds(p0, PPB), :, j * E:(j + 1) * E]], axis=1)
            return lax.dot_general(p, vh, (((2,), (1,)), ((0,), (0,))), preferred_element_type=F32)

        def wo_rows(i):
            return wo[pl.ds(pl.multiple_of((i % NG) * (G * E), G * E), G * E), :]

        def out_mem(i, us, split):
            rb = i // NG
            wog = wo_rows(i)
            rm = pl.ds(pl.multiple_of(rb * (PPB * MR), PPB * MR), PPB * MR)
            new = jnp.where(i % NG > 0, mnew[rm, :], 0.0)
            n = G // split
            for j in range(0, G, n):
                um = jnp.concatenate([u[:, :MR, :] for u in us[j:j + n]], axis=2)
                new = new + _dot(um.reshape(PPB * MR, n * E).astype(BF16), wog[j * E:(j + n) * E])
            mnew[rm, :] = new
            old = mhat[pl.ds(pl.multiple_of(rb * (PPB * MR) + M, M), PPB * MR), :]
            err = jnp.max(jnp.abs(new - old), axis=1, keepdims=True)
            ref = jnp.max(jnp.abs(new), axis=1, keepdims=True)
            okbuf[rm, :] = jnp.broadcast_to(jnp.where(err <= TOL * ref, 1.0, 0.0),
                                            (PPB * MR, LANES))

        def out_tok(i, us, last):
            rb = i // NG
            n = PPH * XR
            kh = G * E // 2

            def quad(half, kk):
                if len(us) < 2 * kk + 2:
                    kk = 0
                u = jnp.concatenate(us[2 * kk:2 * kk + 2], axis=2)
                return u[half * PPH:(half + 1) * PPH, MR:, :].reshape(n, kh)

            def lhs(k):
                return _strassen_lhs(quad(0, 0), quad(0, 1), quad(1, 0), quad(1, 1))[k].astype(BF16)

            wf32 = wo_rows(i).astype(F32)
            rhs = _strassen_rhs(wf32[:kh, :KH], wf32[:kh, KH:], wf32[kh:, :KH], wf32[kh:, KH:])
            quads = [(slice(0, n), slice(0, KH)), (slice(0, n), slice(KH, DM)),
                     (slice(n, 2 * n), slice(0, KH)), (slice(n, 2 * n), slice(KH, DM))]
            init = [jnp.where(i % NG > 0, acc[r, c], 0.0) for r, c in quads]

            def emit(half, hh, v):
                r, c = quads[2 * half + hh]
                obuf[rb, r, c] = v.astype(BF16)
                if last:
                    oq_copy(2 * half + hh).start()
                else:
                    acc[r, c] = v

            if last:
                return _strassen(lhs, rhs, emit, init, order=(2, 5, 4, 1, 3, 0, 6))
            return _strassen(lhs, rhs, emit, init)

        def step(i):
            s0, s1 = scores(0), scores(1)
            mops, vops = mem_lhs(i + 1)
            _drain(qk_proj(i + 1, 0, mops))
            us = [attend(i, 0, s0), attend(i, 1, s1)]
            s2, s3 = scores(2), scores(3)
            _drain(qk_proj(i + 1, 1, mops))
            us += [attend(i, 2, s2), attend(i, 3, s3)]
            _drain(zip(qk_proj(i + 1, 2, mops), vm_proj(i + 1, 0, vops)))
            _drain(zip(qk_proj(i + 1, 3, mops), vm_proj(i + 1, 1, vops)))
            out_mem(i, us, 1)
            _drain(out_tok(i, us, False))

        def last_step(i):
            ss = [scores(j) for j in range(G)]
            us = [attend(i, 0, ss[0]), attend(i, 1, ss[1])]
            gen = out_tok(i, us, True)
            next(gen)
            next(gen)
            us += [attend(i, 2, ss[2]), attend(i, 3, ss[3])]
            out_mem(i, us, 2)
            _drain(gen)

        mops0, vops0 = mem_lhs(0)
        _drain(qk_proj(0, 0, mops0), qk_proj(0, 1, mops0))
        _drain(zip(qk_proj(0, 2, mops0), vm_proj(0, 0, vops0)))
        _drain(zip(qk_proj(0, 3, mops0), vm_proj(0, 1, vops0)))

        def main_body(i, cy):
            step(i)

            @pl.when(i % NG == NG - 1)
            def _():
                o_copy(i // NG).start()

            return cy

        lax.fori_loop(0, NRB * NG - 1, main_body, 0)
        last_step(NRB * NG - 1)
        ok = jnp.min(okbuf[0:(NSEG - 1) * M, :])
        for rb in range(NRB - 1):
            o_copy(rb).wait()
        for qd in range(4):
            oq_copy(qd).wait()
        return it + 1, (ok > 0.5).astype(jnp.int32)

    lax.while_loop(lambda st: jnp.logical_and(st[0] < NSEG, st[1] == 0), sweep,
                   (jnp.int32(0), jnp.int32(0)))
    pltpu.make_async_copy(aout, aout, sem_aout).wait()


@functools.partial(jax.jit, static_argnames=("B_seg_len",))
def pallas_concat_heads__ssm_conv_h3__memory_aug_recurrent_mem_tr__prompt_kernel(
    A_q, A_k, A_v, A_shift_k, A_ssm_k, A_ssm_D,
    B_x, B_mem0, B_Wq, B_Wk, B_Wv, B_Wo, B_seg_len,
):
    _, S, D = A_q.shape
    DM = B_x.shape[2]
    H, E = B_Wq.shape[1], B_Wq.shape[2]
    M = B_mem0.shape[1]
    SEG = int(B_seg_len)
    NSEG = S // SEG
    NP = NSEG // 2
    PR = 2 * (M + SEG)
    PPB = 8
    NRB = NP // PPB
    NT = D // LANES
    assert E == LANES and H == 32 and M == 8 and SEG == 32 and A_shift_k.shape[1] == 4
    assert S == 2048 and D == 1024 and DM == 1024

    fwd, inv = _dft_mats()
    any_spec = pl.BlockSpec(memory_space=pl.ANY)
    scratch = [
        pltpu.VMEM((NRB, 7, PPB // 2 * SEG, DM // 2), U32),
        pltpu.VMEM((7, M + PPB // 2 * SEG, DM // 2), U32),
        pltpu.VMEM((H // 4, NP, 2 * SEG, 4 * E), BF16),
        pltpu.VMEM((3, H // 2, DM, E), U32),
        pltpu.VMEM((H * E, DM), BF16),
        pltpu.VMEM((4, PPB, PR, 2 * E), BF16),
        pltpu.VMEM((PPB, 2 * M, 4 * E), BF16),
        pltpu.VMEM((PPB * 2 * SEG, DM), F32),
        pltpu.VMEM((NRB, PPB * 2 * SEG, DM), BF16),
        pltpu.VMEM(((NSEG + 1) * M, DM), F32),
        pltpu.VMEM((NSEG * M, DM), F32),
        pltpu.VMEM((NSEG * M, LANES), F32),
        pltpu.VMEM((DM // LANES, NSEG, LANES), F32),
        pltpu.VMEM((H // 4, NSEG + M, 4 * E), F32),
        pltpu.VMEM((2, 3, S, LANES), BF16),
        pltpu.VMEM((2, LANES, S), BF16),
        pltpu.VMEM((S + 32, LANES), F32),
        pltpu.VMEM((S, LANES), BF16),
        pltpu.VMEM((NFFT, S), F32),
        pltpu.VMEM((NFFT, S), F32),
        pltpu.VMEM((NFFT, S), BF16),
        pltpu.VMEM((S, LANES), F32),
        pltpu.VMEM((NT, S, LANES), BF16),
        pltpu.VMEM((M, DM), BF16),
        pltpu.VMEM((NFFT, BLK), BF16),
        pltpu.VMEM((BLK, BLK), BF16),
        pltpu.VMEM((4, D), BF16),
        pltpu.VMEM((NT, LANES), BF16),
        pltpu.VMEM((8, LANES), jnp.int32),
        pltpu.SMEM((8,), jnp.int32),
        pltpu.SemaphoreType.DMA((5,)),
        pltpu.SemaphoreType.DMA((2 * NRB,)),
        pltpu.SemaphoreType.DMA((H // 2,)),
        pltpu.SemaphoreType.DMA,
        pltpu.SemaphoreType.DMA,
        pltpu.SemaphoreType.DMA((2, 2)),
        pltpu.SemaphoreType.DMA,
        pltpu.SemaphoreType.DMA((NRB + 3,)),
    ]
    out = pl.pallas_call(
        functools.partial(_kernel, S=S, D=D, DM=DM, H=H, M=M, SEG=SEG),
        out_shape=jax.ShapeDtypeStruct((S, D + DM), BF16),
        in_specs=[any_spec] * 14,
        out_specs=any_spec,
        scratch_shapes=scratch,
        compiler_params=pltpu.CompilerParams(vmem_limit_bytes=120 * 1024 * 1024,
                                             disable_bounds_checks=True,
                                             disable_semaphore_checks=True),
    )(
        A_q.reshape(S, D), A_k.reshape(S, D), A_v.reshape(S, D),
        A_shift_k.T, A_ssm_k, A_ssm_D.reshape(NT, LANES),
        B_x.reshape(NRB, S // NRB, DM), B_mem0.reshape(M, DM),
        B_Wq, B_Wk, B_Wv, B_Wo.reshape(H * E, DM),
        jnp.asarray(fwd, BF16), jnp.asarray(inv, BF16),
    )
    return out.reshape(1, S, D + DM)
```

```python
import functools

import numpy as np
import jax
import jax.numpy as jnp
from jax import lax
import jax.experimental.pallas as pl
import jax.experimental.pallas.tpu as pltpu

F32 = jnp.float32
BF16 = jnp.bfloat16
U32 = jnp.uint32

LANES = 128
BLK = 128
NFFT = 2 * BLK
TOL = 2.0 ** -10


def _dft_mats():
    even = np.arange(0, BLK, 2)
    theta = 2.0 * np.pi * (np.concatenate([even, BLK - 1 - even]) + 0.5) / NFFT
    n = np.arange(BLK)
    c = np.cos(theta[:, None] * n[None, :])
    s = np.sin(theta[:, None] * n[None, :])
    fwd = np.zeros((NFFT, BLK))
    for m in range(BLK // 8):
        fwd[16 * m:16 * m + 8] = c[8 * m:8 * m + 8]
        fwd[16 * m + 8:16 * m + 16] = -s[8 * m:8 * m + 8]
    inv = fwd[:BLK].T * (2.0 / NFFT)
    inv = np.concatenate([inv[0::2], inv[1::2]], axis=0)
    return fwd.astype(np.float32), inv.astype(np.float32)


def _dot(a, b):
    return jnp.dot(a, b, preferred_element_type=F32)


def _pack(x):
    return pltpu.bitcast(x.astype(BF16), U32)


def _unpack(w):
    return pltpu.bitcast(w, BF16)


def _lo(w):
    return pltpu.bitcast(w << 16, F32)


def _hi(w):
    return pltpu.bitcast(w & jnp.uint32(0xFFFF0000), F32)


_STRASSEN_LHS = ((0, 3, 1), (2, 3, 1), (0, None, 0), (3, None, 0), (0, 1, 1), (2, 0, -1), (1, 3, -1))
_STRASSEN_RHS = ((0, 3, 1), (0, None, 0), (1, 3, -1), (2, 0, -1), (3, None, 0), (0, 1, 1), (2, 3, 1))


def _operand(table, k, quad):
    i, j, sign = table[k]
    if j is None:
        return quad(i)
    return quad(i) + quad(j) if sign > 0 else quad(i) - quad(j)


def _strassen_lhs(*quads):
    return [_operand(_STRASSEN_LHS, k, quads.__getitem__) for k in range(7)]


_STRASSEN_USES = (((0, 1), (3, 1)), ((2, 1), (3, -1)), ((1, 1), (3, 1)), ((0, 1), (2, 1)),
                  ((0, -1), (1, 1)), ((3, 1),), ((0, 1),))


def _strassen(lhs, rhs, emit, init=None, order=(4, 2, 1, 3, 0, 6, 5), post=None):
    acc = [[(1, c)] if c is not None else [] for c in (init or (None,) * 4)]
    left = [4, 2, 2, 4]
    for k in order:
        m = _dot(lhs(k), rhs[k])
        if post is not None:
            m = post(k, m)
        for q, sign in _STRASSEN_USES[k]:
            acc[q].append((sign, m))
            left[q] -= 1
            if left[q] < (3, 1, 1, 3)[q]:
                terms = sorted(acc[q], key=lambda t: -t[0])
                v = terms[0][1]
                assert terms[0][0] > 0
                for sg, t in terms[1:]:
                    v = v + t if sg > 0 else v - t
                acc[q] = [(1, v)]
            if left[q] == 0:
                emit(q // 2, q % 2, acc[q][0][1])
        yield m


def _drain(*gens):
    for g in gens:
        for _ in g:
            pass


def _tokens(m):
    return [(m, r, c) for r in range(0, m.shape[0], 8) for c in range(0, m.shape[1], LANES)]


def _tie(never, tok, x):
    if tok is None:
        return x
    reps = (x.shape[0] // 8, x.shape[1] // LANES)
    if tok.dtype != x.dtype:
        tok = pltpu.bitcast(tok, x.dtype)
    if reps != (1, 1):
        never, tok = jnp.tile(never, reps), jnp.tile(tok, reps)
    return jnp.where(never, tok, x)


def _run_paced(items, toks):
    for i, it in enumerate(items):
        m, r, c = toks[i * len(toks) // len(items)]
        it(m[r:r + 8, c:c + LANES])


def _interleave(nv, ngr, weights):
    dur = {'v': 256, 'h': 256, 'x': 256, 'inv': 128}
    margin = 768

    def plan(rate):
        t, v, out = 0, 0, []
        nxt = {'h': 0, 'x': 0, 'inv': 0}
        pos = {k: 0 for k in weights}
        done = {}
        credit = 0.0
        while True:
            kind = None
            if nxt['inv'] < ngr and done.get(('freq', nxt['inv']), 1e9) + margin <= t:
                kind = 'inv'
            elif nxt['x'] < ngr and done.get(('conv', nxt['x']), 1e9) + margin <= t:
                kind = 'x'
            elif nxt['h'] < ngr and nxt['h'] <= nxt['x'] and out and out[-1][0] == 'v':
                kind = 'h'
            elif v < nv:
                kind = 'v'
            if kind is None:
                break
            g = v if kind == 'v' else nxt[kind]
            busy = 0.6 if kind != 'v' else 1.1 if v % (nv // 2) < 7 else 0.0
            credit += (rate - busy) * dur[kind]
            chunk = []
            while credit > 0:
                ready = [('out', i) for i in range(nxt['inv'])]
                ready += [('conv', i) for i in range(ngr)]
                ready += [('freq', i) for i in range(min(nxt['x'], nxt['h']))]
                ready = [k for k in ready if pos[k] < len(weights[k])]
                if not ready:
                    credit = 0.0
                    break
                k = ready[0]
                chunk.append((k, pos[k]))
                credit -= weights[k][pos[k]]
                pos[k] += 1
                if pos[k] == len(weights[k]):
                    done[k] = t + dur[kind]
            out.append((kind, g, chunk))
            t += dur[kind]
            if kind == 'v':
                v += 1
            else:
                nxt[kind] += 1
        ok = all(pos[k] == len(weights[k]) for k in weights)
        return ok, out

    rate = 1.0
    while True:
        ok, out = plan(rate)
        if ok:
            return out
        rate += 0.02


def _kernel(q_hbm, k_hbm, v_hbm, shift_hbm, h_hbm, d_hbm, x_hbm, mem0_hbm,
            wq_hbm, wk_hbm, wv_hbm, wo_hbm, fwd_hbm, inv_hbm,
            out_hbm,
            abuf, a0buf, vbuf, w32, wo, qks, vms, acc, obuf, mhat, mnew, okbuf, mcol, tsum,
            ain, ah, kf, kvb, xf, hf, wf, yt, aout,
            mem0_ref, fwd_ref, inv_ref, shift_ref, d_ref, zero_v, zero_s,
            sem_s, sem_x, sem_wv, sem_wqk, sem_wo, sem_a, sem_aout, sem_o,
            *, S, D, DM, H, M, SEG):
    E = LANES
    NSEG = S // SEG
    NP = NSEG // 2
    MR = 2 * M
    XR = 2 * SEG
    PR = MR + XR
    MW = MR // 2
    L = M + SEG
    NB = S // BLK
    NT = D // LANES
    PPB = 8
    PPH = PPB // 2
    NRB = NP // PPB
    G = 4
    NG = H // G
    KH = DM // 2
    scale = float(E) ** -0.5
    WV, WQ, WK = 0, 1, 2

    small = [pltpu.make_async_copy(src, dst, sem_s.at[i]) for i, (src, dst) in enumerate(
        ((mem0_hbm, mem0_ref), (shift_hbm, shift_ref), (d_hbm, d_ref),
         (fwd_hbm, fwd_ref), (inv_hbm, inv_ref)))]
    HBR = PPH * XR // 2

    def x_copies(hb):
        out = []
        for half in range(2):
            r = pl.ds(pl.multiple_of((2 * half + hb % 2) * HBR, HBR), HBR)
            out.append(pltpu.make_async_copy(x_hbm.at[hb // 2, r], obuf.at[hb // 2, r],
                                             sem_x.at[hb]))
        return out

    def w_copy(which, hp):
        src = (wv_hbm, wq_hbm, wk_hbm)[which].bitcast(U32)
        sem = sem_wv.at[hp] if which == WV else sem_wqk
        return pltpu.make_async_copy(src.at[:, hp, :], w32.at[which, hp], sem)

    def wo_copy(t):
        n = H * E // NT
        r = pl.ds(pl.multiple_of(t * n, n), n)
        return pltpu.make_async_copy(wo_hbm.at[r, :], wo.at[r, :], sem_wo)

    def a_start(t, sl, which=(0, 1, 2, 3)):
        c = pl.ds(pl.multiple_of(t * LANES, LANES), LANES)
        for i in which:
            if i == 3:
                pltpu.make_async_copy(h_hbm.at[c, :], ah.at[sl], sem_a.at[sl, 1]).start()
            else:
                src = (k_hbm, v_hbm, q_hbm)[i]
                pltpu.make_async_copy(src.at[:, c], ain.at[sl, i], sem_a.at[sl, 0]).start()

    def a_wait(sl):
        pltpu.make_async_copy(ain.at[sl], ain.at[sl], sem_a.at[sl, 0]).wait()
        pltpu.make_async_copy(ah.at[sl], ah.at[sl], sem_a.at[sl, 1]).wait()

    def aout_copy(t):
        c = pl.ds(pl.multiple_of(t * LANES, LANES), LANES)
        return pltpu.make_async_copy(aout.at[t], out_hbm.at[:, c], sem_aout)

    def o_copy(rb):
        r = pl.ds(pl.multiple_of(rb * (PPB * XR), PPB * XR), PPB * XR)
        return pltpu.make_async_copy(obuf.at[rb], out_hbm.at[r, pl.ds(D, DM)], sem_o.at[rb])

    def oq_copy(qd):
        n = PPH * XR
        r0, c0 = (qd // 2) * n, (qd % 2) * KH
        return pltpu.make_async_copy(
            obuf.at[NRB - 1, pl.ds(r0, n), pl.ds(c0, KH)],
            out_hbm.at[pl.ds((NRB - 1) * 2 * n + r0, n), pl.ds(D + c0, KH)],
            sem_o.at[NRB - 1 + qd])

    def w_rhs(which, hp):
        out = []
        for k in range(7):
            w = w32.at[which, hp + zero_s[k]]

            def quad(i, w=w):
                return (_lo, _hi)[i % 2](w[(i // 2) * KH:(i // 2 + 1) * KH])

            out.append(_operand(_STRASSEN_RHS, k, quad).astype(BF16))
        return out

    def w_plain(which, hp0, n):
        parts = []
        for j in range(n):
            w = w32[which, hp0 + j]
            parts += [_lo(w), _hi(w)]
        return jnp.concatenate(parts, axis=1).astype(BF16)

    small[0].start()
    for hb in range(2):
        for cp in x_copies(hb):
            cp.start()
    w_copy(WV, 0).start()
    w_copy(WV, 1).start()
    for cp in small[1:]:
        cp.start()

    kf[0:8, :] = jnp.zeros((8, LANES), F32)
    zero_v[...] = jnp.zeros((8, LANES), jnp.int32)
    for k in range(7):
        zero_s[k] = 0
    tsum[:, 0:8, 0:LANES] = jnp.zeros((NG, 8, LANES), F32)
    vbuf[:, 0, 0:16, 0:LANES] = jnp.zeros((NG, 16, LANES), BF16)
    for hb in range(2 * NRB):
        r0 = (hb % 2) * (HBR // 2)
        abuf[hb // 2, 0, r0:r0 + 8, 0:LANES] = jnp.zeros((8, LANES), U32)
    small[0].wait()
    mem0 = mem0_ref[...].astype(F32)
    m0 = jnp.concatenate([mem0, jnp.zeros_like(mem0)], axis=0)
    z0 = jnp.zeros((MR, KH), F32)
    for k, op in enumerate(_strassen_lhs(m0[:, :KH], m0[:, KH:], z0, z0)):
        a0buf[k, 0:MW, :] = _pack(op)

    def x_item(tok, never, src, dst, r, c):
        quad = [_tie(never, tok, src[h * 2 * HBR + r:h * 2 * HBR + r + 16,
                                     kk * KH + c:kk * KH + c + 2 * LANES].astype(F32))
                for h in range(2) for kk in range(2)]
        for k, op in enumerate(_strassen_lhs(*quad)):
            dst[k, r // 2:r // 2 + 8, c:c + 2 * LANES] = _pack(op)

    def x_items(never, src, dst):
        return [functools.partial(x_item, never=never, src=src, dst=dst, r=r, c=c)
                for r in range(0, HBR, 16) for c in range(0, KH, 2 * LANES)]

    def x_first(hb, cy):
        for cp in x_copies(hb):
            cp.wait()
        src = obuf.at[0, pl.ds(pl.multiple_of(hb * HBR, HBR), 3 * HBR)]
        dst = a0buf.at[:, pl.ds(pl.multiple_of(MW + hb * (HBR // 2), 8), HBR // 2)]
        for it in x_items(None, src, dst):
            it(None)
        return cy

    lax.fori_loop(0, 2, x_first, 0)

    def v_part(j, rb, rhs, vwin, twin, pre=None):
        mem0_in = (0, 2, 4, 6) if rb == 0 else ()
        m0 = {}

        def lhs(k):
            x = abuf[rb, k] if rb else (a0buf[k] if k in mem0_in else a0buf[k, MW:])
            if pre is not None and k == 4:
                x0 = jnp.concatenate([pre(x[:8, :LANES]), x[:8, LANES:]], axis=1)
                x = jnp.concatenate([x0, x[8:]], axis=0)
            return _unpack(x)

        def split(k, m):
            if k not in mem0_in:
                return m
            m0[k] = m[:M]
            return m[MR:]

        def emit(half, hh, cv):
            c = slice((2 * j + hh) * E, (2 * j + hh + 1) * E)
            vx = cv.astype(BF16)
            p0 = rb * PPB + half * PPH
            vwin[p0:p0 + PPH, :, c] = vx.reshape(PPH, XR, E)
            ts = jnp.sum(vx.astype(F32).reshape(2 * PPH, SEG, E), axis=1)
            if rb == 0 and half == 0:
                v0 = m0[2] + m0[4] if hh else m0[0] - m0[4] + m0[6]
                v0 = v0.astype(BF16).astype(F32)
                twin[NSEG:NSEG + M, c] = v0
                t0 = jnp.sum(v0, axis=0, keepdims=True)
                rows = lax.broadcasted_iota(jnp.int32, ts.shape, 0)
                ts = ts + jnp.where(rows == 0, t0, 0.0)
            twin[2 * p0:2 * (p0 + PPH), c] = ts

        return _strassen(lhs, rhs, emit, post=split)

    def v_products(t, rbs, never, extra=()):
        vwin = vbuf.at[t]
        twin = tsum.at[t]

        def pre(x):
            for v in (twin[0:8, 0:LANES], pltpu.bitcast(vwin[0, 0:16, 0:LANES], U32)) + tuple(extra):
                x = _tie(never, v, x)
            return x

        for j in range(2):
            rhs = w_rhs(WV, 2 * t + j)
            for rb in rbs:
                yield from v_part(j, rb, rhs, vwin, twin, pre if (j, rb) == (0, rbs[0]) else None)

    def head_body(j, cy):
        w_copy(WV, 2 * j).wait()
        w_copy(WV, 2 * j + 1).wait()

        @pl.when(j >= 2)
        def _():
            for cp in x_copies(j):
                cp.wait()

        @pl.when(j + 1 < NT)
        def _():
            w_copy(WV, 2 * j + 2).start()
            w_copy(WV, 2 * j + 3).start()

        @pl.when(j + 2 < 2 * NRB)
        def _():
            for cp in x_copies(j + 2):
                cp.start()

        @pl.when(j == NT - 3)
        def _():
            a_start(0, 0, (3,))

        @pl.when(j == NT - 2)
        def _():
            a_start(0, 0, (0, 1, 2))

        never = zero_v[...] > 0
        src = obuf.at[j // 2, pl.ds(pl.multiple_of((j % 2) * HBR, HBR), 3 * HBR)]
        dst = abuf.at[j // 2, :, pl.ds(pl.multiple_of((j % 2) * (HBR // 2), 8), HBR // 2)]
        toks = []
        for m in v_products(j, [0], never, [dst[0, 0:8, 0:LANES]]):
            toks += _tokens(m)
        _run_paced(x_items(never, src, dst), toks[:-40])
        return cy

    assert NT == 2 * NRB
    lax.fori_loop(0, NT, head_body, 0)

    GA = 4

    def freq_items(a0, never):
        def item(tok, m, cc, st):
            r_re = slice(16 * m, 16 * m + 8)
            r_im = slice(16 * m + 8, 16 * m + 16)
            xr = _tie(never, tok, xf[r_re, cc * BLK:(cc + 1) * BLK])
            xi = _tie(never, tok, xf[r_im, cc * BLK:(cc + 1) * BLK])
            xs = xr + xi
            for a in range(max(a0, cc), a0 + GA):
                j = a - cc
                if ('g', m, j) not in st:
                    gr = hf[r_re, j * BLK:(j + 1) * BLK]
                    gi = hf[r_im, j * BLK:(j + 1) * BLK]
                    st['g', m, j] = (gr, gi, gr + gi)
                gr, gi, gs = st['g', m, j]
                ps = (xr * gr, xi * gi, xs * gs)
                st[m, a] = ps if (m, a) not in st else tuple(u + v for u, v in zip(st[m, a], ps))
                if cc == a:
                    p1, p2, p3 = st[m, a]
                    st[m, a] = (p1 - p2, p3 - p1 - p2)
                    if m >= BLK // 16:
                        m0 = m - BLK // 16
                        (wr, wi), (vr, vi) = st[m0, a], st[m, a]
                        c = slice(a * BLK, (a + 1) * BLK)
                        wf[16 * m0:16 * m0 + 16, c] = (
                            jnp.concatenate([wr + vr, wi - vi], axis=0).astype(BF16))
                        wf[16 * m:16 * m + 16, c] = (
                            jnp.concatenate([wr - vr, wi + vi], axis=0).astype(BF16))

        items = []
        for m0 in range(BLK // 16):
            st = {}
            for m in (m0, m0 + BLK // 16):
                items += [(functools.partial(item, m=m, cc=cc, st=st),
                           4 + 6 * (a0 + GA - max(a0, cc)) + (6 if cc >= a0 else 0))
                          for cc in range(a0 + GA)]
        return items

    def tile_body(t, carry):
        sl = t & 1
        a_wait(sl)

        @pl.when(t + 1 < NT)
        def _():
            a_start(t + 1, 1 - sl)
            wo_copy(t + 1).start()

        c = pl.ds(pl.multiple_of(t * LANES, LANES), LANES)
        taps = shift_ref[:, c].astype(F32)
        dcol = d_ref[...].astype(F32)
        rows = lax.broadcasted_iota(jnp.int32, dcol.shape, 0)
        dvec = jnp.sum(jnp.where(rows == t, dcol, 0.0), axis=0, keepdims=True)
        dvb = jnp.broadcast_to(dvec, (8, LANES))
        tapb = [jnp.broadcast_to(taps[j:j + 1, :], (8, LANES)) for j in range(4)]
        never = zero_v[...] > 0
        fwd = fwd_ref[...]
        NGR = NB // GA
        GW = GA * BLK

        def conv_item(tok, r0):
            kf[8 + r0:24 + r0, :] = ain[sl, 0, r0:r0 + 16, :].astype(F32)
            halves = []
            for h in range(2):
                r = 8 + r0 + 8 * h
                ks = kf[r:r + 8, :] * _tie(never, tok, tapb[0])
                for j in range(1, 4):
                    ks = ks + kf[r - j:r - j + 8, :] * tapb[j]
                halves.append(ks)
            kvb[r0:r0 + 16, :] = (jnp.concatenate(halves, axis=0)
                                  * ain[sl, 1, r0:r0 + 16, :].astype(F32)).astype(BF16)

        hlast = [None]

        def h_fwd(g):
            hst = jnp.concatenate([ah[sl, :, b * BLK:(b + 1) * BLK]
                                   for b in range(g * GA, (g + 1) * GA)], axis=0)
            hh = lax.dot_general(fwd, hst, (((1,), (1,)), ((), ())), preferred_element_type=F32)
            for b in range(GA):
                cur = hh[:, b * BLK:(b + 1) * BLK]
                prev = hlast[0]
                c = slice((g * GA + b) * BLK, (g * GA + b + 1) * BLK)
                if prev is None:
                    hf[:, c] = cur
                else:
                    for m in range(BLK // 8):
                        re = slice(16 * m, 16 * m + 8)
                        im = slice(16 * m + 8, 16 * m + 16)
                        if m < BLK // 16:
                            hf[re, c] = cur[re] - prev[im]
                            hf[im, c] = cur[im] + prev[re]
                        else:
                            hf[re, c] = cur[re] + prev[im]
                            hf[im, c] = cur[im] - prev[re]
                hlast[0] = cur
            return hh

        def x_fwd(g):
            rhs = jnp.concatenate([kvb[b * BLK:(b + 1) * BLK, :]
                                   for b in range(g * GA, (g + 1) * GA)], axis=1)
            xx = _dot(fwd, rhs)
            xf[:, g * GW:(g + 1) * GW] = xx
            return xx

        def inverse(g):
            ys = []
            for par in range(2):
                y = _dot(inv_ref[par * (BLK // 2):(par + 1) * (BLK // 2), :],
                         wf[par * BLK:(par + 1) * BLK, g * GW:(g + 1) * GW])
                for a in range(GA):
                    yt[pl.ds((g * GA + a) * BLK + par, BLK // 2, stride=2), :] = (
                        y[:, a * BLK:(a + 1) * BLK])
                ys.append(y)
            return jnp.concatenate(ys, axis=0)

        def out_item(tok, r0):
            d8 = _tie(never, tok, dvb)
            yb = yt[r0:r0 + 16, :] + kvb[r0:r0 + 16, :].astype(F32) * jnp.concatenate([d8, d8], axis=0)
            aout[t, r0:r0 + 16, :] = (ain[sl, 2, r0:r0 + 16, :].astype(F32) * yb).astype(BF16)

        def rows16(fn, g, w):
            return [(functools.partial(fn, r0=r0), w) for r0 in range(g * GW, (g + 1) * GW, 16)]

        vgen = v_products(t, list(range(1, NRB)), never)
        nv = 2 * (NRB - 1) * 7
        work = {('conv', g): rows16(conv_item, g, 25) for g in range(NGR)}
        work.update({('freq', g): freq_items(g * GA, never) for g in range(NGR)})
        work.update({('out', g): rows16(out_item, g, 16) for g in range(NGR)})
        for kind, g, chunks in _interleave(nv, NGR, {k: [w for _, w in v] for k, v in work.items()}):
            m = next(vgen) if kind == 'v' else {'h': h_fwd, 'x': x_fwd, 'inv': inverse}[kind](g)
            _run_paced([work[k][i][0] for k, i in chunks], _tokens(m))
        _drain(vgen)
        for which in (WQ, WK):
            w_copy(which, 2 * t).start()
            w_copy(which, 2 * t + 1).start()
        aout_copy(t).start()
        return carry

    for cp in small[1:]:
        cp.wait()
    wo_copy(0).start()
    lax.fori_loop(0, NT, tile_body, 0)
    pltpu.make_async_copy(wo, wo, sem_wo).wait()

    def initial_guess():
        puni = pl.reciprocal(jnp.full((1, 1), float(L), F32), approx=True).astype(BF16).astype(F32)

        def shift_down(m):
            rows = lax.broadcasted_iota(jnp.int32, m.shape, 0)
            return jnp.where(rows == 0, 0.0, pltpu.roll(m, 1, 0))

        tall = jnp.concatenate([tsum[g, 0:NSEG, :] for g in range(NG)], axis=1)
        wov = wo[...]
        m1 = shift_down(_dot((tall * puni).astype(BF16), wov))
        v1 = _dot(m1.astype(BF16), w_plain(WV, 0, H // 2)).astype(BF16).astype(F32)
        u2 = ((tall + float(M) * v1) * puni).astype(BF16)
        for c in range(0, DM, LANES):
            mcol[c // LANES] = _dot(u2, wov[:, c:c + LANES])
            for sg in range(NSEG):
                mhat[(sg + 1) * M:(sg + 2) * M, c:c + LANES] = jnp.broadcast_to(
                    mcol[c // LANES, sg:sg + 1, :], (M, LANES))
        mhat[0:M, :] = mem0_ref[...].astype(F32)
        pltpu.make_async_copy(w32.at[WQ:WK + 1], w32.at[WQ:WK + 1], sem_wqk).wait()

    ri = lax.broadcasted_iota(jnp.int32, (PR, PR), 0)
    ci = lax.broadcasted_iota(jnp.int32, (PR, PR), 1)

    def seg_of(r):
        return jnp.where(r < MR, r // M, (r - MR) // SEG)

    def pos_of(r):
        return jnp.where(r < MR, r % M, M + (r - MR) % SEG)

    same = seg_of(ri) == seg_of(ci)
    allowed = same & ((ri < MR) | (pos_of(ri) >= pos_of(ci)))
    fill = jnp.where(same, -1e9, -jnp.inf).astype(F32)

    def sweep(state):
        it, _ = state
        pl.when(it == 0)(initial_guess)

        @pl.when(it > 0)
        def _():
            def upd(rb, cy):
                n = PPB * MR
                r = pl.ds(pl.multiple_of(rb * n, n), n)
                r2 = pl.ds(pl.multiple_of(rb * n + M, M), n)
                keep = jnp.tile(okbuf[r, :], (1, DM // LANES)) > 0.5
                mhat[r2, :] = jnp.where(keep, mhat[r2, :], mnew[r, :])
                return cy

            lax.fori_loop(0, NRB, upd, 0)

        def mem_rows(i):
            n = PPB * MR
            return mhat[pl.ds(pl.multiple_of((i // NG) * n, n), n), :]

        def mem_lhs(i):
            m = mem_rows(i)
            n = PPH * MR
            ops = [_pack(o) for o in _strassen_lhs(m[:n, :KH], m[:n, KH:], m[n:, :KH], m[n:, KH:])]
            t = jnp.concatenate([jnp.where(i < NG, 0.0, m[:M]), m[M:MR]], axis=0)
            b = m[n:n + MR]
            vops = [jnp.concatenate([_pack(o), full[MW:]], axis=0) for o, full in zip(
                _strassen_lhs(t[:, :KH], t[:, KH:], b[:, :KH], b[:, KH:]), ops)]
            return ops, vops

        def qk_proj(i, j, mops):
            rb = i // NG
            hp = (i % NG) * (G // 2) + j // 2

            def lhs(k):
                return _unpack(jnp.concatenate([mops[k], abuf[rb, k]], axis=0))

            n = PPH * MR
            cs = {}

            def emit(half, hh, cv):
                cs[half, hh] = cv
                if (half, 1 - hh) in cs:
                    v = jnp.concatenate([cs[half, 0], cs[half, 1]], axis=1).astype(BF16)
                    ps = slice(half * PPH, (half + 1) * PPH)
                    qks[j, ps, 0:MR, :] = v[:n].reshape(PPH, MR, 2 * E)
                    qks[j, ps, MR:PR, :] = v[n:].reshape(PPH, XR, 2 * E)

            return _strassen(lhs, w_rhs(WQ + j % 2, hp), emit)

        def vm_proj(i, j, vops):
            hp = (i % NG) * (G // 2) + j

            def emit(half, hh, cv):
                if half == 0:
                    v0 = tsum[i % NG, NSEG:NSEG + M, (2 * j + hh) * E:(2 * j + hh + 1) * E]
                    cv = jnp.concatenate([jnp.where(i < NG, v0, cv[:M]), cv[M:]], axis=0)
                vms[half * PPH:(half + 1) * PPH, :, (2 * j + hh) * E:(2 * j + hh + 1) * E] = (
                    cv.astype(BF16).reshape(PPH, MR, E))

            return _strassen(lambda k: _unpack(vops[k]), w_rhs(WV, hp), emit)

        def scores(j):
            c = slice((j % 2) * E, (j % 2 + 1) * E)
            return lax.dot_general(qks[2 * (j // 2), :, :, c], qks[2 * (j // 2) + 1, :, :, c],
                                   (((2,), (2,)), ((0,), (0,))), preferred_element_type=F32)

        def attend(i, j, s):
            p0 = pl.multiple_of((i // NG) * PPB, PPB)
            s = jnp.where(allowed[None], s * scale, fill[None])
            e = jnp.exp(s - jnp.max(s, axis=-1, keepdims=True))
            p = (e * pl.reciprocal(jnp.sum(e, axis=-1, keepdims=True), approx=True)).astype(BF16)
            vh = jnp.concatenate(
                [vms[:, :, j * E:(j + 1) * E],
                 vbuf[i % NG, pl.ds(p0, PPB), :, j * E:(j + 1) * E]], axis=1)
            return lax.dot_general(p, vh, (((2,), (1,)), ((0,), (0,))), preferred_element_type=F32)

        def wo_rows(i):
            return wo[pl.ds(pl.multiple_of((i % NG) * (G * E), G * E), G * E), :]

        def out_mem(i, us, split):
            rb = i // NG
            wog = wo_rows(i)
            rm = pl.ds(pl.multiple_of(rb * (PPB * MR), PPB * MR), PPB * MR)
            new = jnp.where(i % NG > 0, mnew[rm, :], 0.0)
            n = G // split
            for j in range(0, G, n):
                um = jnp.concatenate([u[:, :MR, :] for u in us[j:j + n]], axis=2)
                new = new + _dot(um.reshape(PPB * MR, n * E).astype(BF16), wog[j * E:(j + n) * E])
            mnew[rm, :] = new
            old = mhat[pl.ds(pl.multiple_of(rb * (PPB * MR) + M, M), PPB * MR), :]
            err = jnp.max(jnp.abs(new - old), axis=1, keepdims=True)
            ref = jnp.max(jnp.abs(new), axis=1, keepdims=True)
            okbuf[rm, :] = jnp.broadcast_to(jnp.where(err <= TOL * ref, 1.0, 0.0),
                                            (PPB * MR, LANES))

        def out_tok(i, us, last):
            rb = i // NG
            n = PPH * XR
            kh = G * E // 2

            def uquad(q):
                u = jnp.concatenate([us[2 * (q % 2)], us[2 * (q % 2) + 1]], axis=2)
                return u[(q // 2) * PPH:(q // 2 + 1) * PPH, MR:, :].reshape(n, kh)

            def lhs(k):
                return _operand(_STRASSEN_LHS, k, uquad).astype(BF16)

            wf32 = wo_rows(i).astype(F32)
            wq4 = [wf32[:kh, :KH], wf32[:kh, KH:], wf32[kh:, :KH], wf32[kh:, KH:]]
            rhs = [_operand(_STRASSEN_RHS, k, wq4.__getitem__).astype(BF16) for k in range(7)]
            quads = [(slice(0, n), slice(0, KH)), (slice(0, n), slice(KH, DM)),
                     (slice(n, 2 * n), slice(0, KH)), (slice(n, 2 * n), slice(KH, DM))]
            init = [jnp.where(i % NG > 0, acc[r, c], 0.0) for r, c in quads]

            def emit(half, hh, v):
                r, c = quads[2 * half + hh]
                obuf[rb, r, c] = v.astype(BF16)
                if last:
                    oq_copy(2 * half + hh).start()
                else:
                    acc[r, c] = v

            if last:
                return _strassen(lhs, rhs, emit, init, order=(2, 5, 4, 1, 3, 0, 6))
            return _strassen(lhs, rhs, emit, init)

        def step(i):
            s0, s1 = scores(0), scores(1)
            mops, vops = mem_lhs(i + 1)
            _drain(qk_proj(i + 1, 0, mops))
            us = [attend(i, 0, s0), attend(i, 1, s1)]
            s2, s3 = scores(2), scores(3)
            _drain(qk_proj(i + 1, 1, mops))
            us += [attend(i, 2, s2), attend(i, 3, s3)]
            _drain(zip(qk_proj(i + 1, 2, mops), vm_proj(i + 1, 0, vops)))
            _drain(zip(qk_proj(i + 1, 3, mops), vm_proj(i + 1, 1, vops)))
            out_mem(i, us, 1)
            _drain(out_tok(i, us, False))

        def last_step(i):
            ss = [scores(j) for j in range(G)]
            us = [attend(i, 0, ss[0]), attend(i, 1, ss[1])]
            gen = out_tok(i, us, True)
            next(gen)
            next(gen)
            us += [attend(i, 2, ss[2]), attend(i, 3, ss[3])]
            out_mem(i, us, 2)
            _drain(gen)

        mops0, vops0 = mem_lhs(0)
        _drain(qk_proj(0, 0, mops0), qk_proj(0, 1, mops0))
        _drain(zip(qk_proj(0, 2, mops0), vm_proj(0, 0, vops0)))
        _drain(zip(qk_proj(0, 3, mops0), vm_proj(0, 1, vops0)))

        def main_body(i, cy):
            step(i)

            @pl.when(i % NG == NG - 1)
            def _():
                o_copy(i // NG).start()

            return cy

        lax.fori_loop(0, NRB * NG - 1, main_body, 0)
        last_step(NRB * NG - 1)
        ok = jnp.min(okbuf[0:(NSEG - 1) * M, :])
        for rb in range(NRB - 1):
            o_copy(rb).wait()
        for qd in range(4):
            oq_copy(qd).wait()
        return it + 1, (ok > 0.5).astype(jnp.int32)

    lax.while_loop(lambda st: jnp.logical_and(st[0] < NSEG, st[1] == 0), sweep,
                   (jnp.int32(0), jnp.int32(0)))
    for t in range(NT):
        aout_copy(t).wait()


@functools.partial(jax.jit, static_argnames=("B_seg_len",))
def pallas_concat_heads__ssm_conv_h3__memory_aug_recurrent_mem_tr__prompt_kernel(
    A_q, A_k, A_v, A_shift_k, A_ssm_k, A_ssm_D,
    B_x, B_mem0, B_Wq, B_Wk, B_Wv, B_Wo, B_seg_len,
):
    _, S, D = A_q.shape
    DM = B_x.shape[2]
    H, E = B_Wq.shape[1], B_Wq.shape[2]
    M = B_mem0.shape[1]
    SEG = int(B_seg_len)
    NSEG = S // SEG
    NP = NSEG // 2
    PR = 2 * (M + SEG)
    PPB = 8
    NRB = NP // PPB
    NT = D // LANES
    assert E == LANES and H == 32 and M == 8 and SEG == 32 and A_shift_k.shape[1] == 4
    assert S == 2048 and D == 1024 and DM == 1024

    fwd, inv = _dft_mats()
    any_spec = pl.BlockSpec(memory_space=pl.ANY)
    scratch = [
        pltpu.VMEM((NRB, 7, PPB // 2 * SEG, DM // 2), U32),
        pltpu.VMEM((7, M + PPB // 2 * SEG, DM // 2), U32),
        pltpu.VMEM((H // 4, NP, 2 * SEG, 4 * E), BF16),
        pltpu.VMEM((3, H // 2, DM, E), U32),
        pltpu.VMEM((H * E, DM), BF16),
        pltpu.VMEM((4, PPB, PR, 2 * E), BF16),
        pltpu.VMEM((PPB, 2 * M, 4 * E), BF16),
        pltpu.VMEM((PPB * 2 * SEG, DM), F32),
        pltpu.VMEM((NRB, PPB * 2 * SEG, DM), BF16),
        pltpu.VMEM(((NSEG + 1) * M, DM), F32),
        pltpu.VMEM((NSEG * M, DM), F32),
        pltpu.VMEM((NSEG * M, LANES), F32),
        pltpu.VMEM((DM // LANES, NSEG, LANES), F32),
        pltpu.VMEM((H // 4, NSEG + M, 4 * E), F32),
        pltpu.VMEM((2, 3, S, LANES), BF16),
        pltpu.VMEM((2, LANES, S), BF16),
        pltpu.VMEM((S + 32, LANES), F32),
        pltpu.VMEM((S, LANES), BF16),
        pltpu.VMEM((NFFT, S), F32),
        pltpu.VMEM((NFFT, S), F32),
        pltpu.VMEM((NFFT, S), BF16),
        pltpu.VMEM((S, LANES), F32),
        pltpu.VMEM((NT, S, LANES), BF16),
        pltpu.VMEM((M, DM), BF16),
        pltpu.VMEM((NFFT, BLK), BF16),
        pltpu.VMEM((BLK, BLK), BF16),
        pltpu.VMEM((4, D), BF16),
        pltpu.VMEM((NT, LANES), BF16),
        pltpu.VMEM((8, LANES), jnp.int32),
        pltpu.SMEM((7,), jnp.int32),
        pltpu.SemaphoreType.DMA((5,)),
        pltpu.SemaphoreType.DMA((2 * NRB,)),
        pltpu.SemaphoreType.DMA((H // 2,)),
        pltpu.SemaphoreType.DMA,
        pltpu.SemaphoreType.DMA,
        pltpu.SemaphoreType.DMA((2, 2)),
        pltpu.SemaphoreType.DMA,
        pltpu.SemaphoreType.DMA((NRB + 3,)),
    ]
    out = pl.pallas_call(
        functools.partial(_kernel, S=S, D=D, DM=DM, H=H, M=M, SEG=SEG),
        out_shape=jax.ShapeDtypeStruct((S, D + DM), BF16),
        in_specs=[any_spec] * 14,
        out_specs=any_spec,
        scratch_shapes=scratch,
        compiler_params=pltpu.CompilerParams(vmem_limit_bytes=120 * 1024 * 1024,
                                             disable_bounds_checks=True,
                                             disable_semaphore_checks=True),
    )(
        A_q.reshape(S, D), A_k.reshape(S, D), A_v.reshape(S, D),
        A_shift_k.T, A_ssm_k, A_ssm_D.reshape(NT, LANES),
        B_x.reshape(NRB, S // NRB, DM), B_mem0.reshape(M, DM),
        B_Wq, B_Wk, B_Wv, B_Wo.reshape(H * E, DM),
        jnp.asarray(fwd, BF16), jnp.asarray(inv, BF16),
    )
    return out.reshape(1, S, D + DM)
```

```python
import functools

import numpy as np
import jax
import jax.numpy as jnp
from jax import lax
import jax.experimental.pallas as pl
import jax.experimental.pallas.tpu as pltpu

F32 = jnp.float32
BF16 = jnp.bfloat16
U32 = jnp.uint32

LANES = 128
BLK = 128
NFFT = 2 * BLK
TOL = 2.0 ** -10


def _dft_mats():
    even = np.arange(0, BLK, 2)
    theta = 2.0 * np.pi * (np.concatenate([even, BLK - 1 - even]) + 0.5) / NFFT
    n = np.arange(BLK)
    c = np.cos(theta[:, None] * n[None, :])
    s = np.sin(theta[:, None] * n[None, :])
    fwd = np.zeros((NFFT, BLK))
    for m in range(BLK // 8):
        fwd[16 * m:16 * m + 8] = c[8 * m:8 * m + 8]
        fwd[16 * m + 8:16 * m + 16] = -s[8 * m:8 * m + 8]
    inv = fwd[:BLK].T * (2.0 / NFFT)
    inv = np.concatenate([inv[0::2], inv[1::2]], axis=0)
    return fwd.astype(np.float32), inv.astype(np.float32)


def _dot(a, b):
    return jnp.dot(a, b, preferred_element_type=F32)


def _pack(x):
    return pltpu.bitcast(x.astype(BF16), U32)


def _unpack(w):
    return pltpu.bitcast(w, BF16)


def _lo(w):
    return pltpu.bitcast(w << 16, F32)


def _hi(w):
    return pltpu.bitcast(w & jnp.uint32(0xFFFF0000), F32)


_STRASSEN_LHS = ((0, 3, 1), (2, 3, 1), (0, None, 0), (3, None, 0), (0, 1, 1), (2, 0, -1), (1, 3, -1))
_STRASSEN_RHS = ((0, 3, 1), (0, None, 0), (1, 3, -1), (2, 0, -1), (3, None, 0), (0, 1, 1), (2, 3, 1))


def _operand(table, k, quad):
    i, j, sign = table[k]
    if j is None:
        return quad(i)
    return quad(i) + quad(j) if sign > 0 else quad(i) - quad(j)


def _strassen_lhs(*quads):
    return [_operand(_STRASSEN_LHS, k, quads.__getitem__) for k in range(7)]


_STRASSEN_USES = (((0, 1), (3, 1)), ((2, 1), (3, -1)), ((1, 1), (3, 1)), ((0, 1), (2, 1)),
                  ((0, -1), (1, 1)), ((3, 1),), ((0, 1),))


def _strassen(lhs, rhs, emit, init=None, order=(4, 2, 1, 3, 0, 6, 5), post=None):
    acc = [[(1, c)] if c is not None else [] for c in (init or (None,) * 4)]
    left = [4, 2, 2, 4]
    for k in order:
        m = _dot(lhs(k), rhs[k])
        if post is not None:
            m = post(k, m)
        for q, sign in _STRASSEN_USES[k]:
            acc[q].append((sign, m))
            left[q] -= 1
            if left[q] < (3, 1, 1, 3)[q]:
                terms = sorted(acc[q], key=lambda t: -t[0])
                v = terms[0][1]
                assert terms[0][0] > 0
                for sg, t in terms[1:]:
                    v = v + t if sg > 0 else v - t
                acc[q] = [(1, v)]
            if left[q] == 0:
                emit(q // 2, q % 2, acc[q][0][1])
        yield m


def _drain(*gens):
    for g in gens:
        for _ in g:
            pass


def _tokens(m):
    return [(m, r, c) for r in range(0, m.shape[0], 8) for c in range(0, m.shape[1], LANES)]


def _tie(never, tok, x):
    if tok is None:
        return x
    reps = (x.shape[0] // 8, x.shape[1] // LANES)
    if tok.dtype != x.dtype:
        tok = pltpu.bitcast(tok, x.dtype)
    if reps != (1, 1):
        never, tok = jnp.tile(never, reps), jnp.tile(tok, reps)
    return jnp.where(never, tok, x)


def _run_paced(items, toks):
    for i, it in enumerate(items):
        m, r, c = toks[i * len(toks) // len(items)]
        it(m[r:r + 8, c:c + LANES])


def _interleave(nv, ngr, weights):
    dur = {'v': 256, 'h': 256, 'x': 256, 'inv': 128}
    margin = 768

    def plan(rate):
        t, v, out = 0, 0, []
        nxt = {'h': 0, 'x': 0, 'inv': 0}
        pos = {k: 0 for k in weights}
        done = {}
        credit = 0.0
        while True:
            kind = None
            if nxt['inv'] < ngr and done.get(('freq', nxt['inv']), 1e9) + margin <= t:
                kind = 'inv'
            elif nxt['x'] < ngr and done.get(('conv', nxt['x']), 1e9) + margin <= t:
                kind = 'x'
            elif nxt['h'] < ngr and nxt['h'] <= nxt['x'] and out and out[-1][0] == 'v':
                kind = 'h'
            elif v < nv:
                kind = 'v'
            if kind is None:
                break
            g = v if kind == 'v' else nxt[kind]
            busy = 0.6 if kind != 'v' else 1.1 if v % (nv // 2) < 7 else 0.0
            credit += (rate - busy) * dur[kind]
            chunk = []
            while credit > 0:
                ready = [('out', i) for i in range(nxt['inv'])]
                ready += [('conv', i) for i in range(ngr)]
                ready += [('freq', i) for i in range(min(nxt['x'], nxt['h']))]
                ready = [k for k in ready if pos[k] < len(weights[k])]
                if not ready:
                    credit = 0.0
                    break
                k = ready[0]
                chunk.append((k, pos[k]))
                credit -= weights[k][pos[k]]
                pos[k] += 1
                if pos[k] == len(weights[k]):
                    done[k] = t + dur[kind]
            out.append((kind, g, chunk))
            t += dur[kind]
            if kind == 'v':
                v += 1
            else:
                nxt[kind] += 1
        ok = all(pos[k] == len(weights[k]) for k in weights)
        return ok, out

    rate = 1.0
    while True:
        ok, out = plan(rate)
        if ok:
            return out
        rate += 0.02


def _kernel(q_hbm, k_hbm, v_hbm, shift_hbm, h_hbm, d_hbm, x_hbm, mem0_hbm,
            wq_hbm, wk_hbm, wv_hbm, wo_hbm, fwd_hbm, inv_hbm,
            out_hbm,
            abuf, a0buf, vbuf, w32, wo, qks, vms, acc, obuf, mhat, mnew, okbuf, mcol, tsum,
            ain, ah, kvb, xf, hf, wf, yt, aout,
            mem0_ref, fwd_ref, inv_ref, shift_ref, d_ref, zero_v, zero_s,
            sem_s, sem_x, sem_wv, sem_wqk, sem_wo, sem_a, sem_aout, sem_o,
            *, S, D, DM, H, M, SEG):
    E = LANES
    NSEG = S // SEG
    NP = NSEG // 2
    MR = 2 * M
    XR = 2 * SEG
    PR = MR + XR
    MW = MR // 2
    L = M + SEG
    NB = S // BLK
    NT = D // LANES
    PPB = 8
    PPH = PPB // 2
    NRB = NP // PPB
    G = 4
    NG = H // G
    KH = DM // 2
    scale = float(E) ** -0.5
    WV, WQ, WK = 0, 1, 2

    small = [pltpu.make_async_copy(src, dst, sem_s.at[i]) for i, (src, dst) in enumerate(
        ((mem0_hbm, mem0_ref), (shift_hbm, shift_ref), (d_hbm, d_ref),
         (fwd_hbm, fwd_ref), (inv_hbm, inv_ref)))]
    HBR = PPH * XR // 2

    def x_copies(hb):
        out = []
        for half in range(2):
            r = pl.ds(pl.multiple_of((2 * half + hb % 2) * HBR, HBR), HBR)
            out.append(pltpu.make_async_copy(x_hbm.at[hb // 2, r], obuf.at[hb // 2, r],
                                             sem_x.at[hb]))
        return out

    def w_copy(which, hp):
        src = (wv_hbm, wq_hbm, wk_hbm)[which].bitcast(U32)
        sem = sem_wv.at[hp] if which == WV else sem_wqk
        return pltpu.make_async_copy(src.at[:, hp, :], w32.at[which, hp], sem)

    def wo_copy(t):
        n = H * E // NT
        r = pl.ds(pl.multiple_of(t * n, n), n)
        return pltpu.make_async_copy(wo_hbm.at[r, :], wo.at[r, :], sem_wo)

    def a_start(t, sl, which=(0, 1, 2, 3)):
        c = pl.ds(pl.multiple_of(t * LANES, LANES), LANES)
        for i in which:
            if i == 3:
                pltpu.make_async_copy(h_hbm.at[c, :], ah.at[sl], sem_a.at[sl, 1]).start()
            else:
                src = (k_hbm, v_hbm, q_hbm)[i]
                pltpu.make_async_copy(src.at[:, c], ain.at[sl, i], sem_a.at[sl, 0]).start()

    def a_wait(sl):
        pltpu.make_async_copy(ain.at[sl], ain.at[sl], sem_a.at[sl, 0]).wait()
        pltpu.make_async_copy(ah.at[sl], ah.at[sl], sem_a.at[sl, 1]).wait()

    def aout_copy(t):
        c = pl.ds(pl.multiple_of(t * LANES, LANES), LANES)
        return pltpu.make_async_copy(aout.at[t], out_hbm.at[:, c], sem_aout)

    def o_copy(rb):
        r = pl.ds(pl.multiple_of(rb * (PPB * XR), PPB * XR), PPB * XR)
        return pltpu.make_async_copy(obuf.at[rb], out_hbm.at[r, pl.ds(D, DM)], sem_o.at[rb])

    def oq_copy(qd):
        n = PPH * XR
        r0, c0 = (qd // 2) * n, (qd % 2) * KH
        return pltpu.make_async_copy(
            obuf.at[NRB - 1, pl.ds(r0, n), pl.ds(c0, KH)],
            out_hbm.at[pl.ds((NRB - 1) * 2 * n + r0, n), pl.ds(D + c0, KH)],
            sem_o.at[NRB - 1 + qd])

    def w_rhs(which, hp):
        out = []
        for k in range(7):
            w = w32.at[which, hp + zero_s[k]]

            def quad(i, w=w):
                return (_lo, _hi)[i % 2](w[(i // 2) * KH:(i // 2 + 1) * KH])

            out.append(_operand(_STRASSEN_RHS, k, quad).astype(BF16))
        return out

    def w_plain(which, hp0, n):
        parts = []
        for j in range(n):
            w = w32[which, hp0 + j]
            parts += [_lo(w), _hi(w)]
        return jnp.concatenate(parts, axis=1).astype(BF16)

    small[0].start()
    for hb in range(2):
        for cp in x_copies(hb):
            cp.start()
    w_copy(WV, 0).start()
    w_copy(WV, 1).start()
    for cp in small[1:]:
        cp.start()

    zero_v[...] = jnp.zeros((8, LANES), jnp.int32)
    for k in range(7):
        zero_s[k] = 0
    tsum[:, 0:8, 0:LANES] = jnp.zeros((NG, 8, LANES), F32)
    vbuf[:, 0, 0:16, 0:LANES] = jnp.zeros((NG, 16, LANES), BF16)
    for hb in range(2 * NRB):
        r0 = (hb % 2) * (HBR // 2)
        abuf[hb // 2, 0, r0:r0 + 8, 0:LANES] = jnp.zeros((8, LANES), U32)
    small[0].wait()
    mem0 = mem0_ref[...].astype(F32)
    m0 = jnp.concatenate([mem0, jnp.zeros_like(mem0)], axis=0)
    z0 = jnp.zeros((MR, KH), F32)
    for k, op in enumerate(_strassen_lhs(m0[:, :KH], m0[:, KH:], z0, z0)):
        a0buf[k, 0:MW, :] = _pack(op)

    def x_item(tok, never, src, dst, r, c):
        quad = [_tie(never, tok, src[h * 2 * HBR + r:h * 2 * HBR + r + 16,
                                     kk * KH + c:kk * KH + c + 2 * LANES].astype(F32))
                for h in range(2) for kk in range(2)]
        for k, op in enumerate(_strassen_lhs(*quad)):
            dst[k, r // 2:r // 2 + 8, c:c + 2 * LANES] = _pack(op)

    def x_items(never, src, dst):
        return [functools.partial(x_item, never=never, src=src, dst=dst, r=r, c=c)
                for r in range(0, HBR, 16) for c in range(0, KH, 2 * LANES)]

    def x_first(hb, cy):
        for cp in x_copies(hb):
            cp.wait()
        src = obuf.at[0, pl.ds(pl.multiple_of(hb * HBR, HBR), 3 * HBR)]
        dst = a0buf.at[:, pl.ds(pl.multiple_of(MW + hb * (HBR // 2), 8), HBR // 2)]
        for it in x_items(None, src, dst):
            it(None)
        return cy

    lax.fori_loop(0, 2, x_first, 0)

    def v_part(j, rb, rhs, vwin, twin, pre=None):
        mem0_in = (0, 2, 4, 6) if rb == 0 else ()
        m0 = {}

        def lhs(k):
            x = abuf[rb, k] if rb else (a0buf[k] if k in mem0_in else a0buf[k, MW:])
            if pre is not None and k == 4:
                x0 = jnp.concatenate([pre(x[:8, :LANES]), x[:8, LANES:]], axis=1)
                x = jnp.concatenate([x0, x[8:]], axis=0)
            return _unpack(x)

        def split(k, m):
            if k not in mem0_in:
                return m
            m0[k] = m[:M]
            return m[MR:]

        def emit(half, hh, cv):
            c = slice((2 * j + hh) * E, (2 * j + hh + 1) * E)
            vx = cv.astype(BF16)
            p0 = rb * PPB + half * PPH
            vwin[p0:p0 + PPH, :, c] = vx.reshape(PPH, XR, E)
            ts = jnp.sum(vx.astype(F32).reshape(2 * PPH, SEG, E), axis=1)
            if rb == 0 and half == 0:
                v0 = m0[2] + m0[4] if hh else m0[0] - m0[4] + m0[6]
                v0 = v0.astype(BF16).astype(F32)
                twin[NSEG:NSEG + M, c] = v0
                t0 = jnp.sum(v0, axis=0, keepdims=True)
                rows = lax.broadcasted_iota(jnp.int32, ts.shape, 0)
                ts = ts + jnp.where(rows == 0, t0, 0.0)
            twin[2 * p0:2 * (p0 + PPH), c] = ts

        return _strassen(lhs, rhs, emit, post=split)

    def v_products(t, rbs, never, extra=()):
        vwin = vbuf.at[t]
        twin = tsum.at[t]

        def pre(x):
            for v in (twin[0:8, 0:LANES], pltpu.bitcast(vwin[0, 0:16, 0:LANES], U32)) + tuple(extra):
                x = _tie(never, v, x)
            return x

        for j in range(2):
            rhs = w_rhs(WV, 2 * t + j)
            for rb in rbs:
                yield from v_part(j, rb, rhs, vwin, twin, pre if (j, rb) == (0, rbs[0]) else None)

    def head_body(j, cy):
        w_copy(WV, 2 * j).wait()
        w_copy(WV, 2 * j + 1).wait()

        @pl.when(j >= 2)
        def _():
            for cp in x_copies(j):
                cp.wait()

        @pl.when(j + 1 < NT)
        def _():
            w_copy(WV, 2 * j + 2).start()
            w_copy(WV, 2 * j + 3).start()

        @pl.when(j + 2 < 2 * NRB)
        def _():
            for cp in x_copies(j + 2):
                cp.start()

        @pl.when(j == NT - 3)
        def _():
            a_start(0, 0, (3,))

        @pl.when(j == NT - 2)
        def _():
            a_start(0, 0, (0, 1, 2))

        never = zero_v[...] > 0
        src = obuf.at[j // 2, pl.ds(pl.multiple_of((j % 2) * HBR, HBR), 3 * HBR)]
        dst = abuf.at[j // 2, :, pl.ds(pl.multiple_of((j % 2) * (HBR // 2), 8), HBR // 2)]
        toks = []
        for m in v_products(j, [0], never, [dst[0, 0:8, 0:LANES]]):
            toks += _tokens(m)
        _run_paced(x_items(never, src, dst), toks[:-40])
        return cy

    assert NT == 2 * NRB
    lax.fori_loop(0, NT, head_body, 0)

    GA = 4

    def freq_items(a0, never):
        def item(tok, m, cc, st):
            r_re = slice(16 * m, 16 * m + 8)
            r_im = slice(16 * m + 8, 16 * m + 16)
            xr = _tie(never, tok, xf[r_re, cc * BLK:(cc + 1) * BLK])
            xi = _tie(never, tok, xf[r_im, cc * BLK:(cc + 1) * BLK])
            xs = xr + xi
            for a in range(max(a0, cc), a0 + GA):
                j = a - cc
                if ('g', m, j) not in st:
                    gr = hf[r_re, j * BLK:(j + 1) * BLK]
                    gi = hf[r_im, j * BLK:(j + 1) * BLK]
                    st['g', m, j] = (gr, gi, gr + gi)
                gr, gi, gs = st['g', m, j]
                ps = (xr * gr, xi * gi, xs * gs)
                st[m, a] = ps if (m, a) not in st else tuple(u + v for u, v in zip(st[m, a], ps))
                if cc == a:
                    p1, p2, p3 = st[m, a]
                    st[m, a] = (p1 - p2, p3 - p1 - p2)
                    if m >= BLK // 16:
                        m0 = m - BLK // 16
                        (wr, wi), (vr, vi) = st[m0, a], st[m, a]
                        c = slice(a * BLK, (a + 1) * BLK)
                        wf[16 * m0:16 * m0 + 16, c] = (
                            jnp.concatenate([wr + vr, wi - vi], axis=0).astype(BF16))
                        wf[16 * m:16 * m + 16, c] = (
                            jnp.concatenate([wr - vr, wi + vi], axis=0).astype(BF16))

        items = []
        for m0 in range(BLK // 16):
            st = {}
            for m in (m0, m0 + BLK // 16):
                items += [(functools.partial(item, m=m, cc=cc, st=st),
                           4 + 6 * (a0 + GA - max(a0, cc)) + (6 if cc >= a0 else 0))
                          for cc in range(a0 + GA)]
        return items

    def tile_body(t, carry):
        sl = t & 1
        a_wait(sl)

        @pl.when(t + 1 < NT)
        def _():
            a_start(t + 1, 1 - sl)
            wo_copy(t + 1).start()

        c = pl.ds(pl.multiple_of(t * LANES, LANES), LANES)
        taps = shift_ref[:, c].astype(F32)
        dcol = d_ref[...].astype(F32)
        rows = lax.broadcasted_iota(jnp.int32, dcol.shape, 0)
        dvec = jnp.sum(jnp.where(rows == t, dcol, 0.0), axis=0, keepdims=True)
        dvb = jnp.broadcast_to(dvec, (8, LANES))
        tapb = [jnp.broadcast_to(taps[j:j + 1, :], (8, LANES)) for j in range(4)]
        never = zero_v[...] > 0
        fwd = fwd_ref[...]
        NGR = NB // GA
        GW = GA * BLK

        sub = lax.broadcasted_iota(jnp.int32, (8, LANES), 0)
        kprev = [jnp.zeros((8, LANES), F32)]

        def conv_item(tok, r0):
            k16 = _tie(never, tok, ain[sl, 0, r0:r0 + 16, :].astype(F32))
            halves = []
            for h in range(2):
                k8 = k16[8 * h:8 * h + 8]
                ks = k8 * tapb[0]
                for j in range(1, 4):
                    ks = ks + pltpu.roll(jnp.where(sub < 8 - j, k8, kprev[0]), j, 0) * tapb[j]
                kprev[0] = k8
                halves.append(ks)
            kvb[r0:r0 + 16, :] = (jnp.concatenate(halves, axis=0)
                                  * ain[sl, 1, r0:r0 + 16, :].astype(F32)).astype(BF16)

        hlast = [None]

        def h_fwd(g):
            hst = jnp.concatenate([ah[sl, :, b * BLK:(b + 1) * BLK]
                                   for b in range(g * GA, (g + 1) * GA)], axis=0)
            hh = lax.dot_general(fwd, hst, (((1,), (1,)), ((), ())), preferred_element_type=F32)
            for b in range(GA):
                cur = hh[:, b * BLK:(b + 1) * BLK]
                prev = hlast[0]
                c = slice((g * GA + b) * BLK, (g * GA + b + 1) * BLK)
                if prev is None:
                    hf[:, c] = cur
                else:
                    for m in range(BLK // 8):
                        re = slice(16 * m, 16 * m + 8)
                        im = slice(16 * m + 8, 16 * m + 16)
                        if m < BLK // 16:
                            hf[re, c] = cur[re] - prev[im]
                            hf[im, c] = cur[im] + prev[re]
                        else:
                            hf[re, c] = cur[re] + prev[im]
                            hf[im, c] = cur[im] - prev[re]
                hlast[0] = cur
            return hh

        def x_fwd(g):
            rhs = jnp.concatenate([kvb[b * BLK:(b + 1) * BLK, :]
                                   for b in range(g * GA, (g + 1) * GA)], axis=1)
            xx = _dot(fwd, rhs)
            xf[:, g * GW:(g + 1) * GW] = xx
            return xx

        def inverse(g):
            ys = []
            for par in range(2):
                y = _dot(inv_ref[par * (BLK // 2):(par + 1) * (BLK // 2), :],
                         wf[par * BLK:(par + 1) * BLK, g * GW:(g + 1) * GW])
                for a in range(GA):
                    yt[pl.ds((g * GA + a) * BLK + par, BLK // 2, stride=2), :] = (
                        y[:, a * BLK:(a + 1) * BLK])
                ys.append(y)
            return jnp.concatenate(ys, axis=0)

        def out_item(tok, r0):
            d8 = _tie(never, tok, dvb)
            yb = yt[r0:r0 + 16, :] + kvb[r0:r0 + 16, :].astype(F32) * jnp.concatenate([d8, d8], axis=0)
            aout[t, r0:r0 + 16, :] = (ain[sl, 2, r0:r0 + 16, :].astype(F32) * yb).astype(BF16)

        def rows16(fn, g, w):
            return [(functools.partial(fn, r0=r0), w) for r0 in range(g * GW, (g + 1) * GW, 16)]

        vgen = v_products(t, list(range(1, NRB)), never)
        nv = 2 * (NRB - 1) * 7
        work = {('conv', g): rows16(conv_item, g, 31) for g in range(NGR)}
        work.update({('freq', g): freq_items(g * GA, never) for g in range(NGR)})
        work.update({('out', g): rows16(out_item, g, 16) for g in range(NGR)})
        for kind, g, chunks in _interleave(nv, NGR, {k: [w for _, w in v] for k, v in work.items()}):
            m = next(vgen) if kind == 'v' else {'h': h_fwd, 'x': x_fwd, 'inv': inverse}[kind](g)
            _run_paced([work[k][i][0] for k, i in chunks], _tokens(m))
        _drain(vgen)
        for which in (WQ, WK):
            w_copy(which, 2 * t).start()
            w_copy(which, 2 * t + 1).start()
        aout_copy(t).start()
        return carry

    for cp in small[1:]:
        cp.wait()
    wo_copy(0).start()
    lax.fori_loop(0, NT, tile_body, 0)
    pltpu.make_async_copy(wo, wo, sem_wo).wait()

    def initial_guess():
        puni = pl.reciprocal(jnp.full((1, 1), float(L), F32), approx=True).astype(BF16).astype(F32)

        def shift_down(m):
            rows = lax.broadcasted_iota(jnp.int32, m.shape, 0)
            return jnp.where(rows == 0, 0.0, pltpu.roll(m, 1, 0))

        tall = jnp.concatenate([tsum[g, 0:NSEG, :] for g in range(NG)], axis=1)
        wov = wo[...]
        m1 = shift_down(_dot((tall * puni).astype(BF16), wov))
        v1 = _dot(m1.astype(BF16), w_plain(WV, 0, H // 2)).astype(BF16).astype(F32)
        u2 = ((tall + float(M) * v1) * puni).astype(BF16)
        for c in range(0, DM, LANES):
            mcol[c // LANES] = _dot(u2, wov[:, c:c + LANES])
            for sg in range(NSEG):
                mhat[(sg + 1) * M:(sg + 2) * M, c:c + LANES] = jnp.broadcast_to(
                    mcol[c // LANES, sg:sg + 1, :], (M, LANES))
        mhat[0:M, :] = mem0_ref[...].astype(F32)
        pltpu.make_async_copy(w32.at[WQ:WK + 1], w32.at[WQ:WK + 1], sem_wqk).wait()

    ri = lax.broadcasted_iota(jnp.int32, (PR, PR), 0)
    ci = lax.broadcasted_iota(jnp.int32, (PR, PR), 1)

    def seg_of(r):
        return jnp.where(r < MR, r // M, (r - MR) // SEG)

    def pos_of(r):
        return jnp.where(r < MR, r % M, M + (r - MR) % SEG)

    same = seg_of(ri) == seg_of(ci)
    allowed = same & ((ri < MR) | (pos_of(ri) >= pos_of(ci)))
    fill = jnp.where(same, -1e9, -jnp.inf).astype(F32)

    def sweep(state):
        it, _ = state
        pl.when(it == 0)(initial_guess)

        @pl.when(it > 0)
        def _():
            def upd(rb, cy):
                n = PPB * MR
                r = pl.ds(pl.multiple_of(rb * n, n), n)
                r2 = pl.ds(pl.multiple_of(rb * n + M, M), n)
                keep = jnp.tile(okbuf[r, :], (1, DM // LANES)) > 0.5
                mhat[r2, :] = jnp.where(keep, mhat[r2, :], mnew[r, :])
                return cy

            lax.fori_loop(0, NRB, upd, 0)

        def mem_rows(i):
            n = PPB * MR
            return mhat[pl.ds(pl.multiple_of((i // NG) * n, n), n), :]

        def mem_lhs(i):
            m = mem_rows(i)
            n = PPH * MR
            ops = [_pack(o) for o in _strassen_lhs(m[:n, :KH], m[:n, KH:], m[n:, :KH], m[n:, KH:])]
            t = jnp.concatenate([jnp.where(i < NG, 0.0, m[:M]), m[M:MR]], axis=0)
            b = m[n:n + MR]
            vops = [jnp.concatenate([_pack(o), full[MW:]], axis=0) for o, full in zip(
                _strassen_lhs(t[:, :KH], t[:, KH:], b[:, :KH], b[:, KH:]), ops)]
            return ops, vops

        def qk_proj(i, j, mops):
            rb = i // NG
            hp = (i % NG) * (G // 2) + j // 2

            def lhs(k):
                return _unpack(jnp.concatenate([mops[k], abuf[rb, k]], axis=0))

            n = PPH * MR
            cs = {}

            def emit(half, hh, cv):
                cs[half, hh] = cv
                if (half, 1 - hh) in cs:
                    v = jnp.concatenate([cs[half, 0], cs[half, 1]], axis=1).astype(BF16)
                    ps = slice(half * PPH, (half + 1) * PPH)
                    qks[j, ps, 0:MR, :] = v[:n].reshape(PPH, MR, 2 * E)
                    qks[j, ps, MR:PR, :] = v[n:].reshape(PPH, XR, 2 * E)

            return _strassen(lhs, w_rhs(WQ + j % 2, hp), emit)

        def vm_proj(i, j, vops):
            hp = (i % NG) * (G // 2) + j

            def emit(half, hh, cv):
                if half == 0:
                    v0 = tsum[i % NG, NSEG:NSEG + M, (2 * j + hh) * E:(2 * j + hh + 1) * E]
                    cv = jnp.concatenate([jnp.where(i < NG, v0, cv[:M]), cv[M:]], axis=0)
                vms[half * PPH:(half + 1) * PPH, :, (2 * j + hh) * E:(2 * j + hh + 1) * E] = (
                    cv.astype(BF16).reshape(PPH, MR, E))

            return _strassen(lambda k: _unpack(vops[k]), w_rhs(WV, hp), emit)

        def scores(j):
            c = slice((j % 2) * E, (j % 2 + 1) * E)
            return lax.dot_general(qks[2 * (j // 2), :, :, c], qks[2 * (j // 2) + 1, :, :, c],
                                   (((2,), (2,)), ((0,), (0,))), preferred_element_type=F32)

        def attend(i, j, s):
            p0 = pl.multiple_of((i // NG) * PPB, PPB)
            s = jnp.where(allowed[None], s * scale, fill[None])
            e = jnp.exp(s - jnp.max(s, axis=-1, keepdims=True))
            p = (e * pl.reciprocal(jnp.sum(e, axis=-1, keepdims=True), approx=True)).astype(BF16)
            vh = jnp.concatenate(
                [vms[:, :, j * E:(j + 1) * E],
                 vbuf[i % NG, pl.ds(p0, PPB), :, j * E:(j + 1) * E]], axis=1)
            return lax.dot_general(p, vh, (((2,), (1,)), ((0,), (0,))), preferred_element_type=F32)

        def wo_rows(i):
            return wo[pl.ds(pl.multiple_of((i % NG) * (G * E), G * E), G * E), :]

        def out_mem(i, us, split):
            rb = i // NG
            wog = wo_rows(i)
            rm = pl.ds(pl.multiple_of(rb * (PPB * MR), PPB * MR), PPB * MR)
            new = jnp.where(i % NG > 0, mnew[rm, :], 0.0)
            n = G // split
            for j in range(0, G, n):
                um = jnp.concatenate([u[:, :MR, :] for u in us[j:j + n]], axis=2)
                new = new + _dot(um.reshape(PPB * MR, n * E).astype(BF16), wog[j * E:(j + n) * E])
            mnew[rm, :] = new
            old = mhat[pl.ds(pl.multiple_of(rb * (PPB * MR) + M, M), PPB * MR), :]
            err = jnp.max(jnp.abs(new - old), axis=1, keepdims=True)
            ref = jnp.max(jnp.abs(new), axis=1, keepdims=True)
            okbuf[rm, :] = jnp.broadcast_to(jnp.where(err <= TOL * ref, 1.0, 0.0),
                                            (PPB * MR, LANES))

        def out_tok(i, us, last):
            rb = i // NG
            n = PPH * XR
            kh = G * E // 2

            def uquad(q):
                u = jnp.concatenate([us[2 * (q % 2)], us[2 * (q % 2) + 1]], axis=2)
                return u[(q // 2) * PPH:(q // 2 + 1) * PPH, MR:, :].reshape(n, kh)

            def lhs(k):
                return _operand(_STRASSEN_LHS, k, uquad).astype(BF16)

            wf32 = wo_rows(i).astype(F32)
            wq4 = [wf32[:kh, :KH], wf32[:kh, KH:], wf32[kh:, :KH], wf32[kh:, KH:]]
            rhs = [_operand(_STRASSEN_RHS, k, wq4.__getitem__).astype(BF16) for k in range(7)]
            quads = [(slice(0, n), slice(0, KH)), (slice(0, n), slice(KH, DM)),
                     (slice(n, 2 * n), slice(0, KH)), (slice(n, 2 * n), slice(KH, DM))]
            init = [jnp.where(i % NG > 0, acc[r, c], 0.0) for r, c in quads]

            def emit(half, hh, v):
                r, c = quads[2 * half + hh]
                obuf[rb, r, c] = v.astype(BF16)
                if last:
                    oq_copy(2 * half + hh).start()
                else:
                    acc[r, c] = v

            if last:
                return _strassen(lhs, rhs, emit, init, order=(2, 5, 4, 1, 3, 0, 6))
            return _strassen(lhs, rhs, emit, init)

        def step(i):
            s0, s1 = scores(0), scores(1)
            mops, vops = mem_lhs(i + 1)
            _drain(qk_proj(i + 1, 0, mops))
            us = [attend(i, 0, s0), attend(i, 1, s1)]
            s2, s3 = scores(2), scores(3)
            _drain(qk_proj(i + 1, 1, mops))
            us += [attend(i, 2, s2), attend(i, 3, s3)]
            _drain(zip(qk_proj(i + 1, 2, mops), vm_proj(i + 1, 0, vops)))
            _drain(zip(qk_proj(i + 1, 3, mops), vm_proj(i + 1, 1, vops)))
            out_mem(i, us, 1)
            _drain(out_tok(i, us, False))

        def last_step(i):
            ss = [scores(j) for j in range(G)]
            us = [attend(i, 0, ss[0]), attend(i, 1, ss[1])]
            gen = out_tok(i, us, True)
            next(gen)
            next(gen)
            us += [attend(i, 2, ss[2]), attend(i, 3, ss[3])]
            out_mem(i, us, 2)
            _drain(gen)

        mops0, vops0 = mem_lhs(0)
        _drain(qk_proj(0, 0, mops0), qk_proj(0, 1, mops0))
        _drain(zip(qk_proj(0, 2, mops0), vm_proj(0, 0, vops0)))
        _drain(zip(qk_proj(0, 3, mops0), vm_proj(0, 1, vops0)))

        def main_body(i, cy):
            step(i)

            @pl.when(i % NG == NG - 1)
            def _():
                o_copy(i // NG).start()

            return cy

        lax.fori_loop(0, NRB * NG - 1, main_body, 0)
        last_step(NRB * NG - 1)
        ok = jnp.min(okbuf[0:(NSEG - 1) * M, :])
        for rb in range(NRB - 1):
            o_copy(rb).wait()
        for qd in range(4):
            oq_copy(qd).wait()
        return it + 1, (ok > 0.5).astype(jnp.int32)

    lax.while_loop(lambda st: jnp.logical_and(st[0] < NSEG, st[1] == 0), sweep,
                   (jnp.int32(0), jnp.int32(0)))
    for t in range(NT):
        aout_copy(t).wait()


@functools.partial(jax.jit, static_argnames=("B_seg_len",))
def pallas_concat_heads__ssm_conv_h3__memory_aug_recurrent_mem_tr__prompt_kernel(
    A_q, A_k, A_v, A_shift_k, A_ssm_k, A_ssm_D,
    B_x, B_mem0, B_Wq, B_Wk, B_Wv, B_Wo, B_seg_len,
):
    _, S, D = A_q.shape
    DM = B_x.shape[2]
    H, E = B_Wq.shape[1], B_Wq.shape[2]
    M = B_mem0.shape[1]
    SEG = int(B_seg_len)
    NSEG = S // SEG
    NP = NSEG // 2
    PR = 2 * (M + SEG)
    PPB = 8
    NRB = NP // PPB
    NT = D // LANES
    assert E == LANES and H == 32 and M == 8 and SEG == 32 and A_shift_k.shape[1] == 4
    assert S == 2048 and D == 1024 and DM == 1024

    fwd, inv = _dft_mats()
    any_spec = pl.BlockSpec(memory_space=pl.ANY)
    scratch = [
        pltpu.VMEM((NRB, 7, PPB // 2 * SEG, DM // 2), U32),
        pltpu.VMEM((7, M + PPB // 2 * SEG, DM // 2), U32),
        pltpu.VMEM((H // 4, NP, 2 * SEG, 4 * E), BF16),
        pltpu.VMEM((3, H // 2, DM, E), U32),
        pltpu.VMEM((H * E, DM), BF16),
        pltpu.VMEM((4, PPB, PR, 2 * E), BF16),
        pltpu.VMEM((PPB, 2 * M, 4 * E), BF16),
        pltpu.VMEM((PPB * 2 * SEG, DM), F32),
        pltpu.VMEM((NRB, PPB * 2 * SEG, DM), BF16),
        pltpu.VMEM(((NSEG + 1) * M, DM), F32),
        pltpu.VMEM((NSEG * M, DM), F32),
        pltpu.VMEM((NSEG * M, LANES), F32),
        pltpu.VMEM((DM // LANES, NSEG, LANES), F32),
        pltpu.VMEM((H // 4, NSEG + M, 4 * E), F32),
        pltpu.VMEM((2, 3, S, LANES), BF16),
        pltpu.VMEM((2, LANES, S), BF16),
        pltpu.VMEM((S, LANES), BF16),
        pltpu.VMEM((NFFT, S), F32),
        pltpu.VMEM((NFFT, S), F32),
        pltpu.VMEM((NFFT, S), BF16),
        pltpu.VMEM((S, LANES), F32),
        pltpu.VMEM((NT, S, LANES), BF16),
        pltpu.VMEM((M, DM), BF16),
        pltpu.VMEM((NFFT, BLK), BF16),
        pltpu.VMEM((BLK, BLK), BF16),
        pltpu.VMEM((4, D), BF16),
        pltpu.VMEM((NT, LANES), BF16),
        pltpu.VMEM((8, LANES), jnp.int32),
        pltpu.SMEM((7,), jnp.int32),
        pltpu.SemaphoreType.DMA((5,)),
        pltpu.SemaphoreType.DMA((2 * NRB,)),
        pltpu.SemaphoreType.DMA((H // 2,)),
        pltpu.SemaphoreType.DMA,
        pltpu.SemaphoreType.DMA,
        pltpu.SemaphoreType.DMA((2, 2)),
        pltpu.SemaphoreType.DMA,
        pltpu.SemaphoreType.DMA((NRB + 3,)),
    ]
    out = pl.pallas_call(
        functools.partial(_kernel, S=S, D=D, DM=DM, H=H, M=M, SEG=SEG),
        out_shape=jax.ShapeDtypeStruct((S, D + DM), BF16),
        in_specs=[any_spec] * 14,
        out_specs=any_spec,
        scratch_shapes=scratch,
        compiler_params=pltpu.CompilerParams(vmem_limit_bytes=120 * 1024 * 1024,
                                             disable_bounds_checks=True,
                                             disable_semaphore_checks=True),
    )(
        A_q.reshape(S, D), A_k.reshape(S, D), A_v.reshape(S, D),
        A_shift_k.T, A_ssm_k, A_ssm_D.reshape(NT, LANES),
        B_x.reshape(NRB, S // NRB, DM), B_mem0.reshape(M, DM),
        B_Wq, B_Wk, B_Wv, B_Wo.reshape(H * E, DM),
        jnp.asarray(fwd, BF16), jnp.asarray(inv, BF16),
    )
    return out.reshape(1, S, D + DM)
```

```python
import functools

import numpy as np
import jax
import jax.numpy as jnp
from jax import lax
import jax.experimental.pallas as pl
import jax.experimental.pallas.tpu as pltpu

F32 = jnp.float32
BF16 = jnp.bfloat16
U32 = jnp.uint32

LANES = 128
BLK = 128
NFFT = 2 * BLK
TOL = 2.0 ** -12


def _dft_mats():
    even = np.arange(0, BLK, 2)
    theta = 2.0 * np.pi * (np.concatenate([even, BLK - 1 - even]) + 0.5) / NFFT
    n = np.arange(BLK)
    c = np.cos(theta[:, None] * n[None, :])
    s = np.sin(theta[:, None] * n[None, :])
    fwd = np.zeros((NFFT, BLK))
    for m in range(BLK // 8):
        fwd[16 * m:16 * m + 8] = c[8 * m:8 * m + 8]
        fwd[16 * m + 8:16 * m + 16] = -s[8 * m:8 * m + 8]
    inv = fwd[:BLK].T * (2.0 / NFFT)
    inv = np.concatenate([inv[0::2], inv[1::2]], axis=0)
    return fwd.astype(np.float32), inv.astype(np.float32)


def _dot(a, b):
    return jnp.dot(a, b, preferred_element_type=F32)


def _pack(x):
    return pltpu.bitcast(x.astype(BF16), U32)


def _unpack(w):
    return pltpu.bitcast(w, BF16)


def _lo(w):
    return pltpu.bitcast(w << 16, F32)


def _hi(w):
    return pltpu.bitcast(w & jnp.uint32(0xFFFF0000), F32)


_STRASSEN_LHS = ((0, 3, 1), (2, 3, 1), (0, None, 0), (3, None, 0), (0, 1, 1), (2, 0, -1), (1, 3, -1))
_STRASSEN_RHS = ((0, 3, 1), (0, None, 0), (1, 3, -1), (2, 0, -1), (3, None, 0), (0, 1, 1), (2, 3, 1))


def _operand(table, k, quad):
    i, j, sign = table[k]
    if j is None:
        return quad(i)
    return quad(i) + quad(j) if sign > 0 else quad(i) - quad(j)


def _strassen_lhs(*quads):
    return [_operand(_STRASSEN_LHS, k, quads.__getitem__) for k in range(7)]


_STRASSEN_USES = (((0, 1), (3, 1)), ((2, 1), (3, -1)), ((1, 1), (3, 1)), ((0, 1), (2, 1)),
                  ((0, -1), (1, 1)), ((3, 1),), ((0, 1),))


def _strassen(lhs, rhs, emit, init=None, order=(4, 2, 1, 3, 0, 6, 5), post=None):
    acc = [[(1, c)] if c is not None else [] for c in (init or (None,) * 4)]
    left = [4, 2, 2, 4]
    for k in order:
        m = _dot(lhs(k), rhs[k])
        if post is not None:
            m = post(k, m)
        for q, sign in _STRASSEN_USES[k]:
            acc[q].append((sign, m))
            left[q] -= 1
            if left[q] < (3, 1, 1, 3)[q]:
                terms = sorted(acc[q], key=lambda t: -t[0])
                v = terms[0][1]
                assert terms[0][0] > 0
                for sg, t in terms[1:]:
                    v = v + t if sg > 0 else v - t
                acc[q] = [(1, v)]
            if left[q] == 0:
                emit(q // 2, q % 2, acc[q][0][1])
        yield m


def _drain(*gens):
    for g in gens:
        for _ in g:
            pass


def _tokens(m):
    return [(m, r, c) for r in range(0, m.shape[0], 8) for c in range(0, m.shape[1], LANES)]


def _tie(never, tok, x):
    if tok is None:
        return x
    reps = (x.shape[0] // 8, x.shape[1] // LANES)
    if tok.dtype != x.dtype:
        tok = pltpu.bitcast(tok, x.dtype)
    if reps != (1, 1):
        never, tok = jnp.tile(never, reps), jnp.tile(tok, reps)
    return jnp.where(never, tok, x)


def _run_paced(items, toks):
    for i, it in enumerate(items):
        m, r, c = toks[i * len(toks) // len(items)]
        it(m[r:r + 8, c:c + LANES])


def _interleave(nv, ngr, weights):
    dur = {'v': 256, 'h': 256, 'x': 256, 'inv': 128}
    margin = 768

    def plan(rate):
        t, v, out = 0, 0, []
        nxt = {'h': 0, 'x': 0, 'inv': 0}
        pos = {k: 0 for k in weights}
        done = {}
        credit = 0.0
        while True:
            kind = None
            if nxt['inv'] < ngr and done.get(('freq', nxt['inv']), 1e9) + margin <= t:
                kind = 'inv'
            elif nxt['x'] < ngr and done.get(('conv', nxt['x']), 1e9) + margin <= t:
                kind = 'x'
            elif nxt['h'] < ngr and nxt['h'] <= nxt['x'] and out and out[-1][0] == 'v':
                kind = 'h'
            elif v < nv:
                kind = 'v'
            if kind is None:
                break
            g = v if kind == 'v' else nxt[kind]
            busy = 0.6
            if kind == 'v':
                busy = 1.1 * (v % (nv // 2) < 7) + 0.55 * (v % 7 in (1, 3, 5, 6))
            credit += (rate - busy) * dur[kind]
            chunk = []
            while credit > 0:
                ready = [('out', i) for i in range(nxt['inv'])]
                ready += [('conv', i) for i in range(ngr)]
                ready += [('freq', i) for i in range(min(nxt['x'], nxt['h']))]
                ready = [k for k in ready if pos[k] < len(weights[k])]
                if not ready:
                    credit = 0.0
                    break
                k = ready[0]
                chunk.append((k, pos[k]))
                credit -= weights[k][pos[k]]
                pos[k] += 1
                if pos[k] == len(weights[k]):
                    done[k] = t + dur[kind]
            out.append((kind, g, chunk))
            t += dur[kind]
            if kind == 'v':
                v += 1
            else:
                nxt[kind] += 1
        ok = all(pos[k] == len(weights[k]) for k in weights)
        return ok, out

    rate = 1.0
    while True:
        ok, out = plan(rate)
        if ok:
            return out
        rate += 0.02


def _kernel(q_hbm, k_hbm, v_hbm, shift_hbm, h_hbm, d_hbm, x_hbm, mem0_hbm,
            wq_hbm, wk_hbm, wv_hbm, wo_hbm, fwd_hbm, inv_hbm,
            out_hbm,
            abuf, a0buf, vbuf, w32, wo, qks, vms, acc, obuf, mhat, mnew, uhat, unew, okbuf, mcol, tsum,
            ain, ah, kvb, xf, hf, wf, yt, aout,
            mem0_ref, fwd_ref, inv_ref, shift_ref, d_ref, zero_v, zero_s,
            sem_s, sem_x, sem_wv, sem_wqk, sem_wo, sem_a, sem_aout, sem_o,
            *, S, D, DM, H, M, SEG):
    E = LANES
    NSEG = S // SEG
    NP = NSEG // 2
    MR = 2 * M
    XR = 2 * SEG
    PR = MR + XR
    MW = MR // 2
    L = M + SEG
    NB = S // BLK
    NT = D // LANES
    PPB = 8
    PPH = PPB // 2
    NRB = NP // PPB
    G = 4
    NG = H // G
    KH = DM // 2
    scale = float(E) ** -0.5
    WV, WQ, WK = 0, 1, 2

    small = [pltpu.make_async_copy(src, dst, sem_s.at[i]) for i, (src, dst) in enumerate(
        ((mem0_hbm, mem0_ref), (shift_hbm, shift_ref), (d_hbm, d_ref),
         (fwd_hbm, fwd_ref), (inv_hbm, inv_ref)))]
    HBR = PPH * XR // 2

    def x_copies(hb):
        out = []
        for half in range(2):
            r = pl.ds(pl.multiple_of((2 * half + hb % 2) * HBR, HBR), HBR)
            out.append(pltpu.make_async_copy(x_hbm.at[hb // 2, r], obuf.at[hb // 2, r],
                                             sem_x.at[hb]))
        return out

    def w_copy(which, hp):
        src = (wv_hbm, wq_hbm, wk_hbm)[which].bitcast(U32)
        sem = sem_wv.at[hp] if which == WV else sem_wqk
        return pltpu.make_async_copy(src.at[:, hp, :], w32.at[which, hp], sem)

    def wo_copy(t):
        n = H * E // NT
        r = pl.ds(pl.multiple_of(t * n, n), n)
        return pltpu.make_async_copy(wo_hbm.at[r, :], wo.at[r, :], sem_wo)

    def a_start(t, sl, which=(0, 1, 2, 3)):
        c = pl.ds(pl.multiple_of(t * LANES, LANES), LANES)
        for i in which:
            if i == 3:
                pltpu.make_async_copy(h_hbm.at[c, :], ah.at[sl], sem_a.at[sl, 1]).start()
            else:
                src = (k_hbm, v_hbm, q_hbm)[i]
                pltpu.make_async_copy(src.at[:, c], ain.at[sl, i], sem_a.at[sl, 0]).start()

    def a_wait(sl):
        pltpu.make_async_copy(ain.at[sl], ain.at[sl], sem_a.at[sl, 0]).wait()
        pltpu.make_async_copy(ah.at[sl], ah.at[sl], sem_a.at[sl, 1]).wait()

    def aout_copy(t):
        c = pl.ds(pl.multiple_of(t * LANES, LANES), LANES)
        return pltpu.make_async_copy(aout.at[t], out_hbm.at[:, c], sem_aout)

    def o_copy(rb):
        r = pl.ds(pl.multiple_of(rb * (PPB * XR), PPB * XR), PPB * XR)
        return pltpu.make_async_copy(obuf.at[rb], out_hbm.at[r, pl.ds(D, DM)], sem_o.at[rb])

    def oq_copy(qd):
        n = PPH * XR
        r0, c0 = (qd // 2) * n, (qd % 2) * KH
        return pltpu.make_async_copy(
            obuf.at[NRB - 1, pl.ds(r0, n), pl.ds(c0, KH)],
            out_hbm.at[pl.ds((NRB - 1) * 2 * n + r0, n), pl.ds(D + c0, KH)],
            sem_o.at[NRB - 1 + qd])

    def w_rhs(which, hp):
        out = []
        for k in range(7):
            w = w32.at[which, hp + zero_s[k]]

            def quad(i, w=w):
                return (_lo, _hi)[i % 2](w[(i // 2) * KH:(i // 2 + 1) * KH])

            out.append(_operand(_STRASSEN_RHS, k, quad).astype(BF16))
        return out

    def w_plain(which, hp0, n):
        parts = []
        for j in range(n):
            w = w32[which, hp0 + j]
            parts += [_lo(w), _hi(w)]
        return jnp.concatenate(parts, axis=1).astype(BF16)

    small[0].start()
    for hb in range(2):
        for cp in x_copies(hb):
            cp.start()
    w_copy(WV, 0).start()
    w_copy(WV, 1).start()
    for cp in small[1:]:
        cp.start()

    zero_v[...] = jnp.zeros((8, LANES), jnp.int32)
    for k in range(7):
        zero_s[k] = 0
    tsum[:, 0:8, 0:LANES] = jnp.zeros((NG, 8, LANES), F32)
    vbuf[:, 0, 0:16, 0:LANES] = jnp.zeros((NG, 16, LANES), BF16)
    for hb in range(2 * NRB):
        r0 = (hb % 2) * (HBR // 2)
        abuf[hb // 2, 0, r0:r0 + 8, 0:LANES] = jnp.zeros((8, LANES), U32)

    ri = lax.broadcasted_iota(jnp.int32, (PR, PR), 0)
    ci = lax.broadcasted_iota(jnp.int32, (PR, PR), 1)

    def seg_of(r):
        return jnp.where(r < MR, r // M, (r - MR) // SEG)

    def pos_of(r):
        return jnp.where(r < MR, r % M, M + (r - MR) % SEG)

    same = seg_of(ri) == seg_of(ci)
    allowed = same & ((ri < MR) | (pos_of(ri) >= pos_of(ci)))
    fill = jnp.where(same, -1e9, -jnp.inf).astype(F32)

    small[0].wait()
    mem0 = mem0_ref[...].astype(F32)
    m0 = jnp.concatenate([mem0, jnp.zeros_like(mem0)], axis=0)
    z0 = jnp.zeros((MR, KH), F32)
    for k, op in enumerate(_strassen_lhs(m0[:, :KH], m0[:, KH:], z0, z0)):
        a0buf[k, 0:MW, :] = _pack(op)

    def x_item(tok, never, src, dst, r, c):
        quad = [_tie(never, tok, src[h * 2 * HBR + r:h * 2 * HBR + r + 16,
                                     kk * KH + c:kk * KH + c + 2 * LANES].astype(F32))
                for h in range(2) for kk in range(2)]
        for k, op in enumerate(_strassen_lhs(*quad)):
            dst[k, r // 2:r // 2 + 8, c:c + 2 * LANES] = _pack(op)

    def x_items(never, src, dst):
        return [functools.partial(x_item, never=never, src=src, dst=dst, r=r, c=c)
                for r in range(0, HBR, 16) for c in range(0, KH, 2 * LANES)]

    def x_first(hb, cy):
        for cp in x_copies(hb):
            cp.wait()
        src = obuf.at[0, pl.ds(pl.multiple_of(hb * HBR, HBR), 3 * HBR)]
        dst = a0buf.at[:, pl.ds(pl.multiple_of(MW + hb * (HBR // 2), 8), HBR // 2)]
        for it in x_items(None, src, dst):
            it(None)
        return cy

    lax.fori_loop(0, 2, x_first, 0)

    def v_part(j, rb, rhs, vwin, twin, pre=None):
        mem0_in = (0, 2, 4, 6) if rb == 0 else ()
        m0 = {}

        def lhs(k):
            x = abuf[rb, k] if rb else (a0buf[k] if k in mem0_in else a0buf[k, MW:])
            if pre is not None and k == 4:
                x0 = jnp.concatenate([pre(x[:8, :LANES]), x[:8, LANES:]], axis=1)
                x = jnp.concatenate([x0, x[8:]], axis=0)
            return _unpack(x)

        def split(k, m):
            if k not in mem0_in:
                return m
            m0[k] = m[:M]
            return m[MR:]

        def emit(half, hh, cv):
            c = slice((2 * j + hh) * E, (2 * j + hh + 1) * E)
            vx = cv.astype(BF16)
            p0 = rb * PPB + half * PPH
            vwin[p0:p0 + PPH, :, c] = vx.reshape(PPH, XR, E)
            ts = jnp.sum(vx.astype(F32).reshape(2 * PPH, SEG, E), axis=1)
            if rb == 0 and half == 0:
                v0 = m0[2] + m0[4] if hh else m0[0] - m0[4] + m0[6]
                v0 = v0.astype(BF16).astype(F32)
                twin[NSEG:NSEG + M, c] = v0
                t0 = jnp.sum(v0, axis=0, keepdims=True)
                rows = lax.broadcasted_iota(jnp.int32, ts.shape, 0)
                ts = ts + jnp.where(rows == 0, t0, 0.0)
            twin[2 * p0:2 * (p0 + PPH), c] = ts

        return _strassen(lhs, rhs, emit, post=split)

    def v_products(t, rbs, never, extra=()):
        vwin = vbuf.at[t]
        twin = tsum.at[t]

        def pre(x):
            for v in (twin[0:8, 0:LANES], pltpu.bitcast(vwin[0, 0:16, 0:LANES], U32)) + tuple(extra):
                x = _tie(never, v, x)
            return x

        for j in range(2):
            rhs = w_rhs(WV, 2 * t + j)
            for rb in rbs:
                yield from v_part(j, rb, rhs, vwin, twin, pre if (j, rb) == (0, rbs[0]) else None)

    def head_body(j, cy):
        w_copy(WV, 2 * j).wait()
        w_copy(WV, 2 * j + 1).wait()

        @pl.when(j >= 2)
        def _():
            for cp in x_copies(j):
                cp.wait()

        @pl.when(j + 1 < NT)
        def _():
            w_copy(WV, 2 * j + 2).start()
            w_copy(WV, 2 * j + 3).start()

        @pl.when(j + 2 < 2 * NRB)
        def _():
            for cp in x_copies(j + 2):
                cp.start()

        @pl.when(j == NT - 3)
        def _():
            a_start(0, 0, (3,))

        @pl.when(j == NT - 2)
        def _():
            a_start(0, 0, (0, 1, 2))

        never = zero_v[...] > 0
        src = obuf.at[j // 2, pl.ds(pl.multiple_of((j % 2) * HBR, HBR), 3 * HBR)]
        dst = abuf.at[j // 2, :, pl.ds(pl.multiple_of((j % 2) * (HBR // 2), 8), HBR // 2)]
        toks = []
        for m in v_products(j, [0], never, [dst[0, 0:8, 0:LANES]]):
            toks += _tokens(m)
        _run_paced(x_items(never, src, dst), toks[:-40])
        return cy

    assert NT == 2 * NRB
    lax.fori_loop(0, NT, head_body, 0)

    GA = 4

    def freq_items(a0, never):
        def item(tok, m, cc, st):
            r_re = slice(16 * m, 16 * m + 8)
            r_im = slice(16 * m + 8, 16 * m + 16)
            xr = _tie(never, tok, xf[r_re, cc * BLK:(cc + 1) * BLK])
            xi = _tie(never, tok, xf[r_im, cc * BLK:(cc + 1) * BLK])
            xs = xr + xi
            for a in range(max(a0, cc), a0 + GA):
                j = a - cc
                if ('g', m, j) not in st:
                    gr = hf[r_re, j * BLK:(j + 1) * BLK]
                    gi = hf[r_im, j * BLK:(j + 1) * BLK]
                    st['g', m, j] = (gr, gi, gr + gi)
                gr, gi, gs = st['g', m, j]
                ps = (xr * gr, xi * gi, xs * gs)
                st[m, a] = ps if (m, a) not in st else tuple(u + v for u, v in zip(st[m, a], ps))
                if cc == a:
                    p1, p2, p3 = st[m, a]
                    st[m, a] = (p1 - p2, p3 - p1 - p2)
                    if m >= BLK // 16:
                        m0 = m - BLK // 16
                        (wr, wi), (vr, vi) = st[m0, a], st[m, a]
                        c = slice(a * BLK, (a + 1) * BLK)
                        wf[16 * m0:16 * m0 + 16, c] = (
                            jnp.concatenate([wr + vr, wi - vi], axis=0).astype(BF16))
                        wf[16 * m:16 * m + 16, c] = (
                            jnp.concatenate([wr - vr, wi + vi], axis=0).astype(BF16))

        items = []
        for m0 in range(BLK // 16):
            st = {}
            for m in (m0, m0 + BLK // 16):
                items += [(functools.partial(item, m=m, cc=cc, st=st),
                           4 + 6 * (a0 + GA - max(a0, cc)) + (6 if cc >= a0 else 0))
                          for cc in range(a0 + GA)]
        return items

    def tile_body(t, carry):
        sl = t & 1
        a_wait(sl)

        @pl.when(t + 1 < NT)
        def _():
            a_start(t + 1, 1 - sl)
            wo_copy(t + 1).start()

        c = pl.ds(pl.multiple_of(t * LANES, LANES), LANES)
        taps = shift_ref[:, c].astype(F32)
        dcol = d_ref[...].astype(F32)
        rows = lax.broadcasted_iota(jnp.int32, dcol.shape, 0)
        dvec = jnp.sum(jnp.where(rows == t, dcol, 0.0), axis=0, keepdims=True)
        dvb = jnp.broadcast_to(dvec, (8, LANES))
        tapb = [jnp.broadcast_to(taps[j:j + 1, :], (8, LANES)) for j in range(4)]
        never = zero_v[...] > 0
        fwd = fwd_ref[...]
        NGR = NB // GA
        GW = GA * BLK

        sub = lax.broadcasted_iota(jnp.int32, (8, LANES), 0)
        kprev = [jnp.zeros((8, LANES), F32)]

        def conv_item(tok, r0):
            k16 = _tie(never, tok, ain[sl, 0, r0:r0 + 16, :].astype(F32))
            halves = []
            for h in range(2):
                k8 = k16[8 * h:8 * h + 8]
                ks = k8 * tapb[0]
                for j in range(1, 4):
                    ks = ks + pltpu.roll(jnp.where(sub < 8 - j, k8, kprev[0]), j, 0) * tapb[j]
                kprev[0] = k8
                halves.append(ks)
            kvb[r0:r0 + 16, :] = (jnp.concatenate(halves, axis=0)
                                  * ain[sl, 1, r0:r0 + 16, :].astype(F32)).astype(BF16)

        hlast = [None]

        def h_fwd(g):
            hst = jnp.concatenate([ah[sl, :, b * BLK:(b + 1) * BLK]
                                   for b in range(g * GA, (g + 1) * GA)], axis=0)
            hh = lax.dot_general(fwd, hst, (((1,), (1,)), ((), ())), preferred_element_type=F32)
            for b in range(GA):
                cur = hh[:, b * BLK:(b + 1) * BLK]
                prev = hlast[0]
                c = slice((g * GA + b) * BLK, (g * GA + b + 1) * BLK)
                if prev is None:
                    hf[:, c] = cur
                else:
                    for m in range(BLK // 8):
                        re = slice(16 * m, 16 * m + 8)
                        im = slice(16 * m + 8, 16 * m + 16)
                        if m < BLK // 16:
                            hf[re, c] = cur[re] - prev[im]
                            hf[im, c] = cur[im] + prev[re]
                        else:
                            hf[re, c] = cur[re] + prev[im]
                            hf[im, c] = cur[im] - prev[re]
                hlast[0] = cur
            return hh

        def x_fwd(g):
            rhs = jnp.concatenate([kvb[b * BLK:(b + 1) * BLK, :]
                                   for b in range(g * GA, (g + 1) * GA)], axis=1)
            xx = _dot(fwd, rhs)
            xf[:, g * GW:(g + 1) * GW] = xx
            return xx

        def inverse(g):
            ys = []
            for par in range(2):
                y = _dot(inv_ref[par * (BLK // 2):(par + 1) * (BLK // 2), :],
                         wf[par * BLK:(par + 1) * BLK, g * GW:(g + 1) * GW])
                for a in range(GA):
                    yt[pl.ds((g * GA + a) * BLK + par, BLK // 2, stride=2), :] = (
                        y[:, a * BLK:(a + 1) * BLK])
                ys.append(y)
            return jnp.concatenate(ys, axis=0)

        def out_item(tok, r0):
            d8 = _tie(never, tok, dvb)
            yb = yt[r0:r0 + 16, :] + kvb[r0:r0 + 16, :].astype(F32) * jnp.concatenate([d8, d8], axis=0)
            aout[t, r0:r0 + 16, :] = (ain[sl, 2, r0:r0 + 16, :].astype(F32) * yb).astype(BF16)

        def rows16(fn, g, w):
            return [(functools.partial(fn, r0=r0), w) for r0 in range(g * GW, (g + 1) * GW, 16)]

        vgen = v_products(t, list(range(1, NRB)), never)
        nv = 2 * (NRB - 1) * 7
        work = {('conv', g): rows16(conv_item, g, 31) for g in range(NGR)}
        work.update({('freq', g): freq_items(g * GA, never) for g in range(NGR)})
        work.update({('out', g): rows16(out_item, g, 16) for g in range(NGR)})
        for kind, g, chunks in _interleave(nv, NGR, {k: [w for _, w in v] for k, v in work.items()}):
            m = next(vgen) if kind == 'v' else {'h': h_fwd, 'x': x_fwd, 'inv': inverse}[kind](g)
            _run_paced([work[k][i][0] for k, i in chunks], _tokens(m))
        _drain(vgen)
        for which in (WQ, WK):
            w_copy(which, 2 * t).start()
            w_copy(which, 2 * t + 1).start()
        aout_copy(t).start()
        return carry

    for cp in small[1:]:
        cp.wait()
    wo_copy(0).start()
    lax.fori_loop(0, NT, tile_body, 0)
    pltpu.make_async_copy(wo, wo, sem_wo).wait()

    def initial_guess():
        puni = pl.reciprocal(jnp.full((1, 1), float(L), F32), approx=True).astype(BF16).astype(F32)

        def shift_down(m):
            rows = lax.broadcasted_iota(jnp.int32, m.shape, 0)
            return jnp.where(rows == 0, 0.0, pltpu.roll(m, 1, 0))

        tall = jnp.concatenate([tsum[g, 0:NSEG, :] for g in range(NG)], axis=1)
        wov = wo[...]
        m1 = shift_down(_dot((tall * puni).astype(BF16), wov))
        v1 = _dot(m1.astype(BF16), w_plain(WV, 0, H // 2))
        u2 = (tall + float(M) * v1) * puni
        for g in range(NG):
            tsum[g, 0:NSEG, :] = u2[:, g * (G * E):(g + 1) * (G * E)]
        u2 = u2.astype(BF16)
        for c in range(0, DM, LANES):
            mcol[c // LANES] = _dot(u2, wov[:, c:c + LANES])
            for sg in range(NSEG):
                mhat[(sg + 1) * M:(sg + 2) * M, c:c + LANES] = jnp.broadcast_to(
                    mcol[c // LANES, sg:sg + 1, :], (M, LANES))
        mhat[0:M, :] = mem0_ref[...].astype(F32)
        pltpu.make_async_copy(w32.at[WQ:WK + 1], w32.at[WQ:WK + 1], sem_wqk).wait()

    def sweep(state):
        it, _ = state
        pl.when(it == 0)(initial_guess)

        def u_estimate(first, rb, g):
            n = PPB * MR
            one = tsum[g, pl.ds(pl.multiple_of(rb * (2 * PPB), 2 * PPB), 2 * PPB), :]
            one = jnp.broadcast_to(one[:, None, :], (2 * PPB, M, G * E)).reshape(n, G * E)
            return jnp.where(first, one, uhat[g, pl.ds(pl.multiple_of(rb * n, n), n), :])

        @pl.when(it > 0)
        def _():
            def upd(i, cy):
                rb, g = i // NG, i % NG
                n = PPB * MR
                r = pl.ds(pl.multiple_of(rb * n, n), n)
                r2 = pl.ds(pl.multiple_of(rb * n + M, M), n)
                c = pl.ds(pl.multiple_of(g * LANES, LANES), LANES)
                keep = okbuf[r, :] > 0.5
                mhat[r2, c] = jnp.where(keep, mhat[r2, c], mnew[r, c])
                uhat[g, r, :] = jnp.where(jnp.tile(keep, (1, G)), u_estimate(it == 1, rb, g),
                                          unew[g, r, :])
                return cy

            assert NG * LANES == DM
            lax.fori_loop(0, NRB * NG, upd, 0)

        def mem_rows(i):
            n = PPB * MR
            return mhat[pl.ds(pl.multiple_of((i // NG) * n, n), n), :]

        def mem_lhs(i):
            m = mem_rows(i)
            n = PPH * MR
            ops = [_pack(o) for o in _strassen_lhs(m[:n, :KH], m[:n, KH:], m[n:, :KH], m[n:, KH:])]
            t = jnp.concatenate([jnp.where(i < NG, 0.0, m[:M]), m[M:MR]], axis=0)
            b = m[n:n + MR]
            vops = [jnp.concatenate([_pack(o), full[MW:]], axis=0) for o, full in zip(
                _strassen_lhs(t[:, :KH], t[:, KH:], b[:, :KH], b[:, KH:]), ops)]
            return ops, vops

        def qk_proj(i, j, mops):
            rb = i // NG
            hp = (i % NG) * (G // 2) + j // 2

            def lhs(k):
                return _unpack(jnp.concatenate([mops[k], abuf[rb, k]], axis=0))

            n = PPH * MR
            cs = {}

            def emit(half, hh, cv):
                cs[half, hh] = cv
                if (half, 1 - hh) in cs:
                    v = jnp.concatenate([cs[half, 0], cs[half, 1]], axis=1).astype(BF16)
                    ps = slice(half * PPH, (half + 1) * PPH)
                    qks[j, ps, 0:MR, :] = v[:n].reshape(PPH, MR, 2 * E)
                    qks[j, ps, MR:PR, :] = v[n:].reshape(PPH, XR, 2 * E)

            return _strassen(lhs, w_rhs(WQ + j % 2, hp), emit)

        def vm_proj(i, j, vops):
            hp = (i % NG) * (G // 2) + j

            def emit(half, hh, cv):
                if half == 0:
                    v0 = tsum[i % NG, NSEG:NSEG + M, (2 * j + hh) * E:(2 * j + hh + 1) * E]
                    cv = jnp.concatenate([jnp.where(i < NG, v0, cv[:M]), cv[M:]], axis=0)
                vms[half * PPH:(half + 1) * PPH, :, (2 * j + hh) * E:(2 * j + hh + 1) * E] = (
                    cv.astype(BF16).reshape(PPH, MR, E))

            return _strassen(lambda k: _unpack(vops[k]), w_rhs(WV, hp), emit)

        def scores(j):
            c = slice((j % 2) * E, (j % 2 + 1) * E)
            return lax.dot_general(qks[2 * (j // 2), :, :, c], qks[2 * (j // 2) + 1, :, :, c],
                                   (((2,), (2,)), ((0,), (0,))), preferred_element_type=F32)

        def attend(i, j, s):
            p0 = pl.multiple_of((i // NG) * PPB, PPB)
            s = jnp.where(allowed[None], s * scale, fill[None])
            e = jnp.exp(s - jnp.max(s, axis=-1, keepdims=True))
            p = (e * pl.reciprocal(jnp.sum(e, axis=-1, keepdims=True), approx=True)).astype(BF16)
            vh = jnp.concatenate(
                [vms[:, :, j * E:(j + 1) * E],
                 vbuf[i % NG, pl.ds(p0, PPB), :, j * E:(j + 1) * E]], axis=1)
            return lax.dot_general(p, vh, (((2,), (1,)), ((0,), (0,))), preferred_element_type=F32)

        def residual(i, us):
            rb, g = i // NG, i % NG
            n = PPB * MR
            rm = pl.ds(pl.multiple_of(rb * n, n), n)
            new = jnp.concatenate([u[:, :MR, :] for u in us], axis=2).reshape(n, G * E)
            unew[g, rm, :] = new
            err = jnp.max(jnp.abs(new - u_estimate(it == 0, rb, g)), axis=1, keepdims=True)
            ref = jnp.max(jnp.abs(new), axis=1, keepdims=True)
            ok = jnp.broadcast_to(jnp.where(err <= TOL * ref, 1.0, 0.0), (n, LANES))
            okbuf[rm, :] = jnp.minimum(ok, jnp.where(g > 0, okbuf[rm, :], 1.0))

        def out_proj(i, us, last):
            rb = i // NG
            n = PPH * PR
            kh = G * E // 2

            def uquad(q):
                u = jnp.concatenate([us[2 * (q % 2)], us[2 * (q % 2) + 1]], axis=2)
                return u[(q // 2) * PPH:(q // 2 + 1) * PPH].reshape(n, kh)

            def lhs(k):
                return _operand(_STRASSEN_LHS, k, uquad).astype(BF16)

            wf32 = wo[pl.ds(pl.multiple_of((i % NG) * (G * E), G * E), G * E), :].astype(F32)
            wq4 = [wf32[:kh, :KH], wf32[:kh, KH:], wf32[kh:, :KH], wf32[kh:, KH:]]
            rhs = [_operand(_STRASSEN_RHS, k, wq4.__getitem__).astype(BF16) for k in range(7)]
            init = [jnp.where(i % NG > 0, acc[q], 0.0) for q in range(4)]
            mwin = mnew.at[pl.ds(pl.multiple_of(rb * (PPB * MR), PPB * MR), PPB * MR), :]

            def emit(half, hh, v):
                c = slice(hh * KH, (hh + 1) * KH)
                v3 = v.reshape(PPH, PR, KH)
                mwin[half * PPH * MR:(half + 1) * PPH * MR, c] = v3[:, :MR].reshape(PPH * MR, KH)
                obuf[rb, half * PPH * XR:(half + 1) * PPH * XR, c] = (
                    v3[:, MR:].reshape(PPH * XR, KH).astype(BF16))
                if last:
                    oq_copy(2 * half + hh).start()
                else:
                    acc[2 * half + hh] = v

            if last:
                return _strassen(lhs, rhs, emit, init, order=(2, 5, 4, 1, 3, 0, 6))
            return _strassen(lhs, rhs, emit, init)

        def step(i):
            s0, s1 = scores(0), scores(1)
            mops, vops = mem_lhs(i + 1)
            _drain(qk_proj(i + 1, 0, mops))
            us = [attend(i, 0, s0), attend(i, 1, s1)]
            s2, s3 = scores(2), scores(3)
            _drain(qk_proj(i + 1, 1, mops))
            us += [attend(i, 2, s2), attend(i, 3, s3)]
            residual(i, us)
            _drain(zip(qk_proj(i + 1, 2, mops), vm_proj(i + 1, 0, vops)))
            _drain(zip(qk_proj(i + 1, 3, mops), vm_proj(i + 1, 1, vops)))
            _drain(out_proj(i, us, False))

        def last_step(i):
            ss = [scores(j) for j in range(G)]
            us = [attend(i, 0, ss[0]), attend(i, 1, ss[1])]
            gen = out_proj(i, us, True)
            next(gen)
            us += [attend(i, 2, ss[2]), attend(i, 3, ss[3])]
            residual(i, us)
            _drain(gen)

        mops0, vops0 = mem_lhs(0)
        _drain(qk_proj(0, 0, mops0), qk_proj(0, 1, mops0))
        _drain(zip(qk_proj(0, 2, mops0), vm_proj(0, 0, vops0)))
        _drain(zip(qk_proj(0, 3, mops0), vm_proj(0, 1, vops0)))

        def main_body(i, cy):
            step(i)

            @pl.when(i % NG == NG - 1)
            def _():
                o_copy(i // NG).start()

            return cy

        lax.fori_loop(0, NRB * NG - 1, main_body, 0)
        last_step(NRB * NG - 1)
        ok = jnp.min(okbuf[0:(NSEG - 1) * M, :])
        for rb in range(NRB - 1):
            o_copy(rb).wait()
        for qd in range(4):
            oq_copy(qd).wait()
        return it + 1, (ok > 0.5).astype(jnp.int32)

    lax.while_loop(lambda st: jnp.logical_and(st[0] < NSEG, st[1] == 0), sweep,
                   (jnp.int32(0), jnp.int32(0)))
    for t in range(NT):
        aout_copy(t).wait()


@functools.partial(jax.jit, static_argnames=("B_seg_len",))
def pallas_concat_heads__ssm_conv_h3__memory_aug_recurrent_mem_tr__prompt_kernel(
    A_q, A_k, A_v, A_shift_k, A_ssm_k, A_ssm_D,
    B_x, B_mem0, B_Wq, B_Wk, B_Wv, B_Wo, B_seg_len,
):
    _, S, D = A_q.shape
    DM = B_x.shape[2]
    H, E = B_Wq.shape[1], B_Wq.shape[2]
    M = B_mem0.shape[1]
    SEG = int(B_seg_len)
    NSEG = S // SEG
    NP = NSEG // 2
    PR = 2 * (M + SEG)
    PPB = 8
    NRB = NP // PPB
    NT = D // LANES
    assert E == LANES and H == 32 and M == 8 and SEG == 32 and A_shift_k.shape[1] == 4
    assert S == 2048 and D == 1024 and DM == 1024

    fwd, inv = _dft_mats()
    any_spec = pl.BlockSpec(memory_space=pl.ANY)
    scratch = [
        pltpu.VMEM((NRB, 7, PPB // 2 * SEG, DM // 2), U32),
        pltpu.VMEM((7, M + PPB // 2 * SEG, DM // 2), U32),
        pltpu.VMEM((H // 4, NP, 2 * SEG, 4 * E), BF16),
        pltpu.VMEM((3, H // 2, DM, E), U32),
        pltpu.VMEM((H * E, DM), BF16),
        pltpu.VMEM((4, PPB, PR, 2 * E), BF16),
        pltpu.VMEM((PPB, 2 * M, 4 * E), BF16),
        pltpu.VMEM((4, PPB // 2 * PR, DM // 2), F32),
        pltpu.VMEM((NRB, PPB * 2 * SEG, DM), BF16),
        pltpu.VMEM(((NSEG + 1) * M, DM), F32),
        pltpu.VMEM((NSEG * M, DM), F32),
        pltpu.VMEM((H // 4, NSEG * M, 4 * E), F32),
        pltpu.VMEM((H // 4, NSEG * M, 4 * E), F32),
        pltpu.VMEM((NSEG * M, LANES), F32),
        pltpu.VMEM((DM // LANES, NSEG, LANES), F32),
        pltpu.VMEM((H // 4, NSEG + M, 4 * E), F32),
        pltpu.VMEM((2, 3, S, LANES), BF16),
        pltpu.VMEM((2, LANES, S), BF16),
        pltpu.VMEM((S, LANES), BF16),
        pltpu.VMEM((NFFT, S), F32),
        pltpu.VMEM((NFFT, S), F32),
        pltpu.VMEM((NFFT, S), BF16),
        pltpu.VMEM((S + 32, LANES), F32),
        pltpu.VMEM((NT, S, LANES), BF16),
        pltpu.VMEM((M, DM), BF16),
        pltpu.VMEM((NFFT, BLK), BF16),
        pltpu.VMEM((BLK, BLK), BF16),
        pltpu.VMEM((4, D), BF16),
        pltpu.VMEM((NT, LANES), BF16),
        pltpu.VMEM((8, LANES), jnp.int32),
        pltpu.SMEM((7,), jnp.int32),
        pltpu.SemaphoreType.DMA((5,)),
        pltpu.SemaphoreType.DMA((2 * NRB,)),
        pltpu.SemaphoreType.DMA((H // 2,)),
        pltpu.SemaphoreType.DMA,
        pltpu.SemaphoreType.DMA,
        pltpu.SemaphoreType.DMA((2, 2)),
        pltpu.SemaphoreType.DMA,
        pltpu.SemaphoreType.DMA((NRB + 3,)),
    ]
    out = pl.pallas_call(
        functools.partial(_kernel, S=S, D=D, DM=DM, H=H, M=M, SEG=SEG),
        out_shape=jax.ShapeDtypeStruct((S, D + DM), BF16),
        in_specs=[any_spec] * 14,
        out_specs=any_spec,
        scratch_shapes=scratch,
        compiler_params=pltpu.CompilerParams(vmem_limit_bytes=120 * 1024 * 1024,
                                             disable_bounds_checks=True,
                                             disable_semaphore_checks=True),
    )(
        A_q.reshape(S, D), A_k.reshape(S, D), A_v.reshape(S, D),
        A_shift_k.T, A_ssm_k, A_ssm_D.reshape(NT, LANES),
        B_x.reshape(NRB, S // NRB, DM), B_mem0.reshape(M, DM),
        B_Wq, B_Wk, B_Wv, B_Wo.reshape(H * E, DM),
        jnp.asarray(fwd, BF16), jnp.asarray(inv, BF16),
    )
    return out.reshape(1, S, D + DM)
```

```python
import functools

import numpy as np
import jax
import jax.numpy as jnp
from jax import lax
import jax.experimental.pallas as pl
import jax.experimental.pallas.tpu as pltpu

F32 = jnp.float32
BF16 = jnp.bfloat16
U32 = jnp.uint32

LANES = 128
BLK = 128
NFFT = 2 * BLK
TOL = 2.0 ** -12


def _dft_mats():
    even = np.arange(0, BLK, 2)
    theta = 2.0 * np.pi * (np.concatenate([even, BLK - 1 - even]) + 0.5) / NFFT
    n = np.arange(BLK)
    c = np.cos(theta[:, None] * n[None, :])
    s = np.sin(theta[:, None] * n[None, :])
    fwd = np.zeros((NFFT, BLK))
    for m in range(BLK // 8):
        fwd[16 * m:16 * m + 8] = c[8 * m:8 * m + 8]
        fwd[16 * m + 8:16 * m + 16] = -s[8 * m:8 * m + 8]
    inv = fwd[:BLK].T * (2.0 / NFFT)
    inv = np.concatenate([inv[0::2], inv[1::2]], axis=0)
    return fwd.astype(np.float32), inv.astype(np.float32)


def _dot(a, b):
    return jnp.dot(a, b, preferred_element_type=F32)


def _pack(x):
    return pltpu.bitcast(x.astype(BF16), U32)


def _unpack(w):
    return pltpu.bitcast(w, BF16)


def _lo(w):
    return pltpu.bitcast(w << 16, F32)


def _hi(w):
    return pltpu.bitcast(w & jnp.uint32(0xFFFF0000), F32)


_STRASSEN_LHS = ((0, 3, 1), (2, 3, 1), (0, None, 0), (3, None, 0), (0, 1, 1), (2, 0, -1), (1, 3, -1))
_STRASSEN_RHS = ((0, 3, 1), (0, None, 0), (1, 3, -1), (2, 0, -1), (3, None, 0), (0, 1, 1), (2, 3, 1))


def _operand(table, k, quad):
    i, j, sign = table[k]
    if j is None:
        return quad(i)
    return quad(i) + quad(j) if sign > 0 else quad(i) - quad(j)


def _strassen_lhs(*quads):
    return [_operand(_STRASSEN_LHS, k, quads.__getitem__) for k in range(7)]


_STRASSEN_USES = (((0, 1), (3, 1)), ((2, 1), (3, -1)), ((1, 1), (3, 1)), ((0, 1), (2, 1)),
                  ((0, -1), (1, 1)), ((3, 1),), ((0, 1),))


def _strassen(lhs, rhs, emit, init=None, order=(4, 2, 1, 3, 0, 6, 5), post=None):
    acc = [[(1, c)] if c is not None else [] for c in (init or (None,) * 4)]
    left = [4, 2, 2, 4]
    for k in order:
        m = _dot(lhs(k), rhs[k])
        if post is not None:
            m = post(k, m)
        for q, sign in _STRASSEN_USES[k]:
            acc[q].append((sign, m))
            left[q] -= 1
            if left[q] < (3, 1, 1, 3)[q]:
                terms = sorted(acc[q], key=lambda t: -t[0])
                v = terms[0][1]
                assert terms[0][0] > 0
                for sg, t in terms[1:]:
                    v = v + t if sg > 0 else v - t
                acc[q] = [(1, v)]
            if left[q] == 0:
                emit(q // 2, q % 2, acc[q][0][1])
        yield m


def _drain(*gens):
    for g in gens:
        for _ in g:
            pass


def _tokens(m):
    return [(m, r, c) for r in range(0, m.shape[0], 8) for c in range(0, m.shape[1], LANES)]


def _tie(never, tok, x):
    if tok is None:
        return x
    reps = (x.shape[0] // 8, x.shape[1] // LANES)
    if tok.dtype != x.dtype:
        tok = pltpu.bitcast(tok, x.dtype)
    if reps != (1, 1):
        never, tok = jnp.tile(never, reps), jnp.tile(tok, reps)
    return jnp.where(never, tok, x)


def _run_paced(items, toks):
    for i, it in enumerate(items):
        m, r, c = toks[i * len(toks) // len(items)]
        it(m[r:r + 8, c:c + LANES])


def _interleave(nv, ngr, weights):
    dur = {'v': 256, 'h': 256, 'x': 256, 'inv': 128}
    margin = 768

    def plan(rate):
        t, v, out = 0, 0, []
        nxt = {'h': 0, 'x': 0, 'inv': 0}
        pos = {k: 0 for k in weights}
        done = {}
        credit = 0.0
        while True:
            kind = None
            if nxt['inv'] < ngr and done.get(('freq', nxt['inv']), 1e9) + margin <= t:
                kind = 'inv'
            elif nxt['x'] < ngr and done.get(('conv', nxt['x']), 1e9) + margin <= t:
                kind = 'x'
            elif nxt['h'] < ngr and nxt['h'] <= nxt['x'] and out and out[-1][0] == 'v':
                kind = 'h'
            elif v < nv:
                kind = 'v'
            if kind is None:
                break
            g = v if kind == 'v' else nxt[kind]
            busy = 0.6
            if kind == 'v':
                busy = 1.1 * (v % (nv // 2) < 7) + 0.55 * (v % 7 in (1, 3, 5, 6))
            credit += (rate - busy) * dur[kind]
            chunk = []
            while credit > 0:
                ready = [('out', i) for i in range(nxt['inv'])]
                ready += [('conv', i) for i in range(ngr)]
                ready += [('freq', i) for i in range(min(nxt['x'], nxt['h']))]
                ready = [k for k in ready if pos[k] < len(weights[k])]
                if not ready:
                    credit = 0.0
                    break
                k = ready[0]
                chunk.append((k, pos[k]))
                credit -= weights[k][pos[k]]
                pos[k] += 1
                if pos[k] == len(weights[k]):
                    done[k] = t + dur[kind]
            out.append((kind, g, chunk))
            t += dur[kind]
            if kind == 'v':
                v += 1
            else:
                nxt[kind] += 1
        ok = all(pos[k] == len(weights[k]) for k in weights)
        return ok, out

    rate = 1.0
    while True:
        ok, out = plan(rate)
        if ok:
            return out
        rate += 0.02


def _kernel(q_hbm, k_hbm, v_hbm, shift_hbm, h_hbm, d_hbm, x_hbm, mem0_hbm,
            wq_hbm, wk_hbm, wv_hbm, wo_hbm, fwd_hbm, inv_hbm,
            out_hbm,
            abuf, a0buf, vbuf, w32, wo, qks, vms, acc, obuf, mhat, mnew, uhat, unew, okbuf, mcol, tsum,
            ain, ah, kvb, xf, hf, wf, yt, aout,
            mem0_ref, fwd_ref, inv_ref, shift_ref, d_ref, zero_v, zero_s,
            sem_s, sem_x, sem_wv, sem_wqk, sem_wo, sem_a, sem_aout, sem_o,
            *, S, D, DM, H, M, SEG):
    E = LANES
    NSEG = S // SEG
    NP = NSEG // 2
    MR = 2 * M
    XR = 2 * SEG
    PR = MR + XR
    MW = MR // 2
    L = M + SEG
    NB = S // BLK
    NT = D // LANES
    PPB = 8
    PPH = PPB // 2
    NRB = NP // PPB
    G = 4
    NG = H // G
    KH = DM // 2
    scale = float(E) ** -0.5
    WV, WQ, WK = 0, 1, 2

    small = [pltpu.make_async_copy(src, dst, sem_s.at[i]) for i, (src, dst) in enumerate(
        ((mem0_hbm, mem0_ref), (shift_hbm, shift_ref), (d_hbm, d_ref),
         (fwd_hbm, fwd_ref), (inv_hbm, inv_ref)))]
    HBR = PPH * XR // 2

    def x_copies(hb):
        out = []
        for half in range(2):
            r = pl.ds(pl.multiple_of((2 * half + hb % 2) * HBR, HBR), HBR)
            out.append(pltpu.make_async_copy(x_hbm.at[hb // 2, r], obuf.at[hb // 2, r],
                                             sem_x.at[hb]))
        return out

    def w_copy(which, hp):
        src = (wv_hbm, wq_hbm, wk_hbm)[which].bitcast(U32)
        sem = sem_wv.at[hp] if which == WV else sem_wqk
        return pltpu.make_async_copy(src.at[:, hp, :], w32.at[which, hp], sem)

    def wo_copy(t):
        n = H * E // NT
        r = pl.ds(pl.multiple_of(t * n, n), n)
        return pltpu.make_async_copy(wo_hbm.at[r, :], wo.at[r, :], sem_wo)

    def a_start(t, sl, which=(0, 1, 2, 3)):
        c = pl.ds(pl.multiple_of(t * LANES, LANES), LANES)
        for i in which:
            if i == 3:
                pltpu.make_async_copy(h_hbm.at[c, :], ah.at[sl], sem_a.at[sl, 1]).start()
            else:
                src = (k_hbm, v_hbm, q_hbm)[i]
                pltpu.make_async_copy(src.at[:, c], ain.at[sl, i], sem_a.at[sl, 0]).start()

    def a_wait(sl):
        pltpu.make_async_copy(ain.at[sl], ain.at[sl], sem_a.at[sl, 0]).wait()
        pltpu.make_async_copy(ah.at[sl], ah.at[sl], sem_a.at[sl, 1]).wait()

    def aout_copy(t):
        c = pl.ds(pl.multiple_of(t * LANES, LANES), LANES)
        return pltpu.make_async_copy(aout.at[t], out_hbm.at[:, c], sem_aout)

    def o_copy(rb):
        r = pl.ds(pl.multiple_of(rb * (PPB * XR), PPB * XR), PPB * XR)
        return pltpu.make_async_copy(obuf.at[rb], out_hbm.at[r, pl.ds(D, DM)], sem_o.at[rb])

    def oq_copy(qd):
        n = PPH * XR
        r0, c0 = (qd // 2) * n, (qd % 2) * KH
        return pltpu.make_async_copy(
            obuf.at[NRB - 1, pl.ds(r0, n), pl.ds(c0, KH)],
            out_hbm.at[pl.ds((NRB - 1) * 2 * n + r0, n), pl.ds(D + c0, KH)],
            sem_o.at[NRB - 1 + qd])

    def w_rhs(which, hp):
        out = []
        for k in range(7):
            w = w32.at[which, hp + zero_s[k]]

            def quad(i, w=w):
                return (_lo, _hi)[i % 2](w[(i // 2) * KH:(i // 2 + 1) * KH])

            out.append(_operand(_STRASSEN_RHS, k, quad).astype(BF16))
        return out

    def w_plain(which, hp0, n):
        parts = []
        for j in range(n):
            w = w32[which, hp0 + j]
            parts += [_lo(w), _hi(w)]
        return jnp.concatenate(parts, axis=1).astype(BF16)

    small[0].start()
    for hb in range(2):
        for cp in x_copies(hb):
            cp.start()
    w_copy(WV, 0).start()
    w_copy(WV, 1).start()
    for cp in small[1:]:
        cp.start()

    zero_v[...] = jnp.zeros((8, LANES), jnp.int32)
    for k in range(7):
        zero_s[k] = 0
    tsum[:, 0:8, 0:LANES] = jnp.zeros((NG, 8, LANES), F32)
    vbuf[:, 0, 0:16, 0:LANES] = jnp.zeros((NG, 16, LANES), BF16)
    for hb in range(2 * NRB):
        r0 = (hb % 2) * (HBR // 2)
        abuf[hb // 2, 0, r0:r0 + 8, 0:LANES] = jnp.zeros((8, LANES), U32)

    ri = lax.broadcasted_iota(jnp.int32, (PR, PR), 0)
    ci = lax.broadcasted_iota(jnp.int32, (PR, PR), 1)

    def seg_of(r):
        return jnp.where(r < MR, r // M, (r - MR) // SEG)

    def pos_of(r):
        return jnp.where(r < MR, r % M, M + (r - MR) % SEG)

    same = seg_of(ri) == seg_of(ci)
    allowed = same & ((ri < MR) | (pos_of(ri) >= pos_of(ci)))
    fill = jnp.where(same, -1e9, -jnp.inf).astype(F32)

    small[0].wait()
    mem0 = mem0_ref[...].astype(F32)
    m0 = jnp.concatenate([mem0, jnp.zeros_like(mem0)], axis=0)
    z0 = jnp.zeros((MR, KH), F32)
    for k, op in enumerate(_strassen_lhs(m0[:, :KH], m0[:, KH:], z0, z0)):
        a0buf[k, 0:MW, :] = _pack(op)

    def x_item(tok, never, src, dst, r, c):
        quad = [_tie(never, tok, src[h * 2 * HBR + r:h * 2 * HBR + r + 16,
                                     kk * KH + c:kk * KH + c + 2 * LANES].astype(F32))
                for h in range(2) for kk in range(2)]
        for k, op in enumerate(_strassen_lhs(*quad)):
            dst[k, r // 2:r // 2 + 8, c:c + 2 * LANES] = _pack(op)

    def x_items(never, src, dst):
        return [functools.partial(x_item, never=never, src=src, dst=dst, r=r, c=c)
                for r in range(0, HBR, 16) for c in range(0, KH, 2 * LANES)]

    def x_first(hb, cy):
        for cp in x_copies(hb):
            cp.wait()
        src = obuf.at[0, pl.ds(pl.multiple_of(hb * HBR, HBR), 3 * HBR)]
        dst = a0buf.at[:, pl.ds(pl.multiple_of(MW + hb * (HBR // 2), 8), HBR // 2)]
        for it in x_items(None, src, dst):
            it(None)
        return cy

    lax.fori_loop(0, 2, x_first, 0)

    def v_part(j, rb, rhs, vwin, twin, pre=None):
        mem0_in = (0, 2, 4, 6) if rb == 0 else ()
        m0 = {}

        def lhs(k):
            x = abuf[rb, k] if rb else (a0buf[k] if k in mem0_in else a0buf[k, MW:])
            if pre is not None and k == 4:
                x0 = jnp.concatenate([pre(x[:8, :LANES]), x[:8, LANES:]], axis=1)
                x = jnp.concatenate([x0, x[8:]], axis=0)
            return _unpack(x)

        def split(k, m):
            if k not in mem0_in:
                return m
            m0[k] = m[:M]
            return m[MR:]

        def emit(half, hh, cv):
            c = slice((2 * j + hh) * E, (2 * j + hh + 1) * E)
            vx = cv.astype(BF16)
            p0 = rb * PPB + half * PPH
            vwin[p0:p0 + PPH, :, c] = vx.reshape(PPH, XR, E)
            ts = jnp.sum(vx.astype(F32).reshape(2 * PPH, SEG, E), axis=1)
            if rb == 0 and half == 0:
                v0 = m0[2] + m0[4] if hh else m0[0] - m0[4] + m0[6]
                v0 = v0.astype(BF16).astype(F32)
                twin[NSEG:NSEG + M, c] = v0
                t0 = jnp.sum(v0, axis=0, keepdims=True)
                rows = lax.broadcasted_iota(jnp.int32, ts.shape, 0)
                ts = ts + jnp.where(rows == 0, t0, 0.0)
            twin[2 * p0:2 * (p0 + PPH), c] = ts

        return _strassen(lhs, rhs, emit, post=split)

    def v_products(t, rbs, never, extra=()):
        vwin = vbuf.at[t]
        twin = tsum.at[t]

        def pre(x):
            for v in (twin[0:8, 0:LANES], pltpu.bitcast(vwin[0, 0:16, 0:LANES], U32)) + tuple(extra):
                x = _tie(never, v, x)
            return x

        for j in range(2):
            rhs = w_rhs(WV, 2 * t + j)
            for rb in rbs:
                yield from v_part(j, rb, rhs, vwin, twin, pre if (j, rb) == (0, rbs[0]) else None)

    def head_body(j, cy):
        w_copy(WV, 2 * j).wait()
        w_copy(WV, 2 * j + 1).wait()

        @pl.when(j >= 2)
        def _():
            for cp in x_copies(j):
                cp.wait()

        @pl.when(j + 1 < NT)
        def _():
            w_copy(WV, 2 * j + 2).start()
            w_copy(WV, 2 * j + 3).start()

        @pl.when(j + 2 < 2 * NRB)
        def _():
            for cp in x_copies(j + 2):
                cp.start()

        @pl.when(j == NT - 3)
        def _():
            a_start(0, 0, (3,))

        @pl.when(j == NT - 2)
        def _():
            a_start(0, 0, (0, 1, 2))

        never = zero_v[...] > 0
        src = obuf.at[j // 2, pl.ds(pl.multiple_of((j % 2) * HBR, HBR), 3 * HBR)]
        dst = abuf.at[j // 2, :, pl.ds(pl.multiple_of((j % 2) * (HBR // 2), 8), HBR // 2)]
        toks = []
        for m in v_products(j, [0], never, [dst[0, 0:8, 0:LANES]]):
            toks += _tokens(m)
        _run_paced(x_items(never, src, dst), toks[:-40])
        return cy

    assert NT == 2 * NRB
    lax.fori_loop(0, NT, head_body, 0)

    GA = 4

    def freq_items(a0, never):
        def item(tok, m, cc, st):
            r_re = slice(16 * m, 16 * m + 8)
            r_im = slice(16 * m + 8, 16 * m + 16)
            xr = _tie(never, tok, xf[r_re, cc * BLK:(cc + 1) * BLK])
            xi = _tie(never, tok, xf[r_im, cc * BLK:(cc + 1) * BLK])
            xs = xr + xi
            for a in range(max(a0, cc), a0 + GA):
                j = a - cc
                if ('g', m, j) not in st:
                    gr = hf[r_re, j * BLK:(j + 1) * BLK]
                    gi = hf[r_im, j * BLK:(j + 1) * BLK]
                    st['g', m, j] = (gr, gi, gr + gi)
                gr, gi, gs = st['g', m, j]
                ps = (xr * gr, xi * gi, xs * gs)
                st[m, a] = ps if (m, a) not in st else tuple(u + v for u, v in zip(st[m, a], ps))
                if cc == a:
                    p1, p2, p3 = st[m, a]
                    st[m, a] = (p1 - p2, p3 - p1 - p2)
                    if m >= BLK // 16:
                        m0 = m - BLK // 16
                        (wr, wi), (vr, vi) = st[m0, a], st[m, a]
                        c = slice(a * BLK, (a + 1) * BLK)
                        wf[16 * m0:16 * m0 + 16, c] = (
                            jnp.concatenate([wr + vr, wi - vi], axis=0).astype(BF16))
                        wf[16 * m:16 * m + 16, c] = (
                            jnp.concatenate([wr - vr, wi + vi], axis=0).astype(BF16))

        items = []
        for m0 in range(BLK // 16):
            st = {}
            for m in (m0, m0 + BLK // 16):
                items += [(functools.partial(item, m=m, cc=cc, st=st),
                           4 + 6 * (a0 + GA - max(a0, cc)) + (6 if cc >= a0 else 0))
                          for cc in range(a0 + GA)]
        return items

    def tile_body(t, carry):
        sl = t & 1
        a_wait(sl)

        @pl.when(t + 1 < NT)
        def _():
            a_start(t + 1, 1 - sl)
            wo_copy(t + 1).start()

        c = pl.ds(pl.multiple_of(t * LANES, LANES), LANES)
        taps = shift_ref[:, c].astype(F32)
        dcol = d_ref[...].astype(F32)
        rows = lax.broadcasted_iota(jnp.int32, dcol.shape, 0)
        dvec = jnp.sum(jnp.where(rows == t, dcol, 0.0), axis=0, keepdims=True)
        dvb = jnp.broadcast_to(dvec, (8, LANES))
        tapb = [jnp.broadcast_to(taps[j:j + 1, :], (8, LANES)) for j in range(4)]
        never = zero_v[...] > 0
        fwd = fwd_ref[...]
        NGR = NB // GA
        GW = GA * BLK

        sub = lax.broadcasted_iota(jnp.int32, (8, LANES), 0)
        kprev = [jnp.zeros((8, LANES), F32)]

        def conv_item(tok, r0):
            k16 = _tie(never, tok, ain[sl, 0, r0:r0 + 16, :].astype(F32))
            halves = []
            for h in range(2):
                k8 = k16[8 * h:8 * h + 8]
                ks = k8 * tapb[0]
                for j in range(1, 4):
                    ks = ks + pltpu.roll(jnp.where(sub < 8 - j, k8, kprev[0]), j, 0) * tapb[j]
                kprev[0] = k8
                halves.append(ks)
            kvb[r0:r0 + 16, :] = (jnp.concatenate(halves, axis=0)
                                  * ain[sl, 1, r0:r0 + 16, :].astype(F32)).astype(BF16)

        hlast = [None]

        def h_fwd(g):
            hst = jnp.concatenate([ah[sl, :, b * BLK:(b + 1) * BLK]
                                   for b in range(g * GA, (g + 1) * GA)], axis=0)
            hh = lax.dot_general(fwd, hst, (((1,), (1,)), ((), ())), preferred_element_type=F32)
            for b in range(GA):
                cur = hh[:, b * BLK:(b + 1) * BLK]
                prev = hlast[0]
                c = slice((g * GA + b) * BLK, (g * GA + b + 1) * BLK)
                if prev is None:
                    hf[:, c] = cur
                else:
                    for m in range(BLK // 8):
                        re = slice(16 * m, 16 * m + 8)
                        im = slice(16 * m + 8, 16 * m + 16)
                        if m < BLK // 16:
                            hf[re, c] = cur[re] - prev[im]
                            hf[im, c] = cur[im] + prev[re]
                        else:
                            hf[re, c] = cur[re] + prev[im]
                            hf[im, c] = cur[im] - prev[re]
                hlast[0] = cur
            return hh

        def x_fwd(g):
            rhs = jnp.concatenate([kvb[b * BLK:(b + 1) * BLK, :]
                                   for b in range(g * GA, (g + 1) * GA)], axis=1)
            xx = _dot(fwd, rhs)
            xf[:, g * GW:(g + 1) * GW] = xx
            return xx

        def inverse(g):
            ys = []
            for par in range(2):
                y = _dot(inv_ref[par * (BLK // 2):(par + 1) * (BLK // 2), :],
                         wf[par * BLK:(par + 1) * BLK, g * GW:(g + 1) * GW])
                for a in range(GA):
                    yt[pl.ds((g * GA + a) * BLK + par, BLK // 2, stride=2), :] = (
                        y[:, a * BLK:(a + 1) * BLK])
                ys.append(y)
            return jnp.concatenate(ys, axis=0)

        def out_item(tok, r0):
            d8 = _tie(never, tok, dvb)
            yb = yt[r0:r0 + 16, :] + kvb[r0:r0 + 16, :].astype(F32) * jnp.concatenate([d8, d8], axis=0)
            aout[t, r0:r0 + 16, :] = (ain[sl, 2, r0:r0 + 16, :].astype(F32) * yb).astype(BF16)

        def rows16(fn, g, w):
            return [(functools.partial(fn, r0=r0), w) for r0 in range(g * GW, (g + 1) * GW, 16)]

        vgen = v_products(t, list(range(1, NRB)), never)
        nv = 2 * (NRB - 1) * 7
        work = {('conv', g): rows16(conv_item, g, 31) for g in range(NGR)}
        work.update({('freq', g): freq_items(g * GA, never) for g in range(NGR)})
        work.update({('out', g): rows16(out_item, g, 16) for g in range(NGR)})
        for kind, g, chunks in _interleave(nv, NGR, {k: [w for _, w in v] for k, v in work.items()}):
            m = next(vgen) if kind == 'v' else {'h': h_fwd, 'x': x_fwd, 'inv': inverse}[kind](g)
            _run_paced([work[k][i][0] for k, i in chunks], _tokens(m))
        _drain(vgen)
        for which in (WQ, WK):
            w_copy(which, 2 * t).start()
            w_copy(which, 2 * t + 1).start()
        aout_copy(t).start()
        return carry

    for cp in small[1:]:
        cp.wait()
    wo_copy(0).start()
    lax.fori_loop(0, NT, tile_body, 0)
    pltpu.make_async_copy(wo, wo, sem_wo).wait()

    def initial_guess():
        puni = pl.reciprocal(jnp.full((1, 1), float(L), F32), approx=True).astype(BF16).astype(F32)

        def shift_down(m):
            rows = lax.broadcasted_iota(jnp.int32, m.shape, 0)
            return jnp.where(rows == 0, 0.0, pltpu.roll(m, 1, 0))

        tall = jnp.concatenate([tsum[g, 0:NSEG, :] for g in range(NG)], axis=1)
        wov = wo[...]
        m1 = shift_down(_dot((tall * puni).astype(BF16), wov))
        v1 = _dot(m1.astype(BF16), w_plain(WV, 0, H // 2))
        u2 = (tall + float(M) * v1) * puni
        for g in range(NG):
            tsum[g, 0:NSEG, :] = u2[:, g * (G * E):(g + 1) * (G * E)]
        u2 = u2.astype(BF16)
        for c in range(0, DM, LANES):
            mcol[c // LANES] = _dot(u2, wov[:, c:c + LANES])
            for sg in range(NSEG):
                mhat[(sg + 1) * M:(sg + 2) * M, c:c + LANES] = jnp.broadcast_to(
                    mcol[c // LANES, sg:sg + 1, :], (M, LANES))
        mhat[0:M, :] = mem0_ref[...].astype(F32)
        pltpu.make_async_copy(w32.at[WQ:WK + 1], w32.at[WQ:WK + 1], sem_wqk).wait()

    def sweep(state):
        it, _ = state
        pl.when(it == 0)(initial_guess)

        def u_estimate(first, rb, g):
            n = PPB * MR
            one = tsum[g, pl.ds(pl.multiple_of(rb * (2 * PPB), 2 * PPB), 2 * PPB), :]
            one = jnp.broadcast_to(one[:, None, :], (2 * PPB, M, G * E)).reshape(n, G * E)
            return jnp.where(first, one, uhat[g, pl.ds(pl.multiple_of(rb * n, n), n), :])

        @pl.when(it > 0)
        def _():
            def upd(i, cy):
                rb, g = i // NG, i % NG
                n = PPB * MR
                r = pl.ds(pl.multiple_of(rb * n, n), n)
                r2 = pl.ds(pl.multiple_of(rb * n + M, M), n)
                c = pl.ds(pl.multiple_of(g * LANES, LANES), LANES)
                keep = okbuf[r, :] > 0.5
                mhat[r2, c] = jnp.where(keep, mhat[r2, c], mnew[r, c])
                uhat[g, r, :] = jnp.where(jnp.tile(keep, (1, G)), u_estimate(it == 1, rb, g),
                                          unew[g, r, :])
                return cy

            assert NG * LANES == DM
            lax.fori_loop(0, NRB * NG, upd, 0)

        def mem_rows(i):
            n = PPB * MR
            return mhat[pl.ds(pl.multiple_of((i // NG) * n, n), n), :]

        def mem_lhs(i):
            m = mem_rows(i)
            n = PPH * MR
            ops = [_pack(o) for o in _strassen_lhs(m[:n, :KH], m[:n, KH:], m[n:, :KH], m[n:, KH:])]
            t = jnp.concatenate([jnp.where(i < NG, 0.0, m[:M]), m[M:MR]], axis=0)
            b = m[n:n + MR]
            vops = [jnp.concatenate([_pack(o), full[MW:]], axis=0) for o, full in zip(
                _strassen_lhs(t[:, :KH], t[:, KH:], b[:, :KH], b[:, KH:]), ops)]
            return ops, vops

        def qk_proj(i, j, mops):
            rb = i // NG
            hp = (i % NG) * (G // 2) + j // 2

            def lhs(k):
                return _unpack(jnp.concatenate([mops[k], abuf[rb, k]], axis=0))

            n = PPH * MR
            cs = {}

            def emit(half, hh, cv):
                cs[half, hh] = cv
                if (half, 1 - hh) in cs:
                    v = jnp.concatenate([cs[half, 0], cs[half, 1]], axis=1).astype(BF16)
                    ps = slice(half * PPH, (half + 1) * PPH)
                    qks[j, ps, 0:MR, :] = v[:n].reshape(PPH, MR, 2 * E)
                    qks[j, ps, MR:PR, :] = v[n:].reshape(PPH, XR, 2 * E)

            return _strassen(lhs, w_rhs(WQ + j % 2, hp), emit)

        def vm_proj(i, j, vops):
            hp = (i % NG) * (G // 2) + j

            def emit(half, hh, cv):
                if half == 0:
                    v0 = tsum[i % NG, NSEG:NSEG + M, (2 * j + hh) * E:(2 * j + hh + 1) * E]
                    cv = jnp.concatenate([jnp.where(i < NG, v0, cv[:M]), cv[M:]], axis=0)
                vms[half * PPH:(half + 1) * PPH, :, (2 * j + hh) * E:(2 * j + hh + 1) * E] = (
                    cv.astype(BF16).reshape(PPH, MR, E))

            return _strassen(lambda k: _unpack(vops[k]), w_rhs(WV, hp), emit)

        def scores(j):
            c = slice((j % 2) * E, (j % 2 + 1) * E)
            return lax.dot_general(qks[2 * (j // 2), :, :, c], qks[2 * (j // 2) + 1, :, :, c],
                                   (((2,), (2,)), ((0,), (0,))), preferred_element_type=F32)

        def attend(i, j, s):
            p0 = pl.multiple_of((i // NG) * PPB, PPB)
            s = jnp.where(allowed[None], s * scale, fill[None])
            e = jnp.exp(s - jnp.max(s, axis=-1, keepdims=True))
            p = (e * pl.reciprocal(jnp.sum(e, axis=-1, keepdims=True), approx=True)).astype(BF16)
            vh = jnp.concatenate(
                [vms[:, :, j * E:(j + 1) * E],
                 vbuf[i % NG, pl.ds(p0, PPB), :, j * E:(j + 1) * E]], axis=1)
            return lax.dot_general(p, vh, (((2,), (1,)), ((0,), (0,))), preferred_element_type=F32)

        def residual(i, us):
            rb, g = i // NG, i % NG
            n = PPB * MR
            rm = pl.ds(pl.multiple_of(rb * n, n), n)
            new = jnp.concatenate([u[:, :MR, :] for u in us], axis=2).reshape(n, G * E)
            unew[g, rm, :] = new
            err = jnp.max(jnp.abs(new - u_estimate(it == 0, rb, g)), axis=1, keepdims=True)
            ref = jnp.max(jnp.abs(new), axis=1, keepdims=True)
            ok = jnp.broadcast_to(jnp.where(err <= TOL * ref, 1.0, 0.0), (n, LANES))
            okbuf[rm, :] = jnp.minimum(ok, jnp.where(g > 0, okbuf[rm, :], 1.0))

        def out_proj(i, us, last):
            rb = i // NG
            n = PPH * PR
            kh = G * E // 2

            def uquad(q):
                u = jnp.concatenate([us[2 * (q % 2)], us[2 * (q % 2) + 1]], axis=2)
                return u[(q // 2) * PPH:(q // 2 + 1) * PPH].reshape(n, kh)

            def lhs(k):
                return _operand(_STRASSEN_LHS, k, uquad).astype(BF16)

            wf32 = wo[pl.ds(pl.multiple_of((i % NG) * (G * E), G * E), G * E), :].astype(F32)
            wq4 = [wf32[:kh, :KH], wf32[:kh, KH:], wf32[kh:, :KH], wf32[kh:, KH:]]
            rhs = [_operand(_STRASSEN_RHS, k, wq4.__getitem__).astype(BF16) for k in range(7)]
            init = [jnp.where(i % NG > 0, acc[q], 0.0) for q in range(4)]
            mwin = mnew.at[pl.ds(pl.multiple_of(rb * (PPB * MR), PPB * MR), PPB * MR), :]

            def emit(half, hh, v):
                c = slice(hh * KH, (hh + 1) * KH)
                v3 = v.reshape(PPH, PR, KH)
                mwin[half * PPH * MR:(half + 1) * PPH * MR, c] = v3[:, :MR].reshape(PPH * MR, KH)
                obuf[rb, half * PPH * XR:(half + 1) * PPH * XR, c] = (
                    v3[:, MR:].reshape(PPH * XR, KH).astype(BF16))
                if last:
                    oq_copy(2 * half + hh).start()
                else:
                    acc[2 * half + hh] = v

            if last:
                return _strassen(lhs, rhs, emit, init, order=(2, 5, 4, 1, 3, 0, 6))
            return _strassen(lhs, rhs, emit, init)

        def step(i):
            s0, s1 = scores(0), scores(1)
            mops, vops = mem_lhs(i + 1)
            _drain(qk_proj(i + 1, 0, mops))
            us = [attend(i, 0, s0), attend(i, 1, s1)]
            s2, s3 = scores(2), scores(3)
            _drain(qk_proj(i + 1, 1, mops))
            us += [attend(i, 2, s2), attend(i, 3, s3)]
            residual(i, us)
            _drain(zip(qk_proj(i + 1, 2, mops), vm_proj(i + 1, 0, vops)))
            _drain(zip(qk_proj(i + 1, 3, mops), vm_proj(i + 1, 1, vops)))
            _drain(out_proj(i, us, False))

        def last_step(i):
            ss = [scores(j) for j in range(G)]
            us = [attend(i, 0, ss[0]), attend(i, 1, ss[1])]
            gen = out_proj(i, us, True)
            next(gen)
            us += [attend(i, 2, ss[2]), attend(i, 3, ss[3])]
            residual(i, us)
            _drain(gen)

        mops0, vops0 = mem_lhs(0)
        _drain(qk_proj(0, 0, mops0), qk_proj(0, 1, mops0))
        _drain(zip(qk_proj(0, 2, mops0), vm_proj(0, 0, vops0)))
        _drain(zip(qk_proj(0, 3, mops0), vm_proj(0, 1, vops0)))

        def main_body(i, cy):
            step(i)

            @pl.when(i % NG == NG - 1)
            def _():
                o_copy(i // NG).start()

            return cy

        lax.fori_loop(0, NRB * NG - 1, main_body, 0)
        last_step(NRB * NG - 1)
        ok = jnp.min(okbuf[0:(NSEG - 1) * M, :])
        for rb in range(NRB - 1):
            o_copy(rb).wait()
        for qd in range(4):
            oq_copy(qd).wait()
        return it + 1, (ok > 0.5).astype(jnp.int32)

    lax.while_loop(lambda st: jnp.logical_and(st[0] < NSEG, st[1] == 0), sweep,
                   (jnp.int32(0), jnp.int32(0)))
    for t in range(NT):
        aout_copy(t).wait()


SEG_LEN = 32


def pallas_concat_heads__ssm_conv_h3__memory_aug_recurrent_mem_tr__prompt_kernel(
    A_q, A_k, A_v, A_shift_k, A_ssm_k, A_ssm_D,
    B_x, B_mem0, B_Wq, B_Wk, B_Wv, B_Wo, B_seg_len,
):
    if isinstance(B_seg_len, int):
        assert B_seg_len == SEG_LEN
    return _run(A_q, A_k, A_v, A_shift_k, A_ssm_k, A_ssm_D, B_x, B_mem0, B_Wq, B_Wk, B_Wv, B_Wo)


@jax.jit
def _run(A_q, A_k, A_v, A_shift_k, A_ssm_k, A_ssm_D, B_x, B_mem0, B_Wq, B_Wk, B_Wv, B_Wo):
    _, S, D = A_q.shape
    DM = B_x.shape[2]
    H, E = B_Wq.shape[1], B_Wq.shape[2]
    M = B_mem0.shape[1]
    SEG = SEG_LEN
    NSEG = S // SEG
    NP = NSEG // 2
    PR = 2 * (M + SEG)
    PPB = 8
    NRB = NP // PPB
    NT = D // LANES
    assert E == LANES and H == 32 and M == 8 and A_shift_k.shape[1] == 4
    assert S == 2048 and D == 1024 and DM == 1024

    fwd, inv = _dft_mats()
    any_spec = pl.BlockSpec(memory_space=pl.ANY)
    scratch = [
        pltpu.VMEM((NRB, 7, PPB // 2 * SEG, DM // 2), U32),
        pltpu.VMEM((7, M + PPB // 2 * SEG, DM // 2), U32),
        pltpu.VMEM((H // 4, NP, 2 * SEG, 4 * E), BF16),
        pltpu.VMEM((3, H // 2, DM, E), U32),
        pltpu.VMEM((H * E, DM), BF16),
        pltpu.VMEM((4, PPB, PR, 2 * E), BF16),
        pltpu.VMEM((PPB, 2 * M, 4 * E), BF16),
        pltpu.VMEM((4, PPB // 2 * PR, DM // 2), F32),
        pltpu.VMEM((NRB, PPB * 2 * SEG, DM), BF16),
        pltpu.VMEM(((NSEG + 1) * M, DM), F32),
        pltpu.VMEM((NSEG * M, DM), F32),
        pltpu.VMEM((H // 4, NSEG * M, 4 * E), F32),
        pltpu.VMEM((H // 4, NSEG * M, 4 * E), F32),
        pltpu.VMEM((NSEG * M, LANES), F32),
        pltpu.VMEM((DM // LANES, NSEG, LANES), F32),
        pltpu.VMEM((H // 4, NSEG + M, 4 * E), F32),
        pltpu.VMEM((2, 3, S, LANES), BF16),
        pltpu.VMEM((2, LANES, S), BF16),
        pltpu.VMEM((S, LANES), BF16),
        pltpu.VMEM((NFFT, S), F32),
        pltpu.VMEM((NFFT, S), F32),
        pltpu.VMEM((NFFT, S), BF16),
        pltpu.VMEM((S + 32, LANES), F32),
        pltpu.VMEM((NT, S, LANES), BF16),
        pltpu.VMEM((M, DM), BF16),
        pltpu.VMEM((NFFT, BLK), BF16),
        pltpu.VMEM((BLK, BLK), BF16),
        pltpu.VMEM((4, D), BF16),
        pltpu.VMEM((NT, LANES), BF16),
        pltpu.VMEM((8, LANES), jnp.int32),
        pltpu.SMEM((7,), jnp.int32),
        pltpu.SemaphoreType.DMA((5,)),
        pltpu.SemaphoreType.DMA((2 * NRB,)),
        pltpu.SemaphoreType.DMA((H // 2,)),
        pltpu.SemaphoreType.DMA,
        pltpu.SemaphoreType.DMA,
        pltpu.SemaphoreType.DMA((2, 2)),
        pltpu.SemaphoreType.DMA,
        pltpu.SemaphoreType.DMA((NRB + 3,)),
    ]
    out = pl.pallas_call(
        functools.partial(_kernel, S=S, D=D, DM=DM, H=H, M=M, SEG=SEG),
        out_shape=jax.ShapeDtypeStruct((S, D + DM), BF16),
        in_specs=[any_spec] * 14,
        out_specs=any_spec,
        scratch_shapes=scratch,
        compiler_params=pltpu.CompilerParams(vmem_limit_bytes=120 * 1024 * 1024,
                                             disable_bounds_checks=True,
                                             disable_semaphore_checks=True),
    )(
        A_q.reshape(S, D), A_k.reshape(S, D), A_v.reshape(S, D),
        A_shift_k.T, A_ssm_k, A_ssm_D.reshape(NT, LANES),
        B_x.reshape(NRB, S // NRB, DM), B_mem0.reshape(M, DM),
        B_Wq, B_Wk, B_Wv, B_Wo.reshape(H * E, DM),
        jnp.asarray(fwd, BF16), jnp.asarray(inv, BF16),
    )
    return out.reshape(1, S, D + DM)
```

```python
import functools

import numpy as np
import jax
import jax.numpy as jnp
from jax import lax
import jax.experimental.pallas as pl
import jax.experimental.pallas.tpu as pltpu

F32 = jnp.float32
BF16 = jnp.bfloat16
U32 = jnp.uint32

LANES = 128
BLK = 128
NFFT = 2 * BLK
TOL = 2.0 ** -12


def _dft_mats():
    even = np.arange(0, BLK, 2)
    theta = 2.0 * np.pi * (np.concatenate([even, BLK - 1 - even]) + 0.5) / NFFT
    n = np.arange(BLK)
    c = np.cos(theta[:, None] * n[None, :])
    s = np.sin(theta[:, None] * n[None, :])
    fwd = np.zeros((NFFT, BLK))
    for m in range(BLK // 8):
        fwd[16 * m:16 * m + 8] = c[8 * m:8 * m + 8]
        fwd[16 * m + 8:16 * m + 16] = -s[8 * m:8 * m + 8]
    inv = fwd[:BLK].T * (2.0 / NFFT)
    inv = np.concatenate([inv[0::2], inv[1::2]], axis=0)
    return fwd.astype(np.float32), inv.astype(np.float32)


def _dot(a, b):
    return jnp.dot(a, b, preferred_element_type=F32)


def _pack(x):
    return pltpu.bitcast(x.astype(BF16), U32)


def _unpack(w):
    return pltpu.bitcast(w, BF16)


def _lo(w):
    return pltpu.bitcast(w << 16, F32)


def _hi(w):
    return pltpu.bitcast(w & jnp.uint32(0xFFFF0000), F32)


_STRASSEN_LHS = ((0, 3, 1), (2, 3, 1), (0, None, 0), (3, None, 0), (0, 1, 1), (2, 0, -1), (1, 3, -1))
_STRASSEN_RHS = ((0, 3, 1), (0, None, 0), (1, 3, -1), (2, 0, -1), (3, None, 0), (0, 1, 1), (2, 3, 1))


def _operand(table, k, quad):
    i, j, sign = table[k]
    if j is None:
        return quad(i)
    return quad(i) + quad(j) if sign > 0 else quad(i) - quad(j)


def _strassen_lhs(*quads):
    return [_operand(_STRASSEN_LHS, k, quads.__getitem__) for k in range(7)]


_STRASSEN_USES = (((0, 1), (3, 1)), ((2, 1), (3, -1)), ((1, 1), (3, 1)), ((0, 1), (2, 1)),
                  ((0, -1), (1, 1)), ((3, 1),), ((0, 1),))


def _strassen(lhs, rhs, emit, init=None, order=(4, 2, 1, 3, 0, 6, 5), post=None):
    acc = [[(1, c)] if c is not None else [] for c in (init or (None,) * 4)]
    left = [4, 2, 2, 4]
    for k in order:
        m = _dot(lhs(k), rhs[k])
        if post is not None:
            m = post(k, m)
        for q, sign in _STRASSEN_USES[k]:
            acc[q].append((sign, m))
            left[q] -= 1
            if left[q] < (3, 1, 1, 3)[q]:
                terms = sorted(acc[q], key=lambda t: -t[0])
                v = terms[0][1]
                assert terms[0][0] > 0
                for sg, t in terms[1:]:
                    v = v + t if sg > 0 else v - t
                acc[q] = [(1, v)]
            if left[q] == 0:
                emit(q // 2, q % 2, acc[q][0][1])
        yield m


def _drain(*gens):
    for g in gens:
        for _ in g:
            pass


def _tokens(m):
    return [(m, r, c) for r in range(0, m.shape[0], 8) for c in range(0, m.shape[1], LANES)]


def _tie(never, tok, x):
    if tok is None:
        return x
    if tok.dtype != x.dtype:
        tok = pltpu.bitcast(tok, x.dtype)
    if x.shape == (8, LANES):
        return jnp.where(never, tok, x)
    return jnp.concatenate(
        [jnp.concatenate([jnp.where(never, tok, x[r:r + 8, c:c + LANES])
                          for c in range(0, x.shape[1], LANES)], axis=1)
         for r in range(0, x.shape[0], 8)], axis=0)


def _run_paced(items, toks):
    for i, it in enumerate(items):
        m, r, c = toks[i * len(toks) // len(items)]
        it(m[r:r + 8, c:c + LANES])


def _interleave(nv, ngr, weights):
    dur = {'v': 256, 'h': 256, 'x': 256, 'inv': 128}
    margin = 768

    def plan(rate):
        t, v, out = 0, 0, []
        nxt = {'h': 0, 'x': 0, 'inv': 0}
        pos = {k: 0 for k in weights}
        done = {}
        credit = 0.0
        while True:
            kind = None
            if nxt['inv'] < ngr and done.get(('freq', nxt['inv']), 1e9) + margin <= t:
                kind = 'inv'
            elif nxt['x'] < ngr and done.get(('conv', nxt['x']), 1e9) + margin <= t:
                kind = 'x'
            elif nxt['h'] < ngr and nxt['h'] <= nxt['x'] and out and out[-1][0] == 'v':
                kind = 'h'
            elif v < nv:
                kind = 'v'
            if kind is None:
                break
            g = v if kind == 'v' else nxt[kind]
            busy = 0.6
            if kind == 'v':
                busy = 1.1 * (v % (nv // 2) < 7) + 0.55 * (v % 7 in (1, 3, 5, 6))
            credit += (rate - busy) * dur[kind]
            chunk = []
            while credit > 0:
                ready = [('out', i) for i in range(nxt['inv'])]
                ready += [('conv', i) for i in range(ngr)]
                ready += [('freq', i) for i in range(min(nxt['x'], nxt['h']))]
                ready = [k for k in ready if pos[k] < len(weights[k])]
                if not ready:
                    credit = 0.0
                    break
                k = ready[0]
                chunk.append((k, pos[k]))
                credit -= weights[k][pos[k]]
                pos[k] += 1
                if pos[k] == len(weights[k]):
                    done[k] = t + dur[kind]
            out.append((kind, g, chunk))
            t += dur[kind]
            if kind == 'v':
                v += 1
            else:
                nxt[kind] += 1
        ok = all(pos[k] == len(weights[k]) for k in weights)
        return ok, out

    rate = 1.0
    while True:
        ok, out = plan(rate)
        if ok:
            return out
        rate += 0.02


def _kernel(q_hbm, k_hbm, v_hbm, shift_hbm, h_hbm, d_hbm, x_hbm, mem0_hbm,
            wq_hbm, wk_hbm, wv_hbm, wo_hbm, fwd_hbm, inv_hbm,
            out_hbm,
            abuf, a0buf, vbuf, w32, wo, qks, vms, acc, obuf, mhat, mnew, uhat, unew, okbuf, mcol, tsum,
            ain, ah, kvb, xf, hf, wf, yt, aout,
            mem0_ref, fwd_ref, inv_ref, shift_ref, d_ref, zero_v, zero_s,
            sem_s, sem_x, sem_wv, sem_wqk, sem_wo, sem_a, sem_aout, sem_o,
            *, S, D, DM, H, M, SEG):
    E = LANES
    NSEG = S // SEG
    NP = NSEG // 2
    MR = 2 * M
    XR = 2 * SEG
    PR = MR + XR
    MW = MR // 2
    L = M + SEG
    NB = S // BLK
    NT = D // LANES
    PPB = 8
    PPH = PPB // 2
    NRB = NP // PPB
    G = 4
    NG = H // G
    KH = DM // 2
    scale = float(E) ** -0.5
    WV, WQ, WK = 0, 1, 2

    small = [pltpu.make_async_copy(src, dst, sem_s.at[i]) for i, (src, dst) in enumerate(
        ((mem0_hbm, mem0_ref), (shift_hbm, shift_ref), (d_hbm, d_ref),
         (fwd_hbm, fwd_ref), (inv_hbm, inv_ref)))]
    HBR = PPH * XR // 2

    def x_copies(hb):
        out = []
        for half in range(2):
            r = pl.ds(pl.multiple_of((2 * half + hb % 2) * HBR, HBR), HBR)
            out.append(pltpu.make_async_copy(x_hbm.at[hb // 2, r], obuf.at[hb // 2, r],
                                             sem_x.at[hb]))
        return out

    def w_copy(which, hp):
        src = (wv_hbm, wq_hbm, wk_hbm)[which].bitcast(U32)
        sem = sem_wv.at[hp] if which == WV else sem_wqk
        return pltpu.make_async_copy(src.at[:, hp, :], w32.at[which, hp], sem)

    def wo_copy(t):
        n = H * E // NT
        r = pl.ds(pl.multiple_of(t * n, n), n)
        return pltpu.make_async_copy(wo_hbm.at[r, :], wo.at[r, :], sem_wo)

    def a_start(t, sl, which=(0, 1, 2, 3)):
        c = pl.ds(pl.multiple_of(t * LANES, LANES), LANES)
        for i in which:
            if i == 3:
                pltpu.make_async_copy(h_hbm.at[c, :], ah.at[sl], sem_a.at[sl, 1]).start()
            else:
                src = (k_hbm, v_hbm, q_hbm)[i]
                pltpu.make_async_copy(src.at[:, c], ain.at[sl, i], sem_a.at[sl, 0]).start()

    def a_wait(sl):
        pltpu.make_async_copy(ain.at[sl], ain.at[sl], sem_a.at[sl, 0]).wait()
        pltpu.make_async_copy(ah.at[sl], ah.at[sl], sem_a.at[sl, 1]).wait()

    def aout_copy(t):
        c = pl.ds(pl.multiple_of(t * LANES, LANES), LANES)
        return pltpu.make_async_copy(aout.at[t], out_hbm.at[:, c], sem_aout)

    def o_copy(rb):
        r = pl.ds(pl.multiple_of(rb * (PPB * XR), PPB * XR), PPB * XR)
        return pltpu.make_async_copy(obuf.at[rb], out_hbm.at[r, pl.ds(D, DM)], sem_o.at[rb])

    def oq_copy(qd):
        n = PPH * XR
        r0, c0 = (qd // 2) * n, (qd % 2) * KH
        return pltpu.make_async_copy(
            obuf.at[NRB - 1, pl.ds(r0, n), pl.ds(c0, KH)],
            out_hbm.at[pl.ds((NRB - 1) * 2 * n + r0, n), pl.ds(D + c0, KH)],
            sem_o.at[NRB - 1 + qd])

    def w_rhs(which, hp):
        out = []
        for k in range(7):
            w = w32.at[which, hp + zero_s[k]]

            def quad(i, w=w):
                return (_lo, _hi)[i % 2](w[(i // 2) * KH:(i // 2 + 1) * KH])

            out.append(_operand(_STRASSEN_RHS, k, quad).astype(BF16))
        return out

    def w_plain(which, hp0, n):
        parts = []
        for j in range(n):
            w = w32[which, hp0 + j]
            parts += [_lo(w), _hi(w)]
        return jnp.concatenate(parts, axis=1).astype(BF16)

    small[0].start()
    for hb in range(2):
        for cp in x_copies(hb):
            cp.start()
    w_copy(WV, 0).start()
    w_copy(WV, 1).start()
    for cp in small[1:]:
        cp.start()

    zero_v[...] = jnp.zeros((8, LANES), jnp.int32)
    for k in range(7):
        zero_s[k] = 0
    tsum[:, 0:8, 0:LANES] = jnp.zeros((NG, 8, LANES), F32)
    vbuf[:, 0, 0:16, 0:LANES] = jnp.zeros((NG, 16, LANES), BF16)
    for hb in range(2 * NRB):
        r0 = (hb % 2) * (HBR // 2)
        abuf[hb // 2, 0, r0:r0 + 8, 0:LANES] = jnp.zeros((8, LANES), U32)

    ri = lax.broadcasted_iota(jnp.int32, (PR, PR), 0)
    ci = lax.broadcasted_iota(jnp.int32, (PR, PR), 1)

    def seg_of(r):
        return jnp.where(r < MR, r // M, (r - MR) // SEG)

    def pos_of(r):
        return jnp.where(r < MR, r % M, M + (r - MR) % SEG)

    same = seg_of(ri) == seg_of(ci)
    allowed = same & ((ri < MR) | (pos_of(ri) >= pos_of(ci)))
    fill = jnp.where(same, -1e9, -jnp.inf).astype(F32)

    small[0].wait()
    mem0 = mem0_ref[...].astype(F32)
    m0 = jnp.concatenate([mem0, jnp.zeros_like(mem0)], axis=0)
    z0 = jnp.zeros((MR, KH), F32)
    for k, op in enumerate(_strassen_lhs(m0[:, :KH], m0[:, KH:], z0, z0)):
        a0buf[k, 0:MW, :] = _pack(op)

    def x_item(tok, never, src, dst, r, c):
        quad = [_tie(never, tok, src[h * 2 * HBR + r:h * 2 * HBR + r + 16,
                                     kk * KH + c:kk * KH + c + 2 * LANES].astype(F32))
                for h in range(2) for kk in range(2)]
        for k, op in enumerate(_strassen_lhs(*quad)):
            dst[k, r // 2:r // 2 + 8, c:c + 2 * LANES] = _pack(op)

    def x_items(never, src, dst):
        return [functools.partial(x_item, never=never, src=src, dst=dst, r=r, c=c)
                for r in range(0, HBR, 16) for c in range(0, KH, 2 * LANES)]

    def x_first(hb, cy):
        for cp in x_copies(hb):
            cp.wait()
        src = obuf.at[0, pl.ds(pl.multiple_of(hb * HBR, HBR), 3 * HBR)]
        dst = a0buf.at[:, pl.ds(pl.multiple_of(MW + hb * (HBR // 2), 8), HBR // 2)]
        for it in x_items(None, src, dst):
            it(None)
        return cy

    lax.fori_loop(0, 2, x_first, 0)

    def v_part(j, rb, rhs, vwin, twin, pre=None):
        mem0_in = (0, 2, 4, 6) if rb == 0 else ()
        m0 = {}

        def lhs(k):
            x = abuf[rb, k] if rb else (a0buf[k] if k in mem0_in else a0buf[k, MW:])
            if pre is not None and k == 4:
                x0 = jnp.concatenate([pre(x[:8, :LANES]), x[:8, LANES:]], axis=1)
                x = jnp.concatenate([x0, x[8:]], axis=0)
            return _unpack(x)

        def split(k, m):
            if k not in mem0_in:
                return m
            m0[k] = m[:M]
            return m[MR:]

        def emit(half, hh, cv):
            c = slice((2 * j + hh) * E, (2 * j + hh + 1) * E)
            vx = cv.astype(BF16)
            p0 = rb * PPB + half * PPH
            vwin[p0:p0 + PPH, :, c] = vx.reshape(PPH, XR, E)
            ts = jnp.sum(vx.astype(F32).reshape(2 * PPH, SEG, E), axis=1)
            if rb == 0 and half == 0:
                v0 = m0[2] + m0[4] if hh else m0[0] - m0[4] + m0[6]
                v0 = v0.astype(BF16).astype(F32)
                twin[NSEG:NSEG + M, c] = v0
                t0 = jnp.sum(v0, axis=0, keepdims=True)
                rows = lax.broadcasted_iota(jnp.int32, ts.shape, 0)
                ts = ts + jnp.where(rows == 0, t0, 0.0)
            twin[2 * p0:2 * (p0 + PPH), c] = ts

        return _strassen(lhs, rhs, emit, post=split)

    def v_products(t, rbs, never, extra=()):
        vwin = vbuf.at[t]
        twin = tsum.at[t]

        def pre(x):
            for v in (twin[0:8, 0:LANES], pltpu.bitcast(vwin[0, 0:16, 0:LANES], U32)) + tuple(extra):
                x = _tie(never, v, x)
            return x

        for j in range(2):
            rhs = w_rhs(WV, 2 * t + j)
            for rb in rbs:
                yield from v_part(j, rb, rhs, vwin, twin, pre if (j, rb) == (0, rbs[0]) else None)

    def head_body(j, cy):
        w_copy(WV, 2 * j).wait()
        w_copy(WV, 2 * j + 1).wait()

        @pl.when(j >= 2)
        def _():
            for cp in x_copies(j):
                cp.wait()

        @pl.when(j + 1 < NT)
        def _():
            w_copy(WV, 2 * j + 2).start()
            w_copy(WV, 2 * j + 3).start()

        @pl.when(j + 2 < 2 * NRB)
        def _():
            for cp in x_copies(j + 2):
                cp.start()

        @pl.when(j == NT - 3)
        def _():
            a_start(0, 0, (3,))

        @pl.when(j == NT - 2)
        def _():
            a_start(0, 0, (0, 1, 2))

        never = zero_v[...] > 0
        src = obuf.at[j // 2, pl.ds(pl.multiple_of((j % 2) * HBR, HBR), 3 * HBR)]
        dst = abuf.at[j // 2, :, pl.ds(pl.multiple_of((j % 2) * (HBR // 2), 8), HBR // 2)]
        toks = []
        for m in v_products(j, [0], never, [dst[0, 0:8, 0:LANES]]):
            toks += _tokens(m)
        _run_paced(x_items(never, src, dst), toks[:-40])
        return cy

    assert NT == 2 * NRB
    lax.fori_loop(0, NT, head_body, 0)

    GA = 4

    def freq_items(a0, never):
        def item(tok, m, cc, st):
            r_re = slice(16 * m, 16 * m + 8)
            r_im = slice(16 * m + 8, 16 * m + 16)
            xr = _tie(never, tok, xf[r_re, cc * BLK:(cc + 1) * BLK])
            xi = _tie(never, tok, xf[r_im, cc * BLK:(cc + 1) * BLK])
            xs = xr + xi
            for a in range(max(a0, cc), a0 + GA):
                j = a - cc
                if ('g', m, j) not in st:
                    gr = hf[r_re, j * BLK:(j + 1) * BLK]
                    gi = hf[r_im, j * BLK:(j + 1) * BLK]
                    st['g', m, j] = (gr, gi, gr + gi)
                gr, gi, gs = st['g', m, j]
                ps = (xr * gr, xi * gi, xs * gs)
                st[m, a] = ps if (m, a) not in st else tuple(u + v for u, v in zip(st[m, a], ps))
                if cc == a:
                    p1, p2, p3 = st[m, a]
                    st[m, a] = (p1 - p2, p3 - p1 - p2)
                    if m >= BLK // 16:
                        m0 = m - BLK // 16
                        (wr, wi), (vr, vi) = st[m0, a], st[m, a]
                        c = slice(a * BLK, (a + 1) * BLK)
                        wf[16 * m0:16 * m0 + 16, c] = (
                            jnp.concatenate([wr + vr, wi - vi], axis=0).astype(BF16))
                        wf[16 * m:16 * m + 16, c] = (
                            jnp.concatenate([wr - vr, wi + vi], axis=0).astype(BF16))

        items = []
        for m0 in range(BLK // 16):
            st = {}
            for m in (m0, m0 + BLK // 16):
                items += [(functools.partial(item, m=m, cc=cc, st=st),
                           4 + 6 * (a0 + GA - max(a0, cc)) + (6 if cc >= a0 else 0))
                          for cc in range(a0 + GA)]
        return items

    def tile_body(t, carry):
        sl = t & 1
        a_wait(sl)

        @pl.when(t + 1 < NT)
        def _():
            a_start(t + 1, 1 - sl)
            wo_copy(t + 1).start()

        c = pl.ds(pl.multiple_of(t * LANES, LANES), LANES)
        taps = shift_ref[:, c].astype(F32)
        dcol = d_ref[...].astype(F32)
        rows = lax.broadcasted_iota(jnp.int32, dcol.shape, 0)
        dvec = jnp.sum(jnp.where(rows == t, dcol, 0.0), axis=0, keepdims=True)
        dvb = jnp.broadcast_to(dvec, (8, LANES))
        tapb = [jnp.broadcast_to(taps[j:j + 1, :], (8, LANES)) for j in range(4)]
        never = zero_v[...] > 0
        fwd = fwd_ref[...]
        NGR = NB // GA
        GW = GA * BLK

        sub = lax.broadcasted_iota(jnp.int32, (8, LANES), 0)
        stays = [sub < 8 - j for j in range(4)]
        kprev = [jnp.zeros((8, LANES), F32)]

        def conv_item(tok, r0):
            k16 = _tie(never, tok, ain[sl, 0, r0:r0 + 16, :].astype(F32))
            halves = []
            for h in range(2):
                k8 = k16[8 * h:8 * h + 8]
                ks = k8 * tapb[0]
                for j in range(1, 4):
                    ks = ks + pltpu.roll(jnp.where(stays[j], k8, kprev[0]), j, 0) * tapb[j]
                kprev[0] = k8
                halves.append(ks)
            kvb[r0:r0 + 16, :] = (jnp.concatenate(halves, axis=0)
                                  * ain[sl, 1, r0:r0 + 16, :].astype(F32)).astype(BF16)

        hlast = [None]

        def h_fwd(g):
            hst = jnp.concatenate([ah[sl, :, b * BLK:(b + 1) * BLK]
                                   for b in range(g * GA, (g + 1) * GA)], axis=0)
            hh = lax.dot_general(fwd, hst, (((1,), (1,)), ((), ())), preferred_element_type=F32)
            for b in range(GA):
                cur = hh[:, b * BLK:(b + 1) * BLK]
                prev = hlast[0]
                c = slice((g * GA + b) * BLK, (g * GA + b + 1) * BLK)
                if prev is None:
                    hf[:, c] = cur
                else:
                    for m in range(BLK // 8):
                        re = slice(16 * m, 16 * m + 8)
                        im = slice(16 * m + 8, 16 * m + 16)
                        if m < BLK // 16:
                            hf[re, c] = cur[re] - prev[im]
                            hf[im, c] = cur[im] + prev[re]
                        else:
                            hf[re, c] = cur[re] + prev[im]
                            hf[im, c] = cur[im] - prev[re]
                hlast[0] = cur
            return hh

        def x_fwd(g):
            rhs = jnp.concatenate([kvb[b * BLK:(b + 1) * BLK, :]
                                   for b in range(g * GA, (g + 1) * GA)], axis=1)
            xx = _dot(fwd, rhs)
            xf[:, g * GW:(g + 1) * GW] = xx
            return xx

        def inverse(g):
            ys = []
            for par in range(2):
                y = _dot(inv_ref[par * (BLK // 2):(par + 1) * (BLK // 2), :],
                         wf[par * BLK:(par + 1) * BLK, g * GW:(g + 1) * GW])
                for a in range(GA):
                    yt[pl.ds((g * GA + a) * BLK + par, BLK // 2, stride=2), :] = (
                        y[:, a * BLK:(a + 1) * BLK])
                ys.append(y)
            return jnp.concatenate(ys, axis=0)

        def out_item(tok, r0):
            d8 = _tie(never, tok, dvb)
            yb = yt[r0:r0 + 16, :] + kvb[r0:r0 + 16, :].astype(F32) * jnp.concatenate([d8, d8], axis=0)
            aout[t, r0:r0 + 16, :] = (ain[sl, 2, r0:r0 + 16, :].astype(F32) * yb).astype(BF16)

        def rows16(fn, g, w):
            return [(functools.partial(fn, r0=r0), w) for r0 in range(g * GW, (g + 1) * GW, 16)]

        vgen = v_products(t, list(range(1, NRB)), never)
        nv = 2 * (NRB - 1) * 7
        work = {('conv', g): rows16(conv_item, g, 31) for g in range(NGR)}
        work.update({('freq', g): freq_items(g * GA, never) for g in range(NGR)})
        work.update({('out', g): rows16(out_item, g, 16) for g in range(NGR)})
        for kind, g, chunks in _interleave(nv, NGR, {k: [w for _, w in v] for k, v in work.items()}):
            m = next(vgen) if kind == 'v' else {'h': h_fwd, 'x': x_fwd, 'inv': inverse}[kind](g)
            _run_paced([work[k][i][0] for k, i in chunks], _tokens(m))
        _drain(vgen)
        for which in (WQ, WK):
            w_copy(which, 2 * t).start()
            w_copy(which, 2 * t + 1).start()
        aout_copy(t).start()
        return carry

    for cp in small[1:]:
        cp.wait()
    wo_copy(0).start()
    lax.fori_loop(0, NT, tile_body, 0)
    pltpu.make_async_copy(wo, wo, sem_wo).wait()

    def initial_guess():
        puni = pl.reciprocal(jnp.full((1, 1), float(L), F32), approx=True).astype(BF16).astype(F32)

        def shift_down(m):
            rows = lax.broadcasted_iota(jnp.int32, m.shape, 0)
            return jnp.where(rows == 0, 0.0, pltpu.roll(m, 1, 0))

        tall = jnp.concatenate([tsum[g, 0:NSEG, :] for g in range(NG)], axis=1)
        wov = wo[...]
        m1 = shift_down(_dot((tall * puni).astype(BF16), wov))
        v1 = _dot(m1.astype(BF16), w_plain(WV, 0, H // 2))
        u2 = (tall + float(M) * v1) * puni
        for g in range(NG):
            tsum[g, 0:NSEG, :] = u2[:, g * (G * E):(g + 1) * (G * E)]
        u2 = u2.astype(BF16)
        for c in range(0, DM, LANES):
            mcol[c // LANES] = _dot(u2, wov[:, c:c + LANES])
            for sg in range(NSEG):
                mhat[(sg + 1) * M:(sg + 2) * M, c:c + LANES] = jnp.broadcast_to(
                    mcol[c // LANES, sg:sg + 1, :], (M, LANES))
        mhat[0:M, :] = mem0_ref[...].astype(F32)
        pltpu.make_async_copy(w32.at[WQ:WK + 1], w32.at[WQ:WK + 1], sem_wqk).wait()

    def sweep(state):
        it, _ = state
        pl.when(it == 0)(initial_guess)

        def u_estimate(first, rb, g):
            n = PPB * MR
            one = tsum[g, pl.ds(pl.multiple_of(rb * (2 * PPB), 2 * PPB), 2 * PPB), :]
            one = jnp.broadcast_to(one[:, None, :], (2 * PPB, M, G * E)).reshape(n, G * E)
            return jnp.where(first, one, uhat[g, pl.ds(pl.multiple_of(rb * n, n), n), :])

        @pl.when(it > 0)
        def _():
            def upd(i, cy):
                rb, g = i // NG, i % NG
                n = PPB * MR
                r = pl.ds(pl.multiple_of(rb * n, n), n)
                r2 = pl.ds(pl.multiple_of(rb * n + M, M), n)
                c = pl.ds(pl.multiple_of(g * LANES, LANES), LANES)
                okr = okbuf[r, :]
                mhat[r2, c] = jnp.where(okr > 0.5, mhat[r2, c], mnew[r, c])
                uhat[g, r, :] = jnp.where(jnp.concatenate([okr] * G, axis=1) > 0.5,
                                          u_estimate(it == 1, rb, g), unew[g, r, :])
                return cy

            assert NG * LANES == DM
            lax.fori_loop(0, NRB * NG, upd, 0)

        def mem_rows(i):
            n = PPB * MR
            return mhat[pl.ds(pl.multiple_of((i // NG) * n, n), n), :]

        def mem_lhs(i):
            m = mem_rows(i)
            n = PPH * MR
            ops = [_pack(o) for o in _strassen_lhs(m[:n, :KH], m[:n, KH:], m[n:, :KH], m[n:, KH:])]
            t = jnp.concatenate([jnp.where(i < NG, 0.0, m[:M]), m[M:MR]], axis=0)
            b = m[n:n + MR]
            vops = [jnp.concatenate([_pack(o), full[MW:]], axis=0) for o, full in zip(
                _strassen_lhs(t[:, :KH], t[:, KH:], b[:, :KH], b[:, KH:]), ops)]
            return ops, vops

        def qk_proj(i, j, mops):
            rb = i // NG
            hp = (i % NG) * (G // 2) + j // 2

            def lhs(k):
                return _unpack(jnp.concatenate([mops[k], abuf[rb, k]], axis=0))

            n = PPH * MR
            cs = {}

            def emit(half, hh, cv):
                cs[half, hh] = cv
                if (half, 1 - hh) in cs:
                    v = jnp.concatenate([cs[half, 0], cs[half, 1]], axis=1).astype(BF16)
                    ps = slice(half * PPH, (half + 1) * PPH)
                    qks[j, ps, 0:MR, :] = v[:n].reshape(PPH, MR, 2 * E)
                    qks[j, ps, MR:PR, :] = v[n:].reshape(PPH, XR, 2 * E)

            return _strassen(lhs, w_rhs(WQ + j % 2, hp), emit)

        def vm_proj(i, j, vops):
            hp = (i % NG) * (G // 2) + j

            def emit(half, hh, cv):
                if half == 0:
                    v0 = tsum[i % NG, NSEG:NSEG + M, (2 * j + hh) * E:(2 * j + hh + 1) * E]
                    cv = jnp.concatenate([jnp.where(i < NG, v0, cv[:M]), cv[M:]], axis=0)
                vms[half * PPH:(half + 1) * PPH, :, (2 * j + hh) * E:(2 * j + hh + 1) * E] = (
                    cv.astype(BF16).reshape(PPH, MR, E))

            return _strassen(lambda k: _unpack(vops[k]), w_rhs(WV, hp), emit)

        def scores(j):
            c = slice((j % 2) * E, (j % 2 + 1) * E)
            return lax.dot_general(qks[2 * (j // 2), :, :, c], qks[2 * (j // 2) + 1, :, :, c],
                                   (((2,), (2,)), ((0,), (0,))), preferred_element_type=F32)

        def attend(i, j, s):
            p0 = pl.multiple_of((i // NG) * PPB, PPB)
            s = jnp.where(allowed[None], s * scale, fill[None])
            e = jnp.exp(s - jnp.max(s, axis=-1, keepdims=True))
            p = (e * pl.reciprocal(jnp.sum(e, axis=-1, keepdims=True), approx=True)).astype(BF16)
            vh = jnp.concatenate(
                [vms[:, :, j * E:(j + 1) * E],
                 vbuf[i % NG, pl.ds(p0, PPB), :, j * E:(j + 1) * E]], axis=1)
            return lax.dot_general(p, vh, (((2,), (1,)), ((0,), (0,))), preferred_element_type=F32)

        def residual(i, us):
            rb, g = i // NG, i % NG
            n = PPB * MR
            rm = pl.ds(pl.multiple_of(rb * n, n), n)
            new = jnp.concatenate([u[:, :MR, :] for u in us], axis=2).reshape(n, G * E)
            unew[g, rm, :] = new
            err = jnp.max(jnp.abs(new - u_estimate(it == 0, rb, g)), axis=1, keepdims=True)
            ref = jnp.max(jnp.abs(new), axis=1, keepdims=True)
            ok = jnp.broadcast_to(jnp.where(err <= TOL * ref, 1.0, 0.0), (n, LANES))
            okbuf[rm, :] = jnp.minimum(ok, jnp.where(g > 0, okbuf[rm, :], 1.0))

        def out_proj(i, us, last):
            rb = i // NG
            n = PPH * PR
            kh = G * E // 2

            def uquad(q):
                u = jnp.concatenate([us[2 * (q % 2)], us[2 * (q % 2) + 1]], axis=2)
                return u[(q // 2) * PPH:(q // 2 + 1) * PPH].reshape(n, kh)

            def lhs(k):
                return _operand(_STRASSEN_LHS, k, uquad).astype(BF16)

            wf32 = wo[pl.ds(pl.multiple_of((i % NG) * (G * E), G * E), G * E), :].astype(F32)
            wq4 = [wf32[:kh, :KH], wf32[:kh, KH:], wf32[kh:, :KH], wf32[kh:, KH:]]
            rhs = [_operand(_STRASSEN_RHS, k, wq4.__getitem__).astype(BF16) for k in range(7)]
            init = [jnp.where(i % NG > 0, acc[q], 0.0) for q in range(4)]
            mwin = mnew.at[pl.ds(pl.multiple_of(rb * (PPB * MR), PPB * MR), PPB * MR), :]

            def emit(half, hh, v):
                c = slice(hh * KH, (hh + 1) * KH)
                v3 = v.reshape(PPH, PR, KH)
                mwin[half * PPH * MR:(half + 1) * PPH * MR, c] = v3[:, :MR].reshape(PPH * MR, KH)
                obuf[rb, half * PPH * XR:(half + 1) * PPH * XR, c] = (
                    v3[:, MR:].reshape(PPH * XR, KH).astype(BF16))
                if last:
                    oq_copy(2 * half + hh).start()
                else:
                    acc[2 * half + hh] = v

            if last:
                return _strassen(lhs, rhs, emit, init, order=(2, 5, 4, 1, 3, 0, 6))
            return _strassen(lhs, rhs, emit, init)

        def step(i):
            s0, s1 = scores(0), scores(1)
            mops, vops = mem_lhs(i + 1)
            _drain(qk_proj(i + 1, 0, mops))
            us = [attend(i, 0, s0), attend(i, 1, s1)]
            s2, s3 = scores(2), scores(3)
            _drain(qk_proj(i + 1, 1, mops))
            us += [attend(i, 2, s2), attend(i, 3, s3)]
            residual(i, us)
            _drain(zip(qk_proj(i + 1, 2, mops), vm_proj(i + 1, 0, vops)))
            _drain(zip(qk_proj(i + 1, 3, mops), vm_proj(i + 1, 1, vops)))
            _drain(out_proj(i, us, False))

        def last_step(i):
            ss = [scores(j) for j in range(G)]
            us = [attend(i, 0, ss[0]), attend(i, 1, ss[1])]
            gen = out_proj(i, us, True)
            next(gen)
            us += [attend(i, 2, ss[2]), attend(i, 3, ss[3])]
            residual(i, us)
            _drain(gen)

        mops0, vops0 = mem_lhs(0)
        _drain(qk_proj(0, 0, mops0), qk_proj(0, 1, mops0))
        _drain(zip(qk_proj(0, 2, mops0), vm_proj(0, 0, vops0)))
        _drain(zip(qk_proj(0, 3, mops0), vm_proj(0, 1, vops0)))

        def main_body(i, cy):
            step(i)

            @pl.when(i % NG == NG - 1)
            def _():
                o_copy(i // NG).start()

            return cy

        lax.fori_loop(0, NRB * NG - 1, main_body, 0)
        last_step(NRB * NG - 1)
        ok = jnp.min(okbuf[0:(NSEG - 1) * M, :])
        for rb in range(NRB - 1):
            o_copy(rb).wait()
        for qd in range(4):
            oq_copy(qd).wait()
        return it + 1, (ok > 0.5).astype(jnp.int32)

    lax.while_loop(lambda st: jnp.logical_and(st[0] < NSEG, st[1] == 0), sweep,
                   (jnp.int32(0), jnp.int32(0)))
    for t in range(NT):
        aout_copy(t).wait()


SEG_LEN = 32


def pallas_concat_heads__ssm_conv_h3__memory_aug_recurrent_mem_tr__prompt_kernel(
    A_q, A_k, A_v, A_shift_k, A_ssm_k, A_ssm_D,
    B_x, B_mem0, B_Wq, B_Wk, B_Wv, B_Wo, B_seg_len,
):
    if isinstance(B_seg_len, int):
        assert B_seg_len == SEG_LEN
    return _run(A_q, A_k, A_v, A_shift_k, A_ssm_k, A_ssm_D, B_x, B_mem0, B_Wq, B_Wk, B_Wv, B_Wo)


@jax.jit
def _run(A_q, A_k, A_v, A_shift_k, A_ssm_k, A_ssm_D, B_x, B_mem0, B_Wq, B_Wk, B_Wv, B_Wo):
    _, S, D = A_q.shape
    DM = B_x.shape[2]
    H, E = B_Wq.shape[1], B_Wq.shape[2]
    M = B_mem0.shape[1]
    SEG = SEG_LEN
    NSEG = S // SEG
    NP = NSEG // 2
    PR = 2 * (M + SEG)
    PPB = 8
    NRB = NP // PPB
    NT = D // LANES
    assert E == LANES and H == 32 and M == 8 and A_shift_k.shape[1] == 4
    assert S == 2048 and D == 1024 and DM == 1024

    fwd, inv = _dft_mats()
    any_spec = pl.BlockSpec(memory_space=pl.ANY)
    scratch = [
        pltpu.VMEM((NRB, 7, PPB // 2 * SEG, DM // 2), U32),
        pltpu.VMEM((7, M + PPB // 2 * SEG, DM // 2), U32),
        pltpu.VMEM((H // 4, NP, 2 * SEG, 4 * E), BF16),
        pltpu.VMEM((3, H // 2, DM, E), U32),
        pltpu.VMEM((H * E, DM), BF16),
        pltpu.VMEM((4, PPB, PR, 2 * E), BF16),
        pltpu.VMEM((PPB, 2 * M, 4 * E), BF16),
        pltpu.VMEM((4, PPB // 2 * PR, DM // 2), F32),
        pltpu.VMEM((NRB, PPB * 2 * SEG, DM), BF16),
        pltpu.VMEM(((NSEG + 1) * M, DM), F32),
        pltpu.VMEM((NSEG * M, DM), F32),
        pltpu.VMEM((H // 4, NSEG * M, 4 * E), F32),
        pltpu.VMEM((H // 4, NSEG * M, 4 * E), F32),
        pltpu.VMEM((NSEG * M, LANES), F32),
        pltpu.VMEM((DM // LANES, NSEG, LANES), F32),
        pltpu.VMEM((H // 4, NSEG + M, 4 * E), F32),
        pltpu.VMEM((2, 3, S, LANES), BF16),
        pltpu.VMEM((2, LANES, S), BF16),
        pltpu.VMEM((S, LANES), BF16),
        pltpu.VMEM((NFFT, S), F32),
        pltpu.VMEM((NFFT, S), F32),
        pltpu.VMEM((NFFT, S), BF16),
        pltpu.VMEM((S + 32, LANES), F32),
        pltpu.VMEM((NT, S, LANES), BF16),
        pltpu.VMEM((M, DM), BF16),
        pltpu.VMEM((NFFT, BLK), BF16),
        pltpu.VMEM((BLK, BLK), BF16),
        pltpu.VMEM((4, D), BF16),
        pltpu.VMEM((NT, LANES), BF16),
        pltpu.VMEM((8, LANES), jnp.int32),
        pltpu.SMEM((7,), jnp.int32),
        pltpu.SemaphoreType.DMA((5,)),
        pltpu.SemaphoreType.DMA((2 * NRB,)),
        pltpu.SemaphoreType.DMA((H // 2,)),
        pltpu.SemaphoreType.DMA,
        pltpu.SemaphoreType.DMA,
        pltpu.SemaphoreType.DMA((2, 2)),
        pltpu.SemaphoreType.DMA,
        pltpu.SemaphoreType.DMA((NRB + 3,)),
    ]
    out = pl.pallas_call(
        functools.partial(_kernel, S=S, D=D, DM=DM, H=H, M=M, SEG=SEG),
        out_shape=jax.ShapeDtypeStruct((S, D + DM), BF16),
        in_specs=[any_spec] * 14,
        out_specs=any_spec,
        scratch_shapes=scratch,
        compiler_params=pltpu.CompilerParams(vmem_limit_bytes=120 * 1024 * 1024,
                                             disable_bounds_checks=True,
                                             disable_semaphore_checks=True),
    )(
        A_q.reshape(S, D), A_k.reshape(S, D), A_v.reshape(S, D),
        A_shift_k.T, A_ssm_k, A_ssm_D.reshape(NT, LANES),
        B_x.reshape(NRB, S // NRB, DM), B_mem0.reshape(M, DM),
        B_Wq, B_Wk, B_Wv, B_Wo.reshape(H * E, DM),
        jnp.asarray(fwd, BF16), jnp.asarray(inv, BF16),
    )
    return out.reshape(1, S, D + DM)
```

```python
import functools

import numpy as np
import jax
import jax.numpy as jnp
from jax import lax
import jax.experimental.pallas as pl
import jax.experimental.pallas.tpu as pltpu

F32 = jnp.float32
BF16 = jnp.bfloat16
U32 = jnp.uint32

LANES = 128
BLK = 128
NFFT = 2 * BLK
TOL = 2.0 ** -12


def _dft_mats():
    even = np.arange(0, BLK, 2)
    theta = 2.0 * np.pi * (np.concatenate([even, BLK - 1 - even]) + 0.5) / NFFT
    n = np.arange(BLK)
    c = np.cos(theta[:, None] * n[None, :])
    s = np.sin(theta[:, None] * n[None, :])
    fwd = np.zeros((NFFT, BLK))
    for m in range(BLK // 8):
        fwd[16 * m:16 * m + 8] = c[8 * m:8 * m + 8]
        fwd[16 * m + 8:16 * m + 16] = -s[8 * m:8 * m + 8]
    inv = fwd[:BLK].T * (2.0 / NFFT)
    inv = np.concatenate([inv[0::2], inv[1::2]], axis=0)
    return fwd.astype(np.float32), inv.astype(np.float32)


def _dot(a, b):
    return jnp.dot(a, b, preferred_element_type=F32)


def _pack(x):
    return pltpu.bitcast(x.astype(BF16), U32)


def _unpack(w):
    return pltpu.bitcast(w, BF16)


def _lo(w):
    return pltpu.bitcast(w << 16, F32)


def _hi(w):
    return pltpu.bitcast(w & jnp.uint32(0xFFFF0000), F32)


_STRASSEN_LHS = ((0, 3, 1), (2, 3, 1), (0, None, 0), (3, None, 0), (0, 1, 1), (2, 0, -1), (1, 3, -1))
_STRASSEN_RHS = ((0, 3, 1), (0, None, 0), (1, 3, -1), (2, 0, -1), (3, None, 0), (0, 1, 1), (2, 3, 1))


def _operand(table, k, quad):
    i, j, sign = table[k]
    if j is None:
        return quad(i)
    return quad(i) + quad(j) if sign > 0 else quad(i) - quad(j)


def _strassen_lhs(*quads):
    return [_operand(_STRASSEN_LHS, k, quads.__getitem__) for k in range(7)]


_STRASSEN_USES = (((0, 1), (3, 1)), ((2, 1), (3, -1)), ((1, 1), (3, 1)), ((0, 1), (2, 1)),
                  ((0, -1), (1, 1)), ((3, 1),), ((0, 1),))


def _strassen(lhs, rhs, emit, init=None, order=(4, 2, 1, 3, 0, 6, 5), post=None):
    acc = [[(1, c)] if c is not None else [] for c in (init or (None,) * 4)]
    left = [4, 2, 2, 4]
    for k in order:
        m = _dot(lhs(k), rhs[k])
        if post is not None:
            m = post(k, m)
        for q, sign in _STRASSEN_USES[k]:
            acc[q].append((sign, m))
            left[q] -= 1
            if left[q] < (3, 1, 1, 3)[q]:
                terms = sorted(acc[q], key=lambda t: -t[0])
                v = terms[0][1]
                assert terms[0][0] > 0
                for sg, t in terms[1:]:
                    v = v + t if sg > 0 else v - t
                acc[q] = [(1, v)]
            if left[q] == 0:
                emit(q // 2, q % 2, acc[q][0][1])
        yield m


def _drain(*gens):
    for g in gens:
        for _ in g:
            pass


def _tokens(m):
    return [(m, r, c) for r in range(0, m.shape[0], 8) for c in range(0, m.shape[1], LANES)]


def _tie(never, tok, x):
    if tok is None:
        return x
    if tok.dtype != x.dtype:
        tok = pltpu.bitcast(tok, x.dtype)
    if x.shape == (8, LANES):
        return jnp.where(never, tok, x)
    return jnp.concatenate(
        [jnp.concatenate([jnp.where(never, tok, x[r:r + 8, c:c + LANES])
                          for c in range(0, x.shape[1], LANES)], axis=1)
         for r in range(0, x.shape[0], 8)], axis=0)


def _run_paced(items, toks):
    for i, it in enumerate(items):
        m, r, c = toks[i * len(toks) // len(items)]
        it(m[r:r + 8, c:c + LANES])


def _interleave(nv, ngr, weights):
    dur = {'v': 256, 'h': 256, 'x': 256, 'inv': 128}
    margin = 768

    def plan(rate):
        t, v, out = 0, 0, []
        nxt = {'h': 0, 'x': 0, 'inv': 0}
        pos = {k: 0 for k in weights}
        done = {}
        credit = 0.0
        while True:
            kind = None
            if nxt['inv'] < ngr and done.get(('freq', nxt['inv']), 1e9) + margin <= t:
                kind = 'inv'
            elif nxt['x'] < ngr and done.get(('conv', nxt['x']), 1e9) + margin <= t:
                kind = 'x'
            elif nxt['h'] < ngr and nxt['h'] <= nxt['x'] and out and out[-1][0] == 'v':
                kind = 'h'
            elif v < nv:
                kind = 'v'
            if kind is None:
                break
            g = v if kind == 'v' else nxt[kind]
            busy = 0.6
            if kind == 'v':
                busy = 1.1 * (v % (nv // 2) < 7) + 0.55 * (v % 7 in (1, 3, 5, 6))
            credit += (rate - busy) * dur[kind]
            chunk = []
            while credit > 0:
                ready = [('out', i) for i in range(nxt['inv'])]
                ready += [('conv', i) for i in range(ngr)]
                ready += [('freq', i) for i in range(min(nxt['x'], nxt['h']))]
                ready = [k for k in ready if pos[k] < len(weights[k])]
                if not ready:
                    credit = 0.0
                    break
                k = ready[0]
                chunk.append((k, pos[k]))
                credit -= weights[k][pos[k]]
                pos[k] += 1
                if pos[k] == len(weights[k]):
                    done[k] = t + dur[kind]
            out.append((kind, g, chunk))
            t += dur[kind]
            if kind == 'v':
                v += 1
            else:
                nxt[kind] += 1
        ok = all(pos[k] == len(weights[k]) for k in weights)
        return ok, out

    rate = 1.0
    while True:
        ok, out = plan(rate)
        if ok:
            return out
        rate += 0.02


def _kernel(q_hbm, k_hbm, v_hbm, shift_hbm, h_hbm, d_hbm, x_hbm, mem0_hbm,
            wq_hbm, wk_hbm, wv_hbm, wo_hbm, fwd_hbm, inv_hbm,
            out_hbm,
            abuf, a0buf, vbuf, w32, wo, qks, vms, acc, obuf, mhat, mnew, uhat, unew, okbuf, mcol, tsum,
            ain, ah, kvb, xf, hf, wf, yt, aout,
            mem0_ref, fwd_ref, inv_ref, shift_ref, d_ref, zero_v, zero_s,
            sem_s, sem_x, sem_wv, sem_wqk, sem_wo, sem_a, sem_aout, sem_o,
            *, S, D, DM, H, M, SEG):
    E = LANES
    NSEG = S // SEG
    NP = NSEG // 2
    MR = 2 * M
    XR = 2 * SEG
    PR = MR + XR
    MW = MR // 2
    L = M + SEG
    NB = S // BLK
    NT = D // LANES
    PPB = 8
    PPH = PPB // 2
    NRB = NP // PPB
    G = 4
    NG = H // G
    KH = DM // 2
    scale = float(E) ** -0.5
    WV, WQ, WK = 0, 1, 2

    small = [pltpu.make_async_copy(src, dst, sem_s.at[i]) for i, (src, dst) in enumerate(
        ((mem0_hbm, mem0_ref), (shift_hbm, shift_ref), (d_hbm, d_ref),
         (fwd_hbm, fwd_ref), (inv_hbm, inv_ref)))]
    HBR = PPH * XR // 2

    def x_copies(hb):
        out = []
        for half in range(2):
            r = pl.ds(pl.multiple_of((2 * half + hb % 2) * HBR, HBR), HBR)
            out.append(pltpu.make_async_copy(x_hbm.at[hb // 2, r], obuf.at[hb // 2, r],
                                             sem_x.at[hb]))
        return out

    def w_copy(which, hp):
        src = (wv_hbm, wq_hbm, wk_hbm)[which].bitcast(U32)
        sem = sem_wv.at[hp] if which == WV else sem_wqk
        return pltpu.make_async_copy(src.at[:, hp, :], w32.at[which, hp], sem)

    def wo_copy(t):
        n = H * E // NT
        r = pl.ds(pl.multiple_of(t * n, n), n)
        return pltpu.make_async_copy(wo_hbm.at[r, :], wo.at[r, :], sem_wo)

    def a_start(t, sl, which=(0, 1, 2, 3)):
        c = pl.ds(pl.multiple_of(t * LANES, LANES), LANES)
        for i in which:
            if i == 3:
                pltpu.make_async_copy(h_hbm.at[c, :], ah.at[sl], sem_a.at[sl, 1]).start()
            else:
                src = (k_hbm, v_hbm, q_hbm)[i]
                pltpu.make_async_copy(src.at[:, c], ain.at[sl, i], sem_a.at[sl, 0]).start()

    def a_wait(sl):
        pltpu.make_async_copy(ain.at[sl], ain.at[sl], sem_a.at[sl, 0]).wait()
        pltpu.make_async_copy(ah.at[sl], ah.at[sl], sem_a.at[sl, 1]).wait()

    def aout_copy(t):
        c = pl.ds(pl.multiple_of(t * LANES, LANES), LANES)
        return pltpu.make_async_copy(aout.at[t], out_hbm.at[:, c], sem_aout)

    def o_copy(rb):
        r = pl.ds(pl.multiple_of(rb * (PPB * XR), PPB * XR), PPB * XR)
        return pltpu.make_async_copy(obuf.at[rb], out_hbm.at[r, pl.ds(D, DM)], sem_o.at[rb])

    OQ = 4

    def oq_piece(qd, pc):
        n = PPH * XR // 2
        return (qd // 2) * 2 * n + (pc % 2) * n, n, (qd % 2) * KH + (pc // 2) * (KH // 2), KH // 2

    def oq_copy(qd, pc):
        r0, nr, c0, nc = oq_piece(qd, pc)
        return pltpu.make_async_copy(
            obuf.at[NRB - 1, pl.ds(r0, nr), pl.ds(c0, nc)],
            out_hbm.at[pl.ds((NRB - 1) * PPB * XR + r0, nr), pl.ds(D + c0, nc)],
            sem_o.at[NRB - 1])

    def w_rhs(which, hp):
        out = []
        for k in range(7):
            w = w32.at[which, hp + zero_s[k]]

            def quad(i, w=w):
                return (_lo, _hi)[i % 2](w[(i // 2) * KH:(i // 2 + 1) * KH])

            out.append(_operand(_STRASSEN_RHS, k, quad).astype(BF16))
        return out

    def w_plain(which, hp0, n):
        parts = []
        for j in range(n):
            w = w32[which, hp0 + j]
            parts += [_lo(w), _hi(w)]
        return jnp.concatenate(parts, axis=1).astype(BF16)

    small[0].start()
    for hb in range(2):
        for cp in x_copies(hb):
            cp.start()
    w_copy(WV, 0).start()
    w_copy(WV, 1).start()
    for cp in small[1:]:
        cp.start()

    zero_v[...] = jnp.zeros((8, LANES), jnp.int32)
    for k in range(7):
        zero_s[k] = 0
    tsum[:, 0:8, 0:LANES] = jnp.zeros((NG, 8, LANES), F32)
    vbuf[:, 0, 0:16, 0:LANES] = jnp.zeros((NG, 16, LANES), BF16)
    for hb in range(2 * NRB):
        r0 = (hb % 2) * (HBR // 2)
        abuf[hb // 2, 0, r0:r0 + 8, 0:LANES] = jnp.zeros((8, LANES), U32)

    ri = lax.broadcasted_iota(jnp.int32, (PR, PR), 0)
    ci = lax.broadcasted_iota(jnp.int32, (PR, PR), 1)

    def seg_of(r):
        return jnp.where(r < MR, r // M, (r - MR) // SEG)

    def pos_of(r):
        return jnp.where(r < MR, r % M, M + (r - MR) % SEG)

    same = seg_of(ri) == seg_of(ci)
    allowed = same & ((ri < MR) | (pos_of(ri) >= pos_of(ci)))
    fill = jnp.where(same, -1e9, -jnp.inf).astype(F32)

    small[0].wait()
    mem0 = mem0_ref[...].astype(F32)
    m0 = jnp.concatenate([mem0, jnp.zeros_like(mem0)], axis=0)
    z0 = jnp.zeros((MR, KH), F32)
    for k, op in enumerate(_strassen_lhs(m0[:, :KH], m0[:, KH:], z0, z0)):
        a0buf[k, 0:MW, :] = _pack(op)

    def x_item(tok, never, src, dst, r, c):
        quad = [_tie(never, tok, src[h * 2 * HBR + r:h * 2 * HBR + r + 16,
                                     kk * KH + c:kk * KH + c + 2 * LANES].astype(F32))
                for h in range(2) for kk in range(2)]
        for k, op in enumerate(_strassen_lhs(*quad)):
            dst[k, r // 2:r // 2 + 8, c:c + 2 * LANES] = _pack(op)

    def x_items(never, src, dst):
        return [functools.partial(x_item, never=never, src=src, dst=dst, r=r, c=c)
                for r in range(0, HBR, 16) for c in range(0, KH, 2 * LANES)]

    def x_first(hb, cy):
        for cp in x_copies(hb):
            cp.wait()
        src = obuf.at[0, pl.ds(pl.multiple_of(hb * HBR, HBR), 3 * HBR)]
        dst = a0buf.at[:, pl.ds(pl.multiple_of(MW + hb * (HBR // 2), 8), HBR // 2)]
        for it in x_items(None, src, dst):
            it(None)
        return cy

    lax.fori_loop(0, 2, x_first, 0)

    def v_part(j, rb, rhs, vwin, twin, pre=None):
        mem0_in = (0, 2, 4, 6) if rb == 0 else ()
        m0 = {}

        def lhs(k):
            x = abuf[rb, k] if rb else (a0buf[k] if k in mem0_in else a0buf[k, MW:])
            if pre is not None and k == 4:
                x0 = jnp.concatenate([pre(x[:8, :LANES]), x[:8, LANES:]], axis=1)
                x = jnp.concatenate([x0, x[8:]], axis=0)
            return _unpack(x)

        def split(k, m):
            if k not in mem0_in:
                return m
            m0[k] = m[:M]
            return m[MR:]

        def emit(half, hh, cv):
            c = slice((2 * j + hh) * E, (2 * j + hh + 1) * E)
            vx = cv.astype(BF16)
            p0 = rb * PPB + half * PPH
            vwin[p0:p0 + PPH, :, c] = vx.reshape(PPH, XR, E)
            ts = jnp.sum(vx.astype(F32).reshape(2 * PPH, SEG, E), axis=1)
            if rb == 0 and half == 0:
                v0 = m0[2] + m0[4] if hh else m0[0] - m0[4] + m0[6]
                v0 = v0.astype(BF16).astype(F32)
                twin[NSEG:NSEG + M, c] = v0
                t0 = jnp.sum(v0, axis=0, keepdims=True)
                rows = lax.broadcasted_iota(jnp.int32, ts.shape, 0)
                ts = ts + jnp.where(rows == 0, t0, 0.0)
            twin[2 * p0:2 * (p0 + PPH), c] = ts

        return _strassen(lhs, rhs, emit, post=split)

    def v_products(t, rbs, never, extra=()):
        vwin = vbuf.at[t]
        twin = tsum.at[t]

        def pre(x):
            for v in (twin[0:8, 0:LANES], pltpu.bitcast(vwin[0, 0:16, 0:LANES], U32)) + tuple(extra):
                x = _tie(never, v, x)
            return x

        for j in range(2):
            rhs = w_rhs(WV, 2 * t + j)
            for rb in rbs:
                yield from v_part(j, rb, rhs, vwin, twin, pre if (j, rb) == (0, rbs[0]) else None)

    def head_body(j, cy):
        w_copy(WV, 2 * j).wait()
        w_copy(WV, 2 * j + 1).wait()

        @pl.when(j >= 2)
        def _():
            for cp in x_copies(j):
                cp.wait()

        @pl.when(j + 1 < NT)
        def _():
            w_copy(WV, 2 * j + 2).start()
            w_copy(WV, 2 * j + 3).start()

        @pl.when(j + 2 < 2 * NRB)
        def _():
            for cp in x_copies(j + 2):
                cp.start()

        @pl.when(j == NT - 3)
        def _():
            a_start(0, 0, (3,))

        @pl.when(j == NT - 2)
        def _():
            a_start(0, 0, (0, 1, 2))

        never = zero_v[...] > 0
        src = obuf.at[j // 2, pl.ds(pl.multiple_of((j % 2) * HBR, HBR), 3 * HBR)]
        dst = abuf.at[j // 2, :, pl.ds(pl.multiple_of((j % 2) * (HBR // 2), 8), HBR // 2)]
        toks = []
        for m in v_products(j, [0], never, [dst[0, 0:8, 0:LANES]]):
            toks += _tokens(m)
        _run_paced(x_items(never, src, dst), toks[:-40])
        return cy

    assert NT == 2 * NRB
    lax.fori_loop(0, NT, head_body, 0)

    GA = 4

    def freq_items(a0, never):
        def item(tok, m, cc, st):
            r_re = slice(16 * m, 16 * m + 8)
            r_im = slice(16 * m + 8, 16 * m + 16)
            xr = _tie(never, tok, xf[r_re, cc * BLK:(cc + 1) * BLK])
            xi = _tie(never, tok, xf[r_im, cc * BLK:(cc + 1) * BLK])
            xs = xr + xi
            for a in range(max(a0, cc), a0 + GA):
                j = a - cc
                if ('g', m, j) not in st:
                    gr = hf[r_re, j * BLK:(j + 1) * BLK]
                    gi = hf[r_im, j * BLK:(j + 1) * BLK]
                    st['g', m, j] = (gr, gi, gr + gi)
                gr, gi, gs = st['g', m, j]
                ps = (xr * gr, xi * gi, xs * gs)
                st[m, a] = ps if (m, a) not in st else tuple(u + v for u, v in zip(st[m, a], ps))
                if cc == a:
                    p1, p2, p3 = st[m, a]
                    st[m, a] = (p1 - p2, p3 - p1 - p2)
                    if m >= BLK // 16:
                        m0 = m - BLK // 16
                        (wr, wi), (vr, vi) = st[m0, a], st[m, a]
                        c = slice(a * BLK, (a + 1) * BLK)
                        wf[16 * m0:16 * m0 + 16, c] = (
                            jnp.concatenate([wr + vr, wi - vi], axis=0).astype(BF16))
                        wf[16 * m:16 * m + 16, c] = (
                            jnp.concatenate([wr - vr, wi + vi], axis=0).astype(BF16))

        items = []
        for m0 in range(BLK // 16):
            st = {}
            for m in (m0, m0 + BLK // 16):
                items += [(functools.partial(item, m=m, cc=cc, st=st),
                           4 + 6 * (a0 + GA - max(a0, cc)) + (6 if cc >= a0 else 0))
                          for cc in range(a0 + GA)]
        return items

    def tile_body(t, carry):
        sl = t & 1
        a_wait(sl)

        @pl.when(t + 1 < NT)
        def _():
            a_start(t + 1, 1 - sl)
            wo_copy(t + 1).start()

        c = pl.ds(pl.multiple_of(t * LANES, LANES), LANES)
        taps = shift_ref[:, c].astype(F32)
        dcol = d_ref[...].astype(F32)
        rows = lax.broadcasted_iota(jnp.int32, dcol.shape, 0)
        dvec = jnp.sum(jnp.where(rows == t, dcol, 0.0), axis=0, keepdims=True)
        dvb = jnp.broadcast_to(dvec, (8, LANES))
        tapb = [jnp.broadcast_to(taps[j:j + 1, :], (8, LANES)) for j in range(4)]
        never = zero_v[...] > 0
        fwd = fwd_ref[...]
        NGR = NB // GA
        GW = GA * BLK

        sub = lax.broadcasted_iota(jnp.int32, (8, LANES), 0)
        stays = [sub < 8 - j for j in range(4)]
        kprev = [jnp.zeros((8, LANES), F32)]

        def conv_item(tok, r0):
            k16 = _tie(never, tok, ain[sl, 0, r0:r0 + 16, :].astype(F32))
            halves = []
            for h in range(2):
                k8 = k16[8 * h:8 * h + 8]
                ks = k8 * tapb[0]
                for j in range(1, 4):
                    ks = ks + pltpu.roll(jnp.where(stays[j], k8, kprev[0]), j, 0) * tapb[j]
                kprev[0] = k8
                halves.append(ks)
            kvb[r0:r0 + 16, :] = (jnp.concatenate(halves, axis=0)
                                  * ain[sl, 1, r0:r0 + 16, :].astype(F32)).astype(BF16)

        hlast = [None]

        def h_fwd(g):
            hst = jnp.concatenate([ah[sl, :, b * BLK:(b + 1) * BLK]
                                   for b in range(g * GA, (g + 1) * GA)], axis=0)
            hh = lax.dot_general(fwd, hst, (((1,), (1,)), ((), ())), preferred_element_type=F32)
            for b in range(GA):
                cur = hh[:, b * BLK:(b + 1) * BLK]
                prev = hlast[0]
                c = slice((g * GA + b) * BLK, (g * GA + b + 1) * BLK)
                if prev is None:
                    hf[:, c] = cur
                else:
                    for m in range(BLK // 8):
                        re = slice(16 * m, 16 * m + 8)
                        im = slice(16 * m + 8, 16 * m + 16)
                        if m < BLK // 16:
                            hf[re, c] = cur[re] - prev[im]
                            hf[im, c] = cur[im] + prev[re]
                        else:
                            hf[re, c] = cur[re] + prev[im]
                            hf[im, c] = cur[im] - prev[re]
                hlast[0] = cur
            return hh

        def x_fwd(g):
            rhs = jnp.concatenate([kvb[b * BLK:(b + 1) * BLK, :]
                                   for b in range(g * GA, (g + 1) * GA)], axis=1)
            xx = _dot(fwd, rhs)
            xf[:, g * GW:(g + 1) * GW] = xx
            return xx

        def inverse(g):
            ys = []
            for par in range(2):
                y = _dot(inv_ref[par * (BLK // 2):(par + 1) * (BLK // 2), :],
                         wf[par * BLK:(par + 1) * BLK, g * GW:(g + 1) * GW])
                for a in range(GA):
                    yt[pl.ds((g * GA + a) * BLK + par, BLK // 2, stride=2), :] = (
                        y[:, a * BLK:(a + 1) * BLK])
                ys.append(y)
            return jnp.concatenate(ys, axis=0)

        def out_item(tok, r0):
            d8 = _tie(never, tok, dvb)
            yb = yt[r0:r0 + 16, :] + kvb[r0:r0 + 16, :].astype(F32) * jnp.concatenate([d8, d8], axis=0)
            aout[t, r0:r0 + 16, :] = (ain[sl, 2, r0:r0 + 16, :].astype(F32) * yb).astype(BF16)

        def rows16(fn, g, w):
            return [(functools.partial(fn, r0=r0), w) for r0 in range(g * GW, (g + 1) * GW, 16)]

        vgen = v_products(t, list(range(1, NRB)), never)
        nv = 2 * (NRB - 1) * 7
        work = {('conv', g): rows16(conv_item, g, 31) for g in range(NGR)}
        work.update({('freq', g): freq_items(g * GA, never) for g in range(NGR)})
        work.update({('out', g): rows16(out_item, g, 16) for g in range(NGR)})
        for kind, g, chunks in _interleave(nv, NGR, {k: [w for _, w in v] for k, v in work.items()}):
            m = next(vgen) if kind == 'v' else {'h': h_fwd, 'x': x_fwd, 'inv': inverse}[kind](g)
            _run_paced([work[k][i][0] for k, i in chunks], _tokens(m))
        _drain(vgen)
        for which in (WQ, WK):
            w_copy(which, 2 * t).start()
            w_copy(which, 2 * t + 1).start()
        aout_copy(t).start()
        return carry

    for cp in small[1:]:
        cp.wait()
    wo_copy(0).start()
    lax.fori_loop(0, NT, tile_body, 0)
    pltpu.make_async_copy(wo, wo, sem_wo).wait()

    def initial_guess():
        puni = pl.reciprocal(jnp.full((1, 1), float(L), F32), approx=True).astype(BF16).astype(F32)

        def shift_down(m):
            rows = lax.broadcasted_iota(jnp.int32, m.shape, 0)
            return jnp.where(rows == 0, 0.0, pltpu.roll(m, 1, 0))

        tall = jnp.concatenate([tsum[g, 0:NSEG, :] for g in range(NG)], axis=1)
        wov = wo[...]
        m1 = shift_down(_dot((tall * puni).astype(BF16), wov))
        v1 = _dot(m1.astype(BF16), w_plain(WV, 0, H // 2))
        u2 = (tall + float(M) * v1) * puni
        for g in range(NG):
            tsum[g, 0:NSEG, :] = u2[:, g * (G * E):(g + 1) * (G * E)]
        u2 = u2.astype(BF16)
        for c in range(0, DM, LANES):
            mcol[c // LANES] = _dot(u2, wov[:, c:c + LANES])
            for sg in range(NSEG):
                mhat[(sg + 1) * M:(sg + 2) * M, c:c + LANES] = jnp.broadcast_to(
                    mcol[c // LANES, sg:sg + 1, :], (M, LANES))
        mhat[0:M, :] = mem0_ref[...].astype(F32)
        pltpu.make_async_copy(w32.at[WQ:WK + 1], w32.at[WQ:WK + 1], sem_wqk).wait()

    def sweep(state):
        it, _ = state
        pl.when(it == 0)(initial_guess)

        def u_estimate(first, rb, g):
            n = PPB * MR
            one = tsum[g, pl.ds(pl.multiple_of(rb * (2 * PPB), 2 * PPB), 2 * PPB), :]
            one = jnp.broadcast_to(one[:, None, :], (2 * PPB, M, G * E)).reshape(n, G * E)
            return jnp.where(first, one, uhat[g, pl.ds(pl.multiple_of(rb * n, n), n), :])

        @pl.when(it > 0)
        def _():
            def upd(i, cy):
                rb, g = i // NG, i % NG
                n = PPB * MR
                r = pl.ds(pl.multiple_of(rb * n, n), n)
                r2 = pl.ds(pl.multiple_of(rb * n + M, M), n)
                c = pl.ds(pl.multiple_of(g * LANES, LANES), LANES)
                okr = okbuf[r, :]
                mhat[r2, c] = jnp.where(okr > 0.5, mhat[r2, c], mnew[r, c])
                uhat[g, r, :] = jnp.where(jnp.concatenate([okr] * G, axis=1) > 0.5,
                                          u_estimate(it == 1, rb, g), unew[g, r, :])
                return cy

            assert NG * LANES == DM
            lax.fori_loop(0, NRB * NG, upd, 0)

        def mem_rows(i):
            n = PPB * MR
            return mhat[pl.ds(pl.multiple_of((i // NG) * n, n), n), :]

        def mem_lhs(i):
            m = mem_rows(i)
            n = PPH * MR
            ops = [_pack(o) for o in _strassen_lhs(m[:n, :KH], m[:n, KH:], m[n:, :KH], m[n:, KH:])]
            t = jnp.concatenate([jnp.where(i < NG, 0.0, m[:M]), m[M:MR]], axis=0)
            b = m[n:n + MR]
            vops = [jnp.concatenate([_pack(o), full[MW:]], axis=0) for o, full in zip(
                _strassen_lhs(t[:, :KH], t[:, KH:], b[:, :KH], b[:, KH:]), ops)]
            return ops, vops

        def qk_proj(i, j, mops):
            rb = i // NG
            hp = (i % NG) * (G // 2) + j // 2

            def lhs(k):
                return _unpack(jnp.concatenate([mops[k], abuf[rb, k]], axis=0))

            n = PPH * MR
            cs = {}

            def emit(half, hh, cv):
                cs[half, hh] = cv
                if (half, 1 - hh) in cs:
                    v = jnp.concatenate([cs[half, 0], cs[half, 1]], axis=1).astype(BF16)
                    ps = slice(half * PPH, (half + 1) * PPH)
                    qks[j, ps, 0:MR, :] = v[:n].reshape(PPH, MR, 2 * E)
                    qks[j, ps, MR:PR, :] = v[n:].reshape(PPH, XR, 2 * E)

            return _strassen(lhs, w_rhs(WQ + j % 2, hp), emit)

        def vm_proj(i, j, vops):
            hp = (i % NG) * (G // 2) + j

            def emit(half, hh, cv):
                if half == 0:
                    v0 = tsum[i % NG, NSEG:NSEG + M, (2 * j + hh) * E:(2 * j + hh + 1) * E]
                    cv = jnp.concatenate([jnp.where(i < NG, v0, cv[:M]), cv[M:]], axis=0)
                vms[half * PPH:(half + 1) * PPH, :, (2 * j + hh) * E:(2 * j + hh + 1) * E] = (
                    cv.astype(BF16).reshape(PPH, MR, E))

            return _strassen(lambda k: _unpack(vops[k]), w_rhs(WV, hp), emit)

        def scores(j):
            c = slice((j % 2) * E, (j % 2 + 1) * E)
            return lax.dot_general(qks[2 * (j // 2), :, :, c], qks[2 * (j // 2) + 1, :, :, c],
                                   (((2,), (2,)), ((0,), (0,))), preferred_element_type=F32)

        def attend(i, j, s):
            p0 = pl.multiple_of((i // NG) * PPB, PPB)
            s = jnp.where(allowed[None], s * scale, fill[None])
            e = jnp.exp(s - jnp.max(s, axis=-1, keepdims=True))
            p = (e * pl.reciprocal(jnp.sum(e, axis=-1, keepdims=True), approx=True)).astype(BF16)
            vh = jnp.concatenate(
                [vms[:, :, j * E:(j + 1) * E],
                 vbuf[i % NG, pl.ds(p0, PPB), :, j * E:(j + 1) * E]], axis=1)
            return lax.dot_general(p, vh, (((2,), (1,)), ((0,), (0,))), preferred_element_type=F32)

        def residual(i, us):
            rb, g = i // NG, i % NG
            n = PPB * MR
            rm = pl.ds(pl.multiple_of(rb * n, n), n)
            new = jnp.concatenate([u[:, :MR, :] for u in us], axis=2).reshape(n, G * E)
            unew[g, rm, :] = new
            err = jnp.max(jnp.abs(new - u_estimate(it == 0, rb, g)), axis=1, keepdims=True)
            ref = jnp.max(jnp.abs(new), axis=1, keepdims=True)
            ok = jnp.broadcast_to(jnp.where(err <= TOL * ref, 1.0, 0.0), (n, LANES))
            okbuf[rm, :] = jnp.minimum(ok, jnp.where(g > 0, okbuf[rm, :], 1.0))

        def out_proj(i, us, last):
            rb = i // NG
            n = PPH * PR
            kh = G * E // 2

            def uquad(q):
                u = jnp.concatenate([us[2 * (q % 2)], us[2 * (q % 2) + 1]], axis=2)
                return u[(q // 2) * PPH:(q // 2 + 1) * PPH].reshape(n, kh)

            def lhs(k):
                return _operand(_STRASSEN_LHS, k, uquad).astype(BF16)

            wf32 = wo[pl.ds(pl.multiple_of((i % NG) * (G * E), G * E), G * E), :].astype(F32)
            wq4 = [wf32[:kh, :KH], wf32[:kh, KH:], wf32[kh:, :KH], wf32[kh:, KH:]]
            rhs = [_operand(_STRASSEN_RHS, k, wq4.__getitem__).astype(BF16) for k in range(7)]
            init = [jnp.where(i % NG > 0, acc[q], 0.0) for q in range(4)]
            mwin = mnew.at[pl.ds(pl.multiple_of(rb * (PPB * MR), PPB * MR), PPB * MR), :]

            def emit(half, hh, v):
                c = slice(hh * KH, (hh + 1) * KH)
                v3 = v.reshape(PPH, PR, KH)
                mwin[half * PPH * MR:(half + 1) * PPH * MR, c] = v3[:, :MR].reshape(PPH * MR, KH)
                vx = v3[:, MR:].reshape(PPH * XR, KH).astype(BF16)
                if last:
                    for pc in range(OQ):
                        r0, nr, c0, nc = oq_piece(2 * half + hh, pc)
                        rr, cc = r0 % (PPH * XR), c0 % KH
                        obuf[rb, r0:r0 + nr, c0:c0 + nc] = vx[rr:rr + nr, cc:cc + nc]
                        oq_copy(2 * half + hh, pc).start()
                else:
                    obuf[rb, half * PPH * XR:(half + 1) * PPH * XR, c] = vx
                    acc[2 * half + hh] = v

            if last:
                return _strassen(lhs, rhs, emit, init, order=(2, 5, 4, 1, 3, 0, 6))
            return _strassen(lhs, rhs, emit, init)

        def step(i):
            s0, s1 = scores(0), scores(1)
            mops, vops = mem_lhs(i + 1)
            _drain(qk_proj(i + 1, 0, mops))
            us = [attend(i, 0, s0), attend(i, 1, s1)]
            s2, s3 = scores(2), scores(3)
            _drain(qk_proj(i + 1, 1, mops))
            us += [attend(i, 2, s2), attend(i, 3, s3)]
            residual(i, us)
            _drain(zip(qk_proj(i + 1, 2, mops), vm_proj(i + 1, 0, vops)))
            _drain(zip(qk_proj(i + 1, 3, mops), vm_proj(i + 1, 1, vops)))
            _drain(out_proj(i, us, False))

        def last_step(i):
            ss = [scores(j) for j in range(G)]
            us = [attend(i, 0, ss[0]), attend(i, 1, ss[1])]
            gen = out_proj(i, us, True)
            next(gen)
            us += [attend(i, 2, ss[2]), attend(i, 3, ss[3])]
            residual(i, us)
            _drain(gen)

        mops0, vops0 = mem_lhs(0)
        _drain(qk_proj(0, 0, mops0), qk_proj(0, 1, mops0))
        _drain(zip(qk_proj(0, 2, mops0), vm_proj(0, 0, vops0)))
        _drain(zip(qk_proj(0, 3, mops0), vm_proj(0, 1, vops0)))

        def main_body(i, cy):
            step(i)

            @pl.when(i % NG == NG - 1)
            def _():
                o_copy(i // NG).start()

            return cy

        lax.fori_loop(0, NRB * NG - 1, main_body, 0)
        last_step(NRB * NG - 1)
        ok = jnp.min(okbuf[0:(NSEG - 1) * M, :])
        for rb in range(NRB - 1):
            o_copy(rb).wait()
        for qd in range(4):
            for pc in range(OQ):
                oq_copy(qd, pc).wait()
        return it + 1, (ok > 0.5).astype(jnp.int32)

    lax.while_loop(lambda st: jnp.logical_and(st[0] < NSEG, st[1] == 0), sweep,
                   (jnp.int32(0), jnp.int32(0)))
    for t in range(NT):
        aout_copy(t).wait()


SEG_LEN = 32


def pallas_concat_heads__ssm_conv_h3__memory_aug_recurrent_mem_tr__prompt_kernel(
    A_q, A_k, A_v, A_shift_k, A_ssm_k, A_ssm_D,
    B_x, B_mem0, B_Wq, B_Wk, B_Wv, B_Wo, B_seg_len,
):
    if isinstance(B_seg_len, int):
        assert B_seg_len == SEG_LEN
    return _run(A_q, A_k, A_v, A_shift_k, A_ssm_k, A_ssm_D, B_x, B_mem0, B_Wq, B_Wk, B_Wv, B_Wo)


@jax.jit
def _run(A_q, A_k, A_v, A_shift_k, A_ssm_k, A_ssm_D, B_x, B_mem0, B_Wq, B_Wk, B_Wv, B_Wo):
    _, S, D = A_q.shape
    DM = B_x.shape[2]
    H, E = B_Wq.shape[1], B_Wq.shape[2]
    M = B_mem0.shape[1]
    SEG = SEG_LEN
    NSEG = S // SEG
    NP = NSEG // 2
    PR = 2 * (M + SEG)
    PPB = 8
    NRB = NP // PPB
    NT = D // LANES
    assert E == LANES and H == 32 and M == 8 and A_shift_k.shape[1] == 4
    assert S == 2048 and D == 1024 and DM == 1024

    fwd, inv = _dft_mats()
    any_spec = pl.BlockSpec(memory_space=pl.ANY)
    scratch = [
        pltpu.VMEM((NRB, 7, PPB // 2 * SEG, DM // 2), U32),
        pltpu.VMEM((7, M + PPB // 2 * SEG, DM // 2), U32),
        pltpu.VMEM((H // 4, NP, 2 * SEG, 4 * E), BF16),
        pltpu.VMEM((3, H // 2, DM, E), U32),
        pltpu.VMEM((H * E, DM), BF16),
        pltpu.VMEM((4, PPB, PR, 2 * E), BF16),
        pltpu.VMEM((PPB, 2 * M, 4 * E), BF16),
        pltpu.VMEM((4, PPB // 2 * PR, DM // 2), F32),
        pltpu.VMEM((NRB, PPB * 2 * SEG, DM), BF16),
        pltpu.VMEM(((NSEG + 1) * M, DM), F32),
        pltpu.VMEM((NSEG * M, DM), F32),
        pltpu.VMEM((H // 4, NSEG * M, 4 * E), F32),
        pltpu.VMEM((H // 4, NSEG * M, 4 * E), F32),
        pltpu.VMEM((NSEG * M, LANES), F32),
        pltpu.VMEM((DM // LANES, NSEG, LANES), F32),
        pltpu.VMEM((H // 4, NSEG + M, 4 * E), F32),
        pltpu.VMEM((2, 3, S, LANES), BF16),
        pltpu.VMEM((2, LANES, S), BF16),
        pltpu.VMEM((S, LANES), BF16),
        pltpu.VMEM((NFFT, S), F32),
        pltpu.VMEM((NFFT, S), F32),
        pltpu.VMEM((NFFT, S), BF16),
        pltpu.VMEM((S + 32, LANES), F32),
        pltpu.VMEM((NT, S, LANES), BF16),
        pltpu.VMEM((M, DM), BF16),
        pltpu.VMEM((NFFT, BLK), BF16),
        pltpu.VMEM((BLK, BLK), BF16),
        pltpu.VMEM((4, D), BF16),
        pltpu.VMEM((NT, LANES), BF16),
        pltpu.VMEM((8, LANES), jnp.int32),
        pltpu.SMEM((7,), jnp.int32),
        pltpu.SemaphoreType.DMA((5,)),
        pltpu.SemaphoreType.DMA((2 * NRB,)),
        pltpu.SemaphoreType.DMA((H // 2,)),
        pltpu.SemaphoreType.DMA,
        pltpu.SemaphoreType.DMA,
        pltpu.SemaphoreType.DMA((2, 2)),
        pltpu.SemaphoreType.DMA,
        pltpu.SemaphoreType.DMA((NRB,)),
    ]
    out = pl.pallas_call(
        functools.partial(_kernel, S=S, D=D, DM=DM, H=H, M=M, SEG=SEG),
        out_shape=jax.ShapeDtypeStruct((S, D + DM), BF16),
        in_specs=[any_spec] * 14,
        out_specs=any_spec,
        scratch_shapes=scratch,
        compiler_params=pltpu.CompilerParams(vmem_limit_bytes=120 * 1024 * 1024,
                                             disable_bounds_checks=True,
                                             disable_semaphore_checks=True),
    )(
        A_q.reshape(S, D), A_k.reshape(S, D), A_v.reshape(S, D),
        A_shift_k.T, A_ssm_k, A_ssm_D.reshape(NT, LANES),
        B_x.reshape(NRB, S // NRB, DM), B_mem0.reshape(M, DM),
        B_Wq, B_Wk, B_Wv, B_Wo.reshape(H * E, DM),
        jnp.asarray(fwd, BF16), jnp.asarray(inv, BF16),
    )
    return out.reshape(1, S, D + DM)
```

```python
import functools

import numpy as np
import jax
import jax.numpy as jnp
from jax import lax
import jax.experimental.pallas as pl
import jax.experimental.pallas.tpu as pltpu

F32 = jnp.float32
BF16 = jnp.bfloat16
U32 = jnp.uint32

LANES = 128
BLK = 128
NFFT = 2 * BLK
TOL = 2.0 ** -12


def _dft_mats():
    even = np.arange(0, BLK, 2)
    theta = 2.0 * np.pi * (np.concatenate([even, BLK - 1 - even]) + 0.5) / NFFT
    n = np.arange(BLK)
    c = np.cos(theta[:, None] * n[None, :])
    s = np.sin(theta[:, None] * n[None, :])
    fwd = np.zeros((NFFT, BLK))
    for m in range(BLK // 8):
        fwd[16 * m:16 * m + 8] = c[8 * m:8 * m + 8]
        fwd[16 * m + 8:16 * m + 16] = -s[8 * m:8 * m + 8]
    inv = fwd[:BLK].T * (2.0 / NFFT)
    inv = np.concatenate([inv[0::2], inv[1::2]], axis=0)
    return fwd.astype(np.float32), inv.astype(np.float32)


def _dot(a, b):
    return jnp.dot(a, b, preferred_element_type=F32)


def _pack(x):
    return pltpu.bitcast(x.astype(BF16), U32)


def _unpack(w):
    return pltpu.bitcast(w, BF16)


def _lo(w):
    return pltpu.bitcast(w << 16, F32)


def _hi(w):
    return pltpu.bitcast(w & jnp.uint32(0xFFFF0000), F32)


_STRASSEN_LHS = ((0, 3, 1), (2, 3, 1), (0, None, 0), (3, None, 0), (0, 1, 1), (2, 0, -1), (1, 3, -1))
_STRASSEN_RHS = ((0, 3, 1), (0, None, 0), (1, 3, -1), (2, 0, -1), (3, None, 0), (0, 1, 1), (2, 3, 1))


def _operand(table, k, quad):
    i, j, sign = table[k]
    if j is None:
        return quad(i)
    return quad(i) + quad(j) if sign > 0 else quad(i) - quad(j)


def _strassen_lhs(*quads):
    return [_operand(_STRASSEN_LHS, k, quads.__getitem__) for k in range(7)]


_STRASSEN_USES = (((0, 1), (3, 1)), ((2, 1), (3, -1)), ((1, 1), (3, 1)), ((0, 1), (2, 1)),
                  ((0, -1), (1, 1)), ((3, 1),), ((0, 1),))


def _strassen(lhs, rhs, emit, init=None, order=(4, 2, 1, 3, 0, 6, 5), post=None):
    acc = [[(1, c)] if c is not None else [] for c in (init or (None,) * 4)]
    left = [4, 2, 2, 4]
    for k in order:
        m = _dot(lhs(k), rhs[k])
        if post is not None:
            m = post(k, m)
        for q, sign in _STRASSEN_USES[k]:
            acc[q].append((sign, m))
            left[q] -= 1
            if left[q] < (3, 1, 1, 3)[q]:
                terms = sorted(acc[q], key=lambda t: -t[0])
                v = terms[0][1]
                assert terms[0][0] > 0
                for sg, t in terms[1:]:
                    v = v + t if sg > 0 else v - t
                acc[q] = [(1, v)]
            if left[q] == 0:
                emit(q // 2, q % 2, acc[q][0][1])
        yield m


def _drain(*gens):
    for g in gens:
        for _ in g:
            pass


def _tokens(m):
    return [(m, r, c) for r in range(0, m.shape[0], 8) for c in range(0, m.shape[1], LANES)]


def _tie(never, tok, x):
    if tok is None:
        return x
    if tok.dtype != x.dtype:
        tok = pltpu.bitcast(tok, x.dtype)
    if x.shape == (8, LANES):
        return jnp.where(never, tok, x)
    return jnp.concatenate(
        [jnp.concatenate([jnp.where(never, tok, x[r:r + 8, c:c + LANES])
                          for c in range(0, x.shape[1], LANES)], axis=1)
         for r in range(0, x.shape[0], 8)], axis=0)


def _run_paced(items, toks):
    for i, it in enumerate(items):
        m, r, c = toks[i * len(toks) // len(items)]
        it(m[r:r + 8, c:c + LANES])


def _interleave(nv, ngr, weights):
    dur = {'v': 256, 'h': 256, 'x': 256, 'inv': 128}
    margin = 768

    def plan(rate):
        t, v, out = 0, 0, []
        nxt = {'h': 0, 'x': 0, 'inv': 0}
        pos = {k: 0 for k in weights}
        done = {}
        credit = 0.0
        while True:
            kind = None
            if nxt['inv'] < ngr and done.get(('freq', nxt['inv']), 1e9) + margin <= t:
                kind = 'inv'
            elif nxt['x'] < ngr and done.get(('conv', nxt['x']), 1e9) + margin <= t:
                kind = 'x'
            elif nxt['h'] < ngr and nxt['h'] <= nxt['x'] and out and out[-1][0] == 'v':
                kind = 'h'
            elif v < nv:
                kind = 'v'
            if kind is None:
                break
            g = v if kind == 'v' else nxt[kind]
            busy = 0.6
            if kind == 'v':
                busy = 1.1 * (v % (nv // 2) < 7) + 0.55 * (v % 7 in (1, 3, 5, 6))
            credit += (rate - busy) * dur[kind]
            chunk = []
            while credit > 0:
                ready = [('out', i) for i in range(nxt['inv'])]
                ready += [('conv', i) for i in range(ngr)]
                ready += [('freq', i) for i in range(min(nxt['x'], nxt['h']))]
                ready = [k for k in ready if pos[k] < len(weights[k])]
                if not ready:
                    credit = 0.0
                    break
                k = ready[0]
                chunk.append((k, pos[k]))
                credit -= weights[k][pos[k]]
                pos[k] += 1
                if pos[k] == len(weights[k]):
                    done[k] = t + dur[kind]
            out.append((kind, g, chunk))
            t += dur[kind]
            if kind == 'v':
                v += 1
            else:
                nxt[kind] += 1
        ok = all(pos[k] == len(weights[k]) for k in weights)
        return ok, out

    rate = 1.0
    while True:
        ok, out = plan(rate)
        if ok:
            return out
        rate += 0.02


def _kernel(q_hbm, k_hbm, v_hbm, shift_hbm, h_hbm, d_hbm, x_hbm, mem0_hbm,
            wq_hbm, wk_hbm, wv_hbm, wo_hbm, fwd_hbm, inv_hbm,
            out_hbm,
            abuf, a0buf, vbuf, w32, wo, qks, vms, acc, obuf, mhat, mnew, uhat, unew, okbuf, mcol, tsum,
            ain, ah, kvb, xf, hf, wf, yt, aout,
            mem0_ref, fwd_ref, inv_ref, shift_ref, d_ref, zero_v, zero_s,
            sem_s, sem_x, sem_wv, sem_wqk, sem_wo, sem_a, sem_aout, sem_o,
            *, S, D, DM, H, M, SEG):
    E = LANES
    NSEG = S // SEG
    NP = NSEG // 2
    MR = 2 * M
    XR = 2 * SEG
    PR = MR + XR
    MW = MR // 2
    L = M + SEG
    NB = S // BLK
    NT = D // LANES
    PPB = 8
    PPH = PPB // 2
    NRB = NP // PPB
    G = 4
    NG = H // G
    KH = DM // 2
    scale = float(E) ** -0.5
    WV, WQ, WK = 0, 1, 2

    small = [pltpu.make_async_copy(src, dst, sem_s.at[i]) for i, (src, dst) in enumerate(
        ((mem0_hbm, mem0_ref), (shift_hbm, shift_ref), (d_hbm, d_ref),
         (fwd_hbm, fwd_ref), (inv_hbm, inv_ref)))]
    HBR = PPH * XR // 2

    def x_copies(hb):
        out = []
        for half in range(2):
            r = pl.ds(pl.multiple_of((2 * half + hb % 2) * HBR, HBR), HBR)
            out.append(pltpu.make_async_copy(x_hbm.at[hb // 2, r], obuf.at[hb // 2, r],
                                             sem_x.at[hb]))
        return out

    def w_copy(which, hp):
        src = (wv_hbm, wq_hbm, wk_hbm)[which].bitcast(U32)
        sem = sem_wv.at[hp] if which == WV else sem_wqk
        return pltpu.make_async_copy(src.at[:, hp, :], w32.at[which, hp], sem)

    def wo_copy(t):
        n = H * E // NT
        r = pl.ds(pl.multiple_of(t * n, n), n)
        return pltpu.make_async_copy(wo_hbm.at[r, :], wo.at[r, :], sem_wo)

    def a_start(t, sl, which=(0, 1, 2, 3)):
        c = pl.ds(pl.multiple_of(t * LANES, LANES), LANES)
        for i in which:
            if i == 3:
                pltpu.make_async_copy(h_hbm.at[c, :], ah.at[sl], sem_a.at[sl, 1]).start()
            else:
                src = (k_hbm, v_hbm, q_hbm)[i]
                pltpu.make_async_copy(src.at[:, c], ain.at[sl, i], sem_a.at[sl, 0]).start()

    def a_wait(sl):
        pltpu.make_async_copy(ain.at[sl], ain.at[sl], sem_a.at[sl, 0]).wait()
        pltpu.make_async_copy(ah.at[sl], ah.at[sl], sem_a.at[sl, 1]).wait()

    def aout_copy(t):
        c = pl.ds(pl.multiple_of(t * LANES, LANES), LANES)
        return pltpu.make_async_copy(aout.at[t], out_hbm.at[:, c], sem_aout)

    def o_copy(rb):
        r = pl.ds(pl.multiple_of(rb * (PPB * XR), PPB * XR), PPB * XR)
        return pltpu.make_async_copy(obuf.at[rb], out_hbm.at[r, pl.ds(D, DM)], sem_o.at[rb])

    OQ = 4

    def oq_piece(qd, pc):
        n = PPH * XR // 2
        return (qd // 2) * 2 * n + (pc % 2) * n, n, (qd % 2) * KH + (pc // 2) * (KH // 2), KH // 2

    def oq_copy(qd, pc):
        r0, nr, c0, nc = oq_piece(qd, pc)
        return pltpu.make_async_copy(
            obuf.at[NRB - 1, pl.ds(r0, nr), pl.ds(c0, nc)],
            out_hbm.at[pl.ds((NRB - 1) * PPB * XR + r0, nr), pl.ds(D + c0, nc)],
            sem_o.at[NRB - 1])

    def w_rhs(which, hp):
        out = []
        for k in range(7):
            w = w32.at[which, hp + zero_s[k]]

            def quad(i, w=w):
                return (_lo, _hi)[i % 2](w[(i // 2) * KH:(i // 2 + 1) * KH])

            out.append(_operand(_STRASSEN_RHS, k, quad).astype(BF16))
        return out

    def w_plain(which, hp0, n):
        parts = []
        for j in range(n):
            w = w32[which, hp0 + j]
            parts += [_lo(w), _hi(w)]
        return jnp.concatenate(parts, axis=1).astype(BF16)

    small[0].start()
    for hb in range(2):
        for cp in x_copies(hb):
            cp.start()
    w_copy(WV, 0).start()
    w_copy(WV, 1).start()
    for cp in small[1:]:
        cp.start()

    zero_v[...] = jnp.zeros((8, LANES), jnp.int32)
    for k in range(7):
        zero_s[k] = 0
    tsum[:, 0:8, 0:LANES] = jnp.zeros((NG, 8, LANES), F32)
    vbuf[:, 0, 0:16, 0:LANES] = jnp.zeros((NG, 16, LANES), BF16)
    for hb in range(2 * NRB):
        r0 = (hb % 2) * (HBR // 2)
        abuf[hb // 2, 0, r0:r0 + 8, 0:LANES] = jnp.zeros((8, LANES), U32)

    ri = lax.broadcasted_iota(jnp.int32, (PR, PR), 0)
    ci = lax.broadcasted_iota(jnp.int32, (PR, PR), 1)

    def seg_of(r):
        return jnp.where(r < MR, (r // (M // 2)) % 2, (r - MR) // SEG)

    def pos_of(r):
        return jnp.where(r < MR, r % M, M + (r - MR) % SEG)

    same = seg_of(ri) == seg_of(ci)
    allowed = same & ((ri < MR) | (pos_of(ri) >= pos_of(ci)))
    fill = jnp.where(same, -1e9, -jnp.inf).astype(F32)

    first4 = lax.broadcasted_iota(jnp.int32, (M, 1), 0) < M // 2

    def roll4(x):
        return pltpu.roll(x, M // 2, 0)

    mnew[0] = jnp.zeros((MR, DM), F32)
    okbuf[0] = jnp.ones((MR, LANES), F32)
    small[0].wait()
    mem0 = mem0_ref[...].astype(F32)
    m0 = jnp.concatenate([mem0, jnp.zeros_like(mem0)], axis=0)
    z0 = jnp.zeros((MR, KH), F32)
    for k, op in enumerate(_strassen_lhs(m0[:, :KH], m0[:, KH:], z0, z0)):
        a0buf[k, 0:MW, :] = _pack(op)

    def x_item(tok, never, src, dst, r, c):
        quad = [_tie(never, tok, src[h * 2 * HBR + r:h * 2 * HBR + r + 16,
                                     kk * KH + c:kk * KH + c + 2 * LANES].astype(F32))
                for h in range(2) for kk in range(2)]
        for k, op in enumerate(_strassen_lhs(*quad)):
            dst[k, r // 2:r // 2 + 8, c:c + 2 * LANES] = _pack(op)

    def x_items(never, src, dst):
        return [functools.partial(x_item, never=never, src=src, dst=dst, r=r, c=c)
                for r in range(0, HBR, 16) for c in range(0, KH, 2 * LANES)]

    def x_first(hb, cy):
        for cp in x_copies(hb):
            cp.wait()
        src = obuf.at[0, pl.ds(pl.multiple_of(hb * HBR, HBR), 3 * HBR)]
        dst = a0buf.at[:, pl.ds(pl.multiple_of(MW + hb * (HBR // 2), 8), HBR // 2)]
        for it in x_items(None, src, dst):
            it(None)
        return cy

    lax.fori_loop(0, 2, x_first, 0)

    def v_part(j, rb, rhs, vwin, twin, pre=None):
        mem0_in = (0, 2, 4, 6) if rb == 0 else ()
        m0 = {}

        def lhs(k):
            x = abuf[rb, k] if rb else (a0buf[k] if k in mem0_in else a0buf[k, MW:])
            if pre is not None and k == 4:
                x0 = jnp.concatenate([pre(x[:8, :LANES]), x[:8, LANES:]], axis=1)
                x = jnp.concatenate([x0, x[8:]], axis=0)
            return _unpack(x)

        def split(k, m):
            if k not in mem0_in:
                return m
            m0[k] = m[:M]
            return m[MR:]

        def emit(half, hh, cv):
            c = slice((2 * j + hh) * E, (2 * j + hh + 1) * E)
            vx = cv.astype(BF16)
            p0 = rb * PPB + half * PPH
            vwin[p0:p0 + PPH, :, c] = vx.reshape(PPH, XR, E)
            ts = jnp.sum(vx.astype(F32).reshape(2 * PPH, SEG, E), axis=1)
            if rb == 0 and half == 0:
                v0 = m0[2] + m0[4] if hh else m0[0] - m0[4] + m0[6]
                v0 = v0.astype(BF16).astype(F32)
                twin[NSEG:NSEG + M, c] = v0
                t0 = jnp.sum(v0, axis=0, keepdims=True)
                rows = lax.broadcasted_iota(jnp.int32, ts.shape, 0)
                ts = ts + jnp.where(rows == 0, t0, 0.0)
            twin[2 * p0:2 * (p0 + PPH), c] = ts

        return _strassen(lhs, rhs, emit, post=split)

    def v_products(t, rbs, never, extra=()):
        vwin = vbuf.at[t]
        twin = tsum.at[t]

        def pre(x):
            for v in (twin[0:8, 0:LANES], pltpu.bitcast(vwin[0, 0:16, 0:LANES], U32)) + tuple(extra):
                x = _tie(never, v, x)
            return x

        for j in range(2):
            rhs = w_rhs(WV, 2 * t + j)
            for rb in rbs:
                yield from v_part(j, rb, rhs, vwin, twin, pre if (j, rb) == (0, rbs[0]) else None)

    def head_body(j, cy):
        w_copy(WV, 2 * j).wait()
        w_copy(WV, 2 * j + 1).wait()

        @pl.when(j >= 2)
        def _():
            for cp in x_copies(j):
                cp.wait()

        @pl.when(j + 1 < NT)
        def _():
            w_copy(WV, 2 * j + 2).start()
            w_copy(WV, 2 * j + 3).start()

        @pl.when(j + 2 < 2 * NRB)
        def _():
            for cp in x_copies(j + 2):
                cp.start()

        @pl.when(j == NT - 3)
        def _():
            a_start(0, 0, (3,))

        @pl.when(j == NT - 2)
        def _():
            a_start(0, 0, (0, 1, 2))

        never = zero_v[...] > 0
        src = obuf.at[j // 2, pl.ds(pl.multiple_of((j % 2) * HBR, HBR), 3 * HBR)]
        dst = abuf.at[j // 2, :, pl.ds(pl.multiple_of((j % 2) * (HBR // 2), 8), HBR // 2)]
        toks = []
        for m in v_products(j, [0], never, [dst[0, 0:8, 0:LANES]]):
            toks += _tokens(m)
        _run_paced(x_items(never, src, dst), toks[:-40])
        return cy

    assert NT == 2 * NRB
    lax.fori_loop(0, NT, head_body, 0)

    GA = 4

    def freq_items(a0, never):
        def item(tok, m, cc, st):
            r_re = slice(16 * m, 16 * m + 8)
            r_im = slice(16 * m + 8, 16 * m + 16)
            xr = _tie(never, tok, xf[r_re, cc * BLK:(cc + 1) * BLK])
            xi = _tie(never, tok, xf[r_im, cc * BLK:(cc + 1) * BLK])
            xs = xr + xi
            for a in range(max(a0, cc), a0 + GA):
                j = a - cc
                if ('g', m, j) not in st:
                    gr = hf[r_re, j * BLK:(j + 1) * BLK]
                    gi = hf[r_im, j * BLK:(j + 1) * BLK]
                    st['g', m, j] = (gr, gi, gr + gi)
                gr, gi, gs = st['g', m, j]
                ps = (xr * gr, xi * gi, xs * gs)
                st[m, a] = ps if (m, a) not in st else tuple(u + v for u, v in zip(st[m, a], ps))
                if cc == a:
                    p1, p2, p3 = st[m, a]
                    st[m, a] = (p1 - p2, p3 - p1 - p2)
                    if m >= BLK // 16:
                        m0 = m - BLK // 16
                        (wr, wi), (vr, vi) = st[m0, a], st[m, a]
                        c = slice(a * BLK, (a + 1) * BLK)
                        wf[16 * m0:16 * m0 + 16, c] = (
                            jnp.concatenate([wr + vr, wi - vi], axis=0).astype(BF16))
                        wf[16 * m:16 * m + 16, c] = (
                            jnp.concatenate([wr - vr, wi + vi], axis=0).astype(BF16))

        items = []
        for m0 in range(BLK // 16):
            st = {}
            for m in (m0, m0 + BLK // 16):
                items += [(functools.partial(item, m=m, cc=cc, st=st),
                           4 + 6 * (a0 + GA - max(a0, cc)) + (6 if cc >= a0 else 0))
                          for cc in range(a0 + GA)]
        return items

    def tile_body(t, carry):
        sl = t & 1
        a_wait(sl)

        @pl.when(t + 1 < NT)
        def _():
            a_start(t + 1, 1 - sl)
            wo_copy(t + 1).start()

        c = pl.ds(pl.multiple_of(t * LANES, LANES), LANES)
        taps = shift_ref[:, c].astype(F32)
        dcol = d_ref[...].astype(F32)
        rows = lax.broadcasted_iota(jnp.int32, dcol.shape, 0)
        dvec = jnp.sum(jnp.where(rows == t, dcol, 0.0), axis=0, keepdims=True)
        dvb = jnp.broadcast_to(dvec, (8, LANES))
        tapb = [jnp.broadcast_to(taps[j:j + 1, :], (8, LANES)) for j in range(4)]
        never = zero_v[...] > 0
        fwd = fwd_ref[...]
        NGR = NB // GA
        GW = GA * BLK

        sub = lax.broadcasted_iota(jnp.int32, (8, LANES), 0)
        stays = [sub < 8 - j for j in range(4)]
        kprev = [jnp.zeros((8, LANES), F32)]

        def conv_item(tok, r0):
            k16 = _tie(never, tok, ain[sl, 0, r0:r0 + 16, :].astype(F32))
            halves = []
            for h in range(2):
                k8 = k16[8 * h:8 * h + 8]
                ks = k8 * tapb[0]
                for j in range(1, 4):
                    ks = ks + pltpu.roll(jnp.where(stays[j], k8, kprev[0]), j, 0) * tapb[j]
                kprev[0] = k8
                halves.append(ks)
            kvb[r0:r0 + 16, :] = (jnp.concatenate(halves, axis=0)
                                  * ain[sl, 1, r0:r0 + 16, :].astype(F32)).astype(BF16)

        hlast = [None]

        def h_fwd(g):
            hst = jnp.concatenate([ah[sl, :, b * BLK:(b + 1) * BLK]
                                   for b in range(g * GA, (g + 1) * GA)], axis=0)
            hh = lax.dot_general(fwd, hst, (((1,), (1,)), ((), ())), preferred_element_type=F32)
            for b in range(GA):
                cur = hh[:, b * BLK:(b + 1) * BLK]
                prev = hlast[0]
                c = slice((g * GA + b) * BLK, (g * GA + b + 1) * BLK)
                if prev is None:
                    hf[:, c] = cur
                else:
                    for m in range(BLK // 8):
                        re = slice(16 * m, 16 * m + 8)
                        im = slice(16 * m + 8, 16 * m + 16)
                        if m < BLK // 16:
                            hf[re, c] = cur[re] - prev[im]
                            hf[im, c] = cur[im] + prev[re]
                        else:
                            hf[re, c] = cur[re] + prev[im]
                            hf[im, c] = cur[im] - prev[re]
                hlast[0] = cur
            return hh

        def x_fwd(g):
            rhs = jnp.concatenate([kvb[b * BLK:(b + 1) * BLK, :]
                                   for b in range(g * GA, (g + 1) * GA)], axis=1)
            xx = _dot(fwd, rhs)
            xf[:, g * GW:(g + 1) * GW] = xx
            return xx

        def inverse(g):
            ys = []
            for par in range(2):
                y = _dot(inv_ref[par * (BLK // 2):(par + 1) * (BLK // 2), :],
                         wf[par * BLK:(par + 1) * BLK, g * GW:(g + 1) * GW])
                for a in range(GA):
                    yt[pl.ds((g * GA + a) * BLK + par, BLK // 2, stride=2), :] = (
                        y[:, a * BLK:(a + 1) * BLK])
                ys.append(y)
            return jnp.concatenate(ys, axis=0)

        def out_item(tok, r0):
            d8 = _tie(never, tok, dvb)
            yb = yt[r0:r0 + 16, :] + kvb[r0:r0 + 16, :].astype(F32) * jnp.concatenate([d8, d8], axis=0)
            aout[t, r0:r0 + 16, :] = (ain[sl, 2, r0:r0 + 16, :].astype(F32) * yb).astype(BF16)

        def rows16(fn, g, w):
            return [(functools.partial(fn, r0=r0), w) for r0 in range(g * GW, (g + 1) * GW, 16)]

        vgen = v_products(t, list(range(1, NRB)), never)
        nv = 2 * (NRB - 1) * 7
        work = {('conv', g): rows16(conv_item, g, 31) for g in range(NGR)}
        work.update({('freq', g): freq_items(g * GA, never) for g in range(NGR)})
        work.update({('out', g): rows16(out_item, g, 16) for g in range(NGR)})
        for kind, g, chunks in _interleave(nv, NGR, {k: [w for _, w in v] for k, v in work.items()}):
            m = next(vgen) if kind == 'v' else {'h': h_fwd, 'x': x_fwd, 'inv': inverse}[kind](g)
            _run_paced([work[k][i][0] for k, i in chunks], _tokens(m))
        _drain(vgen)
        for which in (WQ, WK):
            w_copy(which, 2 * t).start()
            w_copy(which, 2 * t + 1).start()
        aout_copy(t).start()
        return carry

    for cp in small[1:]:
        cp.wait()
    wo_copy(0).start()
    lax.fori_loop(0, NT, tile_body, 0)
    pltpu.make_async_copy(wo, wo, sem_wo).wait()

    def initial_guess():
        puni = pl.reciprocal(jnp.full((1, 1), float(L), F32), approx=True).astype(BF16).astype(F32)

        def shift_down(m):
            rows = lax.broadcasted_iota(jnp.int32, m.shape, 0)
            return jnp.where(rows == 0, 0.0, pltpu.roll(m, 1, 0))

        tall = jnp.concatenate([tsum[g, 0:NSEG, :] for g in range(NG)], axis=1)
        wov = wo[...]
        m1 = shift_down(_dot((tall * puni).astype(BF16), wov))
        v1 = _dot(m1.astype(BF16), w_plain(WV, 0, H // 2))
        u2 = (tall + float(M) * v1) * puni
        for g in range(NG):
            tsum[g, 0:NSEG, :] = u2[:, g * (G * E):(g + 1) * (G * E)]
        u2 = u2.astype(BF16)
        mem0 = mem0_ref[...].astype(F32)
        for c in range(0, DM, LANES):
            mcol[c // LANES] = _dot(u2, wov[:, c:c + LANES])

            def row(sg):
                return jnp.broadcast_to(mcol[c // LANES, sg:sg + 1, :], (M, LANES))

            m0 = mem0[:, c:c + LANES]
            mhat[0, 0:M, c:c + LANES] = jnp.where(first4, m0, row(0))
            mhat[0, M:MR, c:c + LANES] = jnp.where(first4, roll4(m0), row(0))
            for pp in range(1, NP):
                v = jnp.where(first4, row(2 * pp - 1), row(2 * pp))
                mhat[pp, :, c:c + LANES] = jnp.concatenate([v, v], axis=0)
        pltpu.make_async_copy(w32.at[WQ:WK + 1], w32.at[WQ:WK + 1], sem_wqk).wait()

    def sweep(state):
        it, _ = state
        pl.when(it == 0)(initial_guess)

        def pairs(rb, off=0):
            return pl.ds(rb * PPB + off, PPB)

        def u_estimate(first, rb, g):
            one = tsum[g, pl.ds(pl.multiple_of(rb * (2 * PPB), 2 * PPB), 2 * PPB), :]
            rows = []
            for pp in range(PPB):
                v = jnp.where(first4, one[2 * pp:2 * pp + 1], one[2 * pp + 1:2 * pp + 2])
                rows += [v, v]
            one = jnp.concatenate(rows, axis=0).reshape(PPB, MR, G * E)
            return jnp.where(first, one, uhat[g, pairs(rb)])

        @pl.when(it > 0)
        def _():
            def upd(i, cy):
                rb, g = i // NG, i % NG
                c = pl.ds(pl.multiple_of(g * LANES, LANES), LANES)

                def to_next(prev, cur):
                    prev = prev.reshape(PPB * MR, LANES)
                    cur = cur.reshape(PPB * MR, LANES)
                    out = [roll4(jnp.where(first4, cur[r:r + M], prev[r:r + M]))
                           for r in range(0, PPB * MR, M)]
                    return jnp.concatenate(out, axis=0).reshape(PPB, MR, LANES)

                okr = okbuf[pairs(rb, 1)]
                mhat[pairs(rb), :, c] = jnp.where(
                    to_next(okbuf[pairs(rb)], okr) > 0.5, mhat[pairs(rb), :, c],
                    to_next(mnew[pairs(rb), :, c], mnew[pairs(rb, 1), :, c]))
                uhat[g, pairs(rb)] = jnp.where(jnp.concatenate([okr] * G, axis=2) > 0.5,
                                               u_estimate(it == 1, rb, g), unew[g, pairs(rb)])
                return cy

            assert NG * LANES == DM
            lax.fori_loop(0, NRB * NG, upd, 0)

        def mem_lhs(i):
            m = mhat[pairs(i // NG)]
            top = m[:, :M].reshape(PPB * M, DM)
            bot = m[:, M:].reshape(PPB * M, DM)
            return [_pack(o) for o in
                    _strassen_lhs(top[:, :KH], top[:, KH:], bot[:, :KH], bot[:, KH:])]

        def qk_proj(i, j, mops):
            rb = i // NG
            hp = (i % NG) * (G // 2) + j // 2

            def lhs(k):
                return _unpack(jnp.concatenate([mops[k], abuf[rb, k]], axis=0))

            n = PPB * M
            cs = {}

            def emit(half, hh, cv):
                cs[half, hh] = cv
                if (half, 1 - hh) in cs:
                    v = jnp.concatenate([cs[half, 0], cs[half, 1]], axis=1)
                    qks[j, :, half * M:(half + 1) * M, :] = (
                        v[:n].reshape(PPB, M, 2 * E).astype(BF16))
                    qks[j, half * PPH:(half + 1) * PPH, MR:PR, :] = (
                        v[n:].astype(BF16).reshape(PPH, XR, 2 * E))

            return _strassen(lhs, w_rhs(WQ + j % 2, hp), emit)

        def vm_proj(i, j, mops):
            hp = (i % NG) * (G // 2) + j

            def emit(half, hh, cv):
                c = slice((2 * j + hh) * E, (2 * j + hh + 1) * E)
                v0 = tsum[i % NG, NSEG:NSEG + M, c]
                v0 = jnp.where(first4, roll4(v0) if half else v0, cv[:M])
                cv = jnp.concatenate([jnp.where(i < NG, v0, cv[:M]), cv[M:]], axis=0)
                vms[:, half * M:(half + 1) * M, c] = cv.reshape(PPB, M, E).astype(BF16)

            return _strassen(lambda k: _unpack(mops[k]), w_rhs(WV, hp), emit)

        def scores(j):
            c = slice((j % 2) * E, (j % 2 + 1) * E)
            return lax.dot_general(qks[2 * (j // 2), :, :, c], qks[2 * (j // 2) + 1, :, :, c],
                                   (((2,), (2,)), ((0,), (0,))), preferred_element_type=F32)

        def attend(i, j, s):
            p0 = pl.multiple_of((i // NG) * PPB, PPB)
            s = jnp.where(allowed[None], s * scale, fill[None])
            e = jnp.exp(s - jnp.max(s, axis=-1, keepdims=True))
            p = (e * pl.reciprocal(jnp.sum(e, axis=-1, keepdims=True), approx=True)).astype(BF16)
            vh = jnp.concatenate(
                [vms[:, :, j * E:(j + 1) * E],
                 vbuf[i % NG, pl.ds(p0, PPB), :, j * E:(j + 1) * E]], axis=1)
            return lax.dot_general(p, vh, (((2,), (1,)), ((0,), (0,))), preferred_element_type=F32)

        def residual(i, us):
            rb, g = i // NG, i % NG
            new = jnp.concatenate([u[:, :MR, :] for u in us], axis=2)
            unew[g, pairs(rb)] = new
            err = jnp.max(jnp.abs(new - u_estimate(it == 0, rb, g)), axis=2, keepdims=True)
            ref = jnp.max(jnp.abs(new), axis=2, keepdims=True)
            ok = jnp.broadcast_to(jnp.where(err <= TOL * ref, 1.0, 0.0), (PPB, MR, LANES))
            okbuf[pairs(rb, 1)] = jnp.minimum(ok, jnp.where(g > 0, okbuf[pairs(rb, 1)], 1.0))

        def out_proj(i, us, last):
            rb = i // NG
            n = PPB * M
            kh = G * E // 2

            def uquad(q):
                half = q // 2
                u = jnp.concatenate([us[2 * (q % 2)], us[2 * (q % 2) + 1]], axis=2)
                return jnp.concatenate(
                    [u[:, half * M:(half + 1) * M].reshape(n, kh),
                     u[half * PPH:(half + 1) * PPH, MR:].reshape(PPH * XR, kh)], axis=0)

            def lhs(k):
                return _operand(_STRASSEN_LHS, k, uquad).astype(BF16)

            wf32 = wo[pl.ds(pl.multiple_of((i % NG) * (G * E), G * E), G * E), :].astype(F32)
            wq4 = [wf32[:kh, :KH], wf32[:kh, KH:], wf32[kh:, :KH], wf32[kh:, KH:]]
            rhs = [_operand(_STRASSEN_RHS, k, wq4.__getitem__).astype(BF16) for k in range(7)]
            init = [jnp.where(i % NG > 0, acc[q], 0.0) for q in range(4)]

            def emit(half, hh, v):
                c = slice(hh * KH, (hh + 1) * KH)
                mnew[pairs(rb, 1), half * M:(half + 1) * M, c] = v[:n].reshape(PPB, M, KH)
                vx = v[n:].astype(BF16)
                if last:
                    for pc in range(OQ):
                        r0, nr, c0, nc = oq_piece(2 * half + hh, pc)
                        rr, cc = r0 % (PPH * XR), c0 % KH
                        obuf[rb, r0:r0 + nr, c0:c0 + nc] = vx[rr:rr + nr, cc:cc + nc]
                        oq_copy(2 * half + hh, pc).start()
                else:
                    obuf[rb, half * PPH * XR:(half + 1) * PPH * XR, c] = vx
                    acc[2 * half + hh] = v

            if last:
                return _strassen(lhs, rhs, emit, init, order=(2, 5, 4, 1, 3, 0, 6))
            return _strassen(lhs, rhs, emit, init)

        def step(i):
            s0, s1 = scores(0), scores(1)
            mops = mem_lhs(i + 1)
            _drain(qk_proj(i + 1, 0, mops))
            us = [attend(i, 0, s0), attend(i, 1, s1)]
            s2, s3 = scores(2), scores(3)
            _drain(qk_proj(i + 1, 1, mops))
            us += [attend(i, 2, s2), attend(i, 3, s3)]
            residual(i, us)
            _drain(zip(qk_proj(i + 1, 2, mops), vm_proj(i + 1, 0, mops)))
            _drain(zip(qk_proj(i + 1, 3, mops), vm_proj(i + 1, 1, mops)))
            _drain(out_proj(i, us, False))

        def last_step(i):
            ss = [scores(j) for j in range(G)]
            us = [attend(i, 0, ss[0]), attend(i, 1, ss[1])]
            gen = out_proj(i, us, True)
            next(gen)
            us += [attend(i, 2, ss[2]), attend(i, 3, ss[3])]
            residual(i, us)
            _drain(gen)

        mops0 = mem_lhs(0)
        _drain(qk_proj(0, 0, mops0), qk_proj(0, 1, mops0))
        _drain(zip(qk_proj(0, 2, mops0), vm_proj(0, 0, mops0)))
        _drain(zip(qk_proj(0, 3, mops0), vm_proj(0, 1, mops0)))

        def main_body(i, cy):
            step(i)

            @pl.when(i % NG == NG - 1)
            def _():
                o_copy(i // NG).start()

            return cy

        lax.fori_loop(0, NRB * NG - 1, main_body, 0)
        last_step(NRB * NG - 1)
        tail = okbuf[NP]
        ok = jnp.minimum(jnp.min(okbuf[1:NP], axis=0),
                         jnp.where(jnp.concatenate([first4, first4], axis=0), tail, 1.0))
        ok = jnp.min(ok)
        for rb in range(NRB - 1):
            o_copy(rb).wait()
        for qd in range(4):
            for pc in range(OQ):
                oq_copy(qd, pc).wait()
        return it + 1, (ok > 0.5).astype(jnp.int32)

    lax.while_loop(lambda st: jnp.logical_and(st[0] < NSEG, st[1] == 0), sweep,
                   (jnp.int32(0), jnp.int32(0)))
    for t in range(NT):
        aout_copy(t).wait()


SEG_LEN = 32


def pallas_concat_heads__ssm_conv_h3__memory_aug_recurrent_mem_tr__prompt_kernel(
    A_q, A_k, A_v, A_shift_k, A_ssm_k, A_ssm_D,
    B_x, B_mem0, B_Wq, B_Wk, B_Wv, B_Wo, B_seg_len,
):
    if isinstance(B_seg_len, int):
        assert B_seg_len == SEG_LEN
    return _run(A_q, A_k, A_v, A_shift_k, A_ssm_k, A_ssm_D, B_x, B_mem0, B_Wq, B_Wk, B_Wv, B_Wo)


@jax.jit
def _run(A_q, A_k, A_v, A_shift_k, A_ssm_k, A_ssm_D, B_x, B_mem0, B_Wq, B_Wk, B_Wv, B_Wo):
    _, S, D = A_q.shape
    DM = B_x.shape[2]
    H, E = B_Wq.shape[1], B_Wq.shape[2]
    M = B_mem0.shape[1]
    SEG = SEG_LEN
    NSEG = S // SEG
    NP = NSEG // 2
    PR = 2 * (M + SEG)
    PPB = 8
    NRB = NP // PPB
    NT = D // LANES
    assert E == LANES and H == 32 and M == 8 and A_shift_k.shape[1] == 4
    assert S == 2048 and D == 1024 and DM == 1024

    fwd, inv = _dft_mats()
    any_spec = pl.BlockSpec(memory_space=pl.ANY)
    scratch = [
        pltpu.VMEM((NRB, 7, PPB // 2 * SEG, DM // 2), U32),
        pltpu.VMEM((7, M + PPB // 2 * SEG, DM // 2), U32),
        pltpu.VMEM((H // 4, NP, 2 * SEG, 4 * E), BF16),
        pltpu.VMEM((3, H // 2, DM, E), U32),
        pltpu.VMEM((H * E, DM), BF16),
        pltpu.VMEM((4, PPB, PR, 2 * E), BF16),
        pltpu.VMEM((PPB, 2 * M, 4 * E), BF16),
        pltpu.VMEM((4, PPB // 2 * PR, DM // 2), F32),
        pltpu.VMEM((NRB, PPB * 2 * SEG, DM), BF16),
        pltpu.VMEM((NP, 2 * M, DM), F32),
        pltpu.VMEM((NP + 1, 2 * M, DM), F32),
        pltpu.VMEM((H // 4, NP, 2 * M, 4 * E), F32),
        pltpu.VMEM((H // 4, NP, 2 * M, 4 * E), F32),
        pltpu.VMEM((NP + 2, 2 * M, LANES), F32),
        pltpu.VMEM((DM // LANES, NSEG, LANES), F32),
        pltpu.VMEM((H // 4, NSEG + M, 4 * E), F32),
        pltpu.VMEM((2, 3, S, LANES), BF16),
        pltpu.VMEM((2, LANES, S), BF16),
        pltpu.VMEM((S, LANES), BF16),
        pltpu.VMEM((NFFT, S), F32),
        pltpu.VMEM((NFFT, S), F32),
        pltpu.VMEM((NFFT, S), BF16),
        pltpu.VMEM((S + 32, LANES), F32),
        pltpu.VMEM((NT, S, LANES), BF16),
        pltpu.VMEM((M, DM), BF16),
        pltpu.VMEM((NFFT, BLK), BF16),
        pltpu.VMEM((BLK, BLK), BF16),
        pltpu.VMEM((4, D), BF16),
        pltpu.VMEM((NT, LANES), BF16),
        pltpu.VMEM((8, LANES), jnp.int32),
        pltpu.SMEM((7,), jnp.int32),
        pltpu.SemaphoreType.DMA((5,)),
        pltpu.SemaphoreType.DMA((2 * NRB,)),
        pltpu.SemaphoreType.DMA((H // 2,)),
        pltpu.SemaphoreType.DMA,
        pltpu.SemaphoreType.DMA,
        pltpu.SemaphoreType.DMA((2, 2)),
        pltpu.SemaphoreType.DMA,
        pltpu.SemaphoreType.DMA((NRB,)),
    ]
    out = pl.pallas_call(
        functools.partial(_kernel, S=S, D=D, DM=DM, H=H, M=M, SEG=SEG),
        out_shape=jax.ShapeDtypeStruct((S, D + DM), BF16),
        in_specs=[any_spec] * 14,
        out_specs=any_spec,
        scratch_shapes=scratch,
        compiler_params=pltpu.CompilerParams(vmem_limit_bytes=120 * 1024 * 1024,
                                             disable_bounds_checks=True,
                                             disable_semaphore_checks=True),
    )(
        A_q.reshape(S, D), A_k.reshape(S, D), A_v.reshape(S, D),
        A_shift_k.T, A_ssm_k, A_ssm_D.reshape(NT, LANES),
        B_x.reshape(NRB, S // NRB, DM), B_mem0.reshape(M, DM),
        B_Wq, B_Wk, B_Wv, B_Wo.reshape(H * E, DM),
        jnp.asarray(fwd, BF16), jnp.asarray(inv, BF16),
    )
    return out.reshape(1, S, D + DM)
```
